```python
import jax
import jax.numpy as jnp

def _softmax(x, axis=-1):
    return jax.nn.softmax(x, axis=axis)
def _gelu(x):
    return jax.nn.gelu(x, approximate=True)
def _silu(x):
    return jax.nn.silu(x)
def _sigmoid(x):
    return jax.nn.sigmoid(x)
def _layernorm(x, axis=-1, eps=1e-5):
    m = jnp.mean(x, axis=axis, keepdims=True)
    v = jnp.var(x, axis=axis, keepdims=True)
    return (x - m) / jnp.sqrt(v + eps)
def _scatter_add(tgt, idx, src, axis=0):
    return tgt.at[idx].add(src)
def _segment_sum(src, seg, n):
    return jax.ops.segment_sum(src, seg, n)
class _Rng:
    def __init__(self, key):
        self._k = key
    def _next(self):
        self._k, sub = jax.random.split(self._k)
        return sub
    def normal(self, shape):
        return jax.random.normal(self._next(), shape, dtype=jnp.bfloat16)
    def randint(self, lo, hi, shape):
        return jax.random.randint(self._next(), shape, lo, hi, dtype=jnp.int32)
    def uniform(self, shape, lo=0.0, hi=1.0):
        return jax.random.uniform(self._next(), shape, jnp.bfloat16, lo, hi)
    def permutation(self, n):
        return jax.random.permutation(self._next(), n)


kernel_name = 'recurrent_scan__linear_kernel_hedgehog__moe_arch_mod__prompt'

def setup_inputs():
    _rng = _Rng(jax.random.key(int.from_bytes(__import__("os").urandom(4), "little")))
    _w = (lambda a: (lambda t: t.astype(jnp.bfloat16) if jnp.issubdtype(t.dtype, jnp.floating) else t)(jnp.asarray(a)))
    def _A_setup():
        B, S, D, H = 1, 2048, 1024, 32
        Dh = D // H
        return {
            "x": _w((lambda *s: _rng.normal(s) * 0.05)(B, S, D)),
            "wqkv": _w((lambda *s: _rng.normal(s) * 0.05)(D, 3 * D)),
            "w_phi": _w((lambda *s: _rng.normal(s) * 0.05)(H, Dh, Dh) * (Dh ** -0.5)),
            "wo": _w((lambda *s: _rng.normal(s) * 0.05)(D, D)),
        }
    _A_in = _A_setup()

    def _B_setup():
        B, S, D, F, C = 1, 2048, 1024, 3584, 1
        return {
            "x": _w((lambda *s: _rng.normal(s) * 0.05)(B, S, D)),
            "w_r": _w((lambda *s: _rng.normal(s) * 0.05)(D)),
            "w_gate": _w((lambda *s: _rng.normal(s) * 0.05)(D, F)),
            "w_up": _w((lambda *s: _rng.normal(s) * 0.05)(D, F)),
            "w_down": _w((lambda *s: _rng.normal(s) * 0.05)(F, D)),
        }
    _B_in = _B_setup()

    return {
        "A_x": _A_in["x"],
        "A_wqkv": _A_in["wqkv"],
        "A_w_phi": _A_in["w_phi"],
        "A_wo": _A_in["wo"],
        "B_x": _B_in["x"],
        "B_w_r": _B_in["w_r"],
        "B_w_gate": _B_in["w_gate"],
        "B_w_up": _B_in["w_up"],
        "B_w_down": _B_in["w_down"],
    }

def reference(A_x, A_wqkv, A_w_phi, A_wo, B_x, B_w_r, B_w_gate, B_w_up, B_w_down):
    def _A_ref(x, wqkv, w_phi, wo):
        B, S, D = x.shape
        H = 32; Dh = D // H
        qkv = (lambda x, *d: x.transpose(*d))((x @ wqkv).reshape(B, S, 3, H, Dh), 2, 0, 3, 1, 4)
        q, k, v = qkv[0], qkv[1], qkv[2]
        pq = jnp.einsum("bhsd,hdf->bhsf", q, w_phi)
        pk = jnp.einsum("bhsd,hdf->bhsf", k, w_phi)
        phi_q = jnp.concatenate([_softmax(pq, axis=-1), _softmax(-pq, axis=-1)], axis=-1)
        phi_k = jnp.concatenate([_softmax(pk, axis=-1), _softmax(-pk, axis=-1)], axis=-1)
        kv = jnp.einsum("bhsf,bhsd->bhfd", phi_k, v)
        z  = jnp.einsum("bhsf->bhf", phi_k)
        num = jnp.einsum("bhqf,bhfd->bhqd", phi_q, kv)
        den = jnp.einsum("bhqf,bhf->bhq", phi_q, z)[..., None] + 1e-6
        o = num / den
        return (lambda x, *d: x.transpose(*d))(o, 0, 2, 1, 3).reshape(B, S, D) @ wo

    def _B_ref(x, w_r, w_gate, w_up, w_down):
        B, S, D = x.shape
        C = 1
        r = x @ w_r
        idx = jnp.argsort(-r, axis=-1)[:, :C]
        idx_e = jnp.repeat(idx.reshape(B, C, 1), D, axis=2)
        x_sel = jnp.take_along_axis(x, idx_e, axis=1)
        g = _silu(x_sel @ w_gate)
        u = x_sel @ w_up
        y = (g * u) @ w_down
        r_sel = _sigmoid(jnp.take_along_axis(r, idx, axis=1))
        y = y * r_sel.reshape(B, C, 1)
        b_off = (jnp.arange(B) * S).reshape(B, 1)
        flat_idx = (idx + b_off).reshape(B * C)
        zero = (x * 0.0).reshape(B * S, D)
        upd = _scatter_add(zero, flat_idx, y.reshape(B * C, D), axis=0)
        return x + upd.reshape(B, S, D)

    x = A_x
    xn = _layernorm(x, axis=-1)
    s = _A_ref(xn, A_wqkv, A_w_phi, A_wo)
    g = _silu(_B_ref(xn, B_w_r, B_w_gate, B_w_up, B_w_down))
    return x + s * g
```

```python
import functools

import jax
import jax.numpy as jnp
import jax.experimental.pallas as pl
import jax.experimental.pallas.tpu as pltpu

S, D, H, DH, F = 2048, 1024, 32, 32, 3584
T = 256
NT = S // T
NG = D // 128
NP = D // 64
MR = 80
LOG2E = 1.4426950408889634
F32, BF16, U32 = jnp.float32, jnp.bfloat16, jnp.uint32

_NT_DIMS = (((1,), (1,)), ((), ()))


def _dot_nt(a, b):
    return jax.lax.dot_general(a, b, _NT_DIMS, preferred_element_type=F32)


def _dot(a, b):
    return jnp.dot(a, b, preferred_element_type=F32)


def _as_u32(v):
    return pltpu.bitcast(v, U32) if v.dtype != U32 else v


def _or_all(vals):
    acc = None
    for v in vals:
        u = _as_u32(v)
        for a in range(u.shape[0] // 8):
            for b in range(u.shape[1] // 128):
                t = u[a * 8:(a + 1) * 8, b * 128:(b + 1) * 128]
                acc = t if acc is None else acc | t
    return acc


def _gate(lhs_u32, deps, never):
    if not deps:
        return lhs_u32
    t = jnp.where(never, _or_all(deps), lhs_u32[0:8, 0:128])
    top = jnp.concatenate([t, lhs_u32[0:8, 128:]], axis=1)
    return jnp.concatenate([top, lhs_u32[8:]], axis=0)


def _layernorm(x):
    x = x.astype(F32)
    m = jnp.mean(x, axis=-1, keepdims=True)
    xc = x - m
    v = jnp.mean(xc * xc, axis=-1, keepdims=True)
    mb = m.astype(BF16).astype(F32)
    vb = (v.astype(BF16).astype(F32) + 1e-5).astype(BF16).astype(F32)
    sd = jnp.sqrt(vb).astype(BF16).astype(F32)
    return ((x - mb) * (1.0 / sd)).astype(BF16)


def _allreduce_pair(x, op):
    x = op(x, pltpu.roll(x, 2, axis=0))
    return op(x, pltpu.roll(x, 4, axis=0))


def _feature_map(p):
    t = p.shape[1]
    p3 = p.reshape(8, 8, t)
    mx = _allreduce_pair(jnp.max(p3, axis=0), jnp.maximum)
    mn = _allreduce_pair(jnp.min(p3, axis=0), jnp.minimum)
    ep = jnp.exp2(p3 - mx[None])
    en = jnp.exp2(mn[None] - p3)
    rp = 1.0 / _allreduce_pair(jnp.sum(ep, axis=0), jnp.add)
    rn = 1.0 / _allreduce_pair(jnp.sum(en, axis=0), jnp.add)
    pos = (ep * rp[None]).reshape(64, t)
    neg = (en * rn[None]).reshape(64, t)
    return jnp.concatenate([pos, neg], axis=0).astype(BF16)


def _silu(x):
    h = 0.5 * x
    return h + h * jnp.tanh(h)


def _kernel(x_hbm, wqkv_hbm, wphi_hbm, wo_hbm, wr_hbm, wg_hbm, wu_hbm, wd_hbm,
            out_hbm,
            x_v, xn_v, w_v, wphi_v, wr_v, wo_v, wg_v, wu_v, wd_v,
            wkt, wvt, wqt, kv_acc, m_v, r_v, y_v, out_v, zero_s,
            sem_x, sem_w, sem_o):
    def x_copy(i):
        return pltpu.make_async_copy(x_hbm.at[0, pl.ds(i * T, T), :],
                                     x_v.at[pl.ds(i * T, T), :], sem_x.at[i])

    def w_copy(j):
        return pltpu.make_async_copy(wqkv_hbm.at[:, j * D:(j + 1) * D],
                                     w_v.at[j], sem_w.at[j])

    wphi_copy = pltpu.make_async_copy(wphi_hbm, wphi_v, sem_w.at[3])
    wr_copy = pltpu.make_async_copy(wr_hbm, wr_v, sem_w.at[4])
    wo_copy = pltpu.make_async_copy(wo_hbm, wo_v, sem_w.at[5])
    wg_copy = pltpu.make_async_copy(wg_hbm, wg_v, sem_w.at[6])
    wu_copy = pltpu.make_async_copy(wu_hbm, wu_v, sem_w.at[7])
    wd_copy = pltpu.make_async_copy(wd_hbm, wd_v, sem_w.at[8])

    def out_copy(i, slot):
        return pltpu.make_async_copy(out_v.at[slot],
                                     out_hbm.at[0, pl.ds(i * T, T), :],
                                     sem_o.at[slot])

    wphi_copy.start()
    wr_copy.start()
    x_copy(0).start()
    w_copy(1).start()
    w_copy(2).start()
    x_copy(1).start()

    zero_s[0] = 0
    kv_acc[...] = jnp.zeros_like(kv_acc)

    wphi_copy.wait()
    wr_copy.wait()
    row = jax.lax.broadcasted_iota(jnp.int32, (128, DH), 0)
    col = jax.lax.broadcasted_iota(jnp.int32, (128, DH), 1)
    sel = jnp.where(((row % 64) // 2) == col, 1.0, 0.0).astype(BF16)
    wall = wphi_v[...].reshape(H * DH, DH)
    phit = _dot_nt(sel, wall)
    row = jax.lax.broadcasted_iota(jnp.int32, (128, D), 0)
    col = jax.lax.broadcasted_iota(jnp.int32, (128, D), 1)
    keep = (2 * (row // 64) + row % 2) == ((col % 128) // DH)
    phit = jnp.where(keep, phit, 0.0).astype(BF16)

    def fold(j, dst):
        for g in range(NG):
            wt = _dot_nt(phit[:, g * 128:(g + 1) * 128],
                         w_v[j, :, g * 128:(g + 1) * 128])
            dst[g * 64:(g + 1) * 64, :] = _as_u32((wt * LOG2E).astype(BF16))

    x_copy(0).wait()
    xn_v[0:T, :] = _layernorm(x_v[0:T, :])

    w_copy(1).wait()
    fold(1, wkt)
    w_copy(2).wait()
    for i in range(2, NT):
        x_copy(i).start()
    w_copy(0).start()
    wo_copy.start()
    wg_copy.start()
    wu_copy.start()
    wd_copy.start()
    for g in range(NG):
        wvt[g * 64:(g + 1) * 64, :] = _as_u32(w_v[2, :, g * 128:(g + 1) * 128].T)
    wvt[D // 2:D // 2 + 8, :] = _as_u32(jnp.broadcast_to(wr_v[...], (16, D)))

    ones = jnp.ones((16, T), BF16)

    def phase1(i, carry):
        never = zero_s[0] > 0
        nxt = jnp.minimum(i + 1, NT - 1)

        @pl.when(i + 1 < NT)
        def _():
            x_copy(i + 1).wait()

        s0 = pl.multiple_of(i * T, T)
        s1 = pl.multiple_of(nxt * T, T)
        xt = xn_v[pl.ds(s0, T), :]
        R = T // NG
        pk = [None] * NG
        vt = [None] * NG
        ln = [None] * NG

        def kv(g):
            for p in range(2):
                phi = _feature_map(pk[g][p * 64:(p + 1) * 64])
                lhs = jnp.concatenate([vt[g][p * 64:(p + 1) * 64], ones], axis=0)
                kv_acc[2 * g + p] += _dot_nt(lhs, phi)

        for g in range(NG):
            lhs = _gate(wkt[g * 64:(g + 1) * 64, :],
                        [ln[g - 1]] if g > 0 else [], never)
            pk[g] = _dot_nt(pltpu.bitcast(lhs, BF16), xt)
            if g > 0:
                kv(g - 1)
            if g == NG - 1:
                vr = _dot_nt(pltpu.bitcast(wvt[g * 64:(g + 1) * 64 + 8, :], BF16), xt)
                vt[g] = vr[0:128].astype(BF16)
                r_v[:, pl.ds(s0, T)] = vr[128:136]
            else:
                vt[g] = _dot_nt(pltpu.bitcast(wvt[g * 64:(g + 1) * 64, :], BF16),
                                xt).astype(BF16)
            sr = pl.multiple_of(s1 + g * R, R)
            ln[g] = _layernorm(x_v[pl.ds(sr, R), :])
            xn_v[pl.ds(sr, R), :] = ln[g]
        kv(NG - 1)
        return carry

    jax.lax.fori_loop(0, NT, phase1, 0)

    row = jax.lax.broadcasted_iota(jnp.int32, (MR, 128), 0)
    col = jax.lax.broadcasted_iota(jnp.int32, (MR, 128), 1)
    head = jnp.where(row < 64, row // DH, (row - 64) // 8)
    keep = head == (col % 2)
    for p in range(NP):
        m_v[p] = _as_u32(jnp.where(keep, kv_acc[p], 0.0).astype(BF16))

    w_copy(0).wait()
    fold(0, wqt)

    r = r_v[0:1, :].astype(BF16).astype(F32)
    rmax = jnp.max(r, axis=1, keepdims=True)
    pos = jax.lax.broadcasted_iota(jnp.int32, (1, S), 1)
    idx = jnp.min(jnp.where(r == rmax, pos, S))
    idx = jnp.clip(idx, 0, S - 1)
    base = pl.multiple_of((idx // 16) * 16, 16)
    xs = xn_v[pl.ds(base, 16), :]
    wg_copy.wait()
    wu_copy.wait()
    wd_copy.wait()
    hg = _dot(xs, wg_v[...]).astype(BF16).astype(F32)
    hu = _dot(xs, wu_v[...]).astype(BF16).astype(F32)
    hh = (_silu(hg).astype(BF16).astype(F32) * hu).astype(BF16)
    y = _dot(hh, wd_v[...]).astype(BF16).astype(F32)
    gate = (0.5 + 0.5 * jnp.tanh(0.5 * rmax)).astype(BF16).astype(F32)
    y = y * gate
    rows16 = jax.lax.broadcasted_iota(jnp.int32, (16, D), 0)
    y_v[...] = jnp.broadcast_to(
        jnp.sum(jnp.where(rows16 == idx - base, y, 0.0), axis=0, keepdims=True), (8, D))
    wo_copy.wait()

    def phase2(i, carry):
        never = zero_s[0] > 0
        slot = i % 2

        @pl.when(i >= 2)
        def _():
            out_copy(i - 2, slot).wait()

        s0 = pl.multiple_of(i * T, T)
        xt = xn_v[pl.ds(s0, T), :]
        pq = [None] * NG
        og = [None] * NG

        def nd(g):
            parts = []
            for p in range(2):
                phi = _feature_map(pq[g][p * 64:(p + 1) * 64])
                r_ = _dot(pltpu.bitcast(m_v[2 * g + p], BF16), phi)
                inv = 1.0 / (r_[64:80] + 1e-6)
                num = r_[0:64].reshape(2, 4, 8, T)
                o = num * inv.reshape(2, 1, 8, T)
                parts.append(o.reshape(64, T))
            og[g] = jnp.concatenate(parts, axis=0).astype(BF16).T

        for g in range(NG):
            pq[g] = _dot_nt(pltpu.bitcast(wqt[g * 64:(g + 1) * 64, :], BF16), xt)
            if g > 0:
                nd(g - 1)
        oa = jnp.concatenate(og[0:4], axis=1)
        sa = [None] * NG
        for n in range(NG):
            sa[n] = _dot(oa, wo_v[0:512, n * 128:(n + 1) * 128])
            if n == 1:
                nd(NG - 1)
        ob = _as_u32(jnp.concatenate(og[4:8], axis=1))
        rows = jax.lax.broadcasted_iota(jnp.int32, (T, 128), 0) + s0
        hit = rows == idx
        res = [None] * NG
        for n in range(NG):
            lhs = _gate(ob, [res[n - 2]] if n >= 2 else [], never)
            s = sa[n] + _dot(pltpu.bitcast(lhs, BF16), wo_v[512:1024, n * 128:(n + 1) * 128])
            cs = slice(n * 128, (n + 1) * 128)
            b = xt[:, cs].astype(F32) + jnp.where(hit, y_v[0:1, cs], 0.0)
            res[n] = (x_v[pl.ds(s0, T), cs].astype(F32) + s * _silu(b)).astype(BF16)
            out_v[slot, :, cs] = res[n]
        out_copy(i, slot).start()
        return carry

    jax.lax.fori_loop(0, NT, phase2, 0)
    out_copy(NT - 2, (NT - 2) % 2).wait()
    out_copy(NT - 1, (NT - 1) % 2).wait()


@jax.jit
def pallas_recurrent_scan__linear_kernel_hedgehog__moe_arch_mod__prompt_kernel(
    A_x: jax.Array,
    A_wqkv: jax.Array,
    A_w_phi: jax.Array,
    A_wo: jax.Array,
    B_x: jax.Array,
    B_w_r: jax.Array,
    B_w_gate: jax.Array,
    B_w_up: jax.Array,
    B_w_down: jax.Array,
):
    del B_x
    any_spec = pl.BlockSpec(memory_space=pl.ANY)
    return pl.pallas_call(
        _kernel,
        out_shape=jax.ShapeDtypeStruct((1, S, D), BF16),
        in_specs=[any_spec] * 8,
        out_specs=any_spec,
        scratch_shapes=[
            pltpu.VMEM((S, D), BF16),
            pltpu.VMEM((S, D), BF16),
            pltpu.VMEM((3, D, D), BF16),
            pltpu.VMEM((H, DH, DH), BF16),
            pltpu.VMEM((1, D), BF16),
            pltpu.VMEM((D, D), BF16),
            pltpu.VMEM((D, F), BF16),
            pltpu.VMEM((D, F), BF16),
            pltpu.VMEM((F, D), BF16),
            pltpu.VMEM((D // 2, D), U32),
            pltpu.VMEM((D // 2 + 8, D), U32),
            pltpu.VMEM((D // 2, D), U32),
            pltpu.VMEM((NP, MR, 128), F32),
            pltpu.VMEM((NP, MR // 2, 128), U32),
            pltpu.VMEM((8, S), F32),
            pltpu.VMEM((8, D), F32),
            pltpu.VMEM((2, T, D), BF16),
            pltpu.SMEM((1,), jnp.int32),
            pltpu.SemaphoreType.DMA((NT,)),
            pltpu.SemaphoreType.DMA((9,)),
            pltpu.SemaphoreType.DMA((2,)),
        ],
        compiler_params=pltpu.CompilerParams(vmem_limit_bytes=100 * 1024 * 1024),
    )(A_x, A_wqkv, A_w_phi, A_wo, B_w_r.reshape(1, D), B_w_gate, B_w_up, B_w_down)
```

```python
import functools

import jax
import jax.numpy as jnp
import jax.experimental.pallas as pl
import jax.experimental.pallas.tpu as pltpu

S, D, H, DH, F = 2048, 1024, 32, 32, 3584
T = 256
TH = T // 2
DHALF = D // 2
NT = S // T
NJ = 4
NP = D // 64
MR = 80
FC = 512
NFC = F // FC
LOG2E = 1.4426950408889634
F32, BF16, U32, I32 = jnp.float32, jnp.bfloat16, jnp.uint32, jnp.int32

_NT_DIMS = (((1,), (1,)), ((), ()))


def _dot_nt(a, b):
    return jax.lax.dot_general(a, b, _NT_DIMS, preferred_element_type=F32)


def _dot(a, b):
    return jnp.dot(a, b, preferred_element_type=F32)


def _u32(v):
    return pltpu.bitcast(v, U32) if v.dtype != U32 else v


def _pack2(even, odd):
    return pltpu.pack_elementwise([even, odd], packed_dtype=BF16)


def _unpack2(u):
    return [pltpu.unpack_elementwise(u, index=i, packed_dtype=BF16, unpacked_dtype=F32)
            for i in range(2)]


def _pack_blocks(v):
    r, c = v.shape
    v4 = v.reshape(r // 16, 2, 8, c)
    return _pack2(v4[:, 0], v4[:, 1]).reshape(r // 2, c)


def _recip(x):
    r = pl.reciprocal(x, approx=True)
    return r * (2.0 - x * r)


def _bf(v):
    return pltpu.bitcast(v, BF16)


def _round(v):
    return v.astype(BF16).astype(F32)


def _or_all(vals):
    ts = []
    for v in vals:
        u = _u32(v)
        for a in range(u.shape[0] // 8):
            for b in range(u.shape[1] // 128):
                ts.append(u[a * 8:(a + 1) * 8, b * 128:(b + 1) * 128])
    while len(ts) > 1:
        ts = [ts[i] | ts[i + 1] if i + 1 < len(ts) else ts[i] for i in range(0, len(ts), 2)]
    return ts[0]


def _gate(lhs_u32, deps, never):
    if not deps:
        return lhs_u32
    t = jnp.where(never, _or_all(deps), lhs_u32[0:8, 0:128])
    top = jnp.concatenate([t, lhs_u32[0:8, 128:]], axis=1)
    return jnp.concatenate([top, lhs_u32[8:]], axis=0)


def _layernorm(x):
    m = jnp.mean(x, axis=-1, keepdims=True)
    mb = _round(m)
    xc = x - mb
    dm = m - mb
    v = jnp.mean(xc * xc, axis=-1, keepdims=True) - dm * dm
    sd = _round(jnp.sqrt(_round(_round(v) + 1e-5)))
    return xc * _recip(sd)


def _lhs_combos(a11, a12, a21, a22):
    return [a11 + a22, a21 + a22, a11, a22, a11 + a12, a21 - a11, a12 - a22]


def _rhs_combos(b11, b12, b21, b22):
    return [b11 + b22, b11, b12 - b22, b21 - b11, b22, b11 + b12, b21 + b22]


def _strassen(prod, after=None):
    done = {}

    def p(k, step):
        return prod(k, step)

    def hook(step):
        if after is not None:
            after(step, done)

    m1 = p(0, 0)
    hook(0)
    m4 = p(3, 1)
    hook(1)
    m5 = p(4, 2)
    hook(2)
    m7 = p(6, 3)
    done[0] = m1 + m4 - m5 + m7
    hook(3)
    m3 = p(2, 4)
    done[1] = m3 + m5
    hook(4)
    m2 = p(1, 5)
    done[2] = m2 + m4
    hook(5)
    m6 = p(5, 6)
    done[3] = m1 - m2 + m3 + m6
    hook(6)
    return done[0], done[1], done[2], done[3]


def _allreduce_pair(x, op):
    x = op(x, pltpu.roll(x, 2, axis=0))
    return op(x, pltpu.roll(x, 4, axis=0))


def _feature_map(p):
    t = p.shape[1]
    p3 = p.reshape(8, 8, t)
    mx = _allreduce_pair(jnp.max(p3, axis=0), jnp.maximum)
    mn = _allreduce_pair(jnp.min(p3, axis=0), jnp.minimum)
    ep = jnp.exp2(p3 - mx[None])
    en = jnp.exp2(mn[None] - p3)
    rp = _recip(_allreduce_pair(jnp.sum(ep, axis=0), jnp.add))
    rn = _recip(_allreduce_pair(jnp.sum(en, axis=0), jnp.add))
    pos = (ep * rp[None]).reshape(64, t)
    neg = (en * rn[None]).reshape(64, t)
    return jnp.concatenate([pos, neg], axis=0).astype(BF16)


def _silu(x):
    h = 0.5 * x
    return h + h * jnp.tanh(h)


def _kernel(x_hbm, wqkv_hbm, wphi_hbm, wo_hbm, wr_hbm, wg_hbm, wu_hbm, wd_hbm,
            out_hbm,
            x_v, w_v, wphi_v, wr_v, wo_v, wg_v, wu_v, wd_v,
            bq, ak, av, aq, bo, kv_acc, m_v, wr2, r_v, y_acc, xb_v, hb_v, pq0_v,
            out_v, zero_s, sem, sem_o):
    def x_copy(i):
        return pltpu.make_async_copy(x_hbm.at[0, pl.ds(i * T, T), :],
                                     x_v.at[pl.ds(i * T, T), :], sem.at[i])

    def w_copy(m, j):
        return pltpu.make_async_copy(
            wqkv_hbm.at[:, m * D + j * 256:m * D + (j + 1) * 256],
            w_v.at[m, :, j * 256:(j + 1) * 256], sem.at[NT + 6 + 4 * m + j])

    wphi_copy = pltpu.make_async_copy(wphi_hbm, wphi_v, sem.at[NT])
    wr_copy = pltpu.make_async_copy(wr_hbm, wr_v, sem.at[NT + 1])
    wo_copy = pltpu.make_async_copy(wo_hbm, wo_v, sem.at[NT + 2])
    wg_copy = pltpu.make_async_copy(wg_hbm, wg_v, sem.at[NT + 3])
    wu_copy = pltpu.make_async_copy(wu_hbm, wu_v, sem.at[NT + 4])
    wd_copy = pltpu.make_async_copy(wd_hbm, wd_v, sem.at[NT + 5])

    def out_copy(i, slot):
        return pltpu.make_async_copy(out_v.at[slot],
                                     out_hbm.at[0, pl.ds(i * T, T), :],
                                     sem_o.at[slot])

    wphi_copy.start()
    wr_copy.start()
    x_copy(0).start()
    for j in range(NJ):
        w_copy(1, j).start()
        w_copy(2, j).start()
    x_copy(1).start()
    x_copy(2).start()
    wo_copy.start()
    for i in range(3, NT):
        x_copy(i).start()
    for j in range(NJ):
        w_copy(0, j).start()
    wg_copy.start()
    wu_copy.start()
    wd_copy.start()

    zero_s[0] = 0
    kv_acc[...] = jnp.zeros_like(kv_acc)
    y_acc[...] = jnp.zeros_like(y_acc)

    with jax.named_scope('wphi'):
        wphi_copy.wait()
    wr_copy.wait()
    row = jax.lax.broadcasted_iota(I32, (128, DH), 0)
    col = jax.lax.broadcasted_iota(I32, (128, DH), 1)
    sel = jnp.where(((row % 64) // 16) * 8 + row % 8 == col, 1.0, 0.0).astype(BF16)
    wall = wphi_v[...].reshape(H * DH, DH)
    phit = _dot_nt(sel, wall)
    row = jax.lax.broadcasted_iota(I32, (128, D), 0)
    col = jax.lax.broadcasted_iota(I32, (128, D), 1)
    keep = (2 * (row // 64) + (row // 8) % 2) == ((col % 128) // DH)
    phit = jnp.where(keep, phit, 0.0).astype(BF16)


    def fold(which, dst, j):
        wt = []
        for g in (2 * j, 2 * j + 1):
            wt.append(_dot_nt(phit[:, g * 128:(g + 1) * 128],
                              w_v[which, :, g * 128:(g + 1) * 128]) * LOG2E)
        w0, w1 = wt
        cs = _lhs_combos(w0[:, :DHALF], w0[:, DHALF:], w1[:, :DHALF], w1[:, DHALF:])
        for k in range(7):
            dst[k, j * 64:(j + 1) * 64, :] = _pack_blocks(cs[k])

    def packed_combos(fn, u11, u12, u21, u22):
        parts = [_unpack2(u) for u in (u11, u12, u21, u22)]
        ev = fn(*[p[0] for p in parts])
        od = fn(*[p[1] for p in parts])
        return [_pack2(e, o) for e, o in zip(ev, od)]

    def prep_v(j):
        w0, w1 = [_u32(w_v[2, :, g * 128:(g + 1) * 128].T) for g in (2 * j, 2 * j + 1)]
        cs = packed_combos(_lhs_combos, w0[:, :DHALF], w0[:, DHALF:],
                           w1[:, :DHALF], w1[:, DHALF:])
        cs[2], cs[3] = w0[:, :DHALF], w1[:, DHALF:]
        for k in range(7):
            av[k, j * 64:(j + 1) * 64, :] = cs[k]

    def ln_chunk(n, c):
        ys = []
        for h in range(2):
            r0 = n * T + h * TH + c * 16
            if not isinstance(r0, int):
                r0 = pl.multiple_of(r0, 16)
            ys += [_layernorm(xr) for xr in _unpack2(_u32(x_v[pl.ds(r0, 16), :]))]
        cs = []
        for t in range(2):
            ya, yb = ys[t], ys[2 + t]
            cs.append(_rhs_combos(ya[:, :DHALF], yb[:, :DHALF], ya[:, DHALF:], yb[:, DHALF:])
                      + [ya[:, DHALF:], yb[:, :DHALF]])
        cs = [_pack2(e, o) for e, o in zip(*cs)]
        for k in range(9):
            bq[n, k, c * 8:(c + 1) * 8, :] = cs[k]
        return cs

    def wo_piece(c, q):
        r0 = (c // 2) * 256 + (c % 2) * 64 + q * 16
        o0 = c * 32 + q * 8
        if not isinstance(c, int):
            r0 = pl.multiple_of(r0, 16)
            o0 = pl.multiple_of(o0, 8)
        w0 = _u32(wo_v[pl.ds(r0, 16), :])
        w1 = _u32(wo_v[pl.ds(r0 + 128, 16), :])

        def cols(w, par):
            return jnp.concatenate(
                [w[:, (2 * q + par) * 128:(2 * q + par + 1) * 128] for q in range(4)], axis=1)
        blocks = [cols(w0, 0), cols(w0, 1), cols(w1, 0), cols(w1, 1)]
        cs = packed_combos(_rhs_combos, *blocks)
        cs[1], cs[4] = blocks[0], blocks[3]
        for k in range(7):
            bo[k, pl.ds(o0, 8), :] = cs[k]
        return cs

    class Sched:
        def __init__(self, never):
            self.never = never
            self.slot = 0
            self.jobs = {}
            self.deps = {}

        def at(self, slot, fn):
            self.jobs.setdefault(slot, []).append(fn)

        def need(self, slot, vals):
            self.deps.setdefault(slot, []).extend(vals)

        def gate(self, lhs):
            return _gate(lhs, self.deps.pop(self.slot, []), self.never)

        def after(self, step, done):
            for fn in self.jobs.pop(self.slot, []):
                fn()
            self.slot += 1

    def proj(sch, a_ref, j, b, extra=None):
        def prod(k, step):
            lhs = sch.gate(a_ref[k, j * 64:(j + 1) * 64, :])
            if extra is not None and k in (1, 2, 3, 4):
                r_ = _dot_nt(_bf(jnp.concatenate([lhs, wr2[...]], axis=0)), b[k])
                extra[k] = r_[128:136]
                return r_[0:128]
            return _dot_nt(_bf(lhs), b[k])
        c11, c12, c21, c22 = _strassen(prod, sch.after)
        return (jnp.concatenate([c11, c12], axis=1),
                jnp.concatenate([c21, c22], axis=1))

    wr = wr_v[...].astype(F32)
    wr2[...] = _pack2(jnp.broadcast_to(wr[:, :DHALF], (8, DHALF)),
                      jnp.broadcast_to(wr[:, DHALF:], (8, DHALF)))

    with jax.named_scope('x0'):
        x_copy(0).wait()
    for c in range(8):
        ln_chunk(0, c)

    ones = jnp.ones((16, T), BF16)

    def phase1(i, carry):
        first = isinstance(i, int)
        never = zero_s[0] > 0
        if first:
            nxt = 1
        else:
            nxt = jnp.minimum(i + 1, NT - 1)

            @pl.when(i + 1 < NT)
            def _():
                x_copy(i + 1).wait()

            @pl.when(i == 1)
            def _():
                wo_copy.wait()

        b = [_bf(bq[i, k]) for k in range(7)]
        pk = [None] * NJ
        vt = [None] * NJ
        sch = Sched(never)

        def kv(j, g, p):
            phi = _feature_map(pk[j][g][p * 64:(p + 1) * 64])
            lhs = jnp.concatenate([vt[j][g][p * 64:(p + 1) * 64], ones], axis=0)
            kv_acc[4 * j + 2 * g + p] += _dot_nt(lhs, phi)

        def ln_job(c, due):
            return lambda: sch.need(due, ln_chunk(nxt, c))

        def wo_job(q, due):
            return lambda: sch.need(due, wo_piece(i - 1, q))

        if first:
            for c in range(8):
                sch.at(42, ln_job(c, 45 + (3 * c) // 2))
        else:
            for c in range(8):
                sch.at(0, ln_job(c, 6 + 7 * c))
            for q in range(4):
                sch.at(0, wo_job(q, 10 + 14 * q))
        for j in range(NJ - 1):
            for g in range(2):
                for p in range(2):
                    sch.at(14 * (j + 1) + 2 * (2 * g + p),
                           functools.partial(kv, j, g, p))
        def wait(name, *copies):
            with jax.named_scope(name):
                for cp in copies:
                    cp.wait()

        if first:
            wait('wk0', w_copy(1, 0))
            fold(1, ak, 0)
        for j in range(NJ):
            if first:
                if j < 2:
                    wait('wv%d' % j, w_copy(2, j))
                if j == 3:
                    wait('x1', x_copy(1))
                prep_v(j)
            pk[j] = proj(sch, ak, j, b)
            if first and j + 1 < NJ:
                if j == 0:
                    wait('wk1', w_copy(1, 1))
                else:
                    wait('wkv%d' % (j + 1), w_copy(1, j + 1), w_copy(2, j + 1))
                fold(1, ak, j + 1)
            ex = {} if j == 0 else None
            vt[j] = [v.astype(BF16) for v in proj(sch, av, j, b, ex)]
            if j == 0:
                r_v[i] = jnp.concatenate(
                    [ex[1][0:1] + ex[1][1:2] + ex[3][1:2],
                     ex[4][0:1] + ex[4][1:2] + ex[2][0:1]], axis=1)
        for g in range(2):
            for p in range(2):
                kv(NJ - 1, g, p)
        return carry

    phase1(0, 0)
    with jax.named_scope('P1'):
        jax.lax.fori_loop(1, NT, phase1, 0)

    row = jax.lax.broadcasted_iota(I32, (MR, 128), 0)
    col = jax.lax.broadcasted_iota(I32, (MR, 128), 1)
    head = jnp.where(row < 64, row // DH, (row - 64) // 8)
    keep = head == (col % 2)
    for p in range(NP):
        m_v[p] = _u32(jnp.where(keep, kv_acc[p], 0.0).astype(BF16))

    for q in range(4):
        wo_piece(NT - 1, q)
    for j in range(NJ):
        w_copy(0, j).wait()
    for j in range(NJ):
        fold(0, aq, j)

    r = _round(r_v[...].reshape(NT, T))
    rmax = jnp.max(jnp.max(r, axis=1, keepdims=True), axis=0, keepdims=True)
    pos = (jax.lax.broadcasted_iota(I32, (NT, T), 0) * T
           + jax.lax.broadcasted_iota(I32, (NT, T), 1))
    idx = jnp.min(jnp.where(r == rmax, pos, S))
    idx = jnp.clip(idx, 0, S - 1)
    tile = idx // T
    half = (idx % T) // TH
    sub = pl.multiple_of(((idx % TH) // 16) * 8, 8)
    xs = jnp.concatenate([bq[tile, 1 + 7 * half, pl.ds(sub, 8), :],
                          bq[tile, 7 - 3 * half, pl.ds(sub, 8), :]], axis=1)
    xs = jnp.where(jax.lax.broadcasted_iota(I32, (16, D), 0) == idx % 16,
                   _bf(xs).astype(F32), 0.0)
    xs = jnp.sum(xs, axis=0, keepdims=True)

    def lane_bcast(dst, row):
        for t in range(row.shape[1] // 128):
            dst[t * 128:(t + 1) * 128, :] = jnp.broadcast_to(
                row[:, t * 128:(t + 1) * 128], (128, 128)).T

    lane_bcast(xb_v, xs)
    router = _round(0.5 + 0.5 * jnp.tanh(0.5 * rmax))
    wg_copy.wait()
    wu_copy.wait()
    wd_copy.wait()

    first = proj(Sched(None), aq, 0, [_bf(bq[(tile + 1) % NT, k]) for k in range(7)])
    for g in range(2):
        pq0_v[g] = first[g]

    def phase2(i, carry):
        never = zero_s[0] > 0
        slot = i % 2
        n = (tile + 1 + i) % NT

        @pl.when(i >= 2)
        def _():
            out_copy((tile + i - 1) % NT, slot).wait()

        s0 = pl.multiple_of(n * T, T)
        b = [_bf(bq[n, k]) for k in range(7)]
        pq = [None] * NJ
        ao = [None] * NJ
        yrow = _round(jnp.sum(y_acc[...], axis=0, keepdims=True)) * router
        sch = Sched(never)
        ot = {}
        pq[0] = [pq0_v[g] for g in range(2)]
        b_next = [_bf(bq[(n + 1) % NT, k]) for k in range(7)]

        def nd(j, g, p):
            phi = _feature_map(pq[j][g][p * 64:(p + 1) * 64])
            r_ = _dot(_bf(m_v[4 * j + 2 * g + p]), phi)
            inv = _recip(r_[64:80] + 1e-6)
            o = r_[0:64].reshape(2, 4, 8, T) * inv.reshape(2, 1, 8, T)
            ot[j, g, p] = o.reshape(64, T)
            if g == 1 and p == 1:
                o0, o1 = [jnp.concatenate([ot[j, g_, 0], ot[j, g_, 1]], axis=0)
                          for g_ in range(2)]
                cs = _lhs_combos(o0[:, :TH], o1[:, :TH], o0[:, TH:], o1[:, TH:])
                ao[j] = [v.astype(BF16).T for v in cs]

        fc = pl.multiple_of(jnp.minimum(i, NFC - 1) * FC, FC)
        ffn = {}

        def matvec(key, w, vb, due):
            t = (w.astype(F32).reshape(16, 8, 256)
                 * jnp.concatenate([vb, vb], axis=1).reshape(16, 8, 256))
            t = jnp.sum(t, axis=0)
            ffn[key] = t if key not in ffn else ffn[key] + t
            sch.need(due, [ffn[key]])

        def ffn_up(w_ref, name, cp, rb, due):
            rs = slice(rb * 128, (rb + 1) * 128)
            matvec((name, cp), w_ref[rs, pl.ds(fc + cp * 256, 256)], xb_v[rs, :], due)

        def ffn_mid():
            hg, hu = [_round(jnp.sum(jnp.concatenate([ffn[nm, 0], ffn[nm, 1]], axis=1),
                                     axis=0, keepdims=True)) for nm in 'gu']
            lane_bcast(hb_v, _round(_round(_silu(hg)) * hu))

        def ffn_down(cp, rb, due):
            cs_ = slice(cp * 256, (cp + 1) * 256)
            matvec(('y', cp), wd_v[pl.ds(fc + rb * 128, 128), cs_],
                   hb_v[rb * 128:(rb + 1) * 128, :], due)
            if rb == 3:
                y_acc[:, cs_] += jnp.where(i < NFC, ffn['y', cp], 0.0)

        t = 0
        for rb in range(8):
            for name, w_ref in (('g', wg_v), ('u', wu_v)):
                for cp in range(2):
                    sch.at(t, functools.partial(ffn_up, w_ref, name, cp, rb, t + 1))
                    t += 1
        sch.at(t, ffn_mid)
        t += 5
        for rb in range(4):
            for cp in range(4):
                sch.at(t, functools.partial(ffn_down, cp, rb, t + 1))
                t += 1
        for j in range(NJ):
            for g in range(2):
                for p in range(2):
                    off = 2 * g + p if j == NJ - 1 else 2 * (2 * g + p)
                    sch.at(7 * j + off, functools.partial(nd, j, g, p))
        for j in range(1, NJ):
            pq[j] = proj(sch, aq, j, b)
        nxt = proj(sch, aq, 0, b_next)
        for g in range(2):
            pq0_v[g] = nxt[g]

        lhs = [_u32(jnp.concatenate([ao[j][k] for j in range(NJ)], axis=1))
               for k in range(7)]
        rows = jax.lax.broadcasted_iota(I32, (64, 256), 0) + s0

        def epilogue(c, cc, e, due):
            h, r0 = e // 2, (e // 2) * TH + (e % 2) * 64
            cs = slice(c * 256, (c + 1) * 256)
            rs = slice((e % 2) * 64, (e % 2) * 64 + 64)
            blk = ((1, 7), (8, 4))[h][c // 2]
            xn = _bf(bq[n, blk, (e % 2) * 32:(e % 2) * 32 + 32,
                        (c % 2) * 256:(c % 2 + 1) * 256]).astype(F32)
            bb = xn + jnp.where(rows + r0 == idx, yrow[:, cs], 0.0)
            xr = x_v[pl.ds(s0 + r0, 64), cs].astype(F32)
            sv = jnp.concatenate([cc[2 * h][rs], cc[2 * h + 1][rs]], axis=1)
            res = xr + sv * _silu(bb)
            out_v[slot, r0:r0 + 64, cs] = res.astype(BF16)
            if due is not None:
                sch.need(due, [res])

        for c in range(4):
            def prod(k, step):
                return _dot(_bf(sch.gate(lhs[k])), _bf(bo[k, :, c * 128:(c + 1) * 128]))
            cc = _strassen(prod, sch.after)
            for e in range(4):
                epilogue(c, cc, e, sch.slot + 2 + e if c < 3 else None)
        out_copy(n, slot).start()
        return carry

    with jax.named_scope('P2'):
        jax.lax.fori_loop(0, NT, phase2, 0)
    out_copy((tile + NT - 1) % NT, (NT - 2) % 2).wait()
    out_copy(tile, (NT - 1) % 2).wait()


@jax.jit
def pallas_recurrent_scan__linear_kernel_hedgehog__moe_arch_mod__prompt_kernel(
    A_x: jax.Array,
    A_wqkv: jax.Array,
    A_w_phi: jax.Array,
    A_wo: jax.Array,
    B_x: jax.Array,
    B_w_r: jax.Array,
    B_w_gate: jax.Array,
    B_w_up: jax.Array,
    B_w_down: jax.Array,
):
    del B_x
    any_spec = pl.BlockSpec(memory_space=pl.ANY)
    return pl.pallas_call(
        _kernel,
        out_shape=jax.ShapeDtypeStruct((1, S, D), BF16),
        in_specs=[any_spec] * 8,
        out_specs=any_spec,
        scratch_shapes=[
            pltpu.VMEM((S, D), BF16),
            pltpu.VMEM((3, D, D), BF16),
            pltpu.VMEM((H, DH, DH), BF16),
            pltpu.VMEM((1, D), BF16),
            pltpu.VMEM((D, D), BF16),
            pltpu.VMEM((D, F), BF16),
            pltpu.VMEM((D, F), BF16),
            pltpu.VMEM((F, D), BF16),
            pltpu.VMEM((NT, 9, TH // 2, DHALF), U32),
            pltpu.VMEM((7, 256, DHALF), U32),
            pltpu.VMEM((7, 256, DHALF), U32),
            pltpu.VMEM((7, 256, DHALF), U32),
            pltpu.VMEM((7, 256, DHALF), U32),
            pltpu.VMEM((NP, MR, 128), F32),
            pltpu.VMEM((NP, MR // 2, 128), U32),
            pltpu.VMEM((8, DHALF), U32),
            pltpu.VMEM((NT, 1, T), F32),
            pltpu.VMEM((8, D), F32),
            pltpu.VMEM((D, 128), F32),
            pltpu.VMEM((FC, 128), F32),
            pltpu.VMEM((2, 128, T), F32),
            pltpu.VMEM((2, T, D), BF16),
            pltpu.SMEM((1,), I32),
            pltpu.SemaphoreType.DMA((NT + 18,)),
            pltpu.SemaphoreType.DMA((2,)),
        ],
        compiler_params=pltpu.CompilerParams(vmem_limit_bytes=100 * 1024 * 1024),
    )(A_x, A_wqkv, A_w_phi, A_wo, B_w_r.reshape(1, D), B_w_gate, B_w_up, B_w_down)
```

```python
import functools
import os
import json
_P = json.loads(os.environ.get('KP', '{}'))

import jax
import jax.numpy as jnp
import jax.experimental.pallas as pl
import jax.experimental.pallas.tpu as pltpu

S, D, H, DH, F = 2048, 1024, 32, 32, 3584
T = 256
TH = T // 2
DHALF = D // 2
NT = S // T
NJ = 4
NP = D // 64
MR = 80
FC = 512
NFC = F // FC
LOG2E = 1.4426950408889634
F32, BF16, U32, I32 = jnp.float32, jnp.bfloat16, jnp.uint32, jnp.int32

_NT_DIMS = (((1,), (1,)), ((), ()))


def _dot_nt(a, b):
    return jax.lax.dot_general(a, b, _NT_DIMS, preferred_element_type=F32)


def _dot(a, b):
    return jnp.dot(a, b, preferred_element_type=F32)


def _u32(v):
    return pltpu.bitcast(v, U32) if v.dtype != U32 else v


def _pack2(even, odd):
    return pltpu.pack_elementwise([even, odd], packed_dtype=BF16)


def _unpack2(u):
    return [pltpu.unpack_elementwise(u, index=i, packed_dtype=BF16, unpacked_dtype=F32)
            for i in range(2)]


def _pack_blocks(v):
    r, c = v.shape
    v4 = v.reshape(r // 16, 2, 8, c)
    return _pack2(v4[:, 0], v4[:, 1]).reshape(r // 2, c)


def _recip(x):
    r = pl.reciprocal(x, approx=True)
    return r * (2.0 - x * r)


def _bf(v):
    return pltpu.bitcast(v, BF16)


def _round(v):
    return v.astype(BF16).astype(F32)


def _or_all(vals):
    ts = []
    for v in vals:
        u = _u32(v)
        for a in range(u.shape[0] // 8):
            for b in range(u.shape[1] // 128):
                ts.append(u[a * 8:(a + 1) * 8, b * 128:(b + 1) * 128])
    while len(ts) > 1:
        ts = [ts[i] | ts[i + 1] if i + 1 < len(ts) else ts[i] for i in range(0, len(ts), 2)]
    return ts[0]


def _gate(lhs_u32, deps, never):
    if not deps:
        return lhs_u32
    rows = []
    for r in range(lhs_u32.shape[0] // 8):
        row = lhs_u32[r * 8:(r + 1) * 8]
        cs = [c for (r_, c) in deps if r_ == r]
        if cs:
            row = jnp.concatenate(
                [jnp.where(never, _or_all(deps[r, c]), row[:, c * 128:(c + 1) * 128])
                 if c in cs else row[:, c * 128:(c + 1) * 128]
                 for c in range(lhs_u32.shape[1] // 128)], axis=1)
        rows.append(row)
    return jnp.concatenate(rows, axis=0)


def _layernorm(x):
    m = jnp.mean(x, axis=-1, keepdims=True)
    mb = _round(m)
    xc = x - mb
    dm = m - mb
    v = jnp.mean(xc * xc, axis=-1, keepdims=True) - dm * dm
    sd = _round(jnp.sqrt(_round(_round(v) + 1e-5)))
    return xc * _recip(sd)


def _lhs_combos(a11, a12, a21, a22):
    return [a11 + a22, a21 + a22, a11, a22, a11 + a12, a21 - a11, a12 - a22]


def _rhs_combos(b11, b12, b21, b22):
    return [b11 + b22, b11, b12 - b22, b21 - b11, b22, b11 + b12, b21 + b22]


def _strassen(prod, after=None):
    done = {}

    def p(k, step):
        return prod(k, step)

    def hook(step):
        if after is not None:
            after(step, done)

    m1 = p(0, 0)
    hook(0)
    m4 = p(3, 1)
    hook(1)
    m5 = p(4, 2)
    hook(2)
    m7 = p(6, 3)
    done[0] = m1 + m4 - m5 + m7
    hook(3)
    m3 = p(2, 4)
    done[1] = m3 + m5
    hook(4)
    m2 = p(1, 5)
    done[2] = m2 + m4
    hook(5)
    m6 = p(5, 6)
    done[3] = m1 - m2 + m3 + m6
    hook(6)
    return done[0], done[1], done[2], done[3]


def _allreduce_pair(x, op):
    x = op(x, pltpu.roll(x, 2, axis=0))
    return op(x, pltpu.roll(x, 4, axis=0))


def _feature_map(p):
    t = p.shape[1]
    p3 = p.reshape(8, 8, t)
    mx = _allreduce_pair(jnp.max(p3, axis=0), jnp.maximum)
    mn = _allreduce_pair(jnp.min(p3, axis=0), jnp.minimum)
    ep = jnp.exp2(p3 - mx[None])
    en = jnp.exp2(mn[None] - p3)
    rp = _recip(_allreduce_pair(jnp.sum(ep, axis=0), jnp.add))
    rn = _recip(_allreduce_pair(jnp.sum(en, axis=0), jnp.add))
    pos = (ep * rp[None]).reshape(64, t)
    neg = (en * rn[None]).reshape(64, t)
    return _pack_blocks(jnp.concatenate([pos, neg], axis=0))


def _silu(x):
    h = 0.5 * x
    return h + h * jnp.tanh(h)


def _kernel(x_hbm, wqkv_hbm, wphi_hbm, wo_hbm, wr_hbm, wg_hbm, wu_hbm, wd_hbm,
            out_hbm,
            x_v, w_v, wphi_v, wr_v, wo_v, wg_v, wu_v, wd_v,
            bq, ak, av, aq, bo, kv_acc, m_v, wr2, r_v, y_acc, xb_v, hb_v, pq0_v,
            out_v, zero_s, sem, sem_o, *ao_v):
    def x_copy(i):
        return pltpu.make_async_copy(x_hbm.at[0, pl.ds(i * T, T), :],
                                     x_v.at[pl.ds(i * T, T), :], sem.at[i])

    def w_copy(m, j):
        return pltpu.make_async_copy(
            wqkv_hbm.at[:, m * D + j * 256:m * D + (j + 1) * 256],
            w_v.at[m, :, j * 256:(j + 1) * 256], sem.at[NT + 6 + 4 * m + j])

    wphi_copy = pltpu.make_async_copy(wphi_hbm, wphi_v, sem.at[NT])
    wr_copy = pltpu.make_async_copy(wr_hbm, wr_v, sem.at[NT + 1])
    wo_copy = pltpu.make_async_copy(wo_hbm, wo_v, sem.at[NT + 2])
    wg_copy = pltpu.make_async_copy(wg_hbm, wg_v, sem.at[NT + 3])
    wu_copy = pltpu.make_async_copy(wu_hbm, wu_v, sem.at[NT + 4])
    wd_copy = pltpu.make_async_copy(wd_hbm, wd_v, sem.at[NT + 5])

    def out_copy(i, slot):
        return pltpu.make_async_copy(out_v.at[slot],
                                     out_hbm.at[0, pl.ds(i * T, T), :],
                                     sem_o.at[slot])

    wphi_copy.start()
    wr_copy.start()
    x_copy(0).start()
    for j in range(NJ):
        w_copy(1, j).start()
        w_copy(2, j).start()
    x_copy(1).start()
    x_copy(2).start()
    wo_copy.start()
    for i in range(3, NT):
        x_copy(i).start()
    for j in range(NJ):
        w_copy(0, j).start()
    wg_copy.start()
    wu_copy.start()
    wd_copy.start()

    zero_s[0] = 0
    kv_acc[...] = jnp.zeros_like(kv_acc)
    y_acc[...] = jnp.zeros_like(y_acc)
    hb_v[...] = jnp.zeros_like(hb_v)

    with jax.named_scope('wphi'):
        wphi_copy.wait()
    wr_copy.wait()
    row = jax.lax.broadcasted_iota(I32, (128, DH), 0)
    col = jax.lax.broadcasted_iota(I32, (128, DH), 1)
    sel = jnp.where(((row % 64) // 16) * 8 + row % 8 == col, 1.0, 0.0).astype(BF16)
    wall = wphi_v[...].reshape(H * DH, DH)
    phit = _dot_nt(sel, wall)
    row = jax.lax.broadcasted_iota(I32, (128, D), 0)
    col = jax.lax.broadcasted_iota(I32, (128, D), 1)
    keep = (2 * (row // 64) + (row // 8) % 2) == ((col % 128) // DH)
    phit = jnp.where(keep, phit, 0.0).astype(BF16)


    def fold(which, dst, j):
        wt = []
        for g in (2 * j, 2 * j + 1):
            wt.append(_dot_nt(phit[:, g * 128:(g + 1) * 128],
                              w_v[which, :, g * 128:(g + 1) * 128]) * LOG2E)
        w0, w1 = wt
        cs = _lhs_combos(w0[:, :DHALF], w0[:, DHALF:], w1[:, :DHALF], w1[:, DHALF:])
        for k in range(7):
            dst[k, j * 64:(j + 1) * 64, :] = _pack_blocks(cs[k])

    def packed_combos(fn, u11, u12, u21, u22):
        parts = [_unpack2(u) for u in (u11, u12, u21, u22)]
        ev = fn(*[p[0] for p in parts])
        od = fn(*[p[1] for p in parts])
        return [_pack2(e, o) for e, o in zip(ev, od)]

    def prep_v(j):
        w0, w1 = [_u32(w_v[2, :, g * 128:(g + 1) * 128].T) for g in (2 * j, 2 * j + 1)]
        cs = packed_combos(_lhs_combos, w0[:, :DHALF], w0[:, DHALF:],
                           w1[:, :DHALF], w1[:, DHALF:])
        cs[2], cs[3] = w0[:, :DHALF], w1[:, DHALF:]
        for k in range(7):
            av[k, j * 64:(j + 1) * 64, :] = cs[k]

    def ln_chunk(n, c):
        ys = []
        for h in range(2):
            r0 = n * T + h * TH + c * 16
            if not isinstance(r0, int):
                r0 = pl.multiple_of(r0, 16)
            ys += [_layernorm(xr) for xr in _unpack2(_u32(x_v[pl.ds(r0, 16), :]))]
        cs = []
        for t in range(2):
            ya, yb = ys[t], ys[2 + t]
            cs.append(_rhs_combos(ya[:, :DHALF], yb[:, :DHALF], ya[:, DHALF:], yb[:, DHALF:])
                      + [ya[:, DHALF:], yb[:, :DHALF]])
        cs = [_pack2(e, o) for e, o in zip(*cs)]
        for k in range(9):
            bq[n, k, c * 8:(c + 1) * 8, :] = cs[k]
        return cs

    def wo_piece(c, q):
        r0 = (c // 2) * 256 + (c % 2) * 64 + q * 16
        o0 = c * 32 + q * 8
        if not isinstance(c, int):
            r0 = pl.multiple_of(r0, 16)
            o0 = pl.multiple_of(o0, 8)
        w0 = _u32(wo_v[pl.ds(r0, 16), :])
        w1 = _u32(wo_v[pl.ds(r0 + 128, 16), :])

        def cols(w, par):
            return jnp.concatenate(
                [w[:, (2 * q + par) * 128:(2 * q + par + 1) * 128] for q in range(4)], axis=1)
        blocks = [cols(w0, 0), cols(w0, 1), cols(w1, 0), cols(w1, 1)]
        cs = packed_combos(_rhs_combos, *blocks)
        cs[1], cs[4] = blocks[0], blocks[3]
        for k in range(7):
            bo[k, pl.ds(o0, 8), :] = cs[k]
        return cs

    class Sched:
        def __init__(self, never):
            self.never = never
            self.slot = 0
            self.jobs = {}
            self.deps = {}

        def at(self, slot, fn):
            self.jobs.setdefault(slot, []).append(fn)

        def need(self, pos, vals):
            slot, r = int(pos), int(round((pos - int(pos)) * 8))
            d = self.deps.setdefault(slot, {})
            c = (slot + r) % 4
            d.setdefault((r, c), []).extend(vals)

        def gate(self, lhs):
            nc = lhs.shape[1] // 128
            deps = {}
            for (r, c), v in self.deps.pop(self.slot, {}).items():
                deps.setdefault((r, c % nc), []).extend(v)
            return _gate(lhs, deps, self.never)

        def after(self, step, done):
            for fn in self.jobs.pop(self.slot, []):
                fn()
            self.slot += 1

    def proj(sch, a_ref, j, b, extra=None):
        def prod(k, step):
            lhs = sch.gate(a_ref[k, j * 64:(j + 1) * 64, :])
            if extra is not None and k in (1, 2, 3, 4):
                r_ = _dot_nt(_bf(jnp.concatenate([lhs, wr2[...]], axis=0)), b[k])
                extra[k] = r_[128:136]
                return r_[0:128]
            return _dot_nt(_bf(lhs), b[k])
        c11, c12, c21, c22 = _strassen(prod, sch.after)
        return (jnp.concatenate([c11, c12], axis=1),
                jnp.concatenate([c21, c22], axis=1))

    wr = wr_v[...].astype(F32)
    wr2[...] = _pack2(*[
        jnp.concatenate([jnp.broadcast_to(wr[4 * h + t:4 * h + t + 1], (8, 128))
                         for t in range(4)], axis=1) for h in range(2)])

    with jax.named_scope('x0'):
        x_copy(0).wait()
    for c in range(8):
        ln_chunk(0, c)

    ones = jnp.ones((16, T), BF16)

    def phase1(i, carry):
        first = isinstance(i, int)
        never = zero_s[0] > 0
        if first:
            nxt = 1
        else:
            nxt = jnp.minimum(i + 1, NT - 1)

            @pl.when(i + 1 < NT)
            def _():
                x_copy(i + 1).wait()

            @pl.when(i == 1)
            def _():
                wo_copy.wait()

        b = [_bf(bq[i, k]) for k in range(7)]
        pk = [None] * NJ
        vt = [None] * NJ
        sch = Sched(never)

        phis = {}

        def sm(j, g, p, due):
            phis[j, g, p] = _feature_map(pk[j][g][p * 64:(p + 1) * 64])
            if due is not None:
                sch.need(due, [phis[j, g, p]])

        def kv(j, g):
            for p in range(2):
                if (j, g, p) not in phis:
                    sm(j, g, p, None)
                lhs = jnp.concatenate([vt[j][g][p * 64:(p + 1) * 64], ones], axis=0)
                kv_acc[4 * j + 2 * g + p] += _dot_nt(lhs, _bf(phis[j, g, p]))

        def spread(vals, due, step):
            for t in range(4):
                sch.need(due + t * step, [v[:, t * 128:(t + 1) * 128] for v in vals])

        def ln_job(c, due):
            return lambda: spread(ln_chunk(nxt, c), due, _P.get('lnstep', 0.25))

        def wo_job(q, due):
            return lambda: spread(wo_piece(i - 1, q), due, _P.get('wostep', 0.25))

        if first:
            for c in range(8):
                sch.at(42, ln_job(c, 44.5 + 1.375 * c))
        else:
            for c in range(8):
                sch.at(0, ln_job(c, 14 * (c // 2) + _P.get('ln', [6, 13])[c % 2]))
            for q in range(4):
                sch.at(0, wo_job(q, 14 * q + _P.get('wo', 10)))
        for j in range(NJ):
            s0 = 14 * j + 7
            smg = _P.get('smg', [None] * 4)
            kvs = _P.get('kvs', [7, 10])
            for q in range(4):
                if smg[q] is not None:
                    due = s0 + smg[q]
                    if j == NJ - 1:
                        due = min(due, 55)
                    sch.at(s0, functools.partial(sm, j, q // 2, q % 2, due))
            if j < NJ - 1:
                sch.at(s0 + kvs[0], functools.partial(kv, j, 0))
                sch.at(s0 + kvs[1], functools.partial(kv, j, 1))

        def wait(name, *copies):
            with jax.named_scope(name):
                for cp in copies:
                    cp.wait()

        if first:
            wait('wk0', w_copy(1, 0))
            fold(1, ak, 0)
        for j in range(NJ):
            if first:
                if j < 2:
                    wait('wv%d' % j, w_copy(2, j))
                if j == 3:
                    wait('x1', x_copy(1))
                prep_v(j)
            pk[j] = proj(sch, ak, j, b)
            if first and j + 1 < NJ:
                if j == 0:
                    wait('wk1', w_copy(1, 1))
                else:
                    wait('wkv%d' % (j + 1), w_copy(1, j + 1), w_copy(2, j + 1))
                fold(1, ak, j + 1)
            ex = {} if j == 0 else None
            vt[j] = [v.astype(BF16) for v in proj(sch, av, j, b, ex)]
            if j == 0:
                r_v[i] = jnp.concatenate(
                    [ex[1][0:1] + ex[1][1:2] + ex[3][1:2],
                     ex[4][0:1] + ex[4][1:2] + ex[2][0:1]], axis=1)
        for g in range(2):
            kv(NJ - 1, g)
        return carry

    phase1(0, 0)
    with jax.named_scope('P1'):
        jax.lax.fori_loop(1, NT, phase1, 0)

    row = jax.lax.broadcasted_iota(I32, (MR, 128), 0)
    col = jax.lax.broadcasted_iota(I32, (MR, 128), 1)
    head = jnp.where(row < 64, row // DH, (row - 64) // 8)
    keep = head == ((col // 2) % 2)
    for p in range(NP):
        m_v[p] = _u32(jnp.where(keep, kv_acc[p], 0.0).astype(BF16))

    for q in range(4):
        wo_piece(NT - 1, q)
    for j in range(NJ):
        w_copy(0, j).wait()
    for j in range(NJ):
        fold(0, aq, j)

    r = _round(r_v[...].reshape(NT, T))
    rmax = jnp.max(jnp.max(r, axis=1, keepdims=True), axis=0, keepdims=True)
    pos = (jax.lax.broadcasted_iota(I32, (NT, T), 0) * T
           + jax.lax.broadcasted_iota(I32, (NT, T), 1))
    idx = jnp.min(jnp.where(r == rmax, pos, S))
    idx = jnp.clip(idx, 0, S - 1)
    tile = idx // T
    half = (idx % T) // TH
    sub = pl.multiple_of(((idx % TH) // 16) * 8, 8)
    xs = jnp.concatenate([bq[tile, 1 + 7 * half, pl.ds(sub, 8), :],
                          bq[tile, 7 - 3 * half, pl.ds(sub, 8), :]], axis=1)
    xs = jnp.where(jax.lax.broadcasted_iota(I32, (16, D), 0) == idx % 16,
                   _bf(xs).astype(F32), 0.0)
    xs = jnp.sum(xs, axis=0, keepdims=True)

    def lane_bcast(dst, row):
        for t in range(row.shape[1] // 128):
            dst[t * 128:(t + 1) * 128, :] = jnp.broadcast_to(
                row[:, t * 128:(t + 1) * 128], (128, 128)).T

    lane_bcast(xb_v, xs)
    router = _round(0.5 + 0.5 * jnp.tanh(0.5 * rmax))
    wg_copy.wait()
    wu_copy.wait()
    wd_copy.wait()

    first = proj(Sched(None), aq, 0, [_bf(bq[(tile + 1) % NT, k]) for k in range(7)])
    for g in range(2):
        pq0_v[g] = first[g]

    def phase2(i, carry):
        last = isinstance(i, int)
        zero = zero_s[0]
        never = zero > 0
        slot = i % 2
        n = tile if last else (tile + 1 + i) % NT

        if last:
            out_copy((tile + i - 1) % NT, slot).wait()
        else:
            @pl.when(i >= 2)
            def _():
                out_copy((tile + i - 1) % NT, slot).wait()

        s0 = pl.multiple_of(n * T, T)
        b = [_bf(bq[n, k]) for k in range(7)]
        pq = [None] * NJ
        ao = [None] * NJ
        sch = Sched(never)
        ot = {}
        pq[0] = [pq0_v[g] for g in range(2)]

        phis = {}

        def sm(j, g, p, due):
            phis[j, g, p] = _feature_map(pq[j][g][p * 64:(p + 1) * 64])
            if due is not None:
                sch.need(due, [phis[j, g, p]])

        def nd(j, g):
            parts = []
            for p in range(2):
                if (j, g, p) not in phis:
                    sm(j, g, p, None)
                r_ = _dot(_bf(m_v[4 * j + 2 * g + p]), _bf(phis[j, g, p]))
                inv = _recip(r_[64:80] + 1e-6)
                o = r_[0:64].reshape(2, 4, 8, T) * inv.reshape(2, 1, 8, T)
                parts.append(o.reshape(64, T))
            ot[j, g] = jnp.concatenate(parts, axis=0)
            if g == 1:
                o0, o1 = ot[j, 0], ot[j, 1]
                cs = _lhs_combos(o0[:, :TH], o1[:, :TH], o0[:, TH:], o1[:, TH:])
                for k in range(7):
                    ao_v[2 * k + j // 2][zero, :, (j % 2) * 128:(j % 2 + 1) * 128] = (
                        _u32(cs[k].astype(BF16).T))

        if last:
            fd = (NFC - 1) * FC
        else:
            fu = pl.multiple_of(i * FC, FC)
            fd = pl.multiple_of(jnp.maximum(i - 1, 0) * FC, FC)
        ffn = {}

        FR = _P.get('fr', 64)

        def matvec(key, w, vb, due):
            t = (w.astype(F32).reshape(FR // 8, 8, 256)
                 * jnp.concatenate([vb, vb], axis=1).reshape(FR // 8, 8, 256))
            t = jnp.sum(t, axis=0)
            ffn[key] = t if key not in ffn else ffn[key] + t
            sch.need(due, [ffn[key]])

        def ffn_up(w_ref, name, cp, rb, due):
            rs = slice(rb * FR, (rb + 1) * FR)
            matvec((name, cp), w_ref[rs, pl.ds(fu + cp * 256, 256)], xb_v[rs, :], due)

        def ffn_mid():
            hg, hu = [_round(jnp.sum(jnp.concatenate([ffn[nm, 0], ffn[nm, 1]], axis=1),
                                     axis=0, keepdims=True)) for nm in 'gu']
            lane_bcast(hb_v, _round(_round(_silu(hg)) * hu))

        def ffn_down(cp, rb, due):
            cs_ = slice(cp * 256, (cp + 1) * 256)
            if rb == 0:
                ffn['y', cp] = y_acc[:, cs_]
            matvec(('y', cp), wd_v[pl.ds(fd + rb * FR, FR), cs_],
                   hb_v[rb * FR:(rb + 1) * FR, :], due)
            if rb == FC // FR - 1:
                if last:
                    ffn['row', cp] = (
                        _round(jnp.sum(ffn['y', cp], axis=0, keepdims=True)) * router)
                else:
                    y_acc[:, cs_] = ffn['y', cp]

        def eighths(x):
            return round(x * 8) / 8

        d0, d1, u0, u1 = _P.get('ffn', [1, 27.5, 28, 53])
        nd_ = 4 * FC // FR
        for t in range(nd_):
            due = eighths(d0 + (d1 - d0) * t / (nd_ - 1))
            sch.at(0, functools.partial(ffn_down, t % 4, t // 4, due))
        if not last:
            nu_ = 4 * D // FR
            for t in range(nu_):
                due = eighths(u0 + (u1 - u0) * t / (nu_ - 1))
                name, w_ref = (('g', wg_v), ('u', wu_v))[(t // 2) % 2]
                sch.at(0, functools.partial(ffn_up, w_ref, name, t % 2, t // 4, due))
            sch.at(int(u1), ffn_mid)
        for j in range(NJ):
            s1 = 7 * j
            nds = (_P.get('nds', [1, 4]) if j < NJ - 1
                   else _P.get('nds3l', [1, 2]) if last else _P.get('nds3', [1, 2]))
            sch.at(s1 + nds[0], functools.partial(nd, j, 0))
            sch.at(s1 + nds[1], functools.partial(nd, j, 1))
        for j in range(1, NJ):
            pq[j] = proj(sch, aq, j, b)
        part = {}
        if last:
            def prod_a(k, step):
                return _dot(_bf(sch.gate(ao_v[2 * k][0])), _bf(bo[k, 0:128, 0:256]))
            part = _strassen(prod_a, sch.after)
        else:
            nxt = proj(sch, aq, 0, [_bf(bq[(n + 1) % NT, k]) for k in range(7)])
            for g in range(2):
                pq0_v[g] = nxt[g]

        ER = _P.get('er', 32)
        rows = jax.lax.broadcasted_iota(I32, (ER, 256), 0) + s0
        ne_ = T // ER
        gates = {}

        def gate_part(c, e, due):
            r0 = e * ER
            h, rh = r0 // TH, r0 % TH
            blk = ((1, 7), (8, 4))[h][c // 2]
            bb = _bf(bq[n, blk, rh // 2:(rh + ER) // 2,
                        (c % 2) * 256:(c % 2 + 1) * 256]).astype(F32)
            if last:
                bb = bb + jnp.where(rows + r0 == idx, ffn['row', c], 0.0)
            gates[c, e] = _silu(bb)
            if due is not None:
                sch.need(due, [gates[c, e]])

        def epilogue(c, cc, e, due):
            r0 = e * ER
            h, rh = r0 // TH, r0 % TH
            cs = slice(c * 256, (c + 1) * 256)
            rs = slice(rh, rh + ER)
            if (c, e) not in gates:
                gate_part(c, e, None)
            xr = x_v[pl.ds(s0 + r0, ER), cs].astype(F32)
            sv = jnp.concatenate([cc[2 * h][rs], cc[2 * h + 1][rs]], axis=1)
            res = xr + sv * gates[c, e]
            out_v[slot, r0:r0 + ER, cs] = res.astype(BF16)
            if due is not None:
                sch.need(due, [res])

        def out_cols(c):
            cs = slice(c * 256, (c + 1) * 256)
            return pltpu.make_async_copy(out_v.at[slot, :, cs],
                                         out_hbm.at[0, pl.ds(s0, T), cs], sem_o.at[2 + c])

        e0, e1 = _P.get('epi', [1.5, 6.5])
        g0, g1 = _P.get('gl', [0.25, 5.5])
        end = sch.slot + 28 - (7 if last else 0)
        for e in range(ne_):
            sch.at(end - 8, functools.partial(
                gate_part, 3, e, eighths(end - 7 + g0 + (g1 - g0) * e / (ne_ - 1))))
        pending = []
        c = 0
        while c < 4:
            if last and c == 0:
                def prod(k, step):
                    return _dot(_bf(sch.gate(ao_v[2 * k + 1][0])),
                                _bf(bo[k, 128:256, 0:256]))
                cc2 = [u + v for u, v in zip(part, _strassen(prod, sch.after))]
                blocks = [(t, [v[:, t * 128:(t + 1) * 128] for v in cc2]) for t in range(2)]
            else:
                def prod(k, step):
                    return _dot(_bf(sch.gate(jnp.concatenate(
                        [ao_v[2 * k][0], ao_v[2 * k + 1][0]], axis=1))),
                                _bf(bo[k, :, c * 128:(c + 1) * 128]))
                blocks = [(c, _strassen(prod, sch.after))]
            if last:
                for t in pending:
                    out_cols(t).start()
                pending = []
            nb = len(blocks) * ne_
            for q in range(nb):
                t, cc = blocks[q // ne_]
                due = eighths(sch.slot + e0 + (e1 - e0) * q / (nb - 1))
                epilogue(t, cc, q % ne_, due if t < 3 else None)
            pending = [t for t, _ in blocks]
            c += len(blocks)
        if last:
            out_cols(3).start()
            out_copy((tile + i) % NT, 1 - slot).wait()
            for t in range(4):
                out_cols(t).wait()
        else:
            out_copy(n, slot).start()
        return carry

    with jax.named_scope('P2'):
        jax.lax.fori_loop(0, NT - 1, phase2, 0)
    phase2(NT - 1, 0)


@jax.jit
def pallas_recurrent_scan__linear_kernel_hedgehog__moe_arch_mod__prompt_kernel(
    A_x: jax.Array,
    A_wqkv: jax.Array,
    A_w_phi: jax.Array,
    A_wo: jax.Array,
    B_x: jax.Array,
    B_w_r: jax.Array,
    B_w_gate: jax.Array,
    B_w_up: jax.Array,
    B_w_down: jax.Array,
):
    del B_x
    any_spec = pl.BlockSpec(memory_space=pl.ANY)
    return pl.pallas_call(
        _kernel,
        out_shape=jax.ShapeDtypeStruct((1, S, D), BF16),
        in_specs=[any_spec] * 8,
        out_specs=any_spec,
        scratch_shapes=[
            pltpu.VMEM((S, D), BF16),
            pltpu.VMEM((3, D, D), BF16),
            pltpu.VMEM((H, DH, DH), BF16),
            pltpu.VMEM((8, 128), BF16),
            pltpu.VMEM((D, D), BF16),
            pltpu.VMEM((D, F), BF16),
            pltpu.VMEM((D, F), BF16),
            pltpu.VMEM((F, D), BF16),
            pltpu.VMEM((NT, 9, TH // 2, DHALF), U32),
            pltpu.VMEM((7, 256, DHALF), U32),
            pltpu.VMEM((7, 256, DHALF), U32),
            pltpu.VMEM((7, 256, DHALF), U32),
            pltpu.VMEM((7, 256, DHALF), U32),
            pltpu.VMEM((NP, MR, 128), F32),
            pltpu.VMEM((NP, MR // 2, 128), U32),
            pltpu.VMEM((8, DHALF), U32),
            pltpu.VMEM((NT, 1, T), F32),
            pltpu.VMEM((8, D), F32),
            pltpu.VMEM((D, 128), F32),
            pltpu.VMEM((FC, 128), F32),
            pltpu.VMEM((2, 128, T), F32),
            pltpu.VMEM((2, T, D), BF16),
            pltpu.SMEM((1,), I32),
            pltpu.SemaphoreType.DMA((NT + 18,)),
            pltpu.SemaphoreType.DMA((6,)),
        ] + [pltpu.VMEM((1, TH // 2, 256), U32)] * 14,
        compiler_params=pltpu.CompilerParams(vmem_limit_bytes=100 * 1024 * 1024),
    )(A_x, A_wqkv, A_w_phi, A_wo, B_w_r.reshape(8, 128), B_w_gate, B_w_up, B_w_down)
```

```python
import functools
import os
import json
_P = json.loads(os.environ.get('KP', '{}'))

import jax
import jax.numpy as jnp
import jax.experimental.pallas as pl
import jax.experimental.pallas.tpu as pltpu

S, D, H, DH, F = 2048, 1024, 32, 32, 3584
T = 256
TH = T // 2
DHALF = D // 2
NT = S // T
NJ = 4
NP = D // 64
MR = 80
FC = 512
NFC = F // FC
NF = _P.get('nf', 2)
ORDER = 'k0 x0 x1 k1 k2 k3 v0 v1 v2 v3 x2'
PROG = ('w:x1 L1:3:6 K0a w:k1 f1 K0b S0a K1a S0b K1b '
        'w:k2,k3,v0 f2 f3 p0:14:18 S1a K2a S1b K2b S2a K3a S2b K3b '
        'w:v1,v2,v3,x2 p1:3:8 p2:16:21 p3:30:35 L2:6:52 V0a X0a V0b '
        'X0b V1a X1a V1b X1b V2a X2a V2b X2b V3a X3a V3b Y3b')
LOG2E = 1.4426950408889634
F32, BF16, U32, I32 = jnp.float32, jnp.bfloat16, jnp.uint32, jnp.int32

_NT_DIMS = (((1,), (1,)), ((), ()))


def _dot_nt(a, b):
    return jax.lax.dot_general(a, b, _NT_DIMS, preferred_element_type=F32)


def _dot(a, b):
    return jnp.dot(a, b, preferred_element_type=F32)


def _u32(v):
    return pltpu.bitcast(v, U32) if v.dtype != U32 else v


def _pack2(even, odd):
    return pltpu.pack_elementwise([even, odd], packed_dtype=BF16)


def _unpack2(u):
    return [pltpu.unpack_elementwise(u, index=i, packed_dtype=BF16, unpacked_dtype=F32)
            for i in range(2)]


def _pack_blocks(v):
    r, c = v.shape
    v4 = v.reshape(r // 16, 2, 8, c)
    return _pack2(v4[:, 0], v4[:, 1]).reshape(r // 2, c)


def _recip(x):
    r = pl.reciprocal(x, approx=True)
    return r * (2.0 - x * r)


def _bf(v):
    return pltpu.bitcast(v, BF16)


def _round(v):
    return v.astype(BF16).astype(F32)


def _or_all(vals):
    ts = []
    for v in vals:
        u = _u32(v)
        for a in range(u.shape[0] // 8):
            for b in range(u.shape[1] // 128):
                ts.append(u[a * 8:(a + 1) * 8, b * 128:(b + 1) * 128])
    while len(ts) > 1:
        ts = [ts[i] | ts[i + 1] if i + 1 < len(ts) else ts[i] for i in range(0, len(ts), 2)]
    return ts[0]


def _gate(lhs_u32, deps, never):
    if not deps:
        return lhs_u32
    rows = []
    for r in range(lhs_u32.shape[0] // 8):
        row = lhs_u32[r * 8:(r + 1) * 8]
        cs = [c for (r_, c) in deps if r_ == r]
        if cs:
            row = jnp.concatenate(
                [jnp.where(never, _or_all(deps[r, c]), row[:, c * 128:(c + 1) * 128])
                 if c in cs else row[:, c * 128:(c + 1) * 128]
                 for c in range(lhs_u32.shape[1] // 128)], axis=1)
        rows.append(row)
    return jnp.concatenate(rows, axis=0)


def _layernorm(x):
    m = jnp.mean(x, axis=-1, keepdims=True)
    mb = _round(m)
    xc = x - mb
    dm = m - mb
    v = jnp.mean(xc * xc, axis=-1, keepdims=True) - dm * dm
    a = _round(_round(v) + 1e-5)
    rs = jax.lax.rsqrt(a)
    sd = a * rs
    sd = _round(sd + (0.5 * rs) * (a - sd * sd))
    return xc * _recip(sd)


def _lhs_combos(a11, a12, a21, a22):
    return [a11 + a22, a21 + a22, a11, a22, a11 + a12, a21 - a11, a12 - a22]


def _rhs_combos(b11, b12, b21, b22):
    return [b11 + b22, b11, b12 - b22, b21 - b11, b22, b11 + b12, b21 + b22]


def _strassen(prod, after=None):
    done = {}

    def p(k, step):
        return prod(k, step)

    def hook(step):
        if after is not None:
            after(step, done)

    m1 = p(0, 0)
    hook(0)
    m4 = p(3, 1)
    hook(1)
    m5 = p(4, 2)
    hook(2)
    m7 = p(6, 3)
    done[0] = m1 + m4 - m5 + m7
    hook(3)
    m3 = p(2, 4)
    done[1] = m3 + m5
    hook(4)
    m2 = p(1, 5)
    done[2] = m2 + m4
    hook(5)
    m6 = p(5, 6)
    done[3] = m1 - m2 + m3 + m6
    hook(6)
    return done[0], done[1], done[2], done[3]


def _allreduce_pair(x, op):
    x = op(x, pltpu.roll(x, 2, axis=0))
    return op(x, pltpu.roll(x, 4, axis=0))


def _feature_map(p):
    t = p.shape[1]
    p3 = p.reshape(8, 8, t)
    mx = _allreduce_pair(jnp.max(p3, axis=0), jnp.maximum)
    mn = _allreduce_pair(jnp.min(p3, axis=0), jnp.minimum)
    ep = jnp.exp2(p3 - mx[None])
    en = jnp.exp2(mn[None] - p3)
    rp = _recip(_allreduce_pair(jnp.sum(ep, axis=0), jnp.add))
    rn = _recip(_allreduce_pair(jnp.sum(en, axis=0), jnp.add))
    pos = (ep * rp[None]).reshape(64, t)
    neg = (en * rn[None]).reshape(64, t)
    return _pack_blocks(jnp.concatenate([pos, neg], axis=0))


def _silu(x):
    h = 0.5 * x
    return h + h * jnp.tanh(h)


def _kernel(x_hbm, wqkv_hbm, wphi_hbm, wo_hbm, wr_hbm, wg_hbm, wu_hbm, wd_hbm,
            out_hbm,
            x_v, w_v, wphi_v, wr_v, wo_v, wg_v, wu_v, wd_v,
            bq, ak, av, aq, bo, kv_acc, m_v, wr2, r_v, y_acc, xb_v, hb_v, pq0_v,
            out_v, zero_s, sem, sem_o, *ao_v):
    def x_copy(i):
        return pltpu.make_async_copy(x_hbm.at[0, pl.ds(i * T, T), :],
                                     x_v.at[pl.ds(i * T, T), :], sem.at[i])

    def w_copy(m, j):
        return pltpu.make_async_copy(
            wqkv_hbm.at[:, m * D + j * 256:m * D + (j + 1) * 256],
            w_v.at[m, :, j * 256:(j + 1) * 256], sem.at[NT + 6 + 4 * m + j])

    wphi_copy = pltpu.make_async_copy(wphi_hbm, wphi_v, sem.at[NT])
    wr_copy = pltpu.make_async_copy(wr_hbm, wr_v, sem.at[NT + 1])
    wo_copy = pltpu.make_async_copy(wo_hbm, wo_v, sem.at[NT + 2])
    wg_copy = pltpu.make_async_copy(wg_hbm, wg_v, sem.at[NT + 3])
    wu_copy = pltpu.make_async_copy(wu_hbm, wu_v, sem.at[NT + 4])
    wd_copy = pltpu.make_async_copy(wd_hbm, wd_v, sem.at[NT + 5])

    def out_copy(i, slot):
        return pltpu.make_async_copy(out_v.at[slot],
                                     out_hbm.at[0, pl.ds(i * T, T), :],
                                     sem_o.at[slot])

    wphi_copy.start()
    wr_copy.start()
    def named_copy(nm):
        t = int(nm[1])
        return x_copy(t) if nm[0] == 'x' else w_copy({'k': 1, 'v': 2}[nm[0]], t)

    for nm in _P.get('order', ORDER).split():
        named_copy(nm).start()
    x_copy(NF + 1).start()
    wo_copy.start()
    for i in range(NF + 2, NT):
        x_copy(i).start()
    for j in range(NJ):
        w_copy(0, j).start()
    wg_copy.start()
    wu_copy.start()
    wd_copy.start()

    zero_s[0] = 0
    kv_acc[...] = jnp.zeros_like(kv_acc)
    y_acc[...] = jnp.zeros_like(y_acc)
    hb_v[...] = jnp.zeros_like(hb_v)

    with jax.named_scope('wphi'):
        wphi_copy.wait()
    wr_copy.wait()
    row = jax.lax.broadcasted_iota(I32, (128, DH), 0)
    col = jax.lax.broadcasted_iota(I32, (128, DH), 1)
    sel = jnp.where(((row % 64) // 16) * 8 + row % 8 == col, 1.0, 0.0).astype(BF16)
    wall = wphi_v[...].reshape(H * DH, DH)
    phit = _dot_nt(sel, wall)
    row = jax.lax.broadcasted_iota(I32, (128, D), 0)
    col = jax.lax.broadcasted_iota(I32, (128, D), 1)
    keep = (2 * (row // 64) + (row // 8) % 2) == ((col % 128) // DH)
    phit = jnp.where(keep, phit, 0.0).astype(BF16)


    def fold(which, dst, j):
        wt = []
        for g in (2 * j, 2 * j + 1):
            wt.append(_dot_nt(phit[:, g * 128:(g + 1) * 128],
                              w_v[which, :, g * 128:(g + 1) * 128]) * LOG2E)
        w0, w1 = wt
        cs = _lhs_combos(w0[:, :DHALF], w0[:, DHALF:], w1[:, :DHALF], w1[:, DHALF:])
        for k in range(7):
            dst[k, j * 64:(j + 1) * 64, :] = _pack_blocks(cs[k])

    def packed_combos(fn, u11, u12, u21, u22):
        parts = [_unpack2(u) for u in (u11, u12, u21, u22)]
        ev = fn(*[p[0] for p in parts])
        od = fn(*[p[1] for p in parts])
        return [_pack2(e, o) for e, o in zip(ev, od)]

    def prep_v(j, sch=None):
        ws = [_u32(w_v[2, :, g * 128:(g + 1) * 128]) for g in (2 * j, 2 * j + 1)]
        if sch is not None:
            ws = [sch.hold(w, [(8 * q, 0) for q in range(8)]) for w in ws]
        w0, w1 = [_u32(_bf(w).T) for w in ws]
        cs = packed_combos(_lhs_combos, w0[:, :DHALF], w0[:, DHALF:],
                           w1[:, :DHALF], w1[:, DHALF:])
        cs[2], cs[3] = w0[:, :DHALF], w1[:, DHALF:]
        for k in range(7):
            av[k, j * 64:(j + 1) * 64, :] = cs[k]
        return w0, w1

    def ln_chunk(n, c, sch=None):
        ys = []
        for h in range(2):
            r0 = n * T + h * TH + c * 16
            if not isinstance(r0, int):
                r0 = pl.multiple_of(r0, 16)
            xu = _u32(x_v[pl.ds(r0, 16), :])
            if sch is not None:
                xu = sch.hold(xu, [(0, 0)])
            ys += [_layernorm(xr) for xr in _unpack2(xu)]
        cs = []
        for t in range(2):
            ya, yb = ys[t], ys[2 + t]
            cs.append(_rhs_combos(ya[:, :DHALF], yb[:, :DHALF], ya[:, DHALF:], yb[:, DHALF:])
                      + [ya[:, DHALF:], yb[:, :DHALF]])
        cs = [_pack2(e, o) for e, o in zip(*cs)]
        for k in range(9):
            bq[n, k, c * 8:(c + 1) * 8, :] = cs[k]
        return cs

    def wo_piece(c, q):
        r0 = (c // 2) * 256 + (c % 2) * 64 + q * 16
        o0 = c * 32 + q * 8
        if not isinstance(c, int):
            r0 = pl.multiple_of(r0, 16)
            o0 = pl.multiple_of(o0, 8)
        w0 = wo_v[pl.ds(r0, 16), :].astype(F32)
        w1 = wo_v[pl.ds(r0 + 128, 16), :].astype(F32)

        def cols(w, par):
            return jnp.concatenate(
                [w[:, (2 * q + par) * 128:(2 * q + par + 1) * 128] for q in range(4)], axis=1)
        cs = [_pack_blocks(v) for v in
              _rhs_combos(cols(w0, 0), cols(w0, 1), cols(w1, 0), cols(w1, 1))]
        for k in range(7):
            bo[k, pl.ds(o0, 8), :] = cs[k]
        return cs

    class Sched:
        def __init__(self, never):
            self.never = never
            self.slot = 0
            self.gated = 0
            self.token = None
            self.jobs = {}
            self.deps = {}

        def at(self, slot, fn):
            self.jobs.setdefault(slot, []).append(fn)

        def need(self, pos, vals):
            slot, r = divmod(int(round(pos * 8)), 8)
            assert slot >= self.gated, (pos, self.slot)
            d = self.deps.setdefault(slot, {})
            c = (slot + r) % 4
            d.setdefault((r, c), []).extend(vals)

        def gate(self, lhs):
            nc = lhs.shape[1] // 128
            self.gated = self.slot + 1
            deps = {}
            for (r, c), v in self.deps.pop(self.slot, {}).items():
                deps.setdefault((r, c % nc), []).extend(v)
            return _gate(lhs, deps, self.never)

        def hold(self, u, blocks):
            if self.token is None:
                return u
            return _gate(u, {rc: [self.token] for rc in blocks}, self.never)

        def after(self, step, done):
            for fn in self.jobs.pop(self.slot, []):
                fn()
            self.slot += 1

    def proj(sch, a_ref, j, b, extra=None, early=None):
        def prod(k, step):
            lhs = sch.gate(a_ref[k, j * 64:(j + 1) * 64, :])
            if extra is not None and k in (1, 2, 3, 4):
                r_ = _dot_nt(_bf(jnp.concatenate([lhs, wr2[...]], axis=0)), b[k])
                extra[k] = r_[128:136]
                r_ = r_[0:128]
            else:
                r_ = _dot_nt(_bf(lhs), b[k])
            sch.token = r_[0:8, 0:128]
            return r_
        def after(step, done):
            if step == 4 and early is not None:
                early[j] = [jnp.concatenate([done[0], done[1]], axis=1), None]
            sch.after(step, done)
        c11, c12, c21, c22 = _strassen(prod, after)
        return (jnp.concatenate([c11, c12], axis=1),
                jnp.concatenate([c21, c22], axis=1))

    wr = wr_v[...].astype(F32)
    wr2[...] = _pack2(*[
        jnp.concatenate([jnp.broadcast_to(wr[4 * h + t:4 * h + t + 1], (8, 128))
                         for t in range(4)], axis=1) for h in range(2)])

    with jax.named_scope('k0'):
        w_copy(1, 0).wait()
    fold(1, ak, 0)
    with jax.named_scope('x0'):
        x_copy(0).wait()
    for c in range(8):
        ln_chunk(0, c)

    ones = _u32(jnp.ones((16, T), BF16))

    class KVTile:
        def __init__(self, sch, i):
            self.sch, self.i = sch, i
            self.b = None
            self.pk, self.vt, self.phis = {}, {}, {}

        def operands(self):
            if self.b is None:
                self.b = [_bf(bq[self.i, k]) for k in range(7)]
            return self.b

        def kproj(self, j):
            self.pk[j] = proj(self.sch, ak, j, self.operands())

        def vproj(self, j):
            ex = {} if j == 0 else None
            self.vt[j] = [_pack_blocks(v)
                          for v in proj(self.sch, av, j, self.operands(), ex)]
            if j == 0:
                r_v[self.i] = jnp.concatenate(
                    [ex[1][0:1] + ex[1][1:2] + ex[3][1:2],
                     ex[4][0:1] + ex[4][1:2] + ex[2][0:1]], axis=1)

        def sm(self, j, g, p, due=None, step=0):
            phi = _feature_map(self.pk[j][g][p * 64:(p + 1) * 64])
            self.phis[j, g, p] = phi
            if due is not None:
                for t in range(2):
                    self.sch.need(due - step * (1 - t), [phi[:, t * 128:(t + 1) * 128]])

        def kv(self, j, g):
            for p in range(2):
                if (j, g, p) not in self.phis:
                    self.sm(j, g, p)
                lhs = _bf(jnp.concatenate(
                    [self.vt[j][g][p * 32:(p + 1) * 32], ones], axis=0))
                kv_acc[4 * j + 2 * g + p] += _dot_nt(lhs, _bf(self.phis[j, g, p]))

    def spread(sch, vals, due, step=0.25):
        for t in range(4):
            sch.need(due + t * step, [v[:, t * 128:(t + 1) * 128] for v in vals])

    def eighths(x):
        return round(x * 8) / 8

    def first_tiles():
        sch = Sched(zero_s[0] > 0)
        tiles = {'a': KVTile(sch, 0), 'b': KVTile(sch, 1)}
        for op in _P.get('prog', PROG).split():
            kind, arg = op[0], op[1:2]
            if kind == 'w':
                with jax.named_scope(op):
                    for nm in op[2:].split(','):
                        named_copy(nm).wait()
            elif kind == 'f':
                fold(1, ak, int(arg))
            elif kind == 'p':
                _, rel, d0 = op.split(':')

                def job(j=int(arg), base=sch.slot + float(d0), rel=int(rel)):
                    ws = prep_v(j, sch if rel >= 0 else None)
                    for q in range(8):
                        sch.need(base + q * _P.get('pvs', 0.5),
                                 [w[:, q * 128:(q + 1) * 128] for w in ws])
                if int(rel) < 0:
                    job()
                else:
                    sch.at(sch.slot + int(rel), job)
            elif kind == 'U':
                for c in range(8):
                    ln_chunk(int(arg), c)
            elif kind == 'L':
                _, l0, l1 = op.split(':')
                for c in range(8):
                    due = eighths(sch.slot + float(l0) + (float(l1) - float(l0)) * c / 7)
                    rel = int(due - _P.get('lrel', 4.5))

                    def job(n=int(arg), c=c, due=due, held=rel >= sch.slot):
                        spread(sch, ln_chunk(n, c, sch if held else None), due)
                    if rel >= sch.slot:
                        sch.at(rel, job)
                    else:
                        job()
            elif kind == 'S':
                a0, a1 = _P.get('s1', [1.5, 6.5])
                st_ = (a1 - a0) / 7
                for q in range(4):
                    tiles[op[2]].sm(int(arg), q // 2, q % 2,
                                    eighths(sch.slot + a0 + st_ * (2 * q + 1)), eighths(st_))
            elif kind == 'K':
                tiles[op[2]].kproj(int(arg))
            elif kind == 'V':
                tiles[op[2]].vproj(int(arg))
            elif kind == 'X':
                sch.at(sch.slot + 1, functools.partial(tiles[op[2]].kv, int(arg), 0))
                sch.at(sch.slot + 4, functools.partial(tiles[op[2]].kv, int(arg), 1))
            elif kind == 'Y':
                for g in range(2):
                    tiles[op[2]].kv(int(arg), g)
        assert not sch.jobs and not sch.deps, (sch.jobs.keys(), sch.deps.keys())

    def phase1(i, carry):
        nxt = jnp.minimum(i + 1, NT - 1)

        @pl.when(i + 1 < NT)
        def _():
            x_copy(i + 1).wait()

        @pl.when(i == NF)
        def _():
            wo_copy.wait()

        sch = Sched(zero_s[0] > 0)
        tl = KVTile(sch, i)
        tl.operands()
        for c in range(8):
            spread(sch, ln_chunk(nxt, c), 14 * (c // 2) + _P.get('ln', [6, 13])[c % 2])
        for q in range(4):
            spread(sch, wo_piece(i - NF, q), 14 * q + _P.get('wo', 10))
        for j in range(NJ - 1):
            for g in range(2):
                sch.at(14 * j + 7 + _P.get('kvs', [7, 10])[g],
                       functools.partial(tl.kv, j, g))
        for j in range(NJ):
            tl.kproj(j)
            tl.vproj(j)
        for g in range(2):
            tl.kv(NJ - 1, g)
        return carry

    first_tiles()
    with jax.named_scope('P1'):
        jax.lax.fori_loop(NF, NT, phase1, 0)

    row = jax.lax.broadcasted_iota(I32, (MR, 128), 0)
    col = jax.lax.broadcasted_iota(I32, (MR, 128), 1)
    head = jnp.where(row < 64, row // DH, (row - 64) // 8)
    keep = head == ((col // 2) % 2)
    for p in range(NP):
        m_v[p] = _u32(jnp.where(keep, kv_acc[p], 0.0).astype(BF16))

    for c in range(NT - NF, NT):
        for q in range(4):
            wo_piece(c, q)
    for j in range(NJ):
        w_copy(0, j).wait()
    for j in range(NJ):
        fold(0, aq, j)

    r = _round(r_v[...].reshape(NT, T))
    rmax = jnp.max(jnp.max(r, axis=1, keepdims=True), axis=0, keepdims=True)
    pos = (jax.lax.broadcasted_iota(I32, (NT, T), 0) * T
           + jax.lax.broadcasted_iota(I32, (NT, T), 1))
    idx = jnp.min(jnp.where(r == rmax, pos, S))
    idx = jnp.clip(idx, 0, S - 1)
    tile = idx // T
    half = (idx % T) // TH
    sub = pl.multiple_of(((idx % TH) // 16) * 8, 8)
    xs = jnp.concatenate([bq[tile, 1 + 7 * half, pl.ds(sub, 8), :],
                          bq[tile, 7 - 3 * half, pl.ds(sub, 8), :]], axis=1)
    xs = jnp.where(jax.lax.broadcasted_iota(I32, (16, D), 0) == idx % 16,
                   _bf(xs).astype(F32), 0.0)
    xs = jnp.sum(xs, axis=0, keepdims=True)

    def lane_bcast(dst, row):
        for t in range(row.shape[1] // 128):
            dst[t * 128:(t + 1) * 128, :] = jnp.broadcast_to(
                row[:, t * 128:(t + 1) * 128], (128, 128)).T

    lane_bcast(xb_v, xs)
    router = _round(0.5 + 0.5 * jnp.tanh(0.5 * rmax))
    wg_copy.wait()
    wu_copy.wait()
    wd_copy.wait()

    first = proj(Sched(None), aq, 0, [_bf(bq[(tile + 1) % NT, k]) for k in range(7)])
    for g in range(2):
        pq0_v[g] = first[g]

    def phase2(i, carry):
        last = isinstance(i, int)
        zero = zero_s[0]
        never = zero > 0
        slot = i % 2
        n = tile if last else (tile + 1 + i) % NT

        if last:
            out_copy((tile + i - 1) % NT, slot).wait()
        else:
            @pl.when(i >= 2)
            def _():
                out_copy((tile + i - 1) % NT, slot).wait()

        s0 = pl.multiple_of(n * T, T)
        b = [_bf(bq[n, k]) for k in range(7)]
        pq = [None] * NJ
        ao = [None] * NJ
        sch = Sched(never)
        ot = {}
        pq[0] = [pq0_v[g] for g in range(2)]

        phis = {}

        def sm(j, g, p, due, step=0):
            phis[j, g, p] = _feature_map(pq[j][g][p * 64:(p + 1) * 64])
            if due is not None:
                for t in range(2):
                    sch.need(max(due - step * (1 - t), sch.slot + 1),
                             [phis[j, g, p][:, t * 128:(t + 1) * 128]])

        def nd(j, g):
            parts = []
            for p in range(2):
                if (j, g, p) not in phis:
                    sm(j, g, p, None)
                r_ = _dot(_bf(m_v[4 * j + 2 * g + p]), _bf(phis[j, g, p]))
                inv = _recip(r_[64:80] + 1e-6)
                o = r_[0:64].reshape(2, 4, 8, T) * inv.reshape(2, 1, 8, T)
                parts.append(o.reshape(64, T))
            ot[j, g] = jnp.concatenate(parts, axis=0)
            if g == 1:
                o0, o1 = ot[j, 0], ot[j, 1]
                cs = _lhs_combos(o0[:, :TH], o1[:, :TH], o0[:, TH:], o1[:, TH:])
                for k in range(7):
                    ao_v[2 * k + j // 2][zero, :, (j % 2) * 128:(j % 2 + 1) * 128] = (
                        _u32(cs[k].astype(BF16).T))

        if last:
            fd = (NFC - 1) * FC
        else:
            fu = pl.multiple_of(i * FC, FC)
            fd = pl.multiple_of(jnp.maximum(i - 1, 0) * FC, FC)
        ffn = {}

        FR = _P.get('fr', 64)

        def matvec(key, w, vb, due):
            t = (w.astype(F32).reshape(FR // 8, 8, 256)
                 * jnp.concatenate([vb, vb], axis=1).reshape(FR // 8, 8, 256))
            t = jnp.sum(t, axis=0)
            ffn[key] = t if key not in ffn else ffn[key] + t
            sch.need(due, [ffn[key]])

        def ffn_up(w_ref, name, cp, rb, due):
            rs = slice(rb * FR, (rb + 1) * FR)
            matvec((name, cp), w_ref[rs, pl.ds(fu + cp * 256, 256)], xb_v[rs, :], due)

        def ffn_mid():
            hg, hu = [_round(jnp.sum(jnp.concatenate([ffn[nm, 0], ffn[nm, 1]], axis=1),
                                     axis=0, keepdims=True)) for nm in 'gu']
            lane_bcast(hb_v, _round(_round(_silu(hg)) * hu))

        def ffn_down(cp, rb, due):
            cs_ = slice(cp * 256, (cp + 1) * 256)
            if rb == 0:
                ffn['y', cp] = y_acc[:, cs_]
            matvec(('y', cp), wd_v[pl.ds(fd + rb * FR, FR), cs_],
                   hb_v[rb * FR:(rb + 1) * FR, :], due)
            if rb == FC // FR - 1:
                if last:
                    ffn['row', cp] = (
                        _round(jnp.sum(ffn['y', cp], axis=0, keepdims=True)) * router)
                else:
                    y_acc[:, cs_] = ffn['y', cp]

        d0, d1, u0, u1 = _P.get('ffn', [1, 27.5, 28, 53])
        nd_ = 4 * FC // FR
        for t in range(nd_):
            due = eighths(d0 + (d1 - d0) * t / (nd_ - 1))
            sch.at(0, functools.partial(ffn_down, t % 4, t // 4, due))
        if not last:
            nu_ = 4 * D // FR
            for t in range(nu_):
                due = eighths(u0 + (u1 - u0) * t / (nu_ - 1))
                name, w_ref = (('g', wg_v), ('u', wu_v))[(t // 2) % 2]
                sch.at(0, functools.partial(ffn_up, w_ref, name, t % 2, t // 4, due))
            sch.at(int(u1), ffn_mid)
        for j in range(NJ):
            s1 = 7 * j
            nds = (_P.get('nds', [1, 4]) if j < NJ - 1
                   else _P.get('nds3l', [1, 2]) if last else _P.get('nds3', [1, 2]))
            phq = _P.get('phq')
            for g in range(2):
                if phq:
                    for p in range(2):
                        sch.at(s1 if (j == 0 or g == 1) else s1 - 2, functools.partial(
                            sm, j, g, p, s1 + nds[g] + 1 - phq[0] - phq[1] * (2 - 2 * p), phq[1]))
                sch.at(s1 + nds[g], functools.partial(nd, j, g))
        for j in range(1, NJ):
            pq[j] = proj(sch, aq, j, b, early=pq)
        part = {}
        if last:
            def prod_a(k, step):
                return _dot(_bf(sch.gate(ao_v[2 * k][0])), _bf(bo[k, 0:128, 0:256]))
            part = _strassen(prod_a, sch.after)
        else:
            nxt = proj(sch, aq, 0, [_bf(bq[(n + 1) % NT, k]) for k in range(7)])
            for g in range(2):
                pq0_v[g] = nxt[g]

        ER = _P.get('er', 32)
        rows = jax.lax.broadcasted_iota(I32, (ER, 256), 0) + s0
        ne_ = T // ER
        gates = {}

        def gate_part(c, e, due):
            r0 = e * ER
            h, rh = r0 // TH, r0 % TH
            blk = ((1, 7), (8, 4))[h][c // 2]
            bb = _bf(bq[n, blk, rh // 2:(rh + ER) // 2,
                        (c % 2) * 256:(c % 2 + 1) * 256]).astype(F32)
            if last:
                bb = bb + jnp.where(rows + r0 == idx, ffn['row', c], 0.0)
            gates[c, e] = _silu(bb)
            if due is not None:
                sch.need(due, [gates[c, e]])

        def epilogue(c, cc, e, due):
            r0 = e * ER
            h, rh = r0 // TH, r0 % TH
            cs = slice(c * 256, (c + 1) * 256)
            rs = slice(rh, rh + ER)
            if (c, e) not in gates:
                gate_part(c, e, None)
            xr = x_v[pl.ds(s0 + r0, ER), cs].astype(F32)
            sv = jnp.concatenate([cc[2 * h][rs], cc[2 * h + 1][rs]], axis=1)
            res = xr + sv * gates[c, e]
            out_v[slot, r0:r0 + ER, cs] = res.astype(BF16)
            if due is not None:
                sch.need(due, [res])

        def out_cols(c):
            cs = slice(c * 256, (c + 1) * 256)
            return pltpu.make_async_copy(out_v.at[slot, :, cs],
                                         out_hbm.at[0, pl.ds(s0, T), cs], sem_o.at[2 + c])

        e0, e1 = _P.get('epi', [1.5, 6.5])
        g0, g1 = _P.get('gl', [0.25, 5.5])
        end = sch.slot + 28 - (7 if last else 0)
        for e in range(ne_):
            sch.at(end - 8, functools.partial(
                gate_part, 3, e, eighths(end - 7 + g0 + (g1 - g0) * e / (ne_ - 1))))
        pending = []
        c = 0
        while c < 4:
            if last and c == 0:
                def prod(k, step):
                    return _dot(_bf(sch.gate(ao_v[2 * k + 1][0])),
                                _bf(bo[k, 128:256, 0:256]))
                cc2 = [u + v for u, v in zip(part, _strassen(prod, sch.after))]
                blocks = [(t, [v[:, t * 128:(t + 1) * 128] for v in cc2]) for t in range(2)]
            else:
                def prod(k, step):
                    return _dot(_bf(sch.gate(jnp.concatenate(
                        [ao_v[2 * k][0], ao_v[2 * k + 1][0]], axis=1))),
                                _bf(bo[k, :, c * 128:(c + 1) * 128]))
                blocks = [(c, _strassen(prod, sch.after))]
            if last:
                for t in pending:
                    out_cols(t).start()
                pending = []
            nb = len(blocks) * ne_
            for q in range(nb):
                t, cc = blocks[q // ne_]
                due = eighths(sch.slot + e0 + (e1 - e0) * q / (nb - 1))
                epilogue(t, cc, q % ne_, due if t < 3 else None)
            pending = [t for t, _ in blocks]
            c += len(blocks)
        if last:
            out_cols(3).start()
            out_copy((tile + i) % NT, 1 - slot).wait()
            for t in range(4):
                out_cols(t).wait()
        else:
            out_copy(n, slot).start()
        return carry

    with jax.named_scope('P2'):
        jax.lax.fori_loop(0, NT - 1, phase2, 0)
    phase2(NT - 1, 0)


@jax.jit
def pallas_recurrent_scan__linear_kernel_hedgehog__moe_arch_mod__prompt_kernel(
    A_x: jax.Array,
    A_wqkv: jax.Array,
    A_w_phi: jax.Array,
    A_wo: jax.Array,
    B_x: jax.Array,
    B_w_r: jax.Array,
    B_w_gate: jax.Array,
    B_w_up: jax.Array,
    B_w_down: jax.Array,
):
    del B_x
    any_spec = pl.BlockSpec(memory_space=pl.ANY)
    return pl.pallas_call(
        _kernel,
        out_shape=jax.ShapeDtypeStruct((1, S, D), BF16),
        in_specs=[any_spec] * 8,
        out_specs=any_spec,
        scratch_shapes=[
            pltpu.VMEM((S, D), BF16),
            pltpu.VMEM((3, D, D), BF16),
            pltpu.VMEM((H, DH, DH), BF16),
            pltpu.VMEM((8, 128), BF16),
            pltpu.VMEM((D, D), BF16),
            pltpu.VMEM((D, F), BF16),
            pltpu.VMEM((D, F), BF16),
            pltpu.VMEM((F, D), BF16),
            pltpu.VMEM((NT, 9, TH // 2, DHALF), U32),
            pltpu.VMEM((7, 256, DHALF), U32),
            pltpu.VMEM((7, 256, DHALF), U32),
            pltpu.VMEM((7, 256, DHALF), U32),
            pltpu.VMEM((7, 256, DHALF), U32),
            pltpu.VMEM((NP, MR, 128), F32),
            pltpu.VMEM((NP, MR // 2, 128), U32),
            pltpu.VMEM((8, DHALF), U32),
            pltpu.VMEM((NT, 1, T), F32),
            pltpu.VMEM((8, D), F32),
            pltpu.VMEM((D, 128), F32),
            pltpu.VMEM((FC, 128), F32),
            pltpu.VMEM((2, 128, T), F32),
            pltpu.VMEM((2, T, D), BF16),
            pltpu.SMEM((1,), I32),
            pltpu.SemaphoreType.DMA((NT + 18,)),
            pltpu.SemaphoreType.DMA((6,)),
        ] + [pltpu.VMEM((1, TH // 2, 256), U32)] * 14,
        compiler_params=pltpu.CompilerParams(vmem_limit_bytes=100 * 1024 * 1024),
    )(A_x, A_wqkv, A_w_phi, A_wo, B_w_r.reshape(8, 128), B_w_gate, B_w_up, B_w_down)
```

```python
import functools
import os
import json
_P = json.loads(os.environ.get('KP', '{}'))

import jax
import jax.numpy as jnp
import jax.experimental.pallas as pl
import jax.experimental.pallas.tpu as pltpu

S, D, H, DH, F = 2048, 1024, 32, 32, 3584
T = 256
TH = T // 2
DHALF = D // 2
NT = S // T
NJ = 4
NP = D // 64
MR = 64
FC = 512
NFC = F // FC
NF = _P.get('nf', 2)
ORDER = 'k0 x0 x1 k1 k2 k3 v0 v1 v2 v3 x2'
PROG = ('w:x1 L1:3:6 K0a w:k1 f1 K0b S0a K1a S0b K1b '
        'w:k2,k3,v0 f2 f3 p0:14:18 S1a K2a S1b K2b S2a K3a S2b K3b '
        'w:v1,v2,v3,x2 p1:3:8 p2:16:21 p3:30:35 L2:6:52 V0a X0a V0b '
        'X0b V1a X1a V1b X1b V2a X2a V2b X2b V3a X3a V3b Y3b')
LOG2E = 1.4426950408889634
F32, BF16, U32, I32 = jnp.float32, jnp.bfloat16, jnp.uint32, jnp.int32

_NT_DIMS = (((1,), (1,)), ((), ()))


def _dot_nt(a, b):
    return jax.lax.dot_general(a, b, _NT_DIMS, preferred_element_type=F32)


def _dot(a, b):
    return jnp.dot(a, b, preferred_element_type=F32)


def _u32(v):
    return pltpu.bitcast(v, U32) if v.dtype != U32 else v


def _pack2(even, odd):
    return pltpu.pack_elementwise([even, odd], packed_dtype=BF16)


def _unpack2(u):
    return [pltpu.unpack_elementwise(u, index=i, packed_dtype=BF16, unpacked_dtype=F32)
            for i in range(2)]


def _pack_blocks(v):
    r, c = v.shape
    v4 = v.reshape(r // 16, 2, 8, c)
    return _pack2(v4[:, 0], v4[:, 1]).reshape(r // 2, c)


def _recip(x):
    r = pl.reciprocal(x, approx=True)
    return r * (2.0 - x * r)


def _bf(v):
    return pltpu.bitcast(v, BF16)


def _round(v):
    return v.astype(BF16).astype(F32)


def _or_all(vals):
    ts = []
    for v in vals:
        u = _u32(v)
        for a in range(u.shape[0] // 8):
            for b in range(u.shape[1] // 128):
                ts.append(u[a * 8:(a + 1) * 8, b * 128:(b + 1) * 128])
    while len(ts) > 1:
        ts = [ts[i] | ts[i + 1] if i + 1 < len(ts) else ts[i] for i in range(0, len(ts), 2)]
    return ts[0]


def _gate(lhs_u32, deps, never):
    if not deps:
        return lhs_u32
    rows = []
    for r in range(lhs_u32.shape[0] // 8):
        row = lhs_u32[r * 8:(r + 1) * 8]
        cs = [c for (r_, c) in deps if r_ == r]
        if cs:
            row = jnp.concatenate(
                [jnp.where(never, _or_all(deps[r, c]), row[:, c * 128:(c + 1) * 128])
                 if c in cs else row[:, c * 128:(c + 1) * 128]
                 for c in range(lhs_u32.shape[1] // 128)], axis=1)
        rows.append(row)
    return jnp.concatenate(rows, axis=0)


def _layernorm(x):
    m = jnp.mean(x, axis=-1, keepdims=True)
    mb = _round(m)
    xc = x - mb
    dm = m - mb
    v = jnp.mean(xc * xc, axis=-1, keepdims=True) - dm * dm
    a = _round(_round(v) + 1e-5)
    rs = jax.lax.rsqrt(a)
    sd = a * rs
    sd = _round(sd + (0.5 * rs) * (a - sd * sd))
    return xc * _recip(sd)


def _lhs_combos(a11, a12, a21, a22):
    return [a11 + a22, a21 + a22, a11, a22, a11 + a12, a21 - a11, a12 - a22]


def _rhs_combos(b11, b12, b21, b22):
    return [b11 + b22, b11, b12 - b22, b21 - b11, b22, b11 + b12, b21 + b22]


def _strassen(prod, after=None):
    done = {}

    def p(k, step):
        return prod(k, step)

    def hook(step):
        if after is not None:
            after(step, done)

    m1 = p(0, 0)
    hook(0)
    m4 = p(3, 1)
    hook(1)
    m5 = p(4, 2)
    hook(2)
    m7 = p(6, 3)
    done[0] = m1 + m4 - m5 + m7
    hook(3)
    m3 = p(2, 4)
    done[1] = m3 + m5
    hook(4)
    m2 = p(1, 5)
    done[2] = m2 + m4
    hook(5)
    m6 = p(5, 6)
    done[3] = m1 - m2 + m3 + m6
    hook(6)
    return done[0], done[1], done[2], done[3]


def _allreduce_pair(x, op):
    x = op(x, pltpu.roll(x, 2, axis=0))
    return op(x, pltpu.roll(x, 4, axis=0))


def _feature_map(p, z=None):
    t = p.shape[1]
    p3 = p.reshape(8, 8, t)
    mx = _allreduce_pair(jnp.max(p3, axis=0), jnp.maximum)
    mn = _allreduce_pair(jnp.min(p3, axis=0), jnp.minimum)
    ep = jnp.exp2(p3 - mx[None])
    en = jnp.exp2(mn[None] - p3)
    rp = _recip(_allreduce_pair(jnp.sum(ep, axis=0), jnp.add))
    rn = _recip(_allreduce_pair(jnp.sum(en, axis=0), jnp.add))
    if z is not None:
        z4 = jnp.concatenate([z] * (t // 128), axis=1).reshape(2, 8, 8, t)
        den = rp * jnp.sum(ep * z4[0], axis=0) + rn * jnp.sum(en * z4[1], axis=0)
        inv = _recip(_allreduce_pair(den, jnp.add) + 1e-6)
        rp, rn = rp * inv, rn * inv
    pos = (ep * rp[None]).reshape(64, t)
    neg = (en * rn[None]).reshape(64, t)
    return jnp.concatenate([pos, neg], axis=0)


def _silu(x):
    h = 0.5 * x
    return h + h * jnp.tanh(h)


def _kernel(x_hbm, wqkv_hbm, wphi_hbm, wo_hbm, wr_hbm, wg_hbm, wu_hbm, wd_hbm,
            out_hbm,
            x_v, w_v, wphi_v, wr_v, wo_v, wg_v, wu_v, wd_v,
            bq, ak, av, aq, bo, kv_acc, z_v, m_v, wr2, r_v, y_acc, xb_v, hb_v, pq0_v,
            out_v, zero_s, sem, sem_o, *ao_v):
    def x_copy(i):
        return pltpu.make_async_copy(x_hbm.at[0, pl.ds(i * T, T), :],
                                     x_v.at[pl.ds(i * T, T), :], sem.at[i])

    def w_copy(m, j):
        return pltpu.make_async_copy(
            wqkv_hbm.at[:, m * D + j * 256:m * D + (j + 1) * 256],
            w_v.at[m, :, j * 256:(j + 1) * 256], sem.at[NT + 6 + 4 * m + j])

    wphi_copy = pltpu.make_async_copy(wphi_hbm, wphi_v, sem.at[NT])
    wr_copy = pltpu.make_async_copy(wr_hbm, wr_v, sem.at[NT + 1])
    wo_copy = pltpu.make_async_copy(wo_hbm, wo_v, sem.at[NT + 2])
    wg_copy = pltpu.make_async_copy(wg_hbm, wg_v, sem.at[NT + 3])
    wu_copy = pltpu.make_async_copy(wu_hbm, wu_v, sem.at[NT + 4])
    wd_copy = pltpu.make_async_copy(wd_hbm, wd_v, sem.at[NT + 5])

    def out_copy(i, slot):
        return pltpu.make_async_copy(out_v.at[slot],
                                     out_hbm.at[0, pl.ds(i * T, T), :],
                                     sem_o.at[slot])

    wphi_copy.start()
    wr_copy.start()
    def named_copy(nm):
        t = int(nm[1])
        return x_copy(t) if nm[0] == 'x' else w_copy({'k': 1, 'v': 2}[nm[0]], t)

    for nm in _P.get('order', ORDER).split():
        named_copy(nm).start()
    x_copy(NF + 1).start()
    wo_copy.start()
    for i in range(NF + 2, NT):
        x_copy(i).start()
    for j in range(NJ):
        w_copy(0, j).start()
    wg_copy.start()
    wu_copy.start()
    wd_copy.start()

    zero_s[0] = 0
    kv_acc[...] = jnp.zeros_like(kv_acc)
    y_acc[...] = jnp.zeros_like(y_acc)
    z_v[...] = jnp.zeros_like(z_v)
    hb_v[...] = jnp.zeros_like(hb_v)

    with jax.named_scope('wphi'):
        wphi_copy.wait()
    wr_copy.wait()
    row = jax.lax.broadcasted_iota(I32, (128, DH), 0)
    col = jax.lax.broadcasted_iota(I32, (128, DH), 1)
    sel = jnp.where(((row % 64) // 16) * 8 + row % 8 == col, 1.0, 0.0).astype(BF16)
    wall = wphi_v[...].reshape(H * DH, DH)
    phit = _dot_nt(sel, wall)
    row = jax.lax.broadcasted_iota(I32, (128, D), 0)
    col = jax.lax.broadcasted_iota(I32, (128, D), 1)
    keep = (2 * (row // 64) + (row // 8) % 2) == ((col % 128) // DH)
    phit = jnp.where(keep, phit, 0.0).astype(BF16)


    def fold(which, dst, j):
        wt = []
        for g in (2 * j, 2 * j + 1):
            wt.append(_dot_nt(phit[:, g * 128:(g + 1) * 128],
                              w_v[which, :, g * 128:(g + 1) * 128]) * LOG2E)
        w0, w1 = wt
        cs = _lhs_combos(w0[:, :DHALF], w0[:, DHALF:], w1[:, :DHALF], w1[:, DHALF:])
        for k in range(7):
            dst[k, j * 64:(j + 1) * 64, :] = _pack_blocks(cs[k])

    def packed_combos(fn, u11, u12, u21, u22):
        parts = [_unpack2(u) for u in (u11, u12, u21, u22)]
        ev = fn(*[p[0] for p in parts])
        od = fn(*[p[1] for p in parts])
        return [_pack2(e, o) for e, o in zip(ev, od)]

    def prep_v(j, sch=None):
        ws = [_u32(w_v[2, :, g * 128:(g + 1) * 128]) for g in (2 * j, 2 * j + 1)]
        if sch is not None:
            ws = [sch.hold(w, [(8 * q, 0) for q in range(8)]) for w in ws]
        w0, w1 = [_u32(_bf(w).T) for w in ws]
        cs = packed_combos(_lhs_combos, w0[:, :DHALF], w0[:, DHALF:],
                           w1[:, :DHALF], w1[:, DHALF:])
        cs[2], cs[3] = w0[:, :DHALF], w1[:, DHALF:]
        for k in range(7):
            av[k, j * 64:(j + 1) * 64, :] = cs[k]
        return w0, w1

    def ln_chunk(n, c, sch=None):
        ys = []
        for h in range(2):
            r0 = n * T + h * TH + c * 16
            if not isinstance(r0, int):
                r0 = pl.multiple_of(r0, 16)
            xu = _u32(x_v[pl.ds(r0, 16), :])
            if sch is not None:
                xu = sch.hold(xu, [(0, 0)])
            ys += [_layernorm(xr) for xr in _unpack2(xu)]
        cs = []
        for t in range(2):
            ya, yb = ys[t], ys[2 + t]
            cs.append(_rhs_combos(ya[:, :DHALF], yb[:, :DHALF], ya[:, DHALF:], yb[:, DHALF:])
                      + [ya[:, DHALF:], yb[:, :DHALF]])
        cs = [_pack2(e, o) for e, o in zip(*cs)]
        for k in range(9):
            bq[n, k, c * 8:(c + 1) * 8, :] = cs[k]
        return cs

    def wo_piece(c, q):
        r0 = (c // 2) * 256 + (c % 2) * 64 + q * 16
        o0 = c * 32 + q * 8
        if not isinstance(c, int):
            r0 = pl.multiple_of(r0, 16)
            o0 = pl.multiple_of(o0, 8)
        w0 = wo_v[pl.ds(r0, 16), :].astype(F32)
        w1 = wo_v[pl.ds(r0 + 128, 16), :].astype(F32)

        def cols(w, par):
            return jnp.concatenate(
                [w[:, (2 * q + par) * 128:(2 * q + par + 1) * 128] for q in range(4)], axis=1)
        cs = [_pack_blocks(v) for v in
              _rhs_combos(cols(w0, 0), cols(w0, 1), cols(w1, 0), cols(w1, 1))]
        for k in range(7):
            bo[k, pl.ds(o0, 8), :] = cs[k]
        return cs

    class Sched:
        def __init__(self, never):
            self.never = never
            self.slot = 0
            self.gated = 0
            self.token = None
            self.jobs = {}
            self.deps = {}

        def at(self, slot, fn):
            self.jobs.setdefault(slot, []).append(fn)

        def need(self, pos, vals):
            slot, r = divmod(int(round(pos * 8)), 8)
            assert slot >= self.gated, (pos, self.slot)
            d = self.deps.setdefault(slot, {})
            c = (slot + r) % 4
            d.setdefault((r, c), []).extend(vals)

        def gate(self, lhs):
            nc = lhs.shape[1] // 128
            self.gated = self.slot + 1
            deps = {}
            for (r, c), v in self.deps.pop(self.slot, {}).items():
                deps.setdefault((r, c % nc), []).extend(v)
            return _gate(lhs, deps, self.never)

        def hold(self, u, blocks):
            if self.token is None:
                return u
            return _gate(u, {rc: [self.token] for rc in blocks}, self.never)

        def after(self, step, done):
            for fn in self.jobs.pop(self.slot, []):
                fn()
            self.slot += 1

    def proj(sch, a_ref, j, b, extra=None, early=None):
        def prod(k, step):
            lhs = sch.gate(a_ref[k, j * 64:(j + 1) * 64, :])
            if extra is not None and k in (1, 2, 3, 4):
                r_ = _dot_nt(_bf(jnp.concatenate([lhs, wr2[...]], axis=0)), b[k])
                extra[k] = r_[128:136]
                r_ = r_[0:128]
            else:
                r_ = _dot_nt(_bf(lhs), b[k])
            sch.token = r_[0:8, 0:128]
            return r_
        def after(step, done):
            if step == 4 and early is not None:
                early[j] = [jnp.concatenate([done[0], done[1]], axis=1), None]
            sch.after(step, done)
        c11, c12, c21, c22 = _strassen(prod, after)
        return (jnp.concatenate([c11, c12], axis=1),
                jnp.concatenate([c21, c22], axis=1))

    wr = wr_v[...].astype(F32)
    wr2[...] = _pack2(*[
        jnp.concatenate([jnp.broadcast_to(wr[4 * h + t:4 * h + t + 1], (8, 128))
                         for t in range(4)], axis=1) for h in range(2)])

    with jax.named_scope('k0'):
        w_copy(1, 0).wait()
    fold(1, ak, 0)
    with jax.named_scope('x0'):
        x_copy(0).wait()
    for c in range(8):
        ln_chunk(0, c)


    class KVTile:
        def __init__(self, sch, i):
            self.sch, self.i = sch, i
            self.b = None
            self.pk, self.vt, self.phis = {}, {}, {}

        def operands(self):
            if self.b is None:
                self.b = [_bf(bq[self.i, k]) for k in range(7)]
            return self.b

        def kproj(self, j):
            self.pk[j] = proj(self.sch, ak, j, self.operands())

        def vproj(self, j):
            ex = {} if j == 0 else None
            self.vt[j] = [_pack_blocks(v)
                          for v in proj(self.sch, av, j, self.operands(), ex)]
            if j == 0:
                r_v[self.i] = jnp.concatenate(
                    [ex[1][0:1] + ex[1][1:2] + ex[3][1:2],
                     ex[4][0:1] + ex[4][1:2] + ex[2][0:1]], axis=1)

        def sm(self, j, g, p, due=None, step=0):
            phi = _feature_map(self.pk[j][g][p * 64:(p + 1) * 64])
            z_v[4 * j + 2 * g + p] += phi[:, :128] + phi[:, 128:]
            phi = _pack_blocks(phi)
            self.phis[j, g, p] = phi
            if due is not None:
                for t in range(2):
                    self.sch.need(due - step * (1 - t), [phi[:, t * 128:(t + 1) * 128]])

        def kv(self, j, g):
            for p in range(2):
                if (j, g, p) not in self.phis:
                    self.sm(j, g, p)
                lhs = _bf(self.vt[j][g][p * 32:(p + 1) * 32])
                kv_acc[4 * j + 2 * g + p] += _dot_nt(lhs, _bf(self.phis[j, g, p]))

    def spread(sch, vals, due, step=0.25):
        for t in range(4):
            sch.need(due + t * step, [v[:, t * 128:(t + 1) * 128] for v in vals])

    def eighths(x):
        return round(x * 8) / 8

    def first_tiles():
        sch = Sched(zero_s[0] > 0)
        tiles = {'a': KVTile(sch, 0), 'b': KVTile(sch, 1)}
        for op in _P.get('prog', PROG).split():
            kind, arg = op[0], op[1:2]
            if kind == 'w':
                with jax.named_scope(op):
                    for nm in op[2:].split(','):
                        named_copy(nm).wait()
            elif kind == 'f':
                fold(1, ak, int(arg))
            elif kind == 'p':
                _, rel, d0 = op.split(':')

                def job(j=int(arg), base=sch.slot + float(d0), rel=int(rel)):
                    ws = prep_v(j, sch if rel >= 0 else None)
                    for q in range(8):
                        sch.need(base + q * _P.get('pvs', 0.5),
                                 [w[:, q * 128:(q + 1) * 128] for w in ws])
                if int(rel) < 0:
                    job()
                else:
                    sch.at(sch.slot + int(rel), job)
            elif kind == 'U':
                for c in range(8):
                    ln_chunk(int(arg), c)
            elif kind == 'L':
                _, l0, l1 = op.split(':')
                for c in range(8):
                    due = eighths(sch.slot + float(l0) + (float(l1) - float(l0)) * c / 7)
                    rel = int(due - _P.get('lrel', 4.5))

                    def job(n=int(arg), c=c, due=due, held=rel >= sch.slot):
                        spread(sch, ln_chunk(n, c, sch if held else None), due)
                    if rel >= sch.slot:
                        sch.at(rel, job)
                    else:
                        job()
            elif kind == 'S':
                a0, a1 = _P.get('s1', [1.5, 6.5])
                st_ = (a1 - a0) / 7
                for q in range(4):
                    tiles[op[2]].sm(int(arg), q // 2, q % 2,
                                    eighths(sch.slot + a0 + st_ * (2 * q + 1)), eighths(st_))
            elif kind == 'K':
                tiles[op[2]].kproj(int(arg))
            elif kind == 'V':
                tiles[op[2]].vproj(int(arg))
            elif kind == 'X':
                sch.at(sch.slot + 1, functools.partial(tiles[op[2]].kv, int(arg), 0))
                sch.at(sch.slot + 4, functools.partial(tiles[op[2]].kv, int(arg), 1))
            elif kind == 'Y':
                for g in range(2):
                    tiles[op[2]].kv(int(arg), g)
        assert not sch.jobs and not sch.deps, (sch.jobs.keys(), sch.deps.keys())

    def phase1(i, carry):
        nxt = jnp.minimum(i + 1, NT - 1)

        @pl.when(i + 1 < NT)
        def _():
            x_copy(i + 1).wait()

        @pl.when(i == NF)
        def _():
            wo_copy.wait()

        sch = Sched(zero_s[0] > 0)
        tl = KVTile(sch, i)
        tl.operands()
        lrel = _P.get('lrel1')
        for c in range(8):
            due = 14 * (c // 2) + _P.get('ln', [6, 13])[c % 2]
            rel = int(due - lrel) if lrel else -1

            def job(c=c, due=due, held=rel >= 0):
                spread(sch, ln_chunk(nxt, c, sch if held else None), due,
                       _P.get('lnstep', 0.25))
            if rel >= 0:
                sch.at(rel, job)
            else:
                job()
        for q in range(4):
            spread(sch, wo_piece(i - NF, q), 14 * q + _P.get('wo', 1), _P.get('wostep', 0.25))
        phg = _P.get('phg')
        for j in range(NJ):
            for g in range(2):
                at = 14 * j + 7 + _P.get('kvs', [7, 9])[g]
                if j == NJ - 1:
                    at = 55 + _P.get('phl', 1) * (g - 1)
                if phg:
                    for p in range(2):
                        sch.at(14 * j + 7, functools.partial(
                            tl.sm, j, g, p, at + 1 - phg[0] - phg[1] * (2 - 2 * p), phg[1]))
                if j < NJ - 1:
                    sch.at(at, functools.partial(tl.kv, j, g))
        for j in range(NJ):
            tl.kproj(j)
            tl.vproj(j)
        for g in range(2):
            tl.kv(NJ - 1, g)
        return carry

    only = _P.get('only')
    if only is None:
        first_tiles()
    else:
        for nm in ORDER.split()[2:]:
            named_copy(nm).wait()
    with jax.named_scope('P1'):
        if only != 'P2':
            jax.lax.fori_loop(NF, NT, phase1, 0)
        else:
            wo_copy.wait()
            for t in range(NF + 1, NT):
                x_copy(t).wait()

    for j in range(NJ):
        w_copy(0, j).wait()
    wg_copy.wait()
    wu_copy.wait()
    wd_copy.wait()
    row = jax.lax.broadcasted_iota(I32, (MR, 128), 0)
    col = jax.lax.broadcasted_iota(I32, (MR, 128), 1)
    keep = (row // DH) == ((col // 2) % 2)
    for p in range(NP):
        m_v[p] = _u32(jnp.where(keep, kv_acc[p], 0.0).astype(BF16))
        z_v[p] = jnp.broadcast_to(jnp.sum(z_v[p], axis=1, keepdims=True), (128, 128))

    for c in range(NT - NF, NT):
        for q in range(4):
            wo_piece(c, q)
    for j in range(NJ):
        fold(0, aq, j)

    r = _round(r_v[...].reshape(NT, T))
    rmax = jnp.max(jnp.max(r, axis=1, keepdims=True), axis=0, keepdims=True)
    pos = (jax.lax.broadcasted_iota(I32, (NT, T), 0) * T
           + jax.lax.broadcasted_iota(I32, (NT, T), 1))
    idx = jnp.min(jnp.where(r == rmax, pos, S))
    idx = jnp.clip(idx, 0, S - 1)
    tile = idx // T
    half = (idx % T) // TH
    sub = pl.multiple_of(((idx % TH) // 16) * 8, 8)
    xs = jnp.concatenate([bq[tile, 1 + 7 * half, pl.ds(sub, 8), :],
                          bq[tile, 7 - 3 * half, pl.ds(sub, 8), :]], axis=1)
    xs = jnp.where(jax.lax.broadcasted_iota(I32, (16, D), 0) == idx % 16,
                   _bf(xs).astype(F32), 0.0)
    xs = jnp.sum(xs, axis=0, keepdims=True)

    def lane_bcast(dst, row):
        for t in range(row.shape[1] // 128):
            dst[t * 128:(t + 1) * 128, :] = jnp.broadcast_to(
                row[:, t * 128:(t + 1) * 128], (128, 128)).T

    lane_bcast(xb_v, xs)
    router = _round(0.5 + 0.5 * jnp.tanh(0.5 * rmax))

    first = proj(Sched(None), aq, 0, [_bf(bq[(tile + 1) % NT, k]) for k in range(7)])
    for g in range(2):
        pq0_v[g] = first[g]

    def phase2(i, carry):
        last = isinstance(i, int)
        zero = zero_s[0]
        never = zero > 0
        slot = i % 2
        n = tile if last else (tile + 1 + i) % NT

        if last:
            out_copy((tile + i - 1) % NT, slot).wait()
        else:
            @pl.when(i >= 2)
            def _():
                out_copy((tile + i - 1) % NT, slot).wait()

        s0 = pl.multiple_of(n * T, T)
        b = [_bf(bq[n, k]) for k in range(7)]
        pq = [None] * NJ
        ao = [None] * NJ
        sch = Sched(never)
        ot = {}
        pq[0] = [pq0_v[g] for g in range(2)]

        phis = {}

        def sm(j, g, p, due, step=0):
            phis[j, g, p] = _pack_blocks(_feature_map(
                pq[j][g][p * 64:(p + 1) * 64], z_v[4 * j + 2 * g + p]))
            if due is not None:
                for t in range(2):
                    sch.need(max(due - step * (1 - t), sch.slot + 1),
                             [phis[j, g, p][:, t * 128:(t + 1) * 128]])

        def nd(j, g):
            parts = []
            for p in range(2):
                if (j, g, p) not in phis:
                    sm(j, g, p, None)
                parts.append(_dot(_bf(m_v[4 * j + 2 * g + p]), _bf(phis[j, g, p])))
            ot[j, g] = jnp.concatenate(parts, axis=0)
            if g == 1:
                o0, o1 = ot[j, 0], ot[j, 1]
                cs = _lhs_combos(o0[:, :TH], o1[:, :TH], o0[:, TH:], o1[:, TH:])
                for k in range(7):
                    ao_v[2 * k + j // 2][zero, :, (j % 2) * 128:(j % 2 + 1) * 128] = (
                        _u32(cs[k].astype(BF16).T))

        if last:
            fd = (NFC - 1) * FC
        else:
            fu = pl.multiple_of(i * FC, FC)
            fd = pl.multiple_of(jnp.maximum(i - 1, 0) * FC, FC)
        ffn = {}

        FR = _P.get('fr', 64)

        def matvec(key, w, vb, due):
            t = (w.astype(F32).reshape(FR // 8, 8, 256)
                 * jnp.concatenate([vb, vb], axis=1).reshape(FR // 8, 8, 256))
            t = jnp.sum(t, axis=0)
            ffn[key] = t if key not in ffn else ffn[key] + t
            sch.need(due, [ffn[key]])

        def ffn_up(w_ref, name, cp, rb, due):
            rs = slice(rb * FR, (rb + 1) * FR)
            matvec((name, cp), w_ref[rs, pl.ds(fu + cp * 256, 256)], xb_v[rs, :], due)

        def ffn_mid():
            hg, hu = [_round(jnp.sum(jnp.concatenate([ffn[nm, 0], ffn[nm, 1]], axis=1),
                                     axis=0, keepdims=True)) for nm in 'gu']
            lane_bcast(hb_v, _round(_round(_silu(hg)) * hu))

        def ffn_down(cp, rb, due):
            cs_ = slice(cp * 256, (cp + 1) * 256)
            if rb == 0:
                ffn['y', cp] = y_acc[:, cs_]
            matvec(('y', cp), wd_v[pl.ds(fd + rb * FR, FR), cs_],
                   hb_v[rb * FR:(rb + 1) * FR, :], due)
            if rb == FC // FR - 1:
                if last:
                    ffn['row', cp] = (
                        _round(jnp.sum(ffn['y', cp], axis=0, keepdims=True)) * router)
                else:
                    y_acc[:, cs_] = ffn['y', cp]

        d0, d1, u0, u1 = _P.get('ffn', [2, 27, 28, 53])
        nd_ = 4 * FC // FR
        for t in range(nd_):
            due = eighths(d0 + (d1 - d0) * t / (nd_ - 1))
            sch.at(0, functools.partial(ffn_down, t % 4, t // 4, due))
        if not last:
            nu_ = 4 * D // FR
            for t in range(nu_):
                due = eighths(u0 + (u1 - u0) * t / (nu_ - 1))
                name, w_ref = (('g', wg_v), ('u', wu_v))[(t // 2) % 2]
                sch.at(0, functools.partial(ffn_up, w_ref, name, t % 2, t // 4, due))
            sch.at(int(u1), ffn_mid)
        for j in range(NJ):
            s1 = 7 * j
            nds = (_P.get('nds0', [2, 4]) if j == 0 else _P.get('nds', [1, 4]) if j < NJ - 1
                   else _P.get('nds3l', [1, 2]) if last else _P.get('nds3', [0, 2]))
            phq = _P.get('phq', [0.5, 0.5])
            for g in range(2):
                if phq:
                    for p in range(2):
                        sch.at(s1 if (j == 0 or g == 1) else s1 - 2, functools.partial(
                            sm, j, g, p, s1 + nds[g] + 1 - phq[0] - phq[1] * (2 - 2 * p), phq[1]))
                sch.at(s1 + nds[g], functools.partial(nd, j, g))
        for j in range(1, NJ):
            pq[j] = proj(sch, aq, j, b, early=pq)
        part = {}
        if last:
            def prod_a(k, step):
                return _dot(_bf(sch.gate(ao_v[2 * k][0])), _bf(bo[k, 0:128, 0:256]))
            part = _strassen(prod_a, sch.after)
        else:
            nxt = proj(sch, aq, 0, [_bf(bq[(n + 1) % NT, k]) for k in range(7)])
            for g in range(2):
                pq0_v[g] = nxt[g]

        ER = _P.get('er', 64)
        rows = jax.lax.broadcasted_iota(I32, (ER, 256), 0) + s0
        ne_ = T // ER
        gates = {}

        def gate_part(c, e, due):
            r0 = e * ER
            h, rh = r0 // TH, r0 % TH
            blk = ((1, 7), (8, 4))[h][c // 2]
            bb = _bf(bq[n, blk, rh // 2:(rh + ER) // 2,
                        (c % 2) * 256:(c % 2 + 1) * 256]).astype(F32)
            if last:
                bb = bb + jnp.where(rows + r0 == idx, ffn['row', c], 0.0)
            gates[c, e] = _silu(bb)
            if due is not None:
                sch.need(due, [gates[c, e]])

        def epilogue(c, cc, e, due):
            r0 = e * ER
            h, rh = r0 // TH, r0 % TH
            cs = slice(c * 256, (c + 1) * 256)
            rs = slice(rh, rh + ER)
            if (c, e) not in gates:
                gate_part(c, e, None)
            xr = x_v[pl.ds(s0 + r0, ER), cs].astype(F32)
            sv = jnp.concatenate([cc[2 * h][rs], cc[2 * h + 1][rs]], axis=1)
            res = xr + sv * gates[c, e]
            out_v[slot, r0:r0 + ER, cs] = res.astype(BF16)
            if due is not None:
                sch.need(due, [res])

        def out_cols(c):
            cs = slice(c * 256, (c + 1) * 256)
            return pltpu.make_async_copy(out_v.at[slot, :, cs],
                                         out_hbm.at[0, pl.ds(s0, T), cs], sem_o.at[2 + c])

        e0, e1 = _P.get('epi', [1, 6.5])
        g0, g1 = _P.get('gl', [0, 4])
        end = sch.slot + 28 - (7 if last else 0)
        for e in range(ne_):
            sch.at(end - 8, functools.partial(
                gate_part, 3, e, eighths(end - 7 + g0 + (g1 - g0) * e / (ne_ - 1))))
        pending = []
        c = 0
        while c < 4:
            if last and c == 0:
                def prod(k, step):
                    return _dot(_bf(sch.gate(ao_v[2 * k + 1][0])),
                                _bf(bo[k, 128:256, 0:256]))
                cc2 = [u + v for u, v in zip(part, _strassen(prod, sch.after))]
                blocks = [(t, [v[:, t * 128:(t + 1) * 128] for v in cc2]) for t in range(2)]
            else:
                def prod(k, step):
                    return _dot(_bf(sch.gate(jnp.concatenate(
                        [ao_v[2 * k][0], ao_v[2 * k + 1][0]], axis=1))),
                                _bf(bo[k, :, c * 128:(c + 1) * 128]))
                blocks = [(c, _strassen(prod, sch.after))]
            if last:
                for t in pending:
                    out_cols(t).start()
                pending = []
            nb = len(blocks) * ne_
            for q in range(nb):
                t, cc = blocks[q // ne_]
                due = eighths(sch.slot + e0 + (e1 - e0) * q / (nb - 1))
                epilogue(t, cc, q % ne_, due if t < 3 else None)
            pending = [t for t, _ in blocks]
            c += len(blocks)
        if last:
            out_cols(3).start()
            out_copy((tile + i) % NT, 1 - slot).wait()
            for t in range(4):
                out_cols(t).wait()
        else:
            out_copy(n, slot).start()
        return carry

    with jax.named_scope('P2'):
        if only != 'P1':
            jax.lax.fori_loop(0, NT - 1, phase2, 0)
    if only is None:
        phase2(NT - 1, 0)
    elif only == 'P2':
        for t in (NT - 3, NT - 2):
            out_copy((tile + 1 + t) % NT, t % 2).wait()


@jax.jit
def pallas_recurrent_scan__linear_kernel_hedgehog__moe_arch_mod__prompt_kernel(
    A_x: jax.Array,
    A_wqkv: jax.Array,
    A_w_phi: jax.Array,
    A_wo: jax.Array,
    B_x: jax.Array,
    B_w_r: jax.Array,
    B_w_gate: jax.Array,
    B_w_up: jax.Array,
    B_w_down: jax.Array,
):
    del B_x
    any_spec = pl.BlockSpec(memory_space=pl.ANY)
    return pl.pallas_call(
        _kernel,
        out_shape=jax.ShapeDtypeStruct((1, S, D), BF16),
        in_specs=[any_spec] * 8,
        out_specs=any_spec,
        scratch_shapes=[
            pltpu.VMEM((S, D), BF16),
            pltpu.VMEM((3, D, D), BF16),
            pltpu.VMEM((H, DH, DH), BF16),
            pltpu.VMEM((8, 128), BF16),
            pltpu.VMEM((D, D), BF16),
            pltpu.VMEM((D, F), BF16),
            pltpu.VMEM((D, F), BF16),
            pltpu.VMEM((F, D), BF16),
            pltpu.VMEM((NT, 9, TH // 2, DHALF), U32),
            pltpu.VMEM((7, 256, DHALF), U32),
            pltpu.VMEM((7, 256, DHALF), U32),
            pltpu.VMEM((7, 256, DHALF), U32),
            pltpu.VMEM((7, 256, DHALF), U32),
            pltpu.VMEM((NP, MR, 128), F32),
            pltpu.VMEM((NP, 128, 128), F32),
            pltpu.VMEM((NP, MR // 2, 128), U32),
            pltpu.VMEM((8, DHALF), U32),
            pltpu.VMEM((NT, 1, T), F32),
            pltpu.VMEM((8, D), F32),
            pltpu.VMEM((D, 128), F32),
            pltpu.VMEM((FC, 128), F32),
            pltpu.VMEM((2, 128, T), F32),
            pltpu.VMEM((2, T, D), BF16),
            pltpu.SMEM((1,), I32),
            pltpu.SemaphoreType.DMA((NT + 18,)),
            pltpu.SemaphoreType.DMA((6,)),
        ] + [pltpu.VMEM((1, TH // 2, 256), U32)] * 14,
        compiler_params=pltpu.CompilerParams(vmem_limit_bytes=100 * 1024 * 1024),
    )(A_x, A_wqkv, A_w_phi, A_wo, B_w_r.reshape(8, 128), B_w_gate, B_w_up, B_w_down)
```

```python
import functools
import os
import json
_P = json.loads(os.environ.get('KP', '{}'))

import jax
import jax.numpy as jnp
import jax.experimental.pallas as pl
import jax.experimental.pallas.tpu as pltpu

S, D, H, DH, F = 2048, 1024, 32, 32, 3584
T = 256
TH = T // 2
DHALF = D // 2
NT = S // T
NJ = 4
NP = D // 64
MR = 64
FC = 512
NFC = F // FC
NF = _P.get('nf', 2)
ORDER = 'ph wr k0 x0 x1 k1 k2 k3 v0 v1 v2 v3 x2'
PROG = ('w:ph,wr P w:k0 f0 w:x0 U0 w:x1 L1:3:6 K0a w:k1 f1 K0b S0a K1a S0b K1b '
        'w:k2,k3,v0 f2 f3 p0:14:18 S1a K2a S1b K2b S2a K3a S2b K3b '
        'w:v1,v2,v3,x2 p1:3:8 p2:16:21 p3:30:35 L2:6:52 V0a X0a V0b '
        'X0b V1a X1a V1b X1b V2a X2a V2b X2b V3a X3a V3b Y3b')
LOG2E = 1.4426950408889634
F32, BF16, U32, I32 = jnp.float32, jnp.bfloat16, jnp.uint32, jnp.int32

_NT_DIMS = (((1,), (1,)), ((), ()))


def _dot_nt(a, b):
    return jax.lax.dot_general(a, b, _NT_DIMS, preferred_element_type=F32)


def _dot(a, b):
    return jnp.dot(a, b, preferred_element_type=F32)


def _u32(v):
    return pltpu.bitcast(v, U32) if v.dtype != U32 else v


def _pack2(even, odd):
    return pltpu.pack_elementwise([even, odd], packed_dtype=BF16)


def _unpack2(u):
    return [pltpu.unpack_elementwise(u, index=i, packed_dtype=BF16, unpacked_dtype=F32)
            for i in range(2)]


def _pack_blocks(v):
    r, c = v.shape
    v4 = v.reshape(r // 16, 2, 8, c)
    return _pack2(v4[:, 0], v4[:, 1]).reshape(r // 2, c)


def _recip(x):
    r = pl.reciprocal(x, approx=True)
    return r * (2.0 - x * r)


def _bf(v):
    return pltpu.bitcast(v, BF16)


def _round(v):
    return v.astype(BF16).astype(F32)


def _or_all(vals):
    ts = []
    for v in vals:
        u = _u32(v)
        for a in range(u.shape[0] // 8):
            for b in range(u.shape[1] // 128):
                ts.append(u[a * 8:(a + 1) * 8, b * 128:(b + 1) * 128])
    while len(ts) > 1:
        ts = [ts[i] | ts[i + 1] if i + 1 < len(ts) else ts[i] for i in range(0, len(ts), 2)]
    return ts[0]


def _gate(lhs_u32, deps, never):
    if not deps:
        return lhs_u32
    rows = []
    for r in range(lhs_u32.shape[0] // 8):
        row = lhs_u32[r * 8:(r + 1) * 8]
        cs = [c for (r_, c) in deps if r_ == r]
        if cs:
            row = jnp.concatenate(
                [jnp.where(never, _or_all(deps[r, c]), row[:, c * 128:(c + 1) * 128])
                 if c in cs else row[:, c * 128:(c + 1) * 128]
                 for c in range(lhs_u32.shape[1] // 128)], axis=1)
        rows.append(row)
    return jnp.concatenate(rows, axis=0)


def _layernorm(x):
    m = jnp.mean(x, axis=-1, keepdims=True)
    mb = _round(m)
    xc = x - mb
    dm = m - mb
    v = jnp.mean(xc * xc, axis=-1, keepdims=True) - dm * dm
    a = _round(_round(v) + 1e-5)
    rs = jax.lax.rsqrt(a)
    sd = a * rs
    sd = _round(sd + (0.5 * rs) * (a - sd * sd))
    return xc * _recip(sd)


def _lhs_combos(a11, a12, a21, a22):
    return [a11 + a22, a21 + a22, a11, a22, a11 + a12, a21 - a11, a12 - a22]


def _rhs_combos(b11, b12, b21, b22):
    return [b11 + b22, b11, b12 - b22, b21 - b11, b22, b11 + b12, b21 + b22]


def _strassen(prod, after=None):
    done = {}

    def p(k, step):
        return prod(k, step)

    def hook(step):
        if after is not None:
            after(step, done)

    m1 = p(0, 0)
    hook(0)
    m4 = p(3, 1)
    hook(1)
    m5 = p(4, 2)
    hook(2)
    m7 = p(6, 3)
    done[0] = m1 + m4 - m5 + m7
    hook(3)
    m3 = p(2, 4)
    done[1] = m3 + m5
    hook(4)
    m2 = p(1, 5)
    done[2] = m2 + m4
    hook(5)
    m6 = p(5, 6)
    done[3] = m1 - m2 + m3 + m6
    hook(6)
    return done[0], done[1], done[2], done[3]


def _allreduce_pair(x, op):
    x = op(x, pltpu.roll(x, 2, axis=0))
    return op(x, pltpu.roll(x, 4, axis=0))


def _feature_map(p, z=None):
    t = p.shape[1]
    p3 = p.reshape(8, 8, t)
    mx = _allreduce_pair(jnp.max(p3, axis=0), jnp.maximum)
    mn = _allreduce_pair(jnp.min(p3, axis=0), jnp.minimum)
    ep = jnp.exp2(p3 - mx[None])
    en = jnp.exp2(mn[None] - p3)
    rp = _recip(_allreduce_pair(jnp.sum(ep, axis=0), jnp.add))
    rn = _recip(_allreduce_pair(jnp.sum(en, axis=0), jnp.add))
    if z is not None:
        z4 = jnp.concatenate([z] * (t // 128), axis=1).reshape(2, 8, 8, t)
        den = rp * jnp.sum(ep * z4[0], axis=0) + rn * jnp.sum(en * z4[1], axis=0)
        inv = _recip(_allreduce_pair(den, jnp.add) + 1e-6)
        rp, rn = rp * inv, rn * inv
    pos = (ep * rp[None]).reshape(64, t)
    neg = (en * rn[None]).reshape(64, t)
    return jnp.concatenate([pos, neg], axis=0)


def _silu(x):
    h = 0.5 * x
    return h + h * jnp.tanh(h)


def _kernel(x_hbm, wqkv_hbm, wphi_hbm, wo_hbm, wr_hbm, wg_hbm, wu_hbm, wd_hbm,
            out_hbm,
            x_v, w_v, wphi_v, wr_v, wo_v, wg_v, wu_v, wd_v,
            bq, ak, av, aq, bo, kv_acc, z_v, m_v, phit, wr2, r_v, y_acc, xb_v, hb_v, pq0_v,
            out_v, zero_s, sem, sem_o, *ao_v):
    def x_copy(i):
        return pltpu.make_async_copy(x_hbm.at[0, pl.ds(i * T, T), :],
                                     x_v.at[pl.ds(i * T, T), :], sem.at[i])

    def w_copy(m, j):
        return pltpu.make_async_copy(
            wqkv_hbm.at[:, m * D + j * 256:m * D + (j + 1) * 256],
            w_v.at[m, :, j * 256:(j + 1) * 256], sem.at[NT + 6 + 4 * m + j])

    wphi_copy = pltpu.make_async_copy(wphi_hbm, wphi_v, sem.at[NT])
    wr_copy = pltpu.make_async_copy(wr_hbm, wr_v, sem.at[NT + 1])
    wo_copy = pltpu.make_async_copy(wo_hbm, wo_v, sem.at[NT + 2])
    wg_copy = pltpu.make_async_copy(wg_hbm, wg_v, sem.at[NT + 3])
    wu_copy = pltpu.make_async_copy(wu_hbm, wu_v, sem.at[NT + 4])
    wd_copy = pltpu.make_async_copy(wd_hbm, wd_v, sem.at[NT + 5])

    def out_copy(i, slot):
        return pltpu.make_async_copy(out_v.at[slot],
                                     out_hbm.at[0, pl.ds(i * T, T), :],
                                     sem_o.at[slot])

    def named_copy(nm):
        if nm in ('ph', 'wr'):
            return wphi_copy if nm == 'ph' else wr_copy
        t = int(nm[1])
        return x_copy(t) if nm[0] == 'x' else w_copy({'k': 1, 'v': 2}[nm[0]], t)

    for nm in _P.get('order', ORDER).split():
        named_copy(nm).start()
    x_copy(NF + 1).start()
    wo_copy.start()
    for i in range(NF + 2, NT):
        x_copy(i).start()
    for j in range(NJ):
        w_copy(0, j).start()
    wg_copy.start()
    wu_copy.start()
    wd_copy.start()

    zero_s[0] = 0
    kv_acc[...] = jnp.zeros_like(kv_acc)
    y_acc[...] = jnp.zeros_like(y_acc)
    z_v[...] = jnp.zeros_like(z_v)
    hb_v[...] = jnp.zeros_like(hb_v)

    def build_phit():
        row = jax.lax.broadcasted_iota(I32, (128, DH), 0)
        col = jax.lax.broadcasted_iota(I32, (128, DH), 1)
        sel = jnp.where(((row % 64) // 16) * 8 + row % 8 == col, 1.0, 0.0).astype(BF16)
        wall = wphi_v[...].reshape(H * DH, DH)
        ph = _dot_nt(sel, wall)
        row = jax.lax.broadcasted_iota(I32, (128, D), 0)
        col = jax.lax.broadcasted_iota(I32, (128, D), 1)
        keep = (2 * (row // 64) + (row // 8) % 2) == ((col % 128) // DH)
        phit[...] = jnp.where(keep, ph, 0.0).astype(BF16)
        wr = wr_v[...].astype(F32)
        wr2[...] = _pack2(*[
            jnp.concatenate([jnp.broadcast_to(wr[4 * h + t:4 * h + t + 1], (8, 128))
                             for t in range(4)], axis=1) for h in range(2)])

    def fold(which, dst, j, sch=None):
        wt = []
        for g in (2 * j, 2 * j + 1):
            r_ = _dot_nt(phit[:, g * 128:(g + 1) * 128],
                         w_v[which, :, g * 128:(g + 1) * 128])
            if sch is not None and g == 2 * j:
                sch.token = r_[0:8, 0:128]
            wt.append(r_ * LOG2E)
        w0, w1 = wt
        cs = _lhs_combos(w0[:, :DHALF], w0[:, DHALF:], w1[:, :DHALF], w1[:, DHALF:])
        for k in range(7):
            dst[k, j * 64:(j + 1) * 64, :] = _pack_blocks(cs[k])

    def packed_combos(fn, u11, u12, u21, u22):
        parts = [_unpack2(u) for u in (u11, u12, u21, u22)]
        ev = fn(*[p[0] for p in parts])
        od = fn(*[p[1] for p in parts])
        return [_pack2(e, o) for e, o in zip(ev, od)]

    def prep_v(j, sch=None):
        ws = [_u32(w_v[2, :, g * 128:(g + 1) * 128]) for g in (2 * j, 2 * j + 1)]
        if sch is not None:
            ws = [sch.hold(w, [(8 * q, 0) for q in range(8)]) for w in ws]
        w0, w1 = [_u32(_bf(w).T) for w in ws]
        cs = packed_combos(_lhs_combos, w0[:, :DHALF], w0[:, DHALF:],
                           w1[:, :DHALF], w1[:, DHALF:])
        cs[2], cs[3] = w0[:, :DHALF], w1[:, DHALF:]
        for k in range(7):
            av[k, j * 64:(j + 1) * 64, :] = cs[k]
        return w0, w1

    def ln_chunk(n, c, sch=None):
        ys = []
        for h in range(2):
            r0 = n * T + h * TH + c * 16
            if not isinstance(r0, int):
                r0 = pl.multiple_of(r0, 16)
            xu = _u32(x_v[pl.ds(r0, 16), :])
            if sch is not None:
                xu = sch.hold(xu, [(0, 0)])
            ys += [_layernorm(xr) for xr in _unpack2(xu)]
        cs = []
        for t in range(2):
            ya, yb = ys[t], ys[2 + t]
            cs.append(_rhs_combos(ya[:, :DHALF], yb[:, :DHALF], ya[:, DHALF:], yb[:, DHALF:])
                      + [ya[:, DHALF:], yb[:, :DHALF]])
        cs = [_pack2(e, o) for e, o in zip(*cs)]
        for k in range(9):
            bq[n, k, c * 8:(c + 1) * 8, :] = cs[k]
        return cs

    def wo_piece(e):
        r0 = pl.multiple_of((e // 8) * 256 + (e % 8) * 16, 16)
        o0 = pl.multiple_of(e * 8, 8)
        w0 = wo_v[pl.ds(r0, 16), :].astype(F32)
        w1 = wo_v[pl.ds(r0 + 128, 16), :].astype(F32)

        def cols(w, par):
            return jnp.concatenate(
                [w[:, (2 * q + par) * 128:(2 * q + par + 1) * 128] for q in range(4)], axis=1)
        cs = [_pack_blocks(v) for v in
              _rhs_combos(cols(w0, 0), cols(w0, 1), cols(w1, 0), cols(w1, 1))]
        for k in range(7):
            bo[k, pl.ds(o0, 8), :] = cs[k]
        return cs

    class Sched:
        def __init__(self, never):
            self.never = never
            self.slot = 0
            self.gated = 0
            self.token = None
            self.jobs = {}
            self.deps = {}

        def at(self, slot, fn):
            self.jobs.setdefault(slot, []).append(fn)

        def need(self, pos, vals):
            slot, r = divmod(int(round(pos * 8)), 8)
            assert slot >= self.gated, (pos, self.slot)
            d = self.deps.setdefault(slot, {})
            c = (slot + r) % 4
            d.setdefault((r, c), []).extend(vals)

        def gate(self, lhs):
            nc = lhs.shape[1] // 128
            self.gated = self.slot + 1
            deps = {}
            for (r, c), v in self.deps.pop(self.slot, {}).items():
                deps.setdefault((r, c % nc), []).extend(v)
            return _gate(lhs, deps, self.never)

        def hold(self, u, blocks):
            if self.token is None:
                return u
            return _gate(u, {rc: [self.token] for rc in blocks}, self.never)

        def after(self, step, done):
            for fn in self.jobs.pop(self.slot, []):
                fn()
            self.slot += 1

    def proj(sch, a_ref, j, b, extra=None, early=None):
        def prod(k, step):
            lhs = sch.gate(a_ref[k, j * 64:(j + 1) * 64, :])
            if extra is not None and k in (1, 2, 3, 4):
                r_ = _dot_nt(_bf(jnp.concatenate([lhs, wr2[...]], axis=0)), b[k])
                extra[k] = r_[128:136]
                r_ = r_[0:128]
            else:
                r_ = _dot_nt(_bf(lhs), b[k])
            sch.token = r_[0:8, 0:128]
            return r_
        def after(step, done):
            if step == 4 and early is not None:
                early[j] = [jnp.concatenate([done[0], done[1]], axis=1), None]
            sch.after(step, done)
        c11, c12, c21, c22 = _strassen(prod, after)
        return (jnp.concatenate([c11, c12], axis=1),
                jnp.concatenate([c21, c22], axis=1))

    class KVTile:
        def __init__(self, sch, i):
            self.sch, self.i = sch, i
            self.b = None
            self.pk, self.vt, self.phis = {}, {}, {}

        def operands(self):
            if self.b is None:
                self.b = [_bf(bq[self.i, k]) for k in range(7)]
            return self.b

        def kproj(self, j):
            self.pk[j] = proj(self.sch, ak, j, self.operands())

        def vproj(self, j):
            ex = {} if j == 0 else None
            self.vt[j] = [_pack_blocks(v)
                          for v in proj(self.sch, av, j, self.operands(), ex)]
            if j == 0:
                r_v[self.i] = jnp.concatenate(
                    [ex[1][0:1] + ex[1][1:2] + ex[3][1:2],
                     ex[4][0:1] + ex[4][1:2] + ex[2][0:1]], axis=1)

        def sm(self, j, g, p, due=None, step=0):
            phi = _feature_map(self.pk[j][g][p * 64:(p + 1) * 64])
            z_v[4 * j + 2 * g + p] += phi[:, :128] + phi[:, 128:]
            phi = _pack_blocks(phi)
            self.phis[j, g, p] = phi
            if due is not None:
                for t in range(2):
                    self.sch.need(due - step * (1 - t), [phi[:, t * 128:(t + 1) * 128]])

        def kv(self, j, g):
            for p in range(2):
                if (j, g, p) not in self.phis:
                    self.sm(j, g, p)
                lhs = _bf(self.vt[j][g][p * 32:(p + 1) * 32])
                kv_acc[4 * j + 2 * g + p] += _dot_nt(lhs, _bf(self.phis[j, g, p]))

    def spread(sch, vals, due, step=0.25):
        for t in range(4):
            sch.need(due + t * step, [v[:, t * 128:(t + 1) * 128] for v in vals])

    def eighths(x):
        return round(x * 8) / 8

    def first_tiles():
        sch = Sched(zero_s[0] > 0)
        tiles = {'a': KVTile(sch, 0), 'b': KVTile(sch, 1)}
        for op in _P.get('prog', PROG).split():
            kind, arg = op[0], op[1:2]
            if kind == 'w':
                with jax.named_scope(op):
                    for nm in op[2:].split(','):
                        named_copy(nm).wait()
            elif kind == 'P':
                build_phit()
            elif kind == 'f':
                fold(1, ak, int(arg))
            elif kind == 'p':
                _, rel, d0 = op.split(':')

                def job(j=int(arg), base=sch.slot + float(d0), rel=int(rel)):
                    ws = prep_v(j, sch if rel >= 0 else None)
                    for q in range(8):
                        sch.need(base + q * _P.get('pvs', 0.5),
                                 [w[:, q * 128:(q + 1) * 128] for w in ws])
                if int(rel) < 0:
                    job()
                else:
                    sch.at(sch.slot + int(rel), job)
            elif kind == 'U':
                for c in range(8):
                    ln_chunk(int(arg), c)
            elif kind == 'L':
                _, l0, l1 = op.split(':')
                for c in range(8):
                    due = eighths(sch.slot + float(l0) + (float(l1) - float(l0)) * c / 7)
                    rel = int(due - _P.get('lrel', 4.5))

                    def job(n=int(arg), c=c, due=due, held=rel >= sch.slot):
                        spread(sch, ln_chunk(n, c, sch if held else None), due)
                    if rel >= sch.slot:
                        sch.at(rel, job)
                    else:
                        job()
            elif kind == 'S':
                a0, a1 = _P.get('s1', [1.5, 6.5])
                st_ = (a1 - a0) / 7
                for q in range(4):
                    tiles[op[2]].sm(int(arg), q // 2, q % 2,
                                    eighths(sch.slot + a0 + st_ * (2 * q + 1)), eighths(st_))
            elif kind == 'K':
                tiles[op[2]].kproj(int(arg))
            elif kind == 'V':
                tiles[op[2]].vproj(int(arg))
            elif kind == 'X':
                sch.at(sch.slot + 1, functools.partial(tiles[op[2]].kv, int(arg), 0))
                sch.at(sch.slot + 4, functools.partial(tiles[op[2]].kv, int(arg), 1))
            elif kind == 'Y':
                for g in range(2):
                    tiles[op[2]].kv(int(arg), g)
        assert not sch.jobs and not sch.deps, (sch.jobs.keys(), sch.deps.keys())

    def phase1_waits(i, n):
        for d in range(n):
            @pl.when(i + 1 + d < NT)
            def _():
                x_copy(i + 1 + d).wait()

        @pl.when(i == NF)
        def _():
            wo_copy.wait()

    def phase1(i, carry):
        phase1_waits(i, 1)
        return phase1_tile(i, carry)

    def phase1x2(m, carry):
        i = NF + 2 * m
        phase1_waits(i, 2)
        phase1_tile(i, carry)
        return phase1_tile(i + 1, carry)

    def phase1_tile(i, carry):
        nxt = jnp.minimum(i + 1, NT - 1)
        sch = Sched(zero_s[0] > 0)
        tl = KVTile(sch, i)
        tl.operands()
        lrel = _P.get('lrel1')
        for c in range(8):
            due = 14 * (c // 2) + _P.get('ln', [6, 13])[c % 2]
            rel = int(due - lrel) if lrel else -1

            def job(c=c, due=due, held=rel >= 0):
                spread(sch, ln_chunk(nxt, c, sch if held else None), due,
                       _P.get('lnstep', 0.25))
            if rel >= 0:
                sch.at(rel, job)
            else:
                job()
        for q, due in enumerate(_P.get('wos', [1, 2.5, 15, 29, 43, 45])):
            spread(sch, wo_piece(jnp.minimum((i - NF) * 6 + q, 31)), due,
                   _P.get('wostep', 0.25))
        phg = _P.get('phg')
        for j in range(NJ):
            for g in range(2):
                at = 14 * j + 7 + _P.get('kvs', [7, 8])[g]
                if j == NJ - 1:
                    at = 55 + _P.get('phl', 1) * (g - 1)
                if phg:
                    for p in range(2):
                        sch.at(14 * j + 7, functools.partial(
                            tl.sm, j, g, p, at + 1 - phg[0] - phg[1] * (2 - 2 * p), phg[1]))
                if j < NJ - 1:
                    sch.at(at, functools.partial(tl.kv, j, g))
        for j in range(NJ):
            tl.kproj(j)
            tl.vproj(j)
        for g in range(2):
            tl.kv(NJ - 1, g)
        return carry

    only = _P.get('only')
    if only in (None, 'A'):
        first_tiles()
    else:
        for nm in ORDER.split():
            named_copy(nm).wait()
        if only == 'P1':
            wd_copy.wait()
    with jax.named_scope('P1'):
        if only in (None, 'P1'):
            if _P.get('u1'):
                jax.lax.fori_loop(0, (NT - NF) // 2, phase1x2, 0)
            else:
                jax.lax.fori_loop(NF, NT, phase1, 0)
        else:
            wo_copy.wait()
            for t in range(NF + 1, NT):
                x_copy(t).wait()

    if only == 'PL':
        for t in range(2):
            out_copy(t, t).start()
    for j in range(NJ):
        w_copy(0, j).wait()
    wg_copy.wait()
    wu_copy.wait()
    if only != 'P1':
        wd_copy.wait()
    sch = Sched(zero_s[0] > 0)
    row = jax.lax.broadcasted_iota(I32, (MR, 128), 0)
    col = jax.lax.broadcasted_iota(I32, (MR, 128), 1)
    keep = (row // DH) == ((col // 2) % 2)
    for j in range(NJ):
        fold(0, aq, j, sch)
        for p in range(4 * j, 4 * j + 4):
            kvp = pltpu.bitcast(sch.hold(_u32(kv_acc[p]), [(r, 0) for r in range(8)]), F32)
            mp = _u32(jnp.where(keep, kvp, 0.0).astype(BF16))
            m_v[p] = mp
            sch.need(1 + p * 0.375, [mp])
            z_v[p] = jnp.broadcast_to(jnp.sum(z_v[p], axis=1, keepdims=True), (128, 128))

    r = _round(r_v[...].reshape(NT, T))
    rmax = jnp.max(jnp.max(r, axis=1, keepdims=True), axis=0, keepdims=True)
    pos = (jax.lax.broadcasted_iota(I32, (NT, T), 0) * T
           + jax.lax.broadcasted_iota(I32, (NT, T), 1))
    idx = jnp.min(jnp.where(r == rmax, pos, S))
    idx = jnp.clip(idx, 0, S - 1)
    tile = idx // T
    half = (idx % T) // TH
    sub = pl.multiple_of(((idx % TH) // 16) * 8, 8)
    xs = jnp.concatenate([bq[tile, 1 + 7 * half, pl.ds(sub, 8), :],
                          bq[tile, 7 - 3 * half, pl.ds(sub, 8), :]], axis=1)
    xs = jnp.where(jax.lax.broadcasted_iota(I32, (16, D), 0) == idx % 16,
                   _bf(xs).astype(F32), 0.0)
    xs = jnp.sum(xs, axis=0, keepdims=True)

    def lane_bcast(dst, row):
        for t in range(row.shape[1] // 128):
            dst[t * 128:(t + 1) * 128, :] = jnp.broadcast_to(
                row[:, t * 128:(t + 1) * 128], (128, 128)).T

    lane_bcast(xb_v, xs)
    router = _round(0.5 + 0.5 * jnp.tanh(0.5 * rmax))

    first = proj(sch, aq, 0, [_bf(bq[(tile + 1) % NT, k]) for k in range(7)])
    for g in range(2):
        pq0_v[g] = first[g]

    def phase2(i, carry):
        last = isinstance(i, int)
        zero = zero_s[0]
        never = zero > 0
        slot = i % 2
        n = tile if last else (tile + 1 + i) % NT

        if last:
            out_copy((tile + i - 1) % NT, slot).wait()
        else:
            @pl.when(i >= 2)
            def _():
                out_copy((tile + i - 1) % NT, slot).wait()

        s0 = pl.multiple_of(n * T, T)
        b = [_bf(bq[n, k]) for k in range(7)]
        pq = [None] * NJ
        ao = [None] * NJ
        sch = Sched(never)
        ot = {}
        pq[0] = [pq0_v[g] for g in range(2)]

        phis = {}

        def sm(j, g, p, due, step=0):
            phis[j, g, p] = _pack_blocks(_feature_map(
                pq[j][g][p * 64:(p + 1) * 64], z_v[4 * j + 2 * g + p]))
            if due is not None:
                for t in range(2):
                    sch.need(max(due - step * (1 - t), sch.slot + 1),
                             [phis[j, g, p][:, t * 128:(t + 1) * 128]])

        def nd(j, g):
            parts = []
            for p in range(2):
                if (j, g, p) not in phis:
                    sm(j, g, p, None)
                parts.append(_dot(_bf(m_v[4 * j + 2 * g + p]), _bf(phis[j, g, p])))
            ot[j, g] = jnp.concatenate(parts, axis=0)
            if g == 1:
                o0, o1 = ot[j, 0], ot[j, 1]
                cs = _lhs_combos(o0[:, :TH], o1[:, :TH], o0[:, TH:], o1[:, TH:])
                for k in range(7):
                    ao_v[2 * k + j // 2][zero, :, (j % 2) * 128:(j % 2 + 1) * 128] = (
                        _u32(cs[k].astype(BF16).T))

        if last:
            fd = (NFC - 1) * FC
        else:
            fu = pl.multiple_of(i * FC, FC)
            fd = pl.multiple_of(jnp.maximum(i - 1, 0) * FC, FC)
        ffn = {}

        FR = _P.get('fr', 64)

        def matvec(key, w, vb, due):
            t = (w.astype(F32).reshape(FR // 8, 8, 256)
                 * jnp.concatenate([vb, vb], axis=1).reshape(FR // 8, 8, 256))
            t = jnp.sum(t, axis=0)
            ffn[key] = t if key not in ffn else ffn[key] + t
            sch.need(due, [ffn[key]])

        def ffn_up(w_ref, name, cp, rb, due):
            rs = slice(rb * FR, (rb + 1) * FR)
            matvec((name, cp), w_ref[rs, pl.ds(fu + cp * 256, 256)], xb_v[rs, :], due)

        def ffn_mid():
            hg, hu = [_round(jnp.sum(jnp.concatenate([ffn[nm, 0], ffn[nm, 1]], axis=1),
                                     axis=0, keepdims=True)) for nm in 'gu']
            lane_bcast(hb_v, _round(_round(_silu(hg)) * hu))

        def ffn_down(cp, rb, due):
            cs_ = slice(cp * 256, (cp + 1) * 256)
            if rb == 0:
                ffn['y', cp] = y_acc[:, cs_]
            matvec(('y', cp), wd_v[pl.ds(fd + rb * FR, FR), cs_],
                   hb_v[rb * FR:(rb + 1) * FR, :], due)
            if rb == FC // FR - 1:
                if last:
                    ffn['row', cp] = (
                        _round(jnp.sum(ffn['y', cp], axis=0, keepdims=True)) * router)
                else:
                    y_acc[:, cs_] = ffn['y', cp]

        d0, d1, u0, u1 = _P.get('ffn', [28, 36.5, 37, 53.5])
        if last:
            d0, d1 = _P.get('ffnl', [2, 27])
        nd_ = 4 * FC // FR
        for t in range(nd_):
            due = eighths(d0 + (d1 - d0) * t / (nd_ - 1))
            sch.at(0, functools.partial(ffn_down, t % 4, t // 4, due))
        if not last:
            nu_ = 4 * D // FR
            for t in range(nu_):
                due = eighths(u0 + (u1 - u0) * t / (nu_ - 1))
                name, w_ref = (('g', wg_v), ('u', wu_v))[(t // 2) % 2]
                sch.at(0, functools.partial(ffn_up, w_ref, name, t % 2, t // 4, due))
            sch.at(int(u1), ffn_mid)
        for j in range(NJ):
            s1 = 7 * j
            sfx = 'l' if last else ''
            nds = (_P.get('nds0' + sfx, [1, 4] if last else [2, 4]) if j == 0
                   else _P.get('nds' + sfx, [1, 4]) if j < NJ - 1
                   else _P.get('nds3l', [2, 3]) if last else _P.get('nds3', [0, 1]))
            phq = _P.get('phq' + sfx, [0.5, 0.5] if last else [0, 0.5])
            for g in range(2):
                if phq:
                    for p in range(2):
                        sch.at(s1 if (j == 0 or g == 1) else s1 - 2, functools.partial(
                            sm, j, g, p, s1 + nds[g] + 1 - phq[0] - phq[1] * (2 - 2 * p), phq[1]))
                sch.at(s1 + nds[g], functools.partial(nd, j, g))
        for j in range(1, NJ):
            pq[j] = proj(sch, aq, j, b, early=pq)
        part = {}
        if last:
            def prod_a(k, step):
                return _dot(_bf(sch.gate(ao_v[2 * k][0])), _bf(bo[k, 0:128, 0:256]))
            part = _strassen(prod_a, sch.after)
        else:
            nxt = proj(sch, aq, 0, [_bf(bq[(n + 1) % NT, k]) for k in range(7)])
            for g in range(2):
                pq0_v[g] = nxt[g]

        ER = _P.get('er' + sfx, 32 if last else 64)
        rows = jax.lax.broadcasted_iota(I32, (ER, 256), 0) + s0
        ne_ = T // ER
        gates = {}

        def gate_part(c, e, due):
            r0 = e * ER
            h, rh = r0 // TH, r0 % TH
            blk = ((1, 7), (8, 4))[h][c // 2]
            bb = _bf(bq[n, blk, rh // 2:(rh + ER) // 2,
                        (c % 2) * 256:(c % 2 + 1) * 256]).astype(F32)
            if last:
                bb = bb + jnp.where(rows + r0 == idx, ffn['row', c], 0.0)
            gates[c, e] = _silu(bb)
            if due is not None:
                sch.need(due, [gates[c, e]])

        def epilogue(c, cc, e, due):
            r0 = e * ER
            h, rh = r0 // TH, r0 % TH
            cs = slice(c * 256, (c + 1) * 256)
            rs = slice(rh, rh + ER)
            if (c, e) not in gates:
                gate_part(c, e, None)
            xr = x_v[pl.ds(s0 + r0, ER), cs].astype(F32)
            sv = jnp.concatenate([cc[2 * h][rs], cc[2 * h + 1][rs]], axis=1)
            res = xr + sv * gates[c, e]
            out_v[slot, r0:r0 + ER, cs] = res.astype(BF16)
            if due is not None:
                sch.need(due, [res])

        def out_cols(c):
            cs = slice(c * 256, (c + 1) * 256)
            return pltpu.make_async_copy(out_v.at[slot, :, cs],
                                         out_hbm.at[0, pl.ds(s0, T), cs], sem_o.at[2 + c])

        e0, e1 = _P.get('epi' + sfx, [1, 6.5] if last else [0.5, 6.5])
        g0, g1 = _P.get('gl' + sfx, [0, 4])
        end = sch.slot + 28 - (7 if last else 0)
        for e in range(ne_):
            sch.at(end - 8, functools.partial(
                gate_part, 3, e, eighths(end - 7 + g0 + (g1 - g0) * e / (ne_ - 1))))
        pending = []
        c = 0
        while c < 4:
            if last and c == 0:
                def prod(k, step):
                    return _dot(_bf(sch.gate(ao_v[2 * k + 1][0])),
                                _bf(bo[k, 128:256, 0:256]))
                cc2 = [u + v for u, v in zip(part, _strassen(prod, sch.after))]
                blocks = [(t, [v[:, t * 128:(t + 1) * 128] for v in cc2]) for t in range(2)]
            else:
                def prod(k, step):
                    return _dot(_bf(sch.gate(jnp.concatenate(
                        [ao_v[2 * k][0], ao_v[2 * k + 1][0]], axis=1))),
                                _bf(bo[k, :, c * 128:(c + 1) * 128]))
                blocks = [(c, _strassen(prod, sch.after))]
            if last:
                for t in pending:
                    out_cols(t).start()
                pending = []
            nb = len(blocks) * ne_
            for q in range(nb):
                t, cc = blocks[q // ne_]
                due = eighths(sch.slot + e0 + (e1 - e0) * q / (nb - 1))
                epilogue(t, cc, q % ne_, due if t < 3 else None)
            pending = [t for t, _ in blocks]
            c += len(blocks)
        if last:
            out_cols(3).start()
            out_copy((tile + i) % NT, 1 - slot).wait()
            for t in range(4):
                out_cols(t).wait()
        else:
            out_copy(n, slot).start()
        return carry

    with jax.named_scope('P2'):
        if only in (None, 'P2'):
            jax.lax.fori_loop(0, NT - 1, phase2, 0)
    if only in (None, 'PL'):
        with jax.named_scope('PL'):
            phase2(NT - 1, 0)
    elif only == 'P2':
        for t in (NT - 3, NT - 2):
            out_copy((tile + 1 + t) % NT, t % 2).wait()


@jax.jit
def pallas_recurrent_scan__linear_kernel_hedgehog__moe_arch_mod__prompt_kernel(
    A_x: jax.Array,
    A_wqkv: jax.Array,
    A_w_phi: jax.Array,
    A_wo: jax.Array,
    B_x: jax.Array,
    B_w_r: jax.Array,
    B_w_gate: jax.Array,
    B_w_up: jax.Array,
    B_w_down: jax.Array,
):
    del B_x
    any_spec = pl.BlockSpec(memory_space=pl.ANY)
    return pl.pallas_call(
        _kernel,
        out_shape=jax.ShapeDtypeStruct((1, S, D), BF16),
        in_specs=[any_spec] * 8,
        out_specs=any_spec,
        scratch_shapes=[
            pltpu.VMEM((S, D), BF16),
            pltpu.VMEM((3, D, D), BF16),
            pltpu.VMEM((H, DH, DH), BF16),
            pltpu.VMEM((8, 128), BF16),
            pltpu.VMEM((D, D), BF16),
            pltpu.VMEM((D, F), BF16),
            pltpu.VMEM((D, F), BF16),
            pltpu.VMEM((F, D), BF16),
            pltpu.VMEM((NT, 9, TH // 2, DHALF), U32),
            pltpu.VMEM((7, 256, DHALF), U32),
            pltpu.VMEM((7, 256, DHALF), U32),
            pltpu.VMEM((7, 256, DHALF), U32),
            pltpu.VMEM((7, 256, DHALF), U32),
            pltpu.VMEM((NP, MR, 128), F32),
            pltpu.VMEM((NP, 128, 128), F32),
            pltpu.VMEM((NP, MR // 2, 128), U32),
            pltpu.VMEM((128, D), BF16),
            pltpu.VMEM((8, DHALF), U32),
            pltpu.VMEM((NT, 1, T), F32),
            pltpu.VMEM((8, D), F32),
            pltpu.VMEM((D, 128), F32),
            pltpu.VMEM((FC, 128), F32),
            pltpu.VMEM((2, 128, T), F32),
            pltpu.VMEM((2, T, D), BF16),
            pltpu.SMEM((1,), I32),
            pltpu.SemaphoreType.DMA((NT + 18,)),
            pltpu.SemaphoreType.DMA((6,)),
        ] + [pltpu.VMEM((1, TH // 2, 256), U32)] * 14,
        compiler_params=pltpu.CompilerParams(vmem_limit_bytes=100 * 1024 * 1024),
    )(A_x, A_wqkv, A_w_phi, A_wo, B_w_r.reshape(8, 128), B_w_gate, B_w_up, B_w_down)
```

```python
import functools
import os
import json
_P = json.loads(os.environ.get('KP', '{}'))

import jax
import jax.numpy as jnp
import jax.experimental.pallas as pl
import jax.experimental.pallas.tpu as pltpu

S, D, H, DH, F = 2048, 1024, 32, 32, 3584
T = 256
TH = T // 2
DHALF = D // 2
NT = S // T
NJ = 4
NP = D // 64
MR = 64
FC = 512
NFC = F // FC
NF = _P.get('nf', 2)
ORDER = 'ph wr k0 x0 x1 k1 k2 k3 v0 v1 v2 v3 x2'
PROG = ('w:ph,wr P w:k0 f0 w:x0 U0 w:x1 L1:3:6 K0a',
        'w:k1 f1 K0b S0a K1a S0b K1b',
        'w:k2,k3,v0 f2 S1a K2a f3 p0:14:18 S1b K2b S2a K3a S2b K3b',
        'w:v1,v2,v3,x2 p1:3:8 p2:16:21 p3:30:35 L2:6:52 V0a X0a V0b '
        'X0b V1a X1a V1b X1b V2a X2a V2b X2b V3a X3a V3b Y3b')
LOG2E = 1.4426950408889634
F32, BF16, U32, I32 = jnp.float32, jnp.bfloat16, jnp.uint32, jnp.int32

_NT_DIMS = (((1,), (1,)), ((), ()))


def _dot_nt(a, b):
    return jax.lax.dot_general(a, b, _NT_DIMS, preferred_element_type=F32)


def _dot(a, b):
    return jnp.dot(a, b, preferred_element_type=F32)


def _u32(v):
    return pltpu.bitcast(v, U32) if v.dtype != U32 else v


def _pack2(even, odd):
    return pltpu.pack_elementwise([even, odd], packed_dtype=BF16)


def _unpack2(u):
    return [pltpu.unpack_elementwise(u, index=i, packed_dtype=BF16, unpacked_dtype=F32)
            for i in range(2)]


def _pack_blocks(v):
    r, c = v.shape
    v4 = v.reshape(r // 16, 2, 8, c)
    return _pack2(v4[:, 0], v4[:, 1]).reshape(r // 2, c)


def _recip(x):
    r = pl.reciprocal(x, approx=True)
    return r * (2.0 - x * r)


def _bf(v):
    return pltpu.bitcast(v, BF16)


def _round(v):
    return v.astype(BF16).astype(F32)


def _or_all(vals):
    ts = []
    for v in vals:
        u = _u32(v)
        for a in range(u.shape[0] // 8):
            for b in range(u.shape[1] // 128):
                ts.append(u[a * 8:(a + 1) * 8, b * 128:(b + 1) * 128])
    while len(ts) > 1:
        ts = [ts[i] | ts[i + 1] if i + 1 < len(ts) else ts[i] for i in range(0, len(ts), 2)]
    return ts[0]


def _gate(lhs_u32, deps, never):
    if not deps:
        return lhs_u32
    rows = []
    for r in range(lhs_u32.shape[0] // 8):
        row = lhs_u32[r * 8:(r + 1) * 8]
        cs = [c for (r_, c) in deps if r_ == r]
        if cs:
            row = jnp.concatenate(
                [jnp.where(never, _or_all(deps[r, c]), row[:, c * 128:(c + 1) * 128])
                 if c in cs else row[:, c * 128:(c + 1) * 128]
                 for c in range(lhs_u32.shape[1] // 128)], axis=1)
        rows.append(row)
    return jnp.concatenate(rows, axis=0)


def _layernorm(x):
    m = jnp.mean(x, axis=-1, keepdims=True)
    mb = _round(m)
    xc = x - mb
    dm = m - mb
    v = jnp.mean(xc * xc, axis=-1, keepdims=True) - dm * dm
    a = _round(_round(v) + 1e-5)
    rs = jax.lax.rsqrt(a)
    sd = a * rs
    sd = _round(sd + (0.5 * rs) * (a - sd * sd))
    return xc * _recip(sd)


def _lhs_combos(a11, a12, a21, a22):
    return [a11 + a22, a21 + a22, a11, a22, a11 + a12, a21 - a11, a12 - a22]


def _rhs_combos(b11, b12, b21, b22):
    return [b11 + b22, b11, b12 - b22, b21 - b11, b22, b11 + b12, b21 + b22]


def _strassen(prod, after=None):
    done = {}

    def p(k, step):
        return prod(k, step)

    def hook(step):
        if after is not None:
            after(step, done)

    m1 = p(0, 0)
    hook(0)
    m4 = p(3, 1)
    hook(1)
    m5 = p(4, 2)
    hook(2)
    m7 = p(6, 3)
    done[0] = m1 + m4 - m5 + m7
    hook(3)
    m3 = p(2, 4)
    done[1] = m3 + m5
    hook(4)
    m2 = p(1, 5)
    done[2] = m2 + m4
    hook(5)
    m6 = p(5, 6)
    done[3] = m1 - m2 + m3 + m6
    hook(6)
    return done[0], done[1], done[2], done[3]


def _allreduce_pair(x, op):
    x = op(x, pltpu.roll(x, 2, axis=0))
    return op(x, pltpu.roll(x, 4, axis=0))


def _feature_map(p, z=None):
    t = p.shape[1]
    p3 = p.reshape(8, 8, t)
    mx = _allreduce_pair(jnp.max(p3, axis=0), jnp.maximum)
    mn = _allreduce_pair(jnp.min(p3, axis=0), jnp.minimum)
    ep = jnp.exp2(p3 - mx[None])
    en = jnp.exp2(mn[None] - p3)
    rp = _recip(_allreduce_pair(jnp.sum(ep, axis=0), jnp.add))
    rn = _recip(_allreduce_pair(jnp.sum(en, axis=0), jnp.add))
    if z is not None:
        z4 = jnp.concatenate([z] * (t // 128), axis=1).reshape(2, 8, 8, t)
        den = rp * jnp.sum(ep * z4[0], axis=0) + rn * jnp.sum(en * z4[1], axis=0)
        inv = _recip(_allreduce_pair(den, jnp.add) + 1e-6)
        rp, rn = rp * inv, rn * inv
    pos = (ep * rp[None]).reshape(64, t)
    neg = (en * rn[None]).reshape(64, t)
    return jnp.concatenate([pos, neg], axis=0)


def _silu(x):
    h = 0.5 * x
    return h + h * jnp.tanh(h)


def _kernel(*refs):
    pl.run_scoped(functools.partial(_body, *refs),
                  pltpu.SemaphoreType.DMA((NT + 18,)), pltpu.SemaphoreType.DMA((6,)))


def _body(x_hbm, wqkv_hbm, wphi_hbm, wo_hbm, wr_hbm, wg_hbm, wu_hbm, wd_hbm,
            out_hbm,
            x_v, w_v, wphi_v, wr_v, wo_v, wg_v, wu_v, wd_v,
            bq, ak, av, aq, bo, kv_acc, z_v, m_v, phit, wr2, r_v, y_acc, xb_v, hb_v, pq0_v,
            out_v, zero_s, *rest):
    ao_v, (sem, sem_o) = rest[:-2], rest[-2:]
    def x_copy(i):
        return pltpu.make_async_copy(x_hbm.at[0, pl.ds(i * T, T), :],
                                     x_v.at[pl.ds(i * T, T), :], sem.at[i])

    def w_copy(m, j):
        return pltpu.make_async_copy(
            wqkv_hbm.at[:, m * D + j * 256:m * D + (j + 1) * 256],
            w_v.at[m, :, j * 256:(j + 1) * 256], sem.at[NT + 6 + 4 * m + j])

    wphi_copy = pltpu.make_async_copy(wphi_hbm, wphi_v, sem.at[NT])
    wr_copy = pltpu.make_async_copy(wr_hbm, wr_v, sem.at[NT + 1])
    wo_copy = pltpu.make_async_copy(wo_hbm, wo_v, sem.at[NT + 2])
    wg_copy = pltpu.make_async_copy(wg_hbm, wg_v, sem.at[NT + 3])
    wu_copy = pltpu.make_async_copy(wu_hbm, wu_v, sem.at[NT + 4])
    wd_copy = pltpu.make_async_copy(wd_hbm, wd_v, sem.at[NT + 5])

    def out_copy(i, slot):
        return pltpu.make_async_copy(out_v.at[slot],
                                     out_hbm.at[0, pl.ds(i * T, T), :],
                                     sem_o.at[slot])

    def named_copy(nm):
        if nm in ('ph', 'wr'):
            return wphi_copy if nm == 'ph' else wr_copy
        t = int(nm[1])
        return x_copy(t) if nm[0] == 'x' else w_copy({'k': 1, 'v': 2}[nm[0]], t)

    for nm in _P.get('order', ORDER).split():
        named_copy(nm).start()
    x_copy(NF + 1).start()
    wo_copy.start()
    for i in range(NF + 2, NT):
        x_copy(i).start()
    for j in range(NJ):
        w_copy(0, j).start()
    wg_copy.start()
    wu_copy.start()
    wd_copy.start()

    zero_s[0] = 0
    kv_acc[...] = jnp.zeros_like(kv_acc)
    y_acc[...] = jnp.zeros_like(y_acc)
    z_v[...] = jnp.zeros_like(z_v)
    hb_v[...] = jnp.zeros_like(hb_v)

    def build_phit():
        row = jax.lax.broadcasted_iota(I32, (128, DH), 0)
        col = jax.lax.broadcasted_iota(I32, (128, DH), 1)
        sel = jnp.where(((row % 64) // 16) * 8 + row % 8 == col, 1.0, 0.0).astype(BF16)
        wall = wphi_v[...].reshape(H * DH, DH)
        ph = _dot_nt(sel, wall)
        row = jax.lax.broadcasted_iota(I32, (128, D), 0)
        col = jax.lax.broadcasted_iota(I32, (128, D), 1)
        keep = (2 * (row // 64) + (row // 8) % 2) == ((col % 128) // DH)
        phit[...] = jnp.where(keep, ph, 0.0).astype(BF16)
        wr = wr_v[...].astype(F32)
        wr2[...] = _pack2(*[
            jnp.concatenate([jnp.broadcast_to(wr[4 * h + t:4 * h + t + 1], (8, 128))
                             for t in range(4)], axis=1) for h in range(2)])

    def fold(which, dst, j, sch=None):
        wt = []
        for g in (2 * j, 2 * j + 1):
            r_ = _dot_nt(phit[:, g * 128:(g + 1) * 128],
                         w_v[which, :, g * 128:(g + 1) * 128])
            if sch is not None and g == 2 * j:
                sch.token = r_[0:8, 0:128]
            wt.append(r_ * LOG2E)
        w0, w1 = wt
        cs = _lhs_combos(w0[:, :DHALF], w0[:, DHALF:], w1[:, :DHALF], w1[:, DHALF:])
        for k in range(7):
            dst[k, j * 64:(j + 1) * 64, :] = _pack_blocks(cs[k])

    def packed_combos(fn, u11, u12, u21, u22):
        parts = [_unpack2(u) for u in (u11, u12, u21, u22)]
        ev = fn(*[p[0] for p in parts])
        od = fn(*[p[1] for p in parts])
        return [_pack2(e, o) for e, o in zip(ev, od)]

    def prep_v(j, sch=None):
        ws = [_u32(w_v[2, :, g * 128:(g + 1) * 128]) for g in (2 * j, 2 * j + 1)]
        if sch is not None:
            ws = [sch.hold(w, [(8 * q, 0) for q in range(8)]) for w in ws]
        w0, w1 = [_u32(_bf(w).T) for w in ws]
        cs = packed_combos(_lhs_combos, w0[:, :DHALF], w0[:, DHALF:],
                           w1[:, :DHALF], w1[:, DHALF:])
        cs[2], cs[3] = w0[:, :DHALF], w1[:, DHALF:]
        for k in range(7):
            av[k, j * 64:(j + 1) * 64, :] = cs[k]
        return w0, w1

    def ln_chunk(n, c, sch=None):
        ys = []
        for h in range(2):
            r0 = n * T + h * TH + c * 16
            if not isinstance(r0, int):
                r0 = pl.multiple_of(r0, 16)
            xu = _u32(x_v[pl.ds(r0, 16), :])
            if sch is not None:
                xu = sch.hold(xu, [(0, 0)])
            ys += [_layernorm(xr) for xr in _unpack2(xu)]
        cs = []
        for t in range(2):
            ya, yb = ys[t], ys[2 + t]
            cs.append(_rhs_combos(ya[:, :DHALF], yb[:, :DHALF], ya[:, DHALF:], yb[:, DHALF:])
                      + [ya[:, DHALF:], yb[:, :DHALF]])
        cs = [_pack2(e, o) for e, o in zip(*cs)]
        for k in range(9):
            bq[n, k, c * 8:(c + 1) * 8, :] = cs[k]
        return cs

    def wo_piece(e):
        r0 = pl.multiple_of((e // 8) * 256 + (e % 8) * 16, 16)
        o0 = pl.multiple_of(e * 8, 8)
        w0 = wo_v[pl.ds(r0, 16), :].astype(F32)
        w1 = wo_v[pl.ds(r0 + 128, 16), :].astype(F32)

        def cols(w, par):
            return jnp.concatenate(
                [w[:, (2 * q + par) * 128:(2 * q + par + 1) * 128] for q in range(4)], axis=1)
        cs = [_pack_blocks(v) for v in
              _rhs_combos(cols(w0, 0), cols(w0, 1), cols(w1, 0), cols(w1, 1))]
        for k in range(7):
            bo[k, pl.ds(o0, 8), :] = cs[k]
        return cs

    class Sched:
        def __init__(self, never):
            self.never = never
            self.slot = 0
            self.gated = 0
            self.token = None
            self.jobs = {}
            self.deps = {}

        def at(self, slot, fn):
            self.jobs.setdefault(slot, []).append(fn)

        def need(self, pos, vals):
            slot, r = divmod(int(round(pos * 8)), 8)
            assert slot >= self.gated, (pos, self.slot)
            d = self.deps.setdefault(slot, {})
            c = (slot + r) % 4
            d.setdefault((r, c), []).extend(vals)

        def gate(self, lhs):
            nc = lhs.shape[1] // 128
            self.gated = self.slot + 1
            deps = {}
            for (r, c), v in self.deps.pop(self.slot, {}).items():
                deps.setdefault((r, c % nc), []).extend(v)
            return _gate(lhs, deps, self.never)

        def hold(self, u, blocks):
            if self.token is None:
                return u
            return _gate(u, {rc: [self.token] for rc in blocks}, self.never)

        def after(self, step, done):
            for fn in self.jobs.pop(self.slot, []):
                fn()
            self.slot += 1

    def proj(sch, a_ref, j, b, extra=None, early=None):
        def prod(k, step):
            lhs = sch.gate(a_ref[k, j * 64:(j + 1) * 64, :])
            if extra is not None and k in (1, 2, 3, 4):
                r_ = _dot_nt(_bf(jnp.concatenate([lhs, wr2[...]], axis=0)), b[k])
                extra[k] = r_[128:136]
                r_ = r_[0:128]
            else:
                r_ = _dot_nt(_bf(lhs), b[k])
            sch.token = r_[0:8, 0:128]
            return r_
        def after(step, done):
            if step == 4 and early is not None:
                early[j] = [jnp.concatenate([done[0], done[1]], axis=1), None]
            sch.after(step, done)
        c11, c12, c21, c22 = _strassen(prod, after)
        return (jnp.concatenate([c11, c12], axis=1),
                jnp.concatenate([c21, c22], axis=1))

    class KVTile:
        def __init__(self, sch, i):
            self.sch, self.i = sch, i
            self.b = None
            self.pk, self.vt, self.phis = {}, {}, {}

        def operands(self):
            if self.b is None:
                self.b = [_bf(bq[self.i, k]) for k in range(7)]
            return self.b

        def kproj(self, j):
            self.pk[j] = proj(self.sch, ak, j, self.operands())

        def vproj(self, j):
            ex = {} if j == 0 else None
            self.vt[j] = [_pack_blocks(v)
                          for v in proj(self.sch, av, j, self.operands(), ex)]
            if j == 0:
                r_v[self.i] = jnp.concatenate(
                    [ex[1][0:1] + ex[1][1:2] + ex[3][1:2],
                     ex[4][0:1] + ex[4][1:2] + ex[2][0:1]], axis=1)

        def sm(self, j, g, p, due=None, step=0):
            phi = _feature_map(self.pk[j][g][p * 64:(p + 1) * 64])
            z_v[4 * j + 2 * g + p] += phi[:, :128] + phi[:, 128:]
            phi = _pack_blocks(phi)
            self.phis[j, g, p] = phi
            if due is not None:
                for t in range(2):
                    self.sch.need(due - step * (1 - t), [phi[:, t * 128:(t + 1) * 128]])

        def kv(self, j, g):
            for p in range(2):
                if (j, g, p) not in self.phis:
                    self.sm(j, g, p)
                lhs = _bf(self.vt[j][g][p * 32:(p + 1) * 32])
                kv_acc[4 * j + 2 * g + p] += _dot_nt(lhs, _bf(self.phis[j, g, p]))

    def spread(sch, vals, due, step=0.25):
        for t in range(4):
            sch.need(due + t * step, [v[:, t * 128:(t + 1) * 128] for v in vals])

    def eighths(x):
        return round(x * 8) / 8

    def first_tiles():
        sch = Sched(zero_s[0] > 0)
        tiles = {'a': KVTile(sch, 0), 'b': KVTile(sch, 1)}
        prog = _P.get('prog') or ' '.join(_P.get('seg%d' % t, PROG[t]) for t in range(4))
        for op in prog.split():
            kind, arg = op[0], op[1:2]
            if kind == 'w':
                with jax.named_scope(op):
                    for nm in op[2:].split(','):
                        named_copy(nm).wait()
            elif kind == 'P':
                build_phit()
            elif kind == 'f':
                fold(1, ak, int(arg))
            elif kind == 'p':
                _, rel, d0 = op.split(':')

                def job(j=int(arg), base=sch.slot + float(d0), rel=int(rel)):
                    ws = prep_v(j, sch if rel >= 0 else None)
                    for q in range(8):
                        sch.need(base + q * _P.get('pvs', 0.5),
                                 [w[:, q * 128:(q + 1) * 128] for w in ws])
                if int(rel) < 0:
                    job()
                else:
                    sch.at(sch.slot + int(rel), job)
            elif kind == 'U':
                for c in range(8):
                    ln_chunk(int(arg), c)
            elif kind == 'L':
                _, l0, l1 = op.split(':')
                for c in range(8):
                    due = eighths(sch.slot + float(l0) + (float(l1) - float(l0)) * c / 7)
                    rel = int(due - _P.get('lrel', 4.5))

                    def job(n=int(arg), c=c, due=due, held=rel >= sch.slot):
                        spread(sch, ln_chunk(n, c, sch if held else None), due)
                    if rel >= sch.slot:
                        sch.at(rel, job)
                    else:
                        job()
            elif kind == 'S':
                a0, a1 = _P.get('s1', [1.5, 6.5])
                st_ = (a1 - a0) / 7
                for q in range(4):
                    tiles[op[2]].sm(int(arg), q // 2, q % 2,
                                    eighths(sch.slot + a0 + st_ * (2 * q + 1)), eighths(st_))
            elif kind == 'K':
                tiles[op[2]].kproj(int(arg))
            elif kind == 'V':
                tiles[op[2]].vproj(int(arg))
            elif kind == 'X':
                for g in range(2):
                    sch.at(sch.slot + _P.get('xo', [1, 4])[g],
                           functools.partial(tiles[op[2]].kv, int(arg), g))
            elif kind == 'Y':
                for g in range(2):
                    tiles[op[2]].kv(int(arg), g)
        assert not sch.jobs and not sch.deps, (sch.jobs.keys(), sch.deps.keys())

    def phase1_waits(i, n):
        if _P.get('early', 1):
            return
        for d in range(n):
            @pl.when(i + 1 + d < NT)
            def _():
                x_copy(i + 1 + d).wait()

        @pl.when(i == NF)
        def _():
            wo_copy.wait()

    def phase1(i, carry):
        phase1_waits(i, 1)
        return phase1_tile(i, carry)

    def phase1x2(m, carry):
        i = NF + 2 * m
        phase1_waits(i, 2)
        phase1_tile(i, carry)
        return phase1_tile(i + 1, carry)

    def phase1_tile(i, carry):
        nxt = jnp.minimum(i + 1, NT - 1)
        sch = Sched(zero_s[0] > 0)
        tl = KVTile(sch, i)
        tl.operands()
        lrel = _P.get('lrel1')
        for c in range(8):
            due = 14 * (c // 2) + _P.get('ln', [6, 13])[c % 2]
            rel = int(due - lrel) if lrel else -1

            def job(c=c, due=due, held=rel >= 0):
                spread(sch, ln_chunk(nxt, c, sch if held else None), due,
                       _P.get('lnstep', 0.25))
            if rel >= 0:
                sch.at(rel, job)
            else:
                job()
        for q, due in enumerate(_P.get('wos', [1, 2.5, 15, 29, 43, 45])):
            spread(sch, wo_piece(jnp.minimum((i - NF) * 6 + q, 31)), due,
                   _P.get('wostep', 0.25))
        phg = _P.get('phg')
        for j in range(NJ):
            for g in range(2):
                at = 14 * j + 7 + _P.get('kvs', [7, 8])[g]
                if j == NJ - 1:
                    at = 55 + _P.get('phl', 1) * (g - 1)
                if phg:
                    for p in range(2):
                        sch.at(14 * j + 7, functools.partial(
                            tl.sm, j, g, p, at + 1 - phg[0] - phg[1] * (2 - 2 * p), phg[1]))
                if j < NJ - 1:
                    sch.at(at, functools.partial(tl.kv, j, g))
        for j in range(NJ):
            tl.kproj(j)
            tl.vproj(j)
        for g in range(2):
            tl.kv(NJ - 1, g)
        return carry

    only = _P.get('only')
    if only in (None, 'A', 'B'):
        first_tiles()
    else:
        for nm in ORDER.split():
            named_copy(nm).wait()
        if only == 'P1':
            wd_copy.wait()
    if _P.get('early', 1) and only in (None, 'P1', 'B'):
        with jax.named_scope('w:rest'):
            wo_copy.wait()
            for t in range(NF + 1, NT):
                x_copy(t).wait()
    with jax.named_scope('P1'):
        if only in (None, 'P1', 'B'):
            if _P.get('u1'):
                jax.lax.fori_loop(0, (NT - NF) // 2, phase1x2, 0)
            else:
                jax.lax.fori_loop(NF, NT, phase1, 0)
        else:
            wo_copy.wait()
            for t in range(NF + 1, NT):
                x_copy(t).wait()

    if only == 'PL':
        for t in range(2):
            out_copy(t, t).start()
    for j in range(NJ):
        w_copy(0, j).wait()
    wg_copy.wait()
    wu_copy.wait()
    if only != 'P1':
        wd_copy.wait()
    sch = Sched(zero_s[0] > 0)
    row = jax.lax.broadcasted_iota(I32, (MR, 128), 0)
    col = jax.lax.broadcasted_iota(I32, (MR, 128), 1)
    keep = (row // DH) == ((col // 2) % 2)
    for j in range(NJ):
        fold(0, aq, j, sch)
        for p in range(4 * j, 4 * j + 4):
            kvp = pltpu.bitcast(sch.hold(_u32(kv_acc[p]), [(r, 0) for r in range(8)]), F32)
            mp = _u32(jnp.where(keep, kvp, 0.0).astype(BF16))
            m_v[p] = mp
            sch.need(1 + p * 0.375, [mp])
            z_v[p] = jnp.broadcast_to(jnp.sum(z_v[p], axis=1, keepdims=True), (128, 128))

    r = _round(r_v[...].reshape(NT, T))
    rmax = jnp.max(jnp.max(r, axis=1, keepdims=True), axis=0, keepdims=True)
    pos = (jax.lax.broadcasted_iota(I32, (NT, T), 0) * T
           + jax.lax.broadcasted_iota(I32, (NT, T), 1))
    idx = jnp.min(jnp.where(r == rmax, pos, S))
    idx = jnp.clip(idx, 0, S - 1)
    tile = idx // T
    half = (idx % T) // TH
    sub = pl.multiple_of(((idx % TH) // 16) * 8, 8)
    xs = jnp.concatenate([bq[tile, 1 + 7 * half, pl.ds(sub, 8), :],
                          bq[tile, 7 - 3 * half, pl.ds(sub, 8), :]], axis=1)
    xs = jnp.where(jax.lax.broadcasted_iota(I32, (16, D), 0) == idx % 16,
                   _bf(xs).astype(F32), 0.0)
    xs = jnp.sum(xs, axis=0, keepdims=True)

    def lane_bcast(dst, row):
        for t in range(row.shape[1] // 128):
            dst[t * 128:(t + 1) * 128, :] = jnp.broadcast_to(
                row[:, t * 128:(t + 1) * 128], (128, 128)).T

    lane_bcast(xb_v, xs)
    router = _round(0.5 + 0.5 * jnp.tanh(0.5 * rmax))

    first = proj(sch, aq, 0, [_bf(bq[(tile + 1) % NT, k]) for k in range(7)])
    for g in range(2):
        pq0_v[g] = first[g]

    def phase2(i, carry):
        last = isinstance(i, int)
        zero = zero_s[0]
        never = zero > 0
        slot = i % 2
        n = tile if last else (tile + 1 + i) % NT

        if last:
            out_copy((tile + i - 1) % NT, slot).wait()
        else:
            @pl.when(i >= 2)
            def _():
                out_copy((tile + i - 1) % NT, slot).wait()

        s0 = pl.multiple_of(n * T, T)
        b = [_bf(bq[n, k]) for k in range(7)]
        pq = [None] * NJ
        ao = [None] * NJ
        sch = Sched(never)
        ot = {}
        pq[0] = [pq0_v[g] for g in range(2)]

        phis = {}

        def sm(j, g, p, due, step=0):
            phis[j, g, p] = _pack_blocks(_feature_map(
                pq[j][g][p * 64:(p + 1) * 64], z_v[4 * j + 2 * g + p]))
            if due is not None:
                for t in range(2):
                    sch.need(max(due - step * (1 - t), sch.slot + 1),
                             [phis[j, g, p][:, t * 128:(t + 1) * 128]])

        def nd(j, g):
            parts = []
            for p in range(2):
                if (j, g, p) not in phis:
                    sm(j, g, p, None)
                parts.append(_dot(_bf(m_v[4 * j + 2 * g + p]), _bf(phis[j, g, p])))
            ot[j, g] = jnp.concatenate(parts, axis=0)
            if g == 1:
                o0, o1 = ot[j, 0], ot[j, 1]
                cs = _lhs_combos(o0[:, :TH], o1[:, :TH], o0[:, TH:], o1[:, TH:])
                for k in range(7):
                    ao_v[2 * k + j // 2][zero, :, (j % 2) * 128:(j % 2 + 1) * 128] = (
                        _u32(cs[k].astype(BF16).T))

        if last:
            fd = (NFC - 1) * FC
        else:
            fu = pl.multiple_of(i * FC, FC)
            fd = pl.multiple_of(jnp.maximum(i - 1, 0) * FC, FC)
        ffn = {}

        FR = _P.get('fr', 64)

        def matvec(key, w, vb, due):
            t = (w.astype(F32).reshape(FR // 8, 8, 256)
                 * jnp.concatenate([vb, vb], axis=1).reshape(FR // 8, 8, 256))
            t = jnp.sum(t, axis=0)
            ffn[key] = t if key not in ffn else ffn[key] + t
            sch.need(due, [ffn[key]])

        def ffn_up(w_ref, name, cp, rb, due):
            rs = slice(rb * FR, (rb + 1) * FR)
            matvec((name, cp), w_ref[rs, pl.ds(fu + cp * 256, 256)], xb_v[rs, :], due)

        def ffn_mid():
            hg, hu = [_round(jnp.sum(jnp.concatenate([ffn[nm, 0], ffn[nm, 1]], axis=1),
                                     axis=0, keepdims=True)) for nm in 'gu']
            lane_bcast(hb_v, _round(_round(_silu(hg)) * hu))

        def ffn_down(cp, rb, due):
            cs_ = slice(cp * 256, (cp + 1) * 256)
            if rb == 0:
                ffn['y', cp] = y_acc[:, cs_]
            matvec(('y', cp), wd_v[pl.ds(fd + rb * FR, FR), cs_],
                   hb_v[rb * FR:(rb + 1) * FR, :], due)
            if rb == FC // FR - 1:
                if last:
                    ffn['row', cp] = (
                        _round(jnp.sum(ffn['y', cp], axis=0, keepdims=True)) * router)
                else:
                    y_acc[:, cs_] = ffn['y', cp]

        d0, d1, u0, u1 = _P.get('ffn', [28, 36.5, 37, 53.5])
        if last:
            d0, d1 = _P.get('ffnl', [2, 27])
        nd_ = 4 * FC // FR
        for t in range(nd_):
            due = eighths(d0 + (d1 - d0) * t / (nd_ - 1))
            sch.at(0, functools.partial(ffn_down, t % 4, t // 4, due))
        if not last:
            nu_ = 4 * D // FR
            for t in range(nu_):
                due = eighths(u0 + (u1 - u0) * t / (nu_ - 1))
                name, w_ref = (('g', wg_v), ('u', wu_v))[(t // 2) % 2]
                sch.at(0, functools.partial(ffn_up, w_ref, name, t % 2, t // 4, due))
            sch.at(int(u1), ffn_mid)
        for j in range(NJ):
            s1 = 7 * j
            sfx = 'l' if last else ''
            nds = (_P.get('nds0' + sfx, [1, 4] if last else [2, 4]) if j == 0
                   else _P.get('nds' + sfx, [1, 4]) if j < NJ - 1
                   else _P.get('nds3l', [2, 3]) if last else _P.get('nds3', [0, 1]))
            phq = _P.get('phq' + sfx, [0.5, 0.5] if last else [0, 0.5])
            for g in range(2):
                if phq:
                    for p in range(2):
                        sch.at(s1 if (j == 0 or g == 1) else s1 - 2, functools.partial(
                            sm, j, g, p, s1 + nds[g] + 1 - phq[0] - phq[1] * (2 - 2 * p), phq[1]))
                sch.at(s1 + nds[g], functools.partial(nd, j, g))
        for j in range(1, NJ):
            pq[j] = proj(sch, aq, j, b, early=pq)
        part = {}
        if last:
            def prod_a(k, step):
                return _dot(_bf(sch.gate(ao_v[2 * k][0])), _bf(bo[k, 0:128, 0:256]))
            part = _strassen(prod_a, sch.after)
        else:
            nxt = proj(sch, aq, 0, [_bf(bq[(n + 1) % NT, k]) for k in range(7)])
            for g in range(2):
                pq0_v[g] = nxt[g]

        ER = _P.get('er' + sfx, 32 if last else 64)
        rows = jax.lax.broadcasted_iota(I32, (ER, 256), 0) + s0
        ne_ = T // ER
        gates = {}

        def gate_part(c, e, due):
            r0 = e * ER
            h, rh = r0 // TH, r0 % TH
            blk = ((1, 7), (8, 4))[h][c // 2]
            bb = _bf(bq[n, blk, rh // 2:(rh + ER) // 2,
                        (c % 2) * 256:(c % 2 + 1) * 256]).astype(F32)
            if last:
                bb = bb + jnp.where(rows + r0 == idx, ffn['row', c], 0.0)
            gates[c, e] = _silu(bb)
            if due is not None:
                sch.need(due, [gates[c, e]])

        def epilogue(c, cc, e, due):
            r0 = e * ER
            h, rh = r0 // TH, r0 % TH
            cs = slice(c * 256, (c + 1) * 256)
            rs = slice(rh, rh + ER)
            if (c, e) not in gates:
                gate_part(c, e, None)
            xr = x_v[pl.ds(s0 + r0, ER), cs].astype(F32)
            sv = jnp.concatenate([cc[2 * h][rs], cc[2 * h + 1][rs]], axis=1)
            res = xr + sv * gates[c, e]
            out_v[slot, r0:r0 + ER, cs] = res.astype(BF16)
            if due is not None:
                sch.need(due, [res])

        def out_cols(c):
            cs = slice(c * 256, (c + 1) * 256)
            return pltpu.make_async_copy(out_v.at[slot, :, cs],
                                         out_hbm.at[0, pl.ds(s0, T), cs], sem_o.at[2 + c])

        e0, e1 = _P.get('epi' + sfx, [1, 6.5] if last else [0.5, 6.5])
        g0, g1 = _P.get('gl' + sfx, [0, 4])
        end = sch.slot + 28 - (7 if last else 0)
        for e in range(ne_):
            sch.at(end - 8, functools.partial(
                gate_part, 3, e, eighths(end - 7 + g0 + (g1 - g0) * e / (ne_ - 1))))
        pending = []
        c = 0
        while c < 4:
            if last and c == 0:
                def prod(k, step):
                    return _dot(_bf(sch.gate(ao_v[2 * k + 1][0])),
                                _bf(bo[k, 128:256, 0:256]))
                cc2 = [u + v for u, v in zip(part, _strassen(prod, sch.after))]
                blocks = [(t, [v[:, t * 128:(t + 1) * 128] for v in cc2]) for t in range(2)]
            else:
                def prod(k, step):
                    return _dot(_bf(sch.gate(jnp.concatenate(
                        [ao_v[2 * k][0], ao_v[2 * k + 1][0]], axis=1))),
                                _bf(bo[k, :, c * 128:(c + 1) * 128]))
                blocks = [(c, _strassen(prod, sch.after))]
            if last:
                for t in pending:
                    out_cols(t).start()
                pending = []
            nb = len(blocks) * ne_
            for q in range(nb):
                t, cc = blocks[q // ne_]
                due = eighths(sch.slot + e0 + (e1 - e0) * q / (nb - 1))
                epilogue(t, cc, q % ne_, due if t < 3 else None)
            pending = [t for t, _ in blocks]
            c += len(blocks)
        if last:
            out_cols(3).start()
            out_copy((tile + i) % NT, 1 - slot).wait()
            for t in range(4):
                out_cols(t).wait()
        else:
            out_copy(n, slot).start()
        return carry

    with jax.named_scope('P2'):
        if only in (None, 'P2'):
            jax.lax.fori_loop(0, NT - 1, phase2, 0)
    if only in (None, 'PL'):
        with jax.named_scope('PL'):
            phase2(NT - 1, 0)
    elif only == 'P2':
        for t in (NT - 3, NT - 2):
            out_copy((tile + 1 + t) % NT, t % 2).wait()


@jax.jit
def pallas_recurrent_scan__linear_kernel_hedgehog__moe_arch_mod__prompt_kernel(
    A_x: jax.Array,
    A_wqkv: jax.Array,
    A_w_phi: jax.Array,
    A_wo: jax.Array,
    B_x: jax.Array,
    B_w_r: jax.Array,
    B_w_gate: jax.Array,
    B_w_up: jax.Array,
    B_w_down: jax.Array,
):
    del B_x
    any_spec = pl.BlockSpec(memory_space=pl.ANY)
    return pl.pallas_call(
        _kernel,
        out_shape=jax.ShapeDtypeStruct((1, S, D), BF16),
        in_specs=[any_spec] * 8,
        out_specs=any_spec,
        scratch_shapes=[
            pltpu.VMEM((S, D), BF16),
            pltpu.VMEM((3, D, D), BF16),
            pltpu.VMEM((H, DH, DH), BF16),
            pltpu.VMEM((8, 128), BF16),
            pltpu.VMEM((D, D), BF16),
            pltpu.VMEM((D, F), BF16),
            pltpu.VMEM((D, F), BF16),
            pltpu.VMEM((F, D), BF16),
            pltpu.VMEM((NT, 9, TH // 2, DHALF), U32),
            pltpu.VMEM((7, 256, DHALF), U32),
            pltpu.VMEM((7, 256, DHALF), U32),
            pltpu.VMEM((7, 256, DHALF), U32),
            pltpu.VMEM((7, 256, DHALF), U32),
            pltpu.VMEM((NP, MR, 128), F32),
            pltpu.VMEM((NP, 128, 128), F32),
            pltpu.VMEM((NP, MR // 2, 128), U32),
            pltpu.VMEM((128, D), BF16),
            pltpu.VMEM((8, DHALF), U32),
            pltpu.VMEM((NT, 1, T), F32),
            pltpu.VMEM((8, D), F32),
            pltpu.VMEM((D, 128), F32),
            pltpu.VMEM((FC, 128), F32),
            pltpu.VMEM((2, 128, T), F32),
            pltpu.VMEM((2, T, D), BF16),
            pltpu.SMEM((1,), I32),
        ] + [pltpu.VMEM((1, TH // 2, 256), U32)] * 14,
        compiler_params=pltpu.CompilerParams(
            vmem_limit_bytes=100 * 1024 * 1024,
            disable_bounds_checks=bool(_P.get('nbc', 1)),
            shape_invariant_numerics=bool(_P.get('sin', 1))),
    )(A_x, A_wqkv, A_w_phi, A_wo, B_w_r.reshape(8, 128), B_w_gate, B_w_up, B_w_down)
```

```python
import functools
import os
import json
_P = json.loads(os.environ.get('KP', '{}'))

import jax
import jax.numpy as jnp
import jax.experimental.pallas as pl
import jax.experimental.pallas.tpu as pltpu

S, D, H, DH, F = 2048, 1024, 32, 32, 3584
T = 256
TH = T // 2
DHALF = D // 2
NT = S // T
NJ = 4
NP = D // 64
MR = 64
FC = 512
NFC = F // FC
NF = _P.get('nf', 2)
ORDER = 'ph wr k0 x0 x1 k1 k2 k3 v0 v1 v2 v3 x2'
PROG = ('w:ph,wr P w:k0 f0 w:x0 U0 w:x1 L1:3:6 K0a',
        'w:k1 f1 K0b S0a K1a S0b K1b',
        'w:k2,k3,v0 f2 S1a K2a f3 p0:14:18 S1b K2b S2a K3a S2b K3b',
        'w:v1,v2,v3,x2 p1:3:8 p2:16:21 p3:30:35 L2:6:52 V0a X0a V0b '
        'X0b V1a X1a V1b X1b V2a X2a V2b X2b V3a X3a V3b Y3b')
LOG2E = 1.4426950408889634
F32, BF16, U32, I32 = jnp.float32, jnp.bfloat16, jnp.uint32, jnp.int32

_NT_DIMS = (((1,), (1,)), ((), ()))


def _dot_nt(a, b):
    return jax.lax.dot_general(a, b, _NT_DIMS, preferred_element_type=F32)


def _dot(a, b):
    return jnp.dot(a, b, preferred_element_type=F32)


def _u32(v):
    return pltpu.bitcast(v, U32) if v.dtype != U32 else v


def _pack(v):
    return pltpu.bitcast(v.astype(BF16), U32)


def _recip(x):
    r = pl.reciprocal(x, approx=True)
    return r * (2.0 - x * r)


def _bf(v):
    return pltpu.bitcast(v, BF16)


def _round(v):
    return v.astype(BF16).astype(F32)


def _or_all(vals):
    ts = []
    for v in vals:
        u = _u32(v)
        for a in range(u.shape[0] // 8):
            for b in range(u.shape[1] // 128):
                ts.append(u[a * 8:(a + 1) * 8, b * 128:(b + 1) * 128])
    while len(ts) > 1:
        ts = [ts[i] | ts[i + 1] if i + 1 < len(ts) else ts[i] for i in range(0, len(ts), 2)]
    return ts[0]


def _gate(lhs_u32, deps, never):
    if not deps:
        return lhs_u32
    rows = []
    for r in range(lhs_u32.shape[0] // 8):
        row = lhs_u32[r * 8:(r + 1) * 8]
        cs = [c for (r_, c) in deps if r_ == r]
        if cs:
            row = jnp.concatenate(
                [jnp.where(never, _or_all(deps[r, c]), row[:, c * 128:(c + 1) * 128])
                 if c in cs else row[:, c * 128:(c + 1) * 128]
                 for c in range(lhs_u32.shape[1] // 128)], axis=1)
        rows.append(row)
    return jnp.concatenate(rows, axis=0)


def _layernorm(x):
    m = jnp.mean(x, axis=-1, keepdims=True)
    mb = _round(m)
    xc = x - mb
    dm = m - mb
    v = jnp.mean(xc * xc, axis=-1, keepdims=True) - dm * dm
    a = _round(_round(v) + 1e-5)
    rs = jax.lax.rsqrt(a)
    sd = a * rs
    sd = _round(sd + (0.5 * rs) * (a - sd * sd))
    return xc * _recip(sd)


def _lhs_combos(a11, a12, a21, a22):
    return [a11 + a22, a21 + a22, a11, a22, a11 + a12, a21 - a11, a12 - a22]


def _rhs_combos(b11, b12, b21, b22):
    return [b11 + b22, b11, b12 - b22, b21 - b11, b22, b11 + b12, b21 + b22]


def _strassen(prod, after=None):
    done = {}

    def p(k, step):
        return prod(k, step)

    def hook(step):
        if after is not None:
            after(step, done)

    m1 = p(0, 0)
    hook(0)
    m4 = p(3, 1)
    hook(1)
    m5 = p(4, 2)
    hook(2)
    m7 = p(6, 3)
    done[0] = m1 + m4 - m5 + m7
    hook(3)
    m3 = p(2, 4)
    done[1] = m3 + m5
    hook(4)
    m2 = p(1, 5)
    done[2] = m2 + m4
    hook(5)
    m6 = p(5, 6)
    done[3] = m1 - m2 + m3 + m6
    hook(6)
    return done[0], done[1], done[2], done[3]


def _allreduce_pair(x, op):
    x = op(x, pltpu.roll(x, 2, axis=0))
    return op(x, pltpu.roll(x, 4, axis=0))


def _feature_map(p, z=None):
    t = p.shape[1]
    p3 = p.reshape(8, 8, t)
    mx = _allreduce_pair(jnp.max(p3, axis=0), jnp.maximum)
    mn = _allreduce_pair(jnp.min(p3, axis=0), jnp.minimum)
    ep = jnp.exp2(p3 - mx[None])
    en = jnp.exp2(mn[None] - p3)
    rp = _recip(_allreduce_pair(jnp.sum(ep, axis=0), jnp.add))
    rn = _recip(_allreduce_pair(jnp.sum(en, axis=0), jnp.add))
    if z is not None:
        z4 = jnp.concatenate([z] * (t // 128), axis=1).reshape(2, 8, 8, t)
        den = rp * jnp.sum(ep * z4[0], axis=0) + rn * jnp.sum(en * z4[1], axis=0)
        inv = _recip(_allreduce_pair(den, jnp.add) + 1e-6)
        rp, rn = rp * inv, rn * inv
    pos = (ep * rp[None]).reshape(64, t)
    neg = (en * rn[None]).reshape(64, t)
    return jnp.concatenate([pos, neg], axis=0), (rp, rn)


def _silu(x):
    h = 0.5 * x
    return h + h * jnp.tanh(h)


def _kernel(*refs):
    pl.run_scoped(functools.partial(_body, *refs),
                  pltpu.SemaphoreType.DMA((NT + 18,)), pltpu.SemaphoreType.DMA((6,)))


def _body(x_hbm, wqkv_hbm, wphi_hbm, wo_hbm, wr_hbm, wg_hbm, wu_hbm, wd_hbm,
            out_hbm,
            x_v, w_v, wphi_v, wr_v, wo_v, wg_v, wu_v, wd_v,
            bq, ak, av, aq, bo, kv_acc, z_v, ph_v, vt_v, m_v, phit, wr2, r_v, y_acc, xb_v, hb_v, pq0_v,
            out_v, zero_s, *rest):
    ao_v, bp, (sem, sem_o) = rest[:-4], rest[-4:-2], rest[-2:]
    def x_copy(i):
        return pltpu.make_async_copy(x_hbm.at[0, pl.ds(i * T, T), :],
                                     x_v.at[pl.ds(i * T, T), :], sem.at[i])

    def w_copy(m, j):
        return pltpu.make_async_copy(
            wqkv_hbm.at[:, m * D + j * 256:m * D + (j + 1) * 256],
            w_v.at[m, :, j * 256:(j + 1) * 256], sem.at[NT + 6 + 4 * m + j])

    wphi_copy = pltpu.make_async_copy(wphi_hbm, wphi_v, sem.at[NT])
    wr_copy = pltpu.make_async_copy(wr_hbm, wr_v, sem.at[NT + 1])
    wo_copy = pltpu.make_async_copy(wo_hbm, wo_v, sem.at[NT + 2])
    wg_copy = pltpu.make_async_copy(wg_hbm, wg_v, sem.at[NT + 3])
    wu_copy = pltpu.make_async_copy(wu_hbm, wu_v, sem.at[NT + 4])
    wd_copy = pltpu.make_async_copy(wd_hbm, wd_v, sem.at[NT + 5])

    def out_copy(i, slot):
        return pltpu.make_async_copy(out_v.at[slot],
                                     out_hbm.at[0, pl.ds(i * T, T), :],
                                     sem_o.at[slot])

    def named_copy(nm):
        if nm in ('ph', 'wr'):
            return wphi_copy if nm == 'ph' else wr_copy
        t = int(nm[1])
        return x_copy(t) if nm[0] == 'x' else w_copy({'k': 1, 'v': 2}[nm[0]], t)

    for nm in _P.get('order', ORDER).split():
        named_copy(nm).start()
    x_copy(NF + 1).start()
    wo_copy.start()
    for i in range(NF + 2, NT):
        x_copy(i).start()
    for j in range(NJ):
        w_copy(0, j).start()
    wg_copy.start()
    wu_copy.start()
    wd_copy.start()

    zero_s[0] = 0
    kv_acc[...] = jnp.zeros_like(kv_acc)
    y_acc[...] = jnp.zeros_like(y_acc)
    z_v[...] = jnp.zeros_like(z_v)
    hb_v[...] = jnp.zeros_like(hb_v)

    def build_phit():
        row = jax.lax.broadcasted_iota(I32, (128, DH), 0)
        col = jax.lax.broadcasted_iota(I32, (128, DH), 1)
        sel = jnp.where((row % 64) // 2 == col, 1.0, 0.0).astype(BF16)
        wall = wphi_v[...].reshape(H * DH, DH)
        ph = _dot_nt(sel, wall)
        row = jax.lax.broadcasted_iota(I32, (128, D), 0)
        col = jax.lax.broadcasted_iota(I32, (128, D), 1)
        keep = (2 * (row // 64) + row % 2) == ((col % 128) // DH)
        phit[...] = jnp.where(keep, ph, 0.0).astype(BF16)
        wr = wr_v[...].astype(F32)
        halves = [jnp.concatenate([jnp.broadcast_to(wr[4 * h + t:4 * h + t + 1], (16, 128))
                                   for t in range(4)], axis=1) for h in range(2)]
        odd = jax.lax.broadcasted_iota(I32, (16, DHALF), 0) % 2 == 1
        wr2[...] = _pack(jnp.where(odd, halves[1], halves[0]))

    def fold(which, dst, j, sch=None):
        wt = []
        for g in (2 * j, 2 * j + 1):
            r_ = _dot_nt(phit[:, g * 128:(g + 1) * 128],
                         w_v[which, :, g * 128:(g + 1) * 128])
            if sch is not None and g == 2 * j:
                sch.token = r_[0:8, 0:128]
            wt.append(r_ * LOG2E)
        w0, w1 = wt
        cs = _lhs_combos(w0[:, :DHALF], w0[:, DHALF:], w1[:, :DHALF], w1[:, DHALF:])
        for k in range(7):
            dst.at[k][j * 64:(j + 1) * 64, :] = _pack(cs[k])

    def prep_v(j, sch=None):
        ws = [_u32(w_v[2, :, g * 128:(g + 1) * 128]) for g in (2 * j, 2 * j + 1)]
        if sch is not None:
            ws = [sch.hold(w, [(8 * q, 0) for q in range(8)]) for w in ws]
        wt = [_bf(w).T for w in ws]
        f0, f1 = [w.astype(F32) for w in wt]
        w0, w1 = [_u32(w) for w in wt]
        cs = _lhs_combos(f0[:, :DHALF], f0[:, DHALF:], f1[:, :DHALF], f1[:, DHALF:])
        for k in range(7):
            u = w0[:, :DHALF] if k == 2 else w1[:, DHALF:] if k == 3 else _pack(cs[k])
            av.at[k][j * 64:(j + 1) * 64, :] = u
        return w0, w1

    def ln_chunk(n, c, sch=None, also=None):
        ys = []
        for h in range(2):
            r0 = n * T + h * TH + c * 16
            if not isinstance(r0, int):
                r0 = pl.multiple_of(r0, 16)
            xr = x_v[pl.ds(r0, 16), :].astype(F32)
            if sch is not None:
                xr = pltpu.bitcast(sch.hold(_u32(xr), [(0, 0), (1, 0)]), F32)
            ys.append(_layernorm(xr))
        ya, yb = ys
        cs = (_rhs_combos(ya[:, :DHALF], yb[:, :DHALF], ya[:, DHALF:], yb[:, DHALF:])
              + [ya[:, DHALF:], yb[:, :DHALF]])
        out = []
        for k in range(9):
            dst = bq.at[n, k]
            u = _pack(cs[k])
            dst[c * 8:(c + 1) * 8, :] = u
            if also is not None and k < 7:
                dst = also.at[k]
                dst[c * 8:(c + 1) * 8, :] = u
            out.append(dst[c * 8:(c + 1) * 8, :])
        mode = _P.get('lng', 'y') if not isinstance(n, int) else 'st'
        if mode == 'y':
            return [ya[:, :DHALF], ya[:, DHALF:], yb[:, :DHALF], yb[:, DHALF:]]
        if mode == 'cs':
            return [cs[k] for k in (0, 2, 3, 5, 6)]
        return out

    def wo_piece(e):
        r0 = pl.multiple_of((e // 8) * 256 + (e % 8) * 16, 16)
        o0 = pl.multiple_of(e * 8, 8)
        w0 = wo_v[pl.ds(r0, 16), :].astype(F32)
        w1 = wo_v[pl.ds(r0 + 128, 16), :].astype(F32)

        def cols(w, par):
            return jnp.concatenate(
                [w[:, (2 * q + par) * 128:(2 * q + par + 1) * 128] for q in range(4)], axis=1)
        cs = _rhs_combos(cols(w0, 0), cols(w0, 1), cols(w1, 0), cols(w1, 1))
        out = []
        for k in range(7):
            dst = bo.at[k]
            dst[pl.ds(o0, 8), :] = _pack(cs[k])
            out.append(dst[pl.ds(o0, 8), :])
        if _P.get('wog', 'cs') == 'cs':
            return [cs[k] for k in (0, 2, 3, 5, 6)]
        return out

    class Sched:
        def __init__(self, never):
            self.never = never
            self.slot = 0
            self.gated = 0
            self.token = None
            self.jobs = {}
            self.deps = {}

        def at(self, slot, fn):
            self.jobs.setdefault(slot, []).append(fn)

        def need(self, pos, vals):
            slot, r = divmod(int(round(pos * 8)), 8)
            assert slot >= self.gated, (pos, self.slot)
            d = self.deps.setdefault(slot, {})
            c = (slot + r) % 4
            d.setdefault((r, c), []).extend(vals)

        def gate(self, lhs):
            nc = lhs.shape[1] // 128
            self.gated = self.slot + 1
            deps = {}
            for (r, c), v in self.deps.pop(self.slot, {}).items():
                deps.setdefault((r, c % nc), []).extend(v)
            return _gate(lhs, deps, self.never)

        def hold(self, u, blocks):
            if self.token is None:
                return u
            return _gate(u, {rc: [self.token] for rc in blocks}, self.never)

        def after(self, step, done):
            for fn in self.jobs.pop(self.slot, []):
                fn()
            self.slot += 1

    def proj(sch, a_ref, j, b, extra=None, early=None):
        def prod(k, step):
            lhs = sch.gate(a_ref[k, j * 64:(j + 1) * 64, :])
            if extra is not None and k in (1, 2, 3, 4):
                r_ = _dot_nt(_bf(jnp.concatenate([lhs, wr2[...]], axis=0)), b[k])
                extra[k] = r_[128:136]
                r_ = r_[0:128]
            else:
                r_ = _dot_nt(_bf(lhs), b[k])
            sch.token = r_[0:8, 0:128]
            return r_
        def after(step, done):
            if step == 4 and early is not None:
                early[j] = [jnp.concatenate([done[0], done[1]], axis=1), None]
            sch.after(step, done)
        c11, c12, c21, c22 = _strassen(prod, after)
        return (jnp.concatenate([c11, c12], axis=1),
                jnp.concatenate([c21, c22], axis=1))

    class KVTile:
        def __init__(self, sch, i, src=None):
            self.src = src
            self.sch, self.i = sch, i
            self.slot = i if isinstance(i, int) else 0
            self.b = None
            self.pk, self.vt, self.phis = {}, {}, {}

        def operands(self):
            if self.b is None:
                if self.src is not None:
                    return [_bf(self.src[k]) for k in range(7)]
                self.b = [_bf(bq[self.i, k]) for k in range(7)]
            return self.b

        def kproj(self, j):
            self.pk[j] = proj(self.sch, ak, j, self.operands())

        def vproj(self, j):
            ex = {} if j == 0 else None
            vs = proj(self.sch, av, j, self.operands(), ex)
            self.vt[j] = vs
            for g in range(2):
                for p in range(2):
                    if isinstance(self.i, int) or not _P.get('vtd'):
                        vt_v.at[self.slot, 2 * j + g][p * 32:(p + 1) * 32, :] = _pack(
                            vs[g][p * 64:(p + 1) * 64])
            if j == 0:
                r_v[self.i] = jnp.concatenate(
                    [ex[1][0:1] + ex[1][1:2] + ex[3][1:2],
                     ex[4][0:1] + ex[4][1:2] + ex[2][0:1]], axis=1)

        def sm(self, j, g, p, due=None, step=0):
            phi, _ = _feature_map(self.pk[j][g][p * 64:(p + 1) * 64])
            z_v[4 * j + 2 * g + p] += phi[:, :128] + phi[:, 128:]
            if due is None:
                self.phis[j, g, p] = lambda: phi.astype(BF16)
                return
            dst = ph_v.at[self.i, 4 * j + 2 * g + p]
            for t in range(2):
                dst[t * 32:(t + 1) * 32, :] = _pack(phi[t * 64:(t + 1) * 64])
            self.phis[j, g, p] = lambda: _bf(dst[...])
            for t in range(2):
                self.sch.need(due - step * (1 - t), [dst[:, t * 128:(t + 1) * 128]])

        def kv(self, j, g):
            for p in range(2):
                if (j, g, p) not in self.phis:
                    self.sm(j, g, p)
                if isinstance(self.i, int) or not _P.get('vtd'):
                    lhs = _bf(vt_v[self.slot, 2 * j + g, p * 32:(p + 1) * 32, :])
                else:
                    lhs = self.vt[j][g][p * 64:(p + 1) * 64].astype(BF16)
                kv_acc[4 * j + 2 * g + p] += _dot_nt(lhs, self.phis[j, g, p]())

    def spread(sch, vals, due, step=0.25):
        for t in range(4):
            sch.need(due + t * step, [v[:, t * 128:(t + 1) * 128] for v in vals])

    def eighths(x):
        return round(x * 8) / 8

    def first_tiles():
        sch = Sched(zero_s[0] > 0)
        tiles = {'a': KVTile(sch, 0), 'b': KVTile(sch, 1)}
        prog = _P.get('prog') or ' '.join(_P.get('seg%d' % t, PROG[t]) for t in range(4))
        for op in prog.split():
            kind, arg = op[0], op[1:2]
            if kind == 'w':
                with jax.named_scope(op):
                    for nm in op[2:].split(','):
                        named_copy(nm).wait()
            elif kind == 'P':
                build_phit()
            elif kind == 'f':
                fold(1, ak, int(arg))
            elif kind == 'p':
                _, rel, d0 = op.split(':')

                def job(j=int(arg), base=sch.slot + float(d0), rel=int(rel)):
                    ws = prep_v(j, sch if rel >= 0 else None)
                    for q in range(8):
                        sch.need(base + q * _P.get('pvs', 0.5),
                                 [w[:, q * 128:(q + 1) * 128] for w in ws])
                if int(rel) < 0:
                    job()
                else:
                    sch.at(sch.slot + int(rel), job)
            elif kind == 'U':
                for c in range(8):
                    ln_chunk(int(arg), c)
            elif kind == 'L':
                _, l0, l1 = op.split(':')
                for c in range(8):
                    due = eighths(sch.slot + float(l0) + (float(l1) - float(l0)) * c / 7)
                    rel = int(due - _P.get('lrel', 4.5))

                    def job(n=int(arg), c=c, due=due, held=rel >= sch.slot):
                        spread(sch, ln_chunk(n, c, sch if held else None,
                                             bp[0] if (n == NF and _P.get('u1', 0)) else None), due)
                    if rel >= sch.slot:
                        sch.at(rel, job)
                    else:
                        job()
            elif kind == 'S':
                a0, a1 = _P.get('s1', [1.5, 6.5])
                st_ = (a1 - a0) / 7
                for q in range(4):
                    tiles[op[2]].sm(int(arg), q // 2, q % 2,
                                    eighths(sch.slot + a0 + st_ * (2 * q + 1)), eighths(st_))
            elif kind == 'K':
                tiles[op[2]].kproj(int(arg))
            elif kind == 'V':
                tiles[op[2]].vproj(int(arg))
            elif kind == 'X':
                for g in range(2):
                    sch.at(sch.slot + _P.get('xo', [1, 4])[g],
                           functools.partial(tiles[op[2]].kv, int(arg), g))
            elif kind == 'Y':
                for g in range(2):
                    tiles[op[2]].kv(int(arg), g)
        assert not sch.jobs and not sch.deps, (sch.jobs.keys(), sch.deps.keys())

    def phase1_waits(i, n):
        if _P.get('early', 1):
            return
        for d in range(n):
            @pl.when(i + 1 + d < NT)
            def _():
                x_copy(i + 1 + d).wait()

        @pl.when(i == NF)
        def _():
            wo_copy.wait()

    def phase1(i, carry):
        phase1_waits(i, 1)
        return phase1_tile(i, carry)

    def phase1x2(m, carry):
        i = NF + 2 * m
        phase1_waits(i, 2)
        phase1_tile(i, carry, 0)
        return phase1_tile(i + 1, carry, 1)

    def phase1_tile(i, carry, par=None):
        nxt = jnp.minimum(i + 1, NT - 1)
        sch = Sched(zero_s[0] > 0)
        tl = KVTile(sch, i, None if par is None else bp[par])
        tl.slot = par or 0
        tl.operands()
        lrel = _P.get('lrel1')
        for c in range(8):
            due = 14 * (c // 2) + _P.get('ln', [6, 13])[c % 2]
            rel = int(due - lrel) if lrel else -1

            def job(c=c, due=due, held=rel >= 0):
                spread(sch, ln_chunk(nxt, c, sch if held else None,
                                     None if par is None else bp[1 - par]), due,
                       _P.get('lnstep', 0.25))
            if rel >= 0:
                sch.at(rel, job)
            else:
                job()
        for q, due in enumerate(_P.get('wos', [1, 15, 17, 29, 31, 43])):
            spread(sch, wo_piece(jnp.minimum((i - NF) * 6 + q, 31)), due,
                   _P.get('wostep', 0.25))
        phg = _P.get('phg')
        for j in range(NJ):
            for g in range(2):
                at = 14 * j + 7 + _P.get('kvs', [7, 8])[g]
                if j == NJ - 1:
                    at = 55 + _P.get('phl', 1) * (g - 1)
                if phg:
                    for p in range(2):
                        sch.at(14 * j + 7, functools.partial(
                            tl.sm, j, g, p, at + 1 - phg[0] - phg[1] * (2 - 2 * p), phg[1]))
                if j < NJ - 1:
                    sch.at(at, functools.partial(tl.kv, j, g))
        for j in range(NJ):
            tl.kproj(j)
            tl.vproj(j)
        for g in range(2):
            tl.kv(NJ - 1, g)
        return carry

    only = _P.get('only')
    if only in (None, 'A', 'B'):
        first_tiles()
    else:
        for nm in ORDER.split():
            named_copy(nm).wait()
        if only == 'P1':
            wd_copy.wait()
    if _P.get('early', 1) and only in (None, 'P1', 'B'):
        with jax.named_scope('w:rest'):
            wo_copy.wait()
            for t in range(NF + 1, NT):
                x_copy(t).wait()
    with jax.named_scope('P1'):
        if only in (None, 'P1', 'B'):
            if _P.get('u1', 0):
                jax.lax.fori_loop(0, (NT - NF) // 2, phase1x2, 0)
            else:
                jax.lax.fori_loop(NF, NT, phase1, 0)
        else:
            wo_copy.wait()
            for t in range(NF + 1, NT):
                x_copy(t).wait()

    if only == 'PL':
        for t in range(2):
            out_copy(t, t).start()
    for j in range(NJ):
        w_copy(0, j).wait()
    wg_copy.wait()
    wu_copy.wait()
    if only != 'P1':
        wd_copy.wait()
    sch = Sched(zero_s[0] > 0)
    row = jax.lax.broadcasted_iota(I32, (MR, 128), 0)
    col = jax.lax.broadcasted_iota(I32, (MR, 128), 1)
    keep = (row // DH) == (col % 2)
    for j in range(NJ):
        fold(0, aq, j, sch)
        for p in range(4 * j, 4 * j + 4):
            kvp = pltpu.bitcast(sch.hold(_u32(kv_acc[p]), [(r, 0) for r in range(8)]), F32)
            mk = jnp.where(keep, kvp, 0.0)
            for t in range(2):
                m_v.at[p][t * 16:(t + 1) * 16, :] = _pack(mk[t * 32:(t + 1) * 32])
            sch.need(1 + p * 0.375, [m_v[p]])
            z_v[p] = jnp.broadcast_to(jnp.sum(z_v[p], axis=1, keepdims=True), (128, 128))

    r = _round(r_v[...].reshape(NT, T))
    rmax = jnp.max(jnp.max(r, axis=1, keepdims=True), axis=0, keepdims=True)
    pos = (jax.lax.broadcasted_iota(I32, (NT, T), 0) * T
           + jax.lax.broadcasted_iota(I32, (NT, T), 1))
    idx = jnp.min(jnp.where(r == rmax, pos, S))
    idx = jnp.clip(idx, 0, S - 1)
    tile = idx // T
    half = (idx % T) // TH
    sub = pl.multiple_of(((idx % TH) // 16) * 8, 8)
    xs = jnp.concatenate([bq[tile, 1 + 7 * half, pl.ds(sub, 8), :],
                          bq[tile, 7 - 3 * half, pl.ds(sub, 8), :]], axis=1)
    xs = jnp.where(jax.lax.broadcasted_iota(I32, (16, D), 0) == idx % 16,
                   _bf(xs).astype(F32), 0.0)
    xs = jnp.sum(xs, axis=0, keepdims=True)

    def lane_bcast(dst, row):
        for t in range(row.shape[1] // 128):
            dst[t * 128:(t + 1) * 128, :] = jnp.broadcast_to(
                row[:, t * 128:(t + 1) * 128], (128, 128)).T

    lane_bcast(xb_v, xs)
    router = _round(0.5 + 0.5 * jnp.tanh(0.5 * rmax))

    first = proj(sch, aq, 0, [_bf(bq[(tile + 1) % NT, k]) for k in range(7)])
    for g in range(2):
        pq0_v[g] = first[g]

    def phase2(i, carry):
        last = isinstance(i, int)
        zero = zero_s[0]
        never = zero > 0
        slot = i % 2
        n = tile if last else (tile + 1 + i) % NT

        if last:
            out_copy((tile + i - 1) % NT, slot).wait()
        else:
            @pl.when(i >= 2)
            def _():
                out_copy((tile + i - 1) % NT, slot).wait()

        s0 = pl.multiple_of(n * T, T)
        b = [_bf(bq[n, k]) for k in range(7)]
        pq = [None] * NJ
        ao = [None] * NJ
        sch = Sched(never)
        ot = {}
        pq[0] = [pq0_v[g] for g in range(2)]

        phis = {}

        def sm(j, g, p, due, step=0):
            phi, scales = _feature_map(pq[j][g][p * 64:(p + 1) * 64], z_v[4 * j + 2 * g + p])
            phis[j, g, p] = phi.astype(BF16)
            if due is not None:
                for t in range(2):
                    sch.need(max(due - step * (1 - t), sch.slot + 1),
                             [v[:, t * 128:(t + 1) * 128] for v in scales])

        def nd(j, g):
            parts = []
            for p in range(2):
                if (j, g, p) not in phis:
                    sm(j, g, p, None)
                parts.append(_dot(_bf(m_v[4 * j + 2 * g + p]), phis[j, g, p]))
            ot[j, g] = jnp.concatenate(parts, axis=0)
            if g == 1:
                o0, o1 = ot[j, 0], ot[j, 1]
                cs = _lhs_combos(o0[:, :TH], o1[:, :TH], o0[:, TH:], o1[:, TH:])
                for k in range(7):
                    ao_v[2 * k + j // 2][zero, :, (j % 2) * 128:(j % 2 + 1) * 128] = (
                        _u32(cs[k].astype(BF16).T))

        if last:
            fd = (NFC - 1) * FC
        else:
            fu = pl.multiple_of(i * FC, FC)
            fd = pl.multiple_of(jnp.maximum(i - 1, 0) * FC, FC)
        ffn = {}

        FR = _P.get('fr', 64)

        def matvec(key, w, vb, due):
            t = (w.astype(F32).reshape(FR // 8, 8, 256)
                 * jnp.concatenate([vb, vb], axis=1).reshape(FR // 8, 8, 256))
            t = jnp.sum(t, axis=0)
            ffn[key] = t if key not in ffn else ffn[key] + t
            sch.need(due, [ffn[key]])

        def ffn_up(w_ref, name, cp, rb, due):
            rs = slice(rb * FR, (rb + 1) * FR)
            matvec((name, cp), w_ref[rs, pl.ds(fu + cp * 256, 256)], xb_v[rs, :], due)

        def ffn_mid():
            hg, hu = [_round(jnp.sum(jnp.concatenate([ffn[nm, 0], ffn[nm, 1]], axis=1),
                                     axis=0, keepdims=True)) for nm in 'gu']
            lane_bcast(hb_v, _round(_round(_silu(hg)) * hu))

        def ffn_down(cp, rb, due):
            cs_ = slice(cp * 256, (cp + 1) * 256)
            if rb == 0:
                ffn['y', cp] = y_acc[:, cs_]
            matvec(('y', cp), wd_v[pl.ds(fd + rb * FR, FR), cs_],
                   hb_v[rb * FR:(rb + 1) * FR, :], due)
            if rb == FC // FR - 1:
                if last:
                    ffn['row', cp] = (
                        _round(jnp.sum(ffn['y', cp], axis=0, keepdims=True)) * router)
                else:
                    y_acc[:, cs_] = ffn['y', cp]

        d0, d1, u0, u1 = _P.get('ffn', [28, 36.5, 37, 53.5])
        if last:
            d0, d1 = _P.get('ffnl', [2, 27])
        nd_ = 4 * FC // FR
        for t in range(nd_):
            due = eighths(d0 + (d1 - d0) * t / (nd_ - 1))
            sch.at(0, functools.partial(ffn_down, t % 4, t // 4, due))
        if not last:
            nu_ = 4 * D // FR
            for t in range(nu_):
                due = eighths(u0 + (u1 - u0) * t / (nu_ - 1))
                name, w_ref = (('g', wg_v), ('u', wu_v))[(t // 2) % 2]
                sch.at(0, functools.partial(ffn_up, w_ref, name, t % 2, t // 4, due))
            sch.at(int(u1), ffn_mid)
        for j in range(NJ):
            s1 = 7 * j
            sfx = 'l' if last else ''
            nds = (_P.get('nds0' + sfx, [1, 4]) if j == 0
                   else _P.get('nds' + sfx, [1, 4] if last else [0, 3]) if j < NJ - 1
                   else _P.get('nds3l', [2, 3]) if last else _P.get('nds3', [0, 1]))
            phq = _P.get('phq' + sfx, [0.5, 0.5] if last else [0, 0.5])
            for g in range(2):
                if phq:
                    for p in range(2):
                        sch.at(s1 if (j == 0 or g == 1) else s1 - 2, functools.partial(
                            sm, j, g, p, s1 + nds[g] + 1 - phq[0] - phq[1] * (2 - 2 * p), phq[1]))
                sch.at(s1 + nds[g], functools.partial(nd, j, g))
        for j in range(1, NJ):
            pq[j] = proj(sch, aq, j, b, early=pq)
        part = {}
        if last:
            def prod_a(k, step):
                return _dot(_bf(sch.gate(ao_v[2 * k][0])), _bf(bo[k, 0:128, 0:256]))
            part = _strassen(prod_a, sch.after)
        else:
            nxt = proj(sch, aq, 0, [_bf(bq[(n + 1) % NT, k]) for k in range(7)])
            for g in range(2):
                pq0_v[g] = nxt[g]

        ER = _P.get('er' + sfx, 32 if last else 64)
        rows = jax.lax.broadcasted_iota(I32, (ER, 256), 0) + s0
        ne_ = T // ER
        gates = {}

        def gate_part(c, e, due):
            r0 = e * ER
            h, rh = r0 // TH, r0 % TH
            blk = ((1, 7), (8, 4))[h][c // 2]
            bb = _bf(bq[n, blk, rh // 2:(rh + ER) // 2,
                        (c % 2) * 256:(c % 2 + 1) * 256]).astype(F32)
            if last:
                bb = bb + jnp.where(rows + r0 == idx, ffn['row', c], 0.0)
            gates[c, e] = _silu(bb)
            if due is not None:
                sch.need(due, [gates[c, e]])

        def epilogue(c, cc, e, due):
            r0 = e * ER
            h, rh = r0 // TH, r0 % TH
            cs = slice(c * 256, (c + 1) * 256)
            rs = slice(rh, rh + ER)
            if (c, e) not in gates:
                gate_part(c, e, None)
            xr = x_v[pl.ds(s0 + r0, ER), cs].astype(F32)
            sv = jnp.concatenate([cc[2 * h][rs], cc[2 * h + 1][rs]], axis=1)
            res = xr + sv * gates[c, e]
            out_v[slot, r0:r0 + ER, cs] = res.astype(BF16)
            if due is not None:
                sch.need(due, [res])

        def out_cols(c):
            cs = slice(c * 256, (c + 1) * 256)
            return pltpu.make_async_copy(out_v.at[slot, :, cs],
                                         out_hbm.at[0, pl.ds(s0, T), cs], sem_o.at[2 + c])

        e0, e1 = _P.get('epi' + sfx, [1, 6.5] if last else [0.5, 6.5])
        g0, g1 = _P.get('gl' + sfx, [0, 4])
        end = sch.slot + 28 - (7 if last else 0)
        for e in range(ne_):
            sch.at(end - 8, functools.partial(
                gate_part, 3, e, eighths(end - 7 + g0 + (g1 - g0) * e / (ne_ - 1))))
        pending = []
        c = 0
        while c < 4:
            if last and c == 0:
                def prod(k, step):
                    return _dot(_bf(sch.gate(ao_v[2 * k + 1][0])),
                                _bf(bo[k, 128:256, 0:256]))
                cc2 = [u + v for u, v in zip(part, _strassen(prod, sch.after))]
                blocks = [(t, [v[:, t * 128:(t + 1) * 128] for v in cc2]) for t in range(2)]
            else:
                def prod(k, step):
                    return _dot(_bf(sch.gate(jnp.concatenate(
                        [ao_v[2 * k][0], ao_v[2 * k + 1][0]], axis=1))),
                                _bf(bo[k, :, c * 128:(c + 1) * 128]))
                blocks = [(c, _strassen(prod, sch.after))]
            if last:
                for t in pending:
                    out_cols(t).start()
                pending = []
            nb = len(blocks) * ne_
            for q in range(nb):
                t, cc = blocks[q // ne_]
                due = eighths(sch.slot + e0 + (e1 - e0) * q / (nb - 1))
                epilogue(t, cc, q % ne_, due if t < 3 else None)
            pending = [t for t, _ in blocks]
            c += len(blocks)
        if last:
            out_cols(3).start()
            out_copy((tile + i) % NT, 1 - slot).wait()
            for t in range(4):
                out_cols(t).wait()
        else:
            out_copy(n, slot).start()
        return carry

    with jax.named_scope('P2'):
        if only in (None, 'P2'):
            jax.lax.fori_loop(0, NT - 1, phase2, 0)
    if only in (None, 'PL'):
        with jax.named_scope('PL'):
            phase2(NT - 1, 0)
    elif only == 'P2':
        for t in (NT - 3, NT - 2):
            out_copy((tile + 1 + t) % NT, t % 2).wait()


@jax.jit
def pallas_recurrent_scan__linear_kernel_hedgehog__moe_arch_mod__prompt_kernel(
    A_x: jax.Array,
    A_wqkv: jax.Array,
    A_w_phi: jax.Array,
    A_wo: jax.Array,
    B_x: jax.Array,
    B_w_r: jax.Array,
    B_w_gate: jax.Array,
    B_w_up: jax.Array,
    B_w_down: jax.Array,
):
    del B_x
    any_spec = pl.BlockSpec(memory_space=pl.ANY)
    return pl.pallas_call(
        _kernel,
        out_shape=jax.ShapeDtypeStruct((1, S, D), BF16),
        in_specs=[any_spec] * 8,
        out_specs=any_spec,
        scratch_shapes=[
            pltpu.VMEM((S, D), BF16),
            pltpu.VMEM((3, D, D), BF16),
            pltpu.VMEM((H, DH, DH), BF16),
            pltpu.VMEM((8, 128), BF16),
            pltpu.VMEM((D, D), BF16),
            pltpu.VMEM((D, F), BF16),
            pltpu.VMEM((D, F), BF16),
            pltpu.VMEM((F, D), BF16),
            pltpu.VMEM((NT, 9, TH // 2, DHALF), U32),
            pltpu.VMEM((7, 256, DHALF), U32),
            pltpu.VMEM((7, 256, DHALF), U32),
            pltpu.VMEM((7, 256, DHALF), U32),
            pltpu.VMEM((7, 256, DHALF), U32),
            pltpu.VMEM((NP, MR, 128), F32),
            pltpu.VMEM((NP, 128, 128), F32),
            pltpu.VMEM((NF, NP, 64, T), U32),
            pltpu.VMEM((NF, 8, 64, T), U32),
            pltpu.VMEM((NP, MR // 2, 128), U32),
            pltpu.VMEM((128, D), BF16),
            pltpu.VMEM((8, DHALF), U32),
            pltpu.VMEM((NT, 1, T), F32),
            pltpu.VMEM((8, D), F32),
            pltpu.VMEM((D, 128), F32),
            pltpu.VMEM((FC, 128), F32),
            pltpu.VMEM((2, 128, T), F32),
            pltpu.VMEM((2, T, D), BF16),
            pltpu.SMEM((1,), I32),
        ] + [pltpu.VMEM((1, TH // 2, 256), U32)] * 14
        + [pltpu.VMEM((7, TH // 2, DHALF), U32)] * 2,
        compiler_params=pltpu.CompilerParams(
            vmem_limit_bytes=100 * 1024 * 1024,
            disable_bounds_checks=bool(_P.get('nbc', 1)),
            shape_invariant_numerics=bool(_P.get('sin', 1))),
    )(A_x, A_wqkv, A_w_phi, A_wo, B_w_r.reshape(8, 128), B_w_gate, B_w_up, B_w_down)
```

```python
import functools

import jax
import jax.numpy as jnp
import jax.experimental.pallas as pl
import jax.experimental.pallas.tpu as pltpu

S, D, H, DH, F = 2048, 1024, 32, 32, 3584
T = 256
TH = T // 2
DHALF = D // 2
NT = S // T
NJ = 4
NP = D // 64
FC = 512
NFC = F // FC
FR = 64
NF = 2
ORDER = 'ph wr k0 x0 x1 k1 k2 k3 v0 v1 v2 v3 x2'
PROG = ('w:ph,wr P w:k0 f0 w:x0 U0 w:x1 L1:3:6 K0a '
        'w:k1 f1 K0b S0a K1a S0b K1b '
        'w:k2,k3,v0 f2 S1a K2a f3 p0:14:18 S1b K2b S2a K3a S2b K3b '
        'w:v1,v2,v3,x2 p1:3:8 p2:16:21 p3:30:35 L2:6:52 V0a X0a V0b '
        'X0b V1a X1a V1b X1b V2a X2a V2b X2b V3a X3a V3b Y3b')
LOG2E = 1.4426950408889634
F32, BF16, U32, I32 = jnp.float32, jnp.bfloat16, jnp.uint32, jnp.int32

_NT_DIMS = (((1,), (1,)), ((), ()))


def _dot_nt(a, b):
    return jax.lax.dot_general(a, b, _NT_DIMS, preferred_element_type=F32)


def _dot(a, b):
    return jnp.dot(a, b, preferred_element_type=F32)


def _u32(v):
    return pltpu.bitcast(v, U32) if v.dtype != U32 else v


def _pack(v):
    return pltpu.bitcast(v.astype(BF16), U32)


def _recip(x):
    r = pl.reciprocal(x, approx=True)
    return r * (2.0 - x * r)


def _bf(v):
    return pltpu.bitcast(v, BF16)


def _round(v):
    return v.astype(BF16).astype(F32)


def _eighths(x):
    return round(x * 8) / 8


def _or_all(vals):
    ts = []
    for v in vals:
        u = _u32(v)
        for a in range(u.shape[0] // 8):
            for b in range(u.shape[1] // 128):
                ts.append(u[a * 8:(a + 1) * 8, b * 128:(b + 1) * 128])
    while len(ts) > 1:
        ts = [ts[i] | ts[i + 1] if i + 1 < len(ts) else ts[i] for i in range(0, len(ts), 2)]
    return ts[0]


def _gate(lhs_u32, deps, never):
    if not deps:
        return lhs_u32
    rows = []
    for r in range(lhs_u32.shape[0] // 8):
        row = lhs_u32[r * 8:(r + 1) * 8]
        cs = [c for (r_, c) in deps if r_ == r]
        if cs:
            row = jnp.concatenate(
                [jnp.where(never, _or_all(deps[r, c]), row[:, c * 128:(c + 1) * 128])
                 if c in cs else row[:, c * 128:(c + 1) * 128]
                 for c in range(lhs_u32.shape[1] // 128)], axis=1)
        rows.append(row)
    return jnp.concatenate(rows, axis=0)


class Sched:
    def __init__(self, never):
        self.never = never
        self.slot = 0
        self.gated = 0
        self.token = None
        self.jobs = {}
        self.deps = {}

    def at(self, slot, fn):
        self.jobs.setdefault(slot, []).append(fn)

    def need(self, pos, vals):
        slot, r = divmod(int(round(pos * 8)), 8)
        assert slot >= self.gated, (pos, self.slot)
        d = self.deps.setdefault(slot, {})
        c = (slot + r) % 4
        d.setdefault((r, c), []).extend(vals)

    def spread(self, vals, due, step=0.25):
        for t in range(4):
            self.need(due + t * step, [v[:, t * 128:(t + 1) * 128] for v in vals])

    def gate(self, lhs):
        nc = lhs.shape[1] // 128
        self.gated = self.slot + 1
        deps = {}
        for (r, c), v in self.deps.pop(self.slot, {}).items():
            deps.setdefault((r, c % nc), []).extend(v)
        return _gate(lhs, deps, self.never)

    def hold(self, u, blocks):
        if self.token is None:
            return u
        return _gate(u, {rc: [self.token] for rc in blocks}, self.never)

    def after(self, step, done):
        for fn in self.jobs.pop(self.slot, []):
            fn()
        self.slot += 1


def _layernorm(x):
    m = jnp.mean(x, axis=-1, keepdims=True)
    mb = _round(m)
    xc = x - mb
    dm = m - mb
    v = jnp.mean(xc * xc, axis=-1, keepdims=True) - dm * dm
    a = _round(_round(v) + 1e-5)
    rs = jax.lax.rsqrt(a)
    sd = a * rs
    sd = _round(sd + (0.5 * rs) * (a - sd * sd))
    return xc * _recip(sd)


def _lhs_combos(a11, a12, a21, a22):
    return [a11 + a22, a21 + a22, a11, a22, a11 + a12, a21 - a11, a12 - a22]


def _rhs_combos(b11, b12, b21, b22):
    return [b11 + b22, b11, b12 - b22, b21 - b11, b22, b11 + b12, b21 + b22]


def _strassen(prod, after):
    done = {}
    m1 = prod(0)
    after(0, done)
    m4 = prod(3)
    after(1, done)
    m5 = prod(4)
    after(2, done)
    m7 = prod(6)
    done[0] = m1 + m4 - m5 + m7
    after(3, done)
    m3 = prod(2)
    done[1] = m3 + m5
    after(4, done)
    m2 = prod(1)
    done[2] = m2 + m4
    after(5, done)
    m6 = prod(5)
    done[3] = m1 - m2 + m3 + m6
    after(6, done)
    return done[0], done[1], done[2], done[3]


def _allreduce_pair(x, op):
    x = op(x, pltpu.roll(x, 2, axis=0))
    return op(x, pltpu.roll(x, 4, axis=0))


def _feature_map(p, z=None):
    t = p.shape[1]
    p3 = p.reshape(8, 8, t)
    mx = _allreduce_pair(jnp.max(p3, axis=0), jnp.maximum)
    mn = _allreduce_pair(jnp.min(p3, axis=0), jnp.minimum)
    ep = jnp.exp2(p3 - mx[None])
    en = jnp.exp2(mn[None] - p3)
    rp = _recip(_allreduce_pair(jnp.sum(ep, axis=0), jnp.add))
    rn = _recip(_allreduce_pair(jnp.sum(en, axis=0), jnp.add))
    if z is not None:
        z4 = jnp.concatenate([z] * (t // 128), axis=1).reshape(2, 8, 8, t)
        den = rp * jnp.sum(ep * z4[0], axis=0) + rn * jnp.sum(en * z4[1], axis=0)
        inv = _recip(_allreduce_pair(den, jnp.add) + 1e-6)
        rp, rn = rp * inv, rn * inv
    pos = (ep * rp[None]).reshape(64, t)
    neg = (en * rn[None]).reshape(64, t)
    return jnp.concatenate([pos, neg], axis=0), (rp, rn)


def _silu(x):
    h = 0.5 * x
    return h + h * jnp.tanh(h)


def _kernel(*refs):
    pl.run_scoped(functools.partial(_body, *refs),
                  pltpu.SemaphoreType.DMA((NT + 18,)), pltpu.SemaphoreType.DMA((7,)))


def _body(x_hbm, wqkv_hbm, wphi_hbm, wo_hbm, wr_hbm, wg_hbm, wu_hbm, wd_hbm,
          out_hbm,
          x_v, w_v, wphi_v, wr_v, wo_v, wg_v, wu_v, wd_v,
          bq, ak, av, aq, bo, kv_acc, z_v, ph_v, vt_v, m_v, phit, wr2, r_v,
          y_acc, xb_v, hb_v, pq0_v, out_v, zero_s, *rest):
    ao_v, (sem, sem_o) = rest[:-2], rest[-2:]

    def x_copy(i):
        return pltpu.make_async_copy(x_hbm.at[0, pl.ds(i * T, T), :],
                                     x_v.at[pl.ds(i * T, T), :], sem.at[i])

    def w_copy(m, j):
        return pltpu.make_async_copy(
            wqkv_hbm.at[:, m * D + j * 256:m * D + (j + 1) * 256],
            w_v.at[m, :, j * 256:(j + 1) * 256], sem.at[NT + 6 + 4 * m + j])

    wphi_copy = pltpu.make_async_copy(wphi_hbm, wphi_v, sem.at[NT])
    wr_copy = pltpu.make_async_copy(wr_hbm, wr_v, sem.at[NT + 1])
    wo_copy = pltpu.make_async_copy(wo_hbm, wo_v, sem.at[NT + 2])
    wg_copy = pltpu.make_async_copy(wg_hbm, wg_v, sem.at[NT + 3])
    wu_copy = pltpu.make_async_copy(wu_hbm, wu_v, sem.at[NT + 4])
    wd_copy = pltpu.make_async_copy(wd_hbm, wd_v, sem.at[NT + 5])

    def out_copy(i, slot):
        return pltpu.make_async_copy(out_v.at[slot],
                                     out_hbm.at[0, pl.ds(i * T, T), :],
                                     sem_o.at[slot])

    def named_copy(nm):
        if nm in ('ph', 'wr'):
            return wphi_copy if nm == 'ph' else wr_copy
        t = int(nm[1])
        return x_copy(t) if nm[0] == 'x' else w_copy({'k': 1, 'v': 2}[nm[0]], t)

    for nm in ORDER.split():
        named_copy(nm).start()
    x_copy(NF + 1).start()
    wo_copy.start()
    for i in range(NF + 2, NT):
        x_copy(i).start()
    for j in range(NJ):
        w_copy(0, j).start()
    wg_copy.start()
    wu_copy.start()
    wd_copy.start()

    zero_s[0] = 0
    kv_acc[...] = jnp.zeros_like(kv_acc)
    y_acc[...] = jnp.zeros_like(y_acc)
    z_v[...] = jnp.zeros_like(z_v)
    hb_v[...] = jnp.zeros_like(hb_v)

    def build_phit():
        row = jax.lax.broadcasted_iota(I32, (128, DH), 0)
        col = jax.lax.broadcasted_iota(I32, (128, DH), 1)
        sel = jnp.where((row % 64) // 2 == col, 1.0, 0.0).astype(BF16)
        wall = wphi_v[...].reshape(H * DH, DH)
        ph = _dot_nt(sel, wall)
        row = jax.lax.broadcasted_iota(I32, (128, D), 0)
        col = jax.lax.broadcasted_iota(I32, (128, D), 1)
        keep = (2 * (row // 64) + row % 2) == ((col % 128) // DH)
        phit[...] = jnp.where(keep, ph * LOG2E, 0.0).astype(BF16)
        wr = wr_v[...].astype(F32)
        halves = [jnp.concatenate([jnp.broadcast_to(wr[4 * h + t:4 * h + t + 1], (16, 128))
                                   for t in range(4)], axis=1) for h in range(2)]
        odd = jax.lax.broadcasted_iota(I32, (16, DHALF), 0) % 2 == 1
        wr2[...] = _pack(jnp.where(odd, halves[1], halves[0]))

    def fold(which, dst, j, sch=None):
        wt = []
        for g in (2 * j, 2 * j + 1):
            r_ = _dot_nt(phit[:, g * 128:(g + 1) * 128],
                         w_v[which, :, g * 128:(g + 1) * 128])
            if sch is not None and g == 2 * j:
                sch.token = r_[0:8, 0:128]
            wt.append(r_)
        w0, w1 = wt
        cs = _lhs_combos(w0[:, :DHALF], w0[:, DHALF:], w1[:, :DHALF], w1[:, DHALF:])
        for k in range(7):
            dst.at[k][j * 64:(j + 1) * 64, :] = _pack(cs[k])

    def prep_v(j, sch):
        ws = [_u32(w_v[2, :, g * 128:(g + 1) * 128]) for g in (2 * j, 2 * j + 1)]
        ws = [sch.hold(w, [(8 * q, 0) for q in range(8)]) for w in ws]
        wt = [_bf(w).T for w in ws]
        f0, f1 = [w.astype(F32) for w in wt]
        w0, w1 = [_u32(w) for w in wt]
        cs = _lhs_combos(f0[:, :DHALF], f0[:, DHALF:], f1[:, :DHALF], f1[:, DHALF:])
        for k in range(7):
            u = w0[:, :DHALF] if k == 2 else w1[:, DHALF:] if k == 3 else _pack(cs[k])
            av.at[k][j * 64:(j + 1) * 64, :] = u
        return w0, w1

    def ln_chunk(n, c, sch=None):
        ys = []
        for h in range(2):
            r0 = n * T + h * TH + c * 16
            if not isinstance(r0, int):
                r0 = pl.multiple_of(r0, 16)
            xr = x_v[pl.ds(r0, 16), :].astype(F32)
            if sch is not None:
                xr = pltpu.bitcast(sch.hold(_u32(xr), [(0, 0), (1, 0)]), F32)
            ys.append(_layernorm(xr))
        ya, yb = ys
        cs = (_rhs_combos(ya[:, :DHALF], yb[:, :DHALF], ya[:, DHALF:], yb[:, DHALF:])
              + [ya[:, DHALF:], yb[:, :DHALF]])
        out = []
        for k in range(9):
            dst = bq.at[n, k]
            dst[c * 8:(c + 1) * 8, :] = _pack(cs[k])
            if isinstance(n, int):
                out.append(dst[c * 8:(c + 1) * 8, :])
        if isinstance(n, int):
            return out
        return [ya[:, :DHALF], ya[:, DHALF:], yb[:, :DHALF], yb[:, DHALF:]]

    def wo_piece(e):
        r0 = pl.multiple_of((e // 8) * 256 + (e % 8) * 16, 16)
        o0 = pl.multiple_of(e * 8, 8)
        w0 = wo_v[pl.ds(r0, 16), :].astype(F32)
        w1 = wo_v[pl.ds(r0 + 128, 16), :].astype(F32)

        def cols(w, par):
            return jnp.concatenate(
                [w[:, (2 * q + par) * 128:(2 * q + par + 1) * 128] for q in range(4)], axis=1)
        cs = _rhs_combos(cols(w0, 0), cols(w0, 1), cols(w1, 0), cols(w1, 1))
        for k in range(7):
            bo.at[k][pl.ds(o0, 8), :] = _pack(cs[k])
        return [cs[k] for k in (0, 2, 3, 5, 6)]

    def proj(sch, a_ref, j, b, extra=None, early=None):
        def prod(k):
            lhs = sch.gate(a_ref[k, j * 64:(j + 1) * 64, :])
            if extra is not None and k in (1, 2, 3, 4):
                r_ = _dot_nt(_bf(jnp.concatenate([lhs, wr2[...]], axis=0)), b[k])
                extra[k] = r_[128:136]
                r_ = r_[0:128]
            else:
                r_ = _dot_nt(_bf(lhs), b[k])
            sch.token = r_[0:8, 0:128]
            return r_

        def after(step, done):
            if step == 4 and early is not None:
                early[j] = [jnp.concatenate([done[0], done[1]], axis=1), None]
            sch.after(step, done)
        c11, c12, c21, c22 = _strassen(prod, after)
        return (jnp.concatenate([c11, c12], axis=1),
                jnp.concatenate([c21, c22], axis=1))

    class KVTile:
        def __init__(self, sch, i):
            self.sch, self.i = sch, i
            self.slot = i if isinstance(i, int) else 0
            self.b = None
            self.pk, self.phis = {}, {}

        def operands(self):
            if self.b is None:
                self.b = [_bf(bq[self.i, k]) for k in range(7)]
            return self.b

        def kproj(self, j):
            self.pk[j] = proj(self.sch, ak, j, self.operands())

        def vproj(self, j):
            ex = {} if j == 0 else None
            vs = proj(self.sch, av, j, self.operands(), ex)
            for g in range(2):
                for p in range(2):
                    vt_v.at[self.slot, 2 * j + g][p * 32:(p + 1) * 32, :] = _pack(
                        vs[g][p * 64:(p + 1) * 64])
            if j == 0:
                r_v[self.i] = jnp.concatenate(
                    [ex[1][0:1] + ex[1][1:2] + ex[3][1:2],
                     ex[4][0:1] + ex[4][1:2] + ex[2][0:1]], axis=1)

        def sm(self, j, g, p, due=None, step=0):
            phi, _ = _feature_map(self.pk[j][g][p * 64:(p + 1) * 64])
            z_v[4 * j + 2 * g + p] += phi[:, :128] + phi[:, 128:]
            if due is None:
                self.phis[j, g, p] = lambda: phi.astype(BF16)
                return
            dst = ph_v.at[self.i, 4 * j + 2 * g + p]
            for t in range(2):
                dst[t * 32:(t + 1) * 32, :] = _pack(phi[t * 64:(t + 1) * 64])
            self.phis[j, g, p] = lambda: _bf(dst[...])
            for t in range(2):
                self.sch.need(due - step * (1 - t), [dst[:, t * 128:(t + 1) * 128]])

        def kv(self, j, g):
            for p in range(2):
                if (j, g, p) not in self.phis:
                    self.sm(j, g, p)
                lhs = _bf(vt_v[self.slot, 2 * j + g, p * 32:(p + 1) * 32, :])
                kv_acc[4 * j + 2 * g + p] += _dot_nt(lhs, self.phis[j, g, p]())

    def first_tiles():
        sch = Sched(zero_s[0] > 0)
        tiles = {'a': KVTile(sch, 0), 'b': KVTile(sch, 1)}
        for op in PROG.split():
            kind, arg = op[0], op[1:2]
            if kind == 'w':
                for nm in op[2:].split(','):
                    named_copy(nm).wait()
            elif kind == 'P':
                build_phit()
            elif kind == 'f':
                fold(1, ak, int(arg))
            elif kind == 'p':
                _, rel, d0 = op.split(':')

                def job(j=int(arg), base=sch.slot + float(d0)):
                    ws = prep_v(j, sch)
                    for q in range(8):
                        sch.need(base + q * 0.5, [w[:, q * 128:(q + 1) * 128] for w in ws])
                sch.at(sch.slot + int(rel), job)
            elif kind == 'U':
                for c in range(8):
                    ln_chunk(int(arg), c)
            elif kind == 'L':
                _, l0, l1 = op.split(':')
                for c in range(8):
                    due = _eighths(sch.slot + float(l0) + (float(l1) - float(l0)) * c / 7)
                    rel = int(due - 4.5)

                    def job(n=int(arg), c=c, due=due, held=rel >= sch.slot):
                        sch.spread(ln_chunk(n, c, sch if held else None), due)
                    if rel >= sch.slot:
                        sch.at(rel, job)
                    else:
                        job()
            elif kind == 'S':
                st_ = 5.0 / 7
                for q in range(4):
                    tiles[op[2]].sm(int(arg), q // 2, q % 2,
                                    _eighths(sch.slot + 1.5 + st_ * (2 * q + 1)), _eighths(st_))
            elif kind == 'K':
                tiles[op[2]].kproj(int(arg))
            elif kind == 'V':
                tiles[op[2]].vproj(int(arg))
            elif kind == 'X':
                for g in range(2):
                    sch.at(sch.slot + 1 + g, functools.partial(tiles[op[2]].kv, int(arg), g))
            elif kind == 'Y':
                for g in range(2):
                    tiles[op[2]].kv(int(arg), g)
        assert not sch.jobs and not sch.deps

    def phase1(i, carry):
        nxt = jnp.minimum(i + 1, NT - 1)
        sch = Sched(zero_s[0] > 0)
        tl = KVTile(sch, i)
        tl.operands()
        for c in range(8):
            sch.spread(ln_chunk(nxt, c), 14 * (c // 2) + (6, 13)[c % 2])
        for q, due in enumerate((1, 15, 17, 29, 31, 43)):
            sch.spread(wo_piece(jnp.minimum((i - NF) * 6 + q, 31)), due)
        for j in range(NJ - 1):
            for g in range(2):
                sch.at(14 * (j + 1) + g, functools.partial(tl.kv, j, g))
        for j in range(NJ):
            tl.kproj(j)
            tl.vproj(j)
        for g in range(2):
            tl.kv(NJ - 1, g)
        return carry

    first_tiles()
    wo_copy.wait()
    for t in range(NF + 1, NT):
        x_copy(t).wait()
    jax.lax.fori_loop(NF, NT, phase1, 0)

    for j in range(NJ):
        w_copy(0, j).wait()
    wg_copy.wait()
    wu_copy.wait()
    wd_copy.wait()
    sch = Sched(zero_s[0] > 0)
    row = jax.lax.broadcasted_iota(I32, (64, 128), 0)
    col = jax.lax.broadcasted_iota(I32, (64, 128), 1)
    keep = (row // DH) == (col % 2)
    for j in range(NJ):
        fold(0, aq, j, sch)
        for p in range(4 * j, 4 * j + 4):
            kvp = pltpu.bitcast(sch.hold(_u32(kv_acc[p]), [(r, 0) for r in range(8)]), F32)
            mk = jnp.where(keep, kvp, 0.0)
            for t in range(2):
                m_v.at[p][t * 16:(t + 1) * 16, :] = _pack(mk[t * 32:(t + 1) * 32])
            sch.need(1 + p * 0.375, [m_v[p]])
            z_v[p] = jnp.broadcast_to(jnp.sum(z_v[p], axis=1, keepdims=True), (128, 128))

    r = _round(r_v[...].reshape(NT, T))
    rmax = jnp.max(jnp.max(r, axis=1, keepdims=True), axis=0, keepdims=True)
    pos = (jax.lax.broadcasted_iota(I32, (NT, T), 0) * T
           + jax.lax.broadcasted_iota(I32, (NT, T), 1))
    idx = jnp.min(jnp.where(r == rmax, pos, S))
    idx = jnp.clip(idx, 0, S - 1)
    tile = idx // T
    half = (idx % T) // TH
    sub = pl.multiple_of(((idx % TH) // 16) * 8, 8)
    xs = jnp.concatenate([bq[tile, 1 + 7 * half, pl.ds(sub, 8), :],
                          bq[tile, 7 - 3 * half, pl.ds(sub, 8), :]], axis=1)
    xs = jnp.where(jax.lax.broadcasted_iota(I32, (16, D), 0) == idx % 16,
                   _bf(xs).astype(F32), 0.0)
    xs = jnp.sum(xs, axis=0, keepdims=True)

    def lane_bcast(dst, row):
        for t in range(row.shape[1] // 128):
            dst[t * 128:(t + 1) * 128, :] = jnp.broadcast_to(
                row[:, t * 128:(t + 1) * 128], (128, 128)).T

    lane_bcast(xb_v, xs)
    router = _round(0.5 + 0.5 * jnp.tanh(0.5 * rmax))

    first = proj(sch, aq, 0, [_bf(bq[(tile + 1) % NT, k]) for k in range(7)])
    for g in range(2):
        pq0_v[g] = first[g]

    def phase2(i, carry):
        last = isinstance(i, int)
        zero = zero_s[0]
        slot = i % 2
        n = tile if last else (tile + 1 + i) % NT

        if last:
            out_copy((tile + i - 1) % NT, slot).wait()
        else:
            @pl.when(i >= 2)
            def _():
                out_copy((tile + i - 1) % NT, slot).wait()

        s0 = pl.multiple_of(n * T, T)
        b = [_bf(bq[n, k]) for k in range(7)]
        pq = [None] * NJ
        sch = Sched(zero > 0)
        ot = {}
        pq[0] = [pq0_v[g] for g in range(2)]
        phis = {}

        def sm(j, g, p, due, step):
            phi, scales = _feature_map(pq[j][g][p * 64:(p + 1) * 64], z_v[4 * j + 2 * g + p])
            phis[j, g, p] = phi.astype(BF16)
            for t in range(2):
                sch.need(max(due - step * (1 - t), sch.slot + 1),
                         [v[:, t * 128:(t + 1) * 128] for v in scales])

        def nd(j, g):
            ot[j, g] = jnp.concatenate(
                [_dot(_bf(m_v[4 * j + 2 * g + p]), phis[j, g, p]) for p in range(2)], axis=0)
            if g == 1:
                o0, o1 = ot[j, 0], ot[j, 1]
                cs = _lhs_combos(o0[:, :TH], o1[:, :TH], o0[:, TH:], o1[:, TH:])
                for k in range(7):
                    ao_v[2 * k + j // 2][zero, :, (j % 2) * 128:(j % 2 + 1) * 128] = (
                        _u32(cs[k].astype(BF16).T))

        if last:
            fd = (NFC - 1) * FC
        else:
            fu = pl.multiple_of(i * FC, FC)
            fd = pl.multiple_of(jnp.maximum(i - 1, 0) * FC, FC)
        ffn = {}

        def matvec(key, w, vb, due):
            t = (w.astype(F32).reshape(FR // 8, 8, 256)
                 * jnp.concatenate([vb, vb], axis=1).reshape(FR // 8, 8, 256))
            t = jnp.sum(t, axis=0)
            ffn[key] = t if key not in ffn else ffn[key] + t
            sch.need(due, [ffn[key]])

        def ffn_up(w_ref, name, cp, rb, due):
            rs = slice(rb * FR, (rb + 1) * FR)
            matvec((name, cp), w_ref[rs, pl.ds(fu + cp * 256, 256)], xb_v[rs, :], due)

        def ffn_mid():
            hg, hu = [_round(jnp.sum(jnp.concatenate([ffn[nm, 0], ffn[nm, 1]], axis=1),
                                     axis=0, keepdims=True)) for nm in 'gu']
            lane_bcast(hb_v, _round(_round(_silu(hg)) * hu))

        def ffn_down(cp, rb, due):
            cs_ = slice(cp * 256, (cp + 1) * 256)
            if rb == 0:
                ffn['y', cp] = y_acc[:, cs_]
            matvec(('y', cp), wd_v[pl.ds(fd + rb * FR, FR), cs_],
                   hb_v[rb * FR:(rb + 1) * FR, :], due)
            if rb == FC // FR - 1:
                if last:
                    ffn['row', cp] = (
                        _round(jnp.sum(ffn['y', cp], axis=0, keepdims=True)) * router)
                else:
                    y_acc[:, cs_] = ffn['y', cp]

        d0, d1 = (2, 27) if last else (28, 36.5)
        nd_ = 4 * FC // FR
        for t in range(nd_):
            due = _eighths(d0 + (d1 - d0) * t / (nd_ - 1))
            sch.at(0, functools.partial(ffn_down, t % 4, t // 4, due))
        if not last:
            nu_ = 4 * D // FR
            for t in range(nu_):
                due = _eighths(37 + 16.5 * t / (nu_ - 1))
                name, w_ref = (('g', wg_v), ('u', wu_v))[(t // 2) % 2]
                sch.at(0, functools.partial(ffn_up, w_ref, name, t % 2, t // 4, due))
            sch.at(53, ffn_mid)
        lead = 0.5 if last else 0
        for j in range(NJ):
            s1 = 7 * j
            nds = (((1, 4), (1, 4), (1, 4), (2, 3)) if last
                   else ((1, 4), (0, 3), (0, 3), (0, 1)))[j]
            for g in range(2):
                for p in range(2):
                    sch.at(s1 if (j == 0 or g == 1) else s1 - 2, functools.partial(
                        sm, j, g, p, s1 + nds[g] + p - lead, 0.5))
                sch.at(s1 + nds[g], functools.partial(nd, j, g))
        for j in range(1, NJ):
            pq[j] = proj(sch, aq, j, b, early=pq)
        if last:
            def prod_a(k):
                return _dot(_bf(sch.gate(ao_v[2 * k][0])), _bf(bo[k, 0:128, 0:256]))
            part = _strassen(prod_a, sch.after)
        else:
            nxt = proj(sch, aq, 0, [_bf(bq[(n + 1) % NT, k]) for k in range(7)])
            for g in range(2):
                pq0_v[g] = nxt[g]

        er = 32 if last else 64
        rows = jax.lax.broadcasted_iota(I32, (er, 256), 0) + s0
        ne_ = T // er
        gates = {}

        def gate_part(c, e, due):
            r0 = e * er
            h, rh = r0 // TH, r0 % TH
            blk = ((1, 7), (8, 4))[h][c // 2]
            bb = _bf(bq[n, blk, rh // 2:(rh + er) // 2,
                        (c % 2) * 256:(c % 2 + 1) * 256]).astype(F32)
            if last:
                bb = bb + jnp.where(rows + r0 == idx, ffn['row', c], 0.0)
            gates[c, e] = _silu(bb)
            if due is not None:
                sch.need(due, [gates[c, e]])

        def epilogue(c, cc, e, due):
            r0 = e * er
            h, rh = r0 // TH, r0 % TH
            cs = slice(c * 256, (c + 1) * 256)
            rs = slice(rh, rh + er)
            if (c, e) not in gates:
                gate_part(c, e, None)
            xr = x_v[pl.ds(s0 + r0, er), cs].astype(F32)
            sv = jnp.concatenate([cc[2 * h][rs], cc[2 * h + 1][rs]], axis=1)
            res = xr + sv * gates[c, e]
            out_v[slot, r0:r0 + er, cs] = res.astype(BF16)
            if due is not None:
                sch.need(due, [res])

        def out_cols(c, h=None):
            cs = slice(c * 256, (c + 1) * 256)
            if h is None:
                return pltpu.make_async_copy(out_v.at[slot, :, cs],
                                             out_hbm.at[0, pl.ds(s0, T), cs], sem_o.at[2 + c])
            return pltpu.make_async_copy(
                out_v.at[slot, h * TH:(h + 1) * TH, cs],
                out_hbm.at[0, pl.ds(s0 + h * TH, TH), cs], sem_o.at[2 + c + h])

        e0, e1 = (1 if last else 0.5), 6.5
        end = sch.slot + 28 - (7 if last else 0)
        for e in range(ne_):
            sch.at(end - 8, functools.partial(
                gate_part, 3, e, _eighths(end - 7 + 4 * e / (ne_ - 1))))
        pending = []
        c = 0
        while c < 4:
            if last and c == 0:
                def prod(k):
                    return _dot(_bf(sch.gate(ao_v[2 * k + 1][0])),
                                _bf(bo[k, 128:256, 0:256]))
                cc2 = [u + v for u, v in zip(part, _strassen(prod, sch.after))]
                blocks = [(t, [v[:, t * 128:(t + 1) * 128] for v in cc2]) for t in range(2)]
            else:
                def prod(k):
                    return _dot(_bf(sch.gate(jnp.concatenate(
                        [ao_v[2 * k][0], ao_v[2 * k + 1][0]], axis=1))),
                                _bf(bo[k, :, c * 128:(c + 1) * 128]))
                blocks = [(c, _strassen(prod, sch.after))]
            if last:
                for t in pending:
                    out_cols(t).start()
            nb = len(blocks) * ne_
            for q in range(nb):
                t, cc = blocks[q // ne_]
                due = _eighths(sch.slot + e0 + (e1 - e0) * q / (nb - 1))
                epilogue(t, cc, q % ne_, due if t < 3 else None)
                if last and t == 3 and (q + 1) % (ne_ // 2) == 0:
                    out_cols(3, (q + 1) // (ne_ // 2) - 1).start()
            pending = [t for t, _ in blocks]
            c += len(blocks)
        if last:
            out_copy((tile + i) % NT, 1 - slot).wait()
            for t in range(3):
                out_cols(t).wait()
            for h in range(2):
                out_cols(3, h).wait()
        else:
            out_copy(n, slot).start()
        return carry

    jax.lax.fori_loop(0, NT - 1, phase2, 0)
    phase2(NT - 1, 0)


@jax.jit
def pallas_recurrent_scan__linear_kernel_hedgehog__moe_arch_mod__prompt_kernel(
    A_x: jax.Array,
    A_wqkv: jax.Array,
    A_w_phi: jax.Array,
    A_wo: jax.Array,
    B_x: jax.Array,
    B_w_r: jax.Array,
    B_w_gate: jax.Array,
    B_w_up: jax.Array,
    B_w_down: jax.Array,
):
    del B_x
    any_spec = pl.BlockSpec(memory_space=pl.ANY)
    return pl.pallas_call(
        _kernel,
        out_shape=jax.ShapeDtypeStruct((1, S, D), BF16),
        in_specs=[any_spec] * 8,
        out_specs=any_spec,
        scratch_shapes=[
            pltpu.VMEM((S, D), BF16),
            pltpu.VMEM((3, D, D), BF16),
            pltpu.VMEM((H, DH, DH), BF16),
            pltpu.VMEM((8, 128), BF16),
            pltpu.VMEM((D, D), BF16),
            pltpu.VMEM((D, F), BF16),
            pltpu.VMEM((D, F), BF16),
            pltpu.VMEM((F, D), BF16),
            pltpu.VMEM((NT, 9, TH // 2, DHALF), U32),
            pltpu.VMEM((7, 256, DHALF), U32),
            pltpu.VMEM((7, 256, DHALF), U32),
            pltpu.VMEM((7, 256, DHALF), U32),
            pltpu.VMEM((7, 256, DHALF), U32),
            pltpu.VMEM((NP, 64, 128), F32),
            pltpu.VMEM((NP, 128, 128), F32),
            pltpu.VMEM((NF, NP, 64, T), U32),
            pltpu.VMEM((NF, 8, 64, T), U32),
            pltpu.VMEM((NP, 32, 128), U32),
            pltpu.VMEM((128, D), BF16),
            pltpu.VMEM((8, DHALF), U32),
            pltpu.VMEM((NT, 1, T), F32),
            pltpu.VMEM((8, D), F32),
            pltpu.VMEM((D, 128), F32),
            pltpu.VMEM((FC, 128), F32),
            pltpu.VMEM((2, 128, T), F32),
            pltpu.VMEM((2, T, D), BF16),
            pltpu.SMEM((1,), I32),
        ] + [pltpu.VMEM((1, TH // 2, 256), U32)] * 14,
        compiler_params=pltpu.CompilerParams(
            vmem_limit_bytes=100 * 1024 * 1024,
            disable_bounds_checks=True),
    )(A_x, A_wqkv, A_w_phi, A_wo, B_w_r.reshape(8, 128), B_w_gate, B_w_up, B_w_down)
```

```python
import functools

import jax
import jax.numpy as jnp
import jax.experimental.pallas as pl
import jax.experimental.pallas.tpu as pltpu

S, D, H, DH, F = 2048, 1024, 32, 32, 3584
T = 256
TH = T // 2
DHALF = D // 2
NT = S // T
NJ = 4
NP = D // 64
FC = 512
NFC = F // FC
FR = 64
NF = 2
ORDER = 'ph wr k0 x0 x1 k1 k2 k3 v0 v1 v2 v3 x2'
PROG = ('w:ph,wr P w:k0 f0 w:x0 U0 w:x1 L1:3:6 K0a '
        'w:k1 f1 K0b S0a K1a S0b K1b '
        'w:k2,k3,v0 f2 S1a K2a f3 p0:14:18 S1b K2b S2a K3a S2b K3b '
        'w:v1,v2,v3,x2 p1:3:8 p2:16:21 p3:30:35 L2:6:52 V0a X0a V0b '
        'X0b V1a X1a V1b X1b V2a X2a V2b X2b V3a X3a V3b Y3b')
LOG2E = 1.4426950408889634
F32, BF16, U32, I32 = jnp.float32, jnp.bfloat16, jnp.uint32, jnp.int32

_NT_DIMS = (((1,), (1,)), ((), ()))


def _dot_nt(a, b):
    return jax.lax.dot_general(a, b, _NT_DIMS, preferred_element_type=F32)


def _dot(a, b):
    return jnp.dot(a, b, preferred_element_type=F32)


def _u32(v):
    return pltpu.bitcast(v, U32) if v.dtype != U32 else v


def _pack(v):
    return pltpu.bitcast(v.astype(BF16), U32)


def _recip(x):
    r = pl.reciprocal(x, approx=True)
    return r * (2.0 - x * r)


def _bf(v):
    return pltpu.bitcast(v, BF16)


def _round(v):
    return v.astype(BF16).astype(F32)


def _eighths(x):
    return round(x * 8) / 8


def _or_all(vals):
    ts = []
    for v in vals:
        u = _u32(v)
        for a in range(u.shape[0] // 8):
            for b in range(u.shape[1] // 128):
                ts.append(u[a * 8:(a + 1) * 8, b * 128:(b + 1) * 128])
    while len(ts) > 1:
        ts = [ts[i] | ts[i + 1] if i + 1 < len(ts) else ts[i] for i in range(0, len(ts), 2)]
    return ts[0]


def _gate(lhs_u32, deps, never):
    if not deps:
        return lhs_u32
    rows = []
    for r in range(lhs_u32.shape[0] // 8):
        row = lhs_u32[r * 8:(r + 1) * 8]
        cs = [c for (r_, c) in deps if r_ == r]
        if cs:
            row = jnp.concatenate(
                [jnp.where(never, _or_all(deps[r, c]), row[:, c * 128:(c + 1) * 128])
                 if c in cs else row[:, c * 128:(c + 1) * 128]
                 for c in range(lhs_u32.shape[1] // 128)], axis=1)
        rows.append(row)
    return jnp.concatenate(rows, axis=0)


class Sched:
    def __init__(self, never):
        self.never = never
        self.slot = 0
        self.gated = 0
        self.token = None
        self.jobs = {}
        self.deps = {}

    def at(self, slot, fn):
        self.jobs.setdefault(slot, []).append(fn)

    def need(self, pos, vals):
        slot, r = divmod(int(round(pos * 8)), 8)
        assert slot >= self.gated, (pos, self.slot)
        d = self.deps.setdefault(slot, {})
        c = (slot + r) % 4
        d.setdefault((r, c), []).extend(vals)

    def spread(self, vals, due, step=0.25):
        for t in range(4):
            self.need(due + t * step, [v[:, t * 128:(t + 1) * 128] for v in vals])

    def gate(self, lhs):
        nc = lhs.shape[1] // 128
        self.gated = self.slot + 1
        deps = {}
        for (r, c), v in self.deps.pop(self.slot, {}).items():
            deps.setdefault((r, c % nc), []).extend(v)
        return _gate(lhs, deps, self.never)

    def hold(self, u, blocks):
        if self.token is None:
            return u
        return _gate(u, {rc: [self.token] for rc in blocks}, self.never)

    def after(self, step, done):
        for fn in self.jobs.pop(self.slot, []):
            fn()
        self.slot += 1


def _layernorm(x):
    m = jnp.mean(x, axis=-1, keepdims=True)
    mb = _round(m)
    xc = x - mb
    dm = m - mb
    v = jnp.mean(xc * xc, axis=-1, keepdims=True) - dm * dm
    a = _round(_round(v) + 1e-5)
    rs = jax.lax.rsqrt(a)
    sd = a * rs
    sd = _round(sd + (0.5 * rs) * (a - sd * sd))
    return xc * _recip(sd)


def _lhs_combos(a11, a12, a21, a22):
    return [a11 + a22, a21 + a22, a11, a22, a11 + a12, a21 - a11, a12 - a22]


def _rhs_combos(b11, b12, b21, b22):
    return [b11 + b22, b11, b12 - b22, b21 - b11, b22, b11 + b12, b21 + b22]


def _strassen(prod, after):
    done = {}
    m1 = prod(0)
    after(0, done)
    m4 = prod(3)
    after(1, done)
    m5 = prod(4)
    after(2, done)
    m7 = prod(6)
    done[0] = m1 + m4 - m5 + m7
    after(3, done)
    m3 = prod(2)
    done[1] = m3 + m5
    after(4, done)
    m2 = prod(1)
    done[2] = m2 + m4
    after(5, done)
    m6 = prod(5)
    done[3] = m1 - m2 + m3 + m6
    after(6, done)
    return done[0], done[1], done[2], done[3]


def _allreduce_pair(x, op):
    x = op(x, pltpu.roll(x, 2, axis=0))
    return op(x, pltpu.roll(x, 4, axis=0))


def _feature_map(p, z=None):
    t = p.shape[1]
    p3 = p.reshape(8, 8, t)
    mx = _allreduce_pair(jnp.max(p3, axis=0), jnp.maximum)
    mn = _allreduce_pair(jnp.min(p3, axis=0), jnp.minimum)
    ep = jnp.exp2(p3 - mx[None])
    en = jnp.exp2(mn[None] - p3)
    rp = _recip(_allreduce_pair(jnp.sum(ep, axis=0), jnp.add))
    rn = _recip(_allreduce_pair(jnp.sum(en, axis=0), jnp.add))
    if z is not None:
        z4 = jnp.concatenate([z] * (t // 128), axis=1).reshape(2, 8, 8, t)
        den = rp * jnp.sum(ep * z4[0], axis=0) + rn * jnp.sum(en * z4[1], axis=0)
        inv = _recip(_allreduce_pair(den, jnp.add) + 1e-6)
        rp, rn = rp * inv, rn * inv
    pos = (ep * rp[None]).reshape(64, t)
    neg = (en * rn[None]).reshape(64, t)
    return jnp.concatenate([pos, neg], axis=0), (rp, rn)


def _silu(x):
    h = 0.5 * x
    return h + h * jnp.tanh(h)


def _kernel(*refs):
    pl.run_scoped(functools.partial(_body, *refs),
                  pltpu.SemaphoreType.DMA((NT + 18,)), pltpu.SemaphoreType.DMA((NT + 5,)))


def _body(x_hbm, wqkv_hbm, wphi_hbm, wo_hbm, wr_hbm, wg_hbm, wu_hbm, wd_hbm,
          out_hbm,
          x_v, w_v, wphi_v, wr_v, wo_v, wg_v, wu_v, wd_v,
          bq, ak, av, aq, bo, kv_acc, z_v, ph_v, vt_v, m_v, phit, wr2, r_v,
          y_acc, xb_v, hb_v, pq0_v, out_v, zero_s, *rest):
    ao_v, bp, (sem, sem_o) = rest[:-4], rest[-4:-2], rest[-2:]

    def x_copy(i):
        return pltpu.make_async_copy(x_hbm.at[0, pl.ds(i * T, T), :],
                                     x_v.at[pl.ds(i * T, T), :], sem.at[i])

    def w_copy(m, j):
        return pltpu.make_async_copy(
            wqkv_hbm.at[:, m * D + j * 256:m * D + (j + 1) * 256],
            w_v.at[m, :, j * 256:(j + 1) * 256], sem.at[NT + 6 + 4 * m + j])

    wphi_copy = pltpu.make_async_copy(wphi_hbm, wphi_v, sem.at[NT])
    wr_copy = pltpu.make_async_copy(wr_hbm, wr_v, sem.at[NT + 1])
    wo_copy = pltpu.make_async_copy(wo_hbm, wo_v, sem.at[NT + 2])
    wg_copy = pltpu.make_async_copy(wg_hbm, wg_v, sem.at[NT + 3])
    wu_copy = pltpu.make_async_copy(wu_hbm, wu_v, sem.at[NT + 4])
    wd_copy = pltpu.make_async_copy(wd_hbm, wd_v, sem.at[NT + 5])

    def out_copy(i, slot):
        return pltpu.make_async_copy(out_v.at[slot],
                                     out_hbm.at[0, pl.ds(i * T, T), :],
                                     sem_o.at[slot])

    def named_copy(nm):
        if nm in ('ph', 'wr'):
            return wphi_copy if nm == 'ph' else wr_copy
        t = int(nm[1])
        return x_copy(t) if nm[0] == 'x' else w_copy({'k': 1, 'v': 2}[nm[0]], t)

    for nm in ORDER.split():
        named_copy(nm).start()
    x_copy(NF + 1).start()
    wo_copy.start()
    for i in range(NF + 2, NT):
        x_copy(i).start()
    for j in range(NJ):
        w_copy(0, j).start()
    wg_copy.start()
    wu_copy.start()
    wd_copy.start()

    zero_s[0] = 0
    kv_acc[...] = jnp.zeros_like(kv_acc)
    y_acc[...] = jnp.zeros_like(y_acc)
    z_v[...] = jnp.zeros_like(z_v)
    hb_v[...] = jnp.zeros_like(hb_v)

    def build_phit():
        row = jax.lax.broadcasted_iota(I32, (128, DH), 0)
        col = jax.lax.broadcasted_iota(I32, (128, DH), 1)
        sel = jnp.where((row % 64) // 2 == col, 1.0, 0.0).astype(BF16)
        wall = wphi_v[...].reshape(H * DH, DH)
        ph = _dot_nt(sel, wall)
        row = jax.lax.broadcasted_iota(I32, (128, D), 0)
        col = jax.lax.broadcasted_iota(I32, (128, D), 1)
        keep = (2 * (row // 64) + row % 2) == ((col % 128) // DH)
        phit[...] = jnp.where(keep, ph * LOG2E, 0.0).astype(BF16)
        wr = wr_v[...].astype(F32)
        halves = [jnp.concatenate([jnp.broadcast_to(wr[4 * h + t:4 * h + t + 1], (16, 128))
                                   for t in range(4)], axis=1) for h in range(2)]
        odd = jax.lax.broadcasted_iota(I32, (16, DHALF), 0) % 2 == 1
        wr2[...] = _pack(jnp.where(odd, halves[1], halves[0]))

    def fold(which, dst, j, sch=None):
        wt = []
        for g in (2 * j, 2 * j + 1):
            r_ = _dot_nt(phit[:, g * 128:(g + 1) * 128],
                         w_v[which, :, g * 128:(g + 1) * 128])
            if sch is not None and g == 2 * j:
                sch.token = r_[0:8, 0:128]
            wt.append(r_)
        w0, w1 = wt
        cs = _lhs_combos(w0[:, :DHALF], w0[:, DHALF:], w1[:, :DHALF], w1[:, DHALF:])
        for k in range(7):
            dst.at[k][j * 64:(j + 1) * 64, :] = _pack(cs[k])

    def prep_v(j, sch):
        ws = [_u32(w_v[2, :, g * 128:(g + 1) * 128]) for g in (2 * j, 2 * j + 1)]
        ws = [sch.hold(w, [(8 * q, 0) for q in range(8)]) for w in ws]
        wt = [_bf(w).T for w in ws]
        f0, f1 = [w.astype(F32) for w in wt]
        w0, w1 = [_u32(w) for w in wt]
        cs = _lhs_combos(f0[:, :DHALF], f0[:, DHALF:], f1[:, :DHALF], f1[:, DHALF:])
        for k in range(7):
            u = w0[:, :DHALF] if k == 2 else w1[:, DHALF:] if k == 3 else _pack(cs[k])
            av.at[k][j * 64:(j + 1) * 64, :] = u
        return w0, w1

    def ln_chunk(n, c, sch=None, also=None):
        ys = []
        for h in range(2):
            r0 = n * T + h * TH + c * 16
            if not isinstance(r0, int):
                r0 = pl.multiple_of(r0, 16)
            xr = x_v[pl.ds(r0, 16), :].astype(F32)
            if sch is not None:
                xr = pltpu.bitcast(sch.hold(_u32(xr), [(0, 0), (1, 0)]), F32)
            ys.append(_layernorm(xr))
        ya, yb = ys
        cs = (_rhs_combos(ya[:, :DHALF], yb[:, :DHALF], ya[:, DHALF:], yb[:, DHALF:])
              + [ya[:, DHALF:], yb[:, :DHALF]])
        out = []
        for k in range(9):
            dst = bq.at[n, k]
            u = _pack(cs[k])
            dst[c * 8:(c + 1) * 8, :] = u
            if also is not None and k < 7:
                dst = also.at[k]
                dst[c * 8:(c + 1) * 8, :] = u
            if isinstance(n, int):
                out.append(dst[c * 8:(c + 1) * 8, :])
        if isinstance(n, int):
            return out
        return [cs[k] for k in (0, 2, 3, 5, 6)]

    def wo_piece(e):
        r0 = pl.multiple_of((e // 8) * 256 + (e % 8) * 16, 16)
        o0 = pl.multiple_of(e * 8, 8)
        w0 = wo_v[pl.ds(r0, 16), :].astype(F32)
        w1 = wo_v[pl.ds(r0 + 128, 16), :].astype(F32)

        def cols(w, par):
            return jnp.concatenate(
                [w[:, (2 * q + par) * 128:(2 * q + par + 1) * 128] for q in range(4)], axis=1)
        cs = _rhs_combos(cols(w0, 0), cols(w0, 1), cols(w1, 0), cols(w1, 1))
        for k in range(7):
            bo.at[k][pl.ds(o0, 8), :] = _pack(cs[k])
        return [cs[k] for k in (0, 2, 3, 5, 6)]

    def proj(sch, a_ref, j, b, extra=None, early=None):
        def prod(k):
            lhs = sch.gate(a_ref[k, j * 64:(j + 1) * 64, :])
            if extra is not None and k in (1, 2, 3, 4):
                r_ = _dot_nt(_bf(jnp.concatenate([lhs, wr2[...]], axis=0)), b[k])
                extra[k] = r_[128:136]
                r_ = r_[0:128]
            else:
                r_ = _dot_nt(_bf(lhs), b[k])
            sch.token = r_[0:8, 0:128]
            return r_

        def after(step, done):
            if step == 4 and early is not None:
                early[j] = [jnp.concatenate([done[0], done[1]], axis=1), None]
            sch.after(step, done)
        c11, c12, c21, c22 = _strassen(prod, after)
        return (jnp.concatenate([c11, c12], axis=1),
                jnp.concatenate([c21, c22], axis=1))

    class KVTile:
        def __init__(self, sch, i, slot, src=None):
            self.sch, self.i, self.slot, self.src = sch, i, slot, src
            self.b = None
            self.pk, self.phis = {}, {}

        def operands(self):
            if self.src is not None:
                return [_bf(self.src[k]) for k in range(7)]
            if self.b is None:
                self.b = [_bf(bq[self.i, k]) for k in range(7)]
            return self.b

        def kproj(self, j):
            self.pk[j] = proj(self.sch, ak, j, self.operands())

        def vproj(self, j):
            ex = {} if j == 0 else None
            vs = proj(self.sch, av, j, self.operands(), ex)
            for g in range(2):
                for p in range(2):
                    vt_v.at[self.slot, 2 * j + g][p * 32:(p + 1) * 32, :] = _pack(
                        vs[g][p * 64:(p + 1) * 64])
            if j == 0:
                r_v[self.i] = jnp.concatenate(
                    [ex[1][0:1] + ex[1][1:2] + ex[3][1:2],
                     ex[4][0:1] + ex[4][1:2] + ex[2][0:1]], axis=1)

        def sm(self, j, g, p, due=None, step=0):
            phi, _ = _feature_map(self.pk[j][g][p * 64:(p + 1) * 64])
            z_v[4 * j + 2 * g + p] += phi[:, :128] + phi[:, 128:]
            if due is None:
                self.phis[j, g, p] = lambda: phi.astype(BF16)
                return
            dst = ph_v.at[self.i, 4 * j + 2 * g + p]
            for t in range(2):
                dst[t * 32:(t + 1) * 32, :] = _pack(phi[t * 64:(t + 1) * 64])
            self.phis[j, g, p] = lambda: _bf(dst[...])
            for t in range(2):
                self.sch.need(due - step * (1 - t), [dst[:, t * 128:(t + 1) * 128]])

        def kv(self, j, g):
            for p in range(2):
                if (j, g, p) not in self.phis:
                    self.sm(j, g, p)
                lhs = _bf(vt_v[self.slot, 2 * j + g, p * 32:(p + 1) * 32, :])
                kv_acc[4 * j + 2 * g + p] += _dot_nt(lhs, self.phis[j, g, p]())

    def first_tiles():
        sch = Sched(zero_s[0] > 0)
        tiles = {'a': KVTile(sch, 0, 0), 'b': KVTile(sch, 1, 1)}
        for op in PROG.split():
            kind, arg = op[0], op[1:2]
            if kind == 'w':
                for nm in op[2:].split(','):
                    named_copy(nm).wait()
            elif kind == 'P':
                build_phit()
            elif kind == 'f':
                fold(1, ak, int(arg))
            elif kind == 'p':
                _, rel, d0 = op.split(':')

                def job(j=int(arg), base=sch.slot + float(d0)):
                    ws = prep_v(j, sch)
                    for q in range(8):
                        sch.need(base + q * 0.5, [w[:, q * 128:(q + 1) * 128] for w in ws])
                sch.at(sch.slot + int(rel), job)
            elif kind == 'U':
                for c in range(8):
                    ln_chunk(int(arg), c)
            elif kind == 'L':
                _, l0, l1 = op.split(':')
                for c in range(8):
                    due = _eighths(sch.slot + float(l0) + (float(l1) - float(l0)) * c / 7)
                    rel = int(due - 4.5)

                    def job(n=int(arg), c=c, due=due, held=rel >= sch.slot):
                        sch.spread(ln_chunk(n, c, sch if held else None,
                                            bp[0] if n == NF else None), due)
                    if rel >= sch.slot:
                        sch.at(rel, job)
                    else:
                        job()
            elif kind == 'S':
                st_ = 5.0 / 7
                for q in range(4):
                    tiles[op[2]].sm(int(arg), q // 2, q % 2,
                                    _eighths(sch.slot + 1.5 + st_ * (2 * q + 1)), _eighths(st_))
            elif kind == 'K':
                tiles[op[2]].kproj(int(arg))
            elif kind == 'V':
                tiles[op[2]].vproj(int(arg))
            elif kind == 'X':
                for g in range(2):
                    sch.at(sch.slot + 1 + g, functools.partial(tiles[op[2]].kv, int(arg), g))
            elif kind == 'Y':
                for g in range(2):
                    tiles[op[2]].kv(int(arg), g)
        assert not sch.jobs and not sch.deps

    def phase1_tile(i, par, sch):
        nxt = jnp.minimum(i + 1, NT - 1)
        o = sch.slot
        tl = KVTile(sch, i, par, bp[par])
        for c in range(8):
            due = 14 * (c // 2) + (6, 13)[c % 2]
            sch.spread(ln_chunk(nxt, c, None, bp[1 - par]),
                       o + (min(due, 53) if par == 0 else due))
        for q, due in enumerate((1, 15, 17, 29, 31, 43)):
            sch.spread(wo_piece(jnp.minimum((i - NF) * 6 + q, 31)), o + due)
        for j in range(NJ if par == 0 else NJ - 1):
            for g in range(2):
                sch.at(o + 14 * (j + 1) + 2 * g, functools.partial(tl.kv, j, g))
        for j in range(NJ):
            tl.kproj(j)
            tl.vproj(j)
        if par == 1:
            for g in range(2):
                tl.kv(NJ - 1, g)

    def phase1(m, carry):
        sch = Sched(zero_s[0] > 0)
        for par in range(2):
            phase1_tile(NF + 2 * m + par, par, sch)
        return carry

    first_tiles()
    wo_copy.wait()
    for t in range(NF + 1, NT):
        x_copy(t).wait()
    jax.lax.fori_loop(0, (NT - NF) // 2, phase1, 0)

    for j in range(NJ):
        w_copy(0, j).wait()
    wg_copy.wait()
    wu_copy.wait()
    wd_copy.wait()
    sch = Sched(zero_s[0] > 0)
    row = jax.lax.broadcasted_iota(I32, (64, 128), 0)
    col = jax.lax.broadcasted_iota(I32, (64, 128), 1)
    keep = (row // DH) == (col % 2)
    for j in range(NJ):
        fold(0, aq, j, sch)
        for p in range(4 * j, 4 * j + 4):
            kvp = pltpu.bitcast(sch.hold(_u32(kv_acc[p]), [(r, 0) for r in range(8)]), F32)
            mk = jnp.where(keep, kvp, 0.0)
            for t in range(2):
                m_v.at[p][t * 16:(t + 1) * 16, :] = _pack(mk[t * 32:(t + 1) * 32])
            sch.need(1 + p * 0.375, [m_v[p]])
            z_v[p] = jnp.broadcast_to(jnp.sum(z_v[p], axis=1, keepdims=True), (128, 128))

    r = _round(r_v[...].reshape(NT, T))
    rmax = jnp.max(jnp.max(r, axis=1, keepdims=True), axis=0, keepdims=True)
    pos = (jax.lax.broadcasted_iota(I32, (NT, T), 0) * T
           + jax.lax.broadcasted_iota(I32, (NT, T), 1))
    idx = jnp.min(jnp.where(r == rmax, pos, S))
    idx = jnp.clip(idx, 0, S - 1)
    tile = idx // T
    half = (idx % T) // TH
    sub = pl.multiple_of(((idx % TH) // 16) * 8, 8)
    xs = jnp.concatenate([bq[tile, 1 + 7 * half, pl.ds(sub, 8), :],
                          bq[tile, 7 - 3 * half, pl.ds(sub, 8), :]], axis=1)
    xs = jnp.where(jax.lax.broadcasted_iota(I32, (16, D), 0) == idx % 16,
                   _bf(xs).astype(F32), 0.0)
    xs = jnp.sum(xs, axis=0, keepdims=True)

    def lane_bcast(dst, row):
        for t in range(row.shape[1] // 128):
            dst[t * 128:(t + 1) * 128, :] = jnp.broadcast_to(
                row[:, t * 128:(t + 1) * 128], (128, 128)).T

    lane_bcast(xb_v, xs)
    router = _round(0.5 + 0.5 * jnp.tanh(0.5 * rmax))

    first = proj(sch, aq, 0, [_bf(bq[(tile + 1) % NT, k]) for k in range(7)])
    for g in range(2):
        pq0_v[g] = first[g]

    def phase2(i, carry):
        last = isinstance(i, int)
        zero = zero_s[0]
        slot = i
        n = tile if last else (tile + 1 + i) % NT

        s0 = pl.multiple_of(n * T, T)
        b = [_bf(bq[n, k]) for k in range(7)]
        pq = [None] * NJ
        sch = Sched(zero > 0)
        ot = {}
        pq[0] = [pq0_v[g] for g in range(2)]
        phis = {}

        def sm(j, g, p, due, step):
            phi, scales = _feature_map(pq[j][g][p * 64:(p + 1) * 64], z_v[4 * j + 2 * g + p])
            phis[j, g, p] = phi.astype(BF16)
            for t in range(2):
                sch.need(max(due - step * (1 - t), sch.slot + 1),
                         [v[:, t * 128:(t + 1) * 128] for v in scales])

        def nd(j, g):
            ot[j, g] = jnp.concatenate(
                [_dot(_bf(m_v[4 * j + 2 * g + p]), phis[j, g, p]) for p in range(2)], axis=0)
            if g == 1:
                o0, o1 = ot[j, 0], ot[j, 1]
                cs = _lhs_combos(o0[:, :TH], o1[:, :TH], o0[:, TH:], o1[:, TH:])
                for k in range(7):
                    ao_v[2 * k + j // 2][zero, :, (j % 2) * 128:(j % 2 + 1) * 128] = (
                        _u32(cs[k].astype(BF16).T))

        if last:
            fd = (NFC - 1) * FC
        else:
            fu = pl.multiple_of(i * FC, FC)
            fd = pl.multiple_of(jnp.maximum(i - 1, 0) * FC, FC)
        ffn = {}

        def matvec(key, w, vb, due):
            t = (w.astype(F32).reshape(FR // 8, 8, 256)
                 * jnp.concatenate([vb, vb], axis=1).reshape(FR // 8, 8, 256))
            t = jnp.sum(t, axis=0)
            ffn[key] = t if key not in ffn else ffn[key] + t
            sch.need(due, [ffn[key]])

        def ffn_up(w_ref, name, cp, rb, due):
            rs = slice(rb * FR, (rb + 1) * FR)
            matvec((name, cp), w_ref[rs, pl.ds(fu + cp * 256, 256)], xb_v[rs, :], due)

        def ffn_mid():
            hg, hu = [_round(jnp.sum(jnp.concatenate([ffn[nm, 0], ffn[nm, 1]], axis=1),
                                     axis=0, keepdims=True)) for nm in 'gu']
            lane_bcast(hb_v, _round(_round(_silu(hg)) * hu))

        def ffn_down(cp, rb, due):
            cs_ = slice(cp * 256, (cp + 1) * 256)
            if rb == 0:
                ffn['y', cp] = y_acc[:, cs_]
            matvec(('y', cp), wd_v[pl.ds(fd + rb * FR, FR), cs_],
                   hb_v[rb * FR:(rb + 1) * FR, :], due)
            if rb == FC // FR - 1:
                if last:
                    ffn['row', cp] = (
                        _round(jnp.sum(ffn['y', cp], axis=0, keepdims=True)) * router)
                else:
                    y_acc[:, cs_] = ffn['y', cp]

        d0, d1 = (2, 27) if last else (28, 36.5)
        nd_ = 4 * FC // FR
        for t in range(nd_):
            due = _eighths(d0 + (d1 - d0) * t / (nd_ - 1))
            sch.at(0, functools.partial(ffn_down, t % 4, t // 4, due))
        if not last:
            nu_ = 4 * D // FR
            for t in range(nu_):
                due = _eighths(37 + 16.5 * t / (nu_ - 1))
                name, w_ref = (('g', wg_v), ('u', wu_v))[(t // 2) % 2]
                sch.at(0, functools.partial(ffn_up, w_ref, name, t % 2, t // 4, due))
            sch.at(53, ffn_mid)
        lead = 0.5 if last else 0
        for j in range(NJ):
            s1 = 7 * j
            nds = (((1, 4), (1, 4), (1, 4), (2, 3)) if last
                   else ((1, 4), (0, 3), (0, 3), (0, 1)))[j]
            for g in range(2):
                for p in range(2):
                    sch.at(s1 if (j == 0 or g == 1) else s1 - 2, functools.partial(
                        sm, j, g, p, s1 + nds[g] + p - lead, 0.5))
                sch.at(s1 + nds[g], functools.partial(nd, j, g))
        for j in range(1, NJ):
            pq[j] = proj(sch, aq, j, b, early=pq)
        if last:
            def prod_a(k):
                return _dot(_bf(sch.gate(ao_v[2 * k][0])), _bf(bo[k, 0:128, 0:256]))
            part = _strassen(prod_a, sch.after)
        else:
            nxt = proj(sch, aq, 0, [_bf(bq[(n + 1) % NT, k]) for k in range(7)])
            for g in range(2):
                pq0_v[g] = nxt[g]

        er = 32 if last else 64
        rows = jax.lax.broadcasted_iota(I32, (er, 256), 0) + s0
        ne_ = T // er
        gates = {}

        def gate_part(c, e, due):
            r0 = e * er
            h, rh = r0 // TH, r0 % TH
            blk = ((1, 7), (8, 4))[h][c // 2]
            bb = _bf(bq[n, blk, rh // 2:(rh + er) // 2,
                        (c % 2) * 256:(c % 2 + 1) * 256]).astype(F32)
            if last:
                bb = bb + jnp.where(rows + r0 == idx, ffn['row', c], 0.0)
            gates[c, e] = _silu(bb)
            if due is not None:
                sch.need(due, [gates[c, e]])

        def epilogue(c, cc, e, due):
            r0 = e * er
            h, rh = r0 // TH, r0 % TH
            cs = slice(c * 256, (c + 1) * 256)
            rs = slice(rh, rh + er)
            if (c, e) not in gates:
                gate_part(c, e, None)
            xr = x_v[pl.ds(s0 + r0, er), cs].astype(F32)
            sv = jnp.concatenate([cc[2 * h][rs], cc[2 * h + 1][rs]], axis=1)
            res = xr + sv * gates[c, e]
            out_v[slot, r0:r0 + er, cs] = res.astype(BF16)
            if due is not None:
                sch.need(due, [res])

        def out_cols(c, h=None):
            cs = slice(c * 256, (c + 1) * 256)
            if h is None:
                return pltpu.make_async_copy(out_v.at[slot, :, cs],
                                             out_hbm.at[0, pl.ds(s0, T), cs], sem_o.at[NT + c])
            return pltpu.make_async_copy(
                out_v.at[slot, h * TH:(h + 1) * TH, cs],
                out_hbm.at[0, pl.ds(s0 + h * TH, TH), cs], sem_o.at[NT + c + h])

        e0, e1 = (1 if last else 0.5), 6.5
        end = sch.slot + 28 - (7 if last else 0)
        for e in range(ne_):
            sch.at(end - 8, functools.partial(
                gate_part, 3, e, _eighths(end - 7 + 4 * e / (ne_ - 1))))
        pending = []
        c = 0
        while c < 4:
            if last and c == 0:
                def prod(k):
                    return _dot(_bf(sch.gate(ao_v[2 * k + 1][0])),
                                _bf(bo[k, 128:256, 0:256]))
                cc2 = [u + v for u, v in zip(part, _strassen(prod, sch.after))]
                blocks = [(t, [v[:, t * 128:(t + 1) * 128] for v in cc2]) for t in range(2)]
            else:
                def prod(k):
                    return _dot(_bf(sch.gate(jnp.concatenate(
                        [ao_v[2 * k][0], ao_v[2 * k + 1][0]], axis=1))),
                                _bf(bo[k, :, c * 128:(c + 1) * 128]))
                blocks = [(c, _strassen(prod, sch.after))]
            if last:
                for t in pending:
                    out_cols(t).start()
            nb = len(blocks) * ne_
            for q in range(nb):
                t, cc = blocks[q // ne_]
                due = _eighths(sch.slot + e0 + (e1 - e0) * q / (nb - 1))
                epilogue(t, cc, q % ne_, due if t < 3 else None)
                if last and t == 3 and (q + 1) % (ne_ // 2) == 0:
                    out_cols(3, (q + 1) // (ne_ // 2) - 1).start()
            pending = [t for t, _ in blocks]
            c += len(blocks)
        if last:
            for t in range(NT - 1):
                out_copy((tile + 1 + t) % NT, t).wait()
            for t in range(3):
                out_cols(t).wait()
            for h in range(2):
                out_cols(3, h).wait()
        else:
            out_copy(n, slot).start()
        return carry

    jax.lax.fori_loop(0, NT - 1, phase2, 0)
    phase2(NT - 1, 0)


@jax.jit
def pallas_recurrent_scan__linear_kernel_hedgehog__moe_arch_mod__prompt_kernel(
    A_x: jax.Array,
    A_wqkv: jax.Array,
    A_w_phi: jax.Array,
    A_wo: jax.Array,
    B_x: jax.Array,
    B_w_r: jax.Array,
    B_w_gate: jax.Array,
    B_w_up: jax.Array,
    B_w_down: jax.Array,
):
    del B_x
    any_spec = pl.BlockSpec(memory_space=pl.ANY)
    return pl.pallas_call(
        _kernel,
        out_shape=jax.ShapeDtypeStruct((1, S, D), BF16),
        in_specs=[any_spec] * 8,
        out_specs=any_spec,
        scratch_shapes=[
            pltpu.VMEM((S, D), BF16),
            pltpu.VMEM((3, D, D), BF16),
            pltpu.VMEM((H, DH, DH), BF16),
            pltpu.VMEM((8, 128), BF16),
            pltpu.VMEM((D, D), BF16),
            pltpu.VMEM((D, F), BF16),
            pltpu.VMEM((D, F), BF16),
            pltpu.VMEM((F, D), BF16),
            pltpu.VMEM((NT, 9, TH // 2, DHALF), U32),
            pltpu.VMEM((7, 256, DHALF), U32),
            pltpu.VMEM((7, 256, DHALF), U32),
            pltpu.VMEM((7, 256, DHALF), U32),
            pltpu.VMEM((7, 256, DHALF), U32),
            pltpu.VMEM((NP, 64, 128), F32),
            pltpu.VMEM((NP, 128, 128), F32),
            pltpu.VMEM((NF, NP, 64, T), U32),
            pltpu.VMEM((NF, 8, 64, T), U32),
            pltpu.VMEM((NP, 32, 128), U32),
            pltpu.VMEM((128, D), BF16),
            pltpu.VMEM((8, DHALF), U32),
            pltpu.VMEM((NT, 1, T), F32),
            pltpu.VMEM((8, D), F32),
            pltpu.VMEM((D, 128), F32),
            pltpu.VMEM((FC, 128), F32),
            pltpu.VMEM((2, 128, T), F32),
            pltpu.VMEM((NT, T, D), BF16),
            pltpu.SMEM((1,), I32),
        ] + [pltpu.VMEM((1, TH // 2, 256), U32)] * 14
        + [pltpu.VMEM((7, TH // 2, DHALF), U32)] * 2,
        compiler_params=pltpu.CompilerParams(
            vmem_limit_bytes=100 * 1024 * 1024,
            disable_bounds_checks=True),
    )(A_x, A_wqkv, A_w_phi, A_wo, B_w_r.reshape(8, 128), B_w_gate, B_w_up, B_w_down)
```

```python
import functools

import jax
import jax.numpy as jnp
import jax.experimental.pallas as pl
import jax.experimental.pallas.tpu as pltpu

S, D, H, DH, F = 2048, 1024, 32, 32, 3584
T = 256
TH = T // 2
DHALF = D // 2
NT = S // T
NJ = 4
NP = D // 64
FC = 512
NFC = F // FC
FR = 64
NF = 2
ORDER = 'ph wr k0 x0 x1 k1 k2 k3 v0 v1 v2 v3 x2'
PROG = ('w:ph,wr P w:k0 f0 w:x0 U0 w:x1 L1:2.75:6:0:4:5.5 K0a '
        'w:k1 f1 L1:2:6:4:8:4.5 K1a S0a K0b S0b K1b '
        'w:k2,k3,v0 f2 S1a K2a f3 p0:14:18 S1b K2b S2a K3a S2b K3b '
        'w:v1,v2,v3,x2 p1:3:8 p2:16:21 p3:30:35 L2:6:52:0:8:5.5 V0a X0a V0b '
        'X0b V1a X1a S3a V1b X1b V2a X2a S3b V2b X2b V3a X3a V3b Y3b')
LOG2E = 1.4426950408889634
F32, BF16, U32, I32 = jnp.float32, jnp.bfloat16, jnp.uint32, jnp.int32

_NT_DIMS = (((1,), (1,)), ((), ()))


def _dot_nt(a, b):
    return jax.lax.dot_general(a, b, _NT_DIMS, preferred_element_type=F32)


def _dot(a, b):
    return jnp.dot(a, b, preferred_element_type=F32)


def _u32(v):
    return pltpu.bitcast(v, U32) if v.dtype != U32 else v


def _pack(v):
    return pltpu.bitcast(v.astype(BF16), U32)


def _recip(x):
    r = pl.reciprocal(x, approx=True)
    return r * (2.0 - x * r)


def _bf(v):
    return pltpu.bitcast(v, BF16)


def _round(v):
    return v.astype(BF16).astype(F32)


def _eighths(x):
    return round(x * 8) / 8


def _or_all(vals):
    ts = []
    for v in vals:
        u = _u32(v)
        for a in range(u.shape[0] // 8):
            for b in range(u.shape[1] // 128):
                ts.append(u[a * 8:(a + 1) * 8, b * 128:(b + 1) * 128])
    while len(ts) > 1:
        ts = [ts[i] | ts[i + 1] if i + 1 < len(ts) else ts[i] for i in range(0, len(ts), 2)]
    return ts[0]


def _gate(lhs_u32, deps, never):
    if not deps:
        return lhs_u32
    rows = []
    for r in range(lhs_u32.shape[0] // 8):
        row = lhs_u32[r * 8:(r + 1) * 8]
        cs = [c for (r_, c) in deps if r_ == r]
        if cs:
            row = jnp.concatenate(
                [jnp.where(never, _or_all(deps[r, c]), row[:, c * 128:(c + 1) * 128])
                 if c in cs else row[:, c * 128:(c + 1) * 128]
                 for c in range(lhs_u32.shape[1] // 128)], axis=1)
        rows.append(row)
    return jnp.concatenate(rows, axis=0)


class Sched:
    def __init__(self, never):
        self.never = never
        self.slot = 0
        self.gated = 0
        self.token = None
        self.jobs = {}
        self.deps = {}

    def at(self, slot, fn):
        self.jobs.setdefault(slot, []).append(fn)

    def need(self, pos, vals):
        slot, r = divmod(int(round(pos * 8)), 8)
        assert slot >= self.gated, (pos, self.slot)
        d = self.deps.setdefault(slot, {})
        c = (slot + r) % 4
        d.setdefault((r, c), []).extend(vals)

    def spread(self, vals, due, step=0.25):
        for t in range(4):
            self.need(due + t * step, [v[:, t * 128:(t + 1) * 128] for v in vals])

    def gate(self, lhs):
        nc = lhs.shape[1] // 128
        self.gated = self.slot + 1
        deps = {}
        for (r, c), v in self.deps.pop(self.slot, {}).items():
            deps.setdefault((r, c % nc), []).extend(v)
        return _gate(lhs, deps, self.never)

    def hold(self, u, blocks):
        if self.token is None:
            return u
        return _gate(u, {rc: [self.token] for rc in blocks}, self.never)

    def after(self, step, done):
        for fn in self.jobs.pop(self.slot, []):
            fn()
        self.slot += 1


def _layernorm(x):
    m = jnp.mean(x, axis=-1, keepdims=True)
    mb = _round(m)
    xc = x - mb
    dm = m - mb
    v = jnp.mean(xc * xc, axis=-1, keepdims=True) - dm * dm
    a = _round(_round(v) + 1e-5)
    rs = jax.lax.rsqrt(a)
    sd = a * rs
    sd = _round(sd + (0.5 * rs) * (a - sd * sd))
    return xc * _recip(sd)


def _lhs_combos(a11, a12, a21, a22):
    return [a11 + a22, a21 + a22, a11, a22, a11 + a12, a21 - a11, a12 - a22]


def _rhs_combos(b11, b12, b21, b22):
    return [b11 + b22, b11, b12 - b22, b21 - b11, b22, b11 + b12, b21 + b22]


def _strassen(prod, after):
    done = {}
    m1 = prod(0)
    after(0, done)
    m4 = prod(3)
    after(1, done)
    m5 = prod(4)
    after(2, done)
    m7 = prod(6)
    done[0] = m1 + m4 - m5 + m7
    after(3, done)
    m3 = prod(2)
    done[1] = m3 + m5
    after(4, done)
    m2 = prod(1)
    done[2] = m2 + m4
    after(5, done)
    m6 = prod(5)
    done[3] = m1 - m2 + m3 + m6
    after(6, done)
    return done[0], done[1], done[2], done[3]


def _allreduce_pair(x, op):
    x = op(x, pltpu.roll(x, 2, axis=0))
    return op(x, pltpu.roll(x, 4, axis=0))


def _feature_map(p, z=None):
    t = p.shape[1]
    p3 = p.reshape(8, 8, t)
    mx = _allreduce_pair(jnp.max(p3, axis=0), jnp.maximum)
    mn = _allreduce_pair(jnp.min(p3, axis=0), jnp.minimum)
    ep = jnp.exp2(p3 - mx[None])
    en = jnp.exp2(mn[None] - p3)
    rp = _recip(_allreduce_pair(jnp.sum(ep, axis=0), jnp.add))
    rn = _recip(_allreduce_pair(jnp.sum(en, axis=0), jnp.add))
    if z is not None:
        z4 = jnp.concatenate([z] * (t // 128), axis=1).reshape(2, 8, 8, t)
        den = rp * jnp.sum(ep * z4[0], axis=0) + rn * jnp.sum(en * z4[1], axis=0)
        inv = _recip(_allreduce_pair(den, jnp.add) + 1e-6)
        rp, rn = rp * inv, rn * inv
    pos = (ep * rp[None]).reshape(64, t)
    neg = (en * rn[None]).reshape(64, t)
    return jnp.concatenate([pos, neg], axis=0), (rp, rn)


def _silu(x):
    h = 0.5 * x
    return h + h * jnp.tanh(h)


def _kernel(*refs):
    pl.run_scoped(functools.partial(_body, *refs),
                  pltpu.SemaphoreType.DMA((NT + 18,)), pltpu.SemaphoreType.DMA((NT + 5,)))


def _body(x_hbm, wqkv_hbm, wphi_hbm, wo_hbm, wr_hbm, wg_hbm, wu_hbm, wd_hbm,
          out_hbm,
          x_v, w_v, wphi_v, wr_v, wo_v, wg_v, wu_v, wd_v,
          bq, ak, av, aq, bo, kv_acc, z_v, ph_v, vt_v, m_v, phit, wr2, r_v,
          y_acc, xb_v, hb_v, pq0_v, out_v, zero_s, *rest):
    ao_v, bp, (sem, sem_o) = rest[:-4], rest[-4:-2], rest[-2:]

    def x_copy(i):
        return pltpu.make_async_copy(x_hbm.at[0, pl.ds(i * T, T), :],
                                     x_v.at[pl.ds(i * T, T), :], sem.at[i])

    def w_copy(m, j):
        return pltpu.make_async_copy(
            wqkv_hbm.at[:, m * D + j * 256:m * D + (j + 1) * 256],
            w_v.at[m, :, j * 256:(j + 1) * 256], sem.at[NT + 6 + 4 * m + j])

    wphi_copy = pltpu.make_async_copy(wphi_hbm, wphi_v, sem.at[NT])
    wr_copy = pltpu.make_async_copy(wr_hbm, wr_v, sem.at[NT + 1])
    wo_copy = pltpu.make_async_copy(wo_hbm, wo_v, sem.at[NT + 2])
    wg_copy = pltpu.make_async_copy(wg_hbm, wg_v, sem.at[NT + 3])
    wu_copy = pltpu.make_async_copy(wu_hbm, wu_v, sem.at[NT + 4])
    wd_copy = pltpu.make_async_copy(wd_hbm, wd_v, sem.at[NT + 5])

    def out_copy(i, slot):
        return pltpu.make_async_copy(out_v.at[slot],
                                     out_hbm.at[0, pl.ds(i * T, T), :],
                                     sem_o.at[slot])

    def named_copy(nm):
        if nm in ('ph', 'wr'):
            return wphi_copy if nm == 'ph' else wr_copy
        t = int(nm[1])
        return x_copy(t) if nm[0] == 'x' else w_copy({'k': 1, 'v': 2}[nm[0]], t)

    for nm in ORDER.split():
        named_copy(nm).start()
    x_copy(NF + 1).start()
    wo_copy.start()
    for i in range(NF + 2, NT):
        x_copy(i).start()
    for j in range(NJ):
        w_copy(0, j).start()
    wg_copy.start()
    wu_copy.start()
    wd_copy.start()

    zero_s[0] = 0
    kv_acc[...] = jnp.zeros_like(kv_acc)
    y_acc[...] = jnp.zeros_like(y_acc)
    z_v[...] = jnp.zeros_like(z_v)
    hb_v[...] = jnp.zeros_like(hb_v)

    def build_phit():
        row = jax.lax.broadcasted_iota(I32, (128, DH), 0)
        col = jax.lax.broadcasted_iota(I32, (128, DH), 1)
        sel = jnp.where((row % 64) // 2 == col, 1.0, 0.0).astype(BF16)
        wall = wphi_v[...].reshape(H * DH, DH)
        ph = _dot_nt(sel, wall)
        row = jax.lax.broadcasted_iota(I32, (128, D), 0)
        col = jax.lax.broadcasted_iota(I32, (128, D), 1)
        keep = (2 * (row // 64) + row % 2) == ((col % 128) // DH)
        phit[...] = jnp.where(keep, ph * LOG2E, 0.0).astype(BF16)
        wr = wr_v[...].astype(F32)
        halves = [jnp.concatenate([jnp.broadcast_to(wr[4 * h + t:4 * h + t + 1], (16, 128))
                                   for t in range(4)], axis=1) for h in range(2)]
        odd = jax.lax.broadcasted_iota(I32, (16, DHALF), 0) % 2 == 1
        wr2[...] = _pack(jnp.where(odd, halves[1], halves[0]))

    def fold(which, dst, j, sch=None):
        wt = []
        for g in (2 * j, 2 * j + 1):
            r_ = _dot_nt(phit[:, g * 128:(g + 1) * 128],
                         w_v[which, :, g * 128:(g + 1) * 128])
            if sch is not None and g == 2 * j:
                sch.token = r_[0:8, 0:128]
            wt.append(r_)
        w0, w1 = wt
        cs = _lhs_combos(w0[:, :DHALF], w0[:, DHALF:], w1[:, :DHALF], w1[:, DHALF:])
        for k in range(7):
            dst.at[k][j * 64:(j + 1) * 64, :] = _pack(cs[k])

    def prep_v(j, sch):
        ws = [_u32(w_v[2, :, g * 128:(g + 1) * 128]) for g in (2 * j, 2 * j + 1)]
        ws = [sch.hold(w, [(8 * q, 0) for q in range(8)]) for w in ws]
        wt = [_bf(w).T for w in ws]
        f0, f1 = [w.astype(F32) for w in wt]
        w0, w1 = [_u32(w) for w in wt]
        cs = _lhs_combos(f0[:, :DHALF], f0[:, DHALF:], f1[:, :DHALF], f1[:, DHALF:])
        for k in range(7):
            u = w0[:, :DHALF] if k == 2 else w1[:, DHALF:] if k == 3 else _pack(cs[k])
            av.at[k][j * 64:(j + 1) * 64, :] = u
        return w0, w1

    def ln_chunk(n, c, sch=None, also=None):
        ys = []
        for h in range(2):
            r0 = n * T + h * TH + c * 16
            if not isinstance(r0, int):
                r0 = pl.multiple_of(r0, 16)
            xr = x_v[pl.ds(r0, 16), :].astype(F32)
            if sch is not None:
                xr = pltpu.bitcast(sch.hold(_u32(xr), [(0, 0), (1, 0)]), F32)
            ys.append(_layernorm(xr))
        ya, yb = ys
        cs = (_rhs_combos(ya[:, :DHALF], yb[:, :DHALF], ya[:, DHALF:], yb[:, DHALF:])
              + [ya[:, DHALF:], yb[:, :DHALF]])
        out = []
        for k in range(9):
            dst = bq.at[n, k]
            u = _pack(cs[k])
            dst[c * 8:(c + 1) * 8, :] = u
            if also is not None and k < 7:
                dst = also.at[k]
                dst[c * 8:(c + 1) * 8, :] = u
            if isinstance(n, int):
                out.append(dst[c * 8:(c + 1) * 8, :])
        if isinstance(n, int):
            return out
        return [cs[k] for k in (0, 2, 3, 5, 6)]

    def wo_piece(e):
        r0 = pl.multiple_of((e // 8) * 256 + (e % 8) * 16, 16)
        o0 = pl.multiple_of(e * 8, 8)
        w0 = wo_v[pl.ds(r0, 16), :].astype(F32)
        w1 = wo_v[pl.ds(r0 + 128, 16), :].astype(F32)

        def cols(w, par):
            return jnp.concatenate(
                [w[:, (2 * q + par) * 128:(2 * q + par + 1) * 128] for q in range(4)], axis=1)
        cs = _rhs_combos(cols(w0, 0), cols(w0, 1), cols(w1, 0), cols(w1, 1))
        for k in range(7):
            bo.at[k][pl.ds(o0, 8), :] = _pack(cs[k])
        return [cs[k] for k in (0, 2, 3, 5, 6)]

    def proj(sch, a_ref, j, b, extra=None, early=None):
        def prod(k):
            lhs = sch.gate(a_ref[k, j * 64:(j + 1) * 64, :])
            if extra is not None and k in (1, 2, 3, 4):
                r_ = _dot_nt(_bf(jnp.concatenate([lhs, wr2[...]], axis=0)), b[k])
                extra[k] = r_[128:136]
                r_ = r_[0:128]
            else:
                r_ = _dot_nt(_bf(lhs), b[k])
            sch.token = r_[0:8, 0:128]
            return r_

        def after(step, done):
            if step == 4 and early is not None:
                early[j] = [jnp.concatenate([done[0], done[1]], axis=1), None]
            sch.after(step, done)
        c11, c12, c21, c22 = _strassen(prod, after)
        return (jnp.concatenate([c11, c12], axis=1),
                jnp.concatenate([c21, c22], axis=1))

    class KVTile:
        def __init__(self, sch, i, slot, src=None):
            self.sch, self.i, self.slot, self.src = sch, i, slot, src
            self.b = None
            self.pk, self.phis = {}, {}

        def operands(self):
            if self.src is not None:
                return [_bf(self.src[k]) for k in range(7)]
            if self.b is None:
                self.b = [_bf(bq[self.i, k]) for k in range(7)]
            return self.b

        def kproj(self, j):
            self.pk[j] = proj(self.sch, ak, j, self.operands())

        def vproj(self, j):
            ex = {} if j == 0 else None
            vs = proj(self.sch, av, j, self.operands(), ex)
            for g in range(2):
                for p in range(2):
                    vt_v.at[self.slot, 2 * j + g][p * 32:(p + 1) * 32, :] = _pack(
                        vs[g][p * 64:(p + 1) * 64])
            if j == 0:
                r_v[self.i] = jnp.concatenate(
                    [ex[1][0:1] + ex[1][1:2] + ex[3][1:2],
                     ex[4][0:1] + ex[4][1:2] + ex[2][0:1]], axis=1)

        def sm(self, j, g, p, due=None, step=0):
            phi, _ = _feature_map(self.pk[j][g][p * 64:(p + 1) * 64])
            z_v[4 * j + 2 * g + p] += phi[:, :128] + phi[:, 128:]
            if due is None:
                self.phis[j, g, p] = lambda: phi.astype(BF16)
                return
            dst = ph_v.at[self.i, 4 * j + 2 * g + p]
            for t in range(2):
                dst[t * 32:(t + 1) * 32, :] = _pack(phi[t * 64:(t + 1) * 64])
            self.phis[j, g, p] = lambda: _bf(dst[...])
            for t in range(2):
                self.sch.need(due - step * (1 - t), [dst[:, t * 128:(t + 1) * 128]])

        def kv(self, j, g):
            for p in range(2):
                if (j, g, p) not in self.phis:
                    self.sm(j, g, p)
                lhs = _bf(vt_v[self.slot, 2 * j + g, p * 32:(p + 1) * 32, :])
                kv_acc[4 * j + 2 * g + p] += _dot_nt(lhs, self.phis[j, g, p]())

    def first_tiles():
        sch = Sched(zero_s[0] > 0)
        tiles = {'a': KVTile(sch, 0, 0), 'b': KVTile(sch, 1, 1)}
        for op in PROG.split():
            kind, arg = op[0], op[1:2]
            if kind == 'w':
                for nm in op[2:].split(','):
                    named_copy(nm).wait()
            elif kind == 'P':
                build_phit()
            elif kind == 'f':
                fold(1, ak, int(arg))
            elif kind == 'p':
                _, rel, d0 = op.split(':')

                def job(j=int(arg), base=sch.slot + float(d0)):
                    ws = prep_v(j, sch)
                    for q in range(8):
                        sch.need(base + q * 0.375, [w[:, q * 128:(q + 1) * 128] for w in ws])
                sch.at(sch.slot + int(rel), job)
            elif kind == 'U':
                for c in range(8):
                    ln_chunk(int(arg), c)
            elif kind == 'L':
                l0, l1, c0, c1, lead = [float(v) for v in op.split(':')[1:]]
                for c in range(int(c0), int(c1)):
                    due = _eighths(sch.slot + l0 + (l1 - l0) * (c - c0) / (c1 - c0 - 1))
                    rel = int(due - lead)

                    def job(n=int(arg), c=c, due=due, held=rel >= sch.slot):
                        sch.spread(ln_chunk(n, c, sch if held else None,
                                            bp[0] if n == NF else None), due)
                    if rel >= sch.slot:
                        sch.at(rel, job)
                    else:
                        job()
            elif kind == 'S':
                st_ = 4.0 / 7
                for q in range(4):
                    tiles[op[2]].sm(int(arg), q // 2, q % 2,
                                    _eighths(sch.slot + 2.5 + st_ * (2 * q + 1)), _eighths(st_))
            elif kind == 'K':
                tiles[op[2]].kproj(int(arg))
            elif kind == 'V':
                tiles[op[2]].vproj(int(arg))
            elif kind == 'X':
                for g in range(2):
                    sch.at(sch.slot + 1 + g, functools.partial(tiles[op[2]].kv, int(arg), g))
            elif kind == 'Y':
                for g in range(2):
                    tiles[op[2]].kv(int(arg), g)
        assert not sch.jobs and not sch.deps

    def phase1_tile(i, par, sch):
        nxt = jnp.minimum(i + 1, NT - 1)
        o = sch.slot
        tl = KVTile(sch, i, par, bp[par])
        for c in range(8):
            due = 14 * (c // 2) + (5, 13)[c % 2]
            sch.spread(ln_chunk(nxt, c, None, bp[1 - par]),
                       o + (min(due, 54) if par == 0 else due))
        for q, due in enumerate((1, 8, 15, 29, 36, 43)):
            sch.spread(wo_piece(jnp.minimum((i - NF) * 6 + q, 31)), o + due)
        for j in range(NJ if par == 0 else NJ - 1):
            for g in range(2):
                sch.at(o + 14 * (j + 1) + g, functools.partial(tl.kv, j, g))
        for j in range(NJ):
            tl.kproj(j)
            tl.vproj(j)
        if par == 1:
            for g in range(2):
                tl.kv(NJ - 1, g)

    def phase1(m, carry):
        sch = Sched(zero_s[0] > 0)
        for par in range(2):
            phase1_tile(NF + 2 * m + par, par, sch)
        return carry

    first_tiles()
    wo_copy.wait()
    for t in range(NF + 1, NT):
        x_copy(t).wait()
    jax.lax.fori_loop(0, (NT - NF) // 2, phase1, 0)

    for j in range(NJ):
        w_copy(0, j).wait()
    wg_copy.wait()
    wu_copy.wait()
    wd_copy.wait()
    sch = Sched(zero_s[0] > 0)
    row = jax.lax.broadcasted_iota(I32, (64, 128), 0)
    col = jax.lax.broadcasted_iota(I32, (64, 128), 1)
    keep = (row // DH) == (col % 2)
    for j in range(NJ):
        fold(0, aq, j, sch)
        for p in range(4 * j, 4 * j + 4):
            kvp = pltpu.bitcast(sch.hold(_u32(kv_acc[p]), [(r, 0) for r in range(8)]), F32)
            mk = jnp.where(keep, kvp, 0.0)
            for t in range(2):
                m_v.at[p][t * 16:(t + 1) * 16, :] = _pack(mk[t * 32:(t + 1) * 32])
            sch.need(1 + p * 0.375, [m_v[p]])
            z_v[p] = jnp.broadcast_to(jnp.sum(z_v[p], axis=1, keepdims=True), (128, 128))

    r = _round(r_v[...].reshape(NT, T))
    rmax = jnp.max(jnp.max(r, axis=1, keepdims=True), axis=0, keepdims=True)
    pos = (jax.lax.broadcasted_iota(I32, (NT, T), 0) * T
           + jax.lax.broadcasted_iota(I32, (NT, T), 1))
    idx = jnp.min(jnp.where(r == rmax, pos, S))
    idx = jnp.clip(idx, 0, S - 1)
    tile = idx // T
    half = (idx % T) // TH
    sub = pl.multiple_of(((idx % TH) // 16) * 8, 8)
    xs = jnp.concatenate([bq[tile, 1 + 7 * half, pl.ds(sub, 8), :],
                          bq[tile, 7 - 3 * half, pl.ds(sub, 8), :]], axis=1)
    xs = jnp.where(jax.lax.broadcasted_iota(I32, (16, D), 0) == idx % 16,
                   _bf(xs).astype(F32), 0.0)
    xs = jnp.sum(xs, axis=0, keepdims=True)

    def lane_bcast(dst, row):
        for t in range(row.shape[1] // 128):
            dst[t * 128:(t + 1) * 128, :] = jnp.broadcast_to(
                row[:, t * 128:(t + 1) * 128], (128, 128)).T

    lane_bcast(xb_v, xs)
    router = _round(0.5 + 0.5 * jnp.tanh(0.5 * rmax))

    n_first = (tile + 1) & (NT - 1)
    first = proj(sch, aq, 0, [_bf(bq[n_first, k]) for k in range(7)])
    for g in range(2):
        pq0_v[g] = first[g]

    def phase2(i, n):
        last = isinstance(i, int)
        zero = zero_s[0]
        slot = i
        n_next = (n + 1) & (NT - 1)

        s0 = pl.multiple_of(n * T, T)
        b = [_bf(bq[n, k]) for k in range(7)]
        pq = [None] * NJ
        sch = Sched(zero > 0)
        ot = {}
        pq[0] = [pq0_v[g] for g in range(2)]
        phis = {}

        def sm(j, g, p, due, step):
            phi, scales = _feature_map(pq[j][g][p * 64:(p + 1) * 64], z_v[4 * j + 2 * g + p])
            phis[j, g, p] = phi.astype(BF16)
            for t in range(2):
                sch.need(max(due - step * (1 - t), sch.slot + 1),
                         [v[:, t * 128:(t + 1) * 128] for v in scales])

        def nd(j, g):
            ot[j, g] = jnp.concatenate(
                [_dot(_bf(m_v[4 * j + 2 * g + p]), phis[j, g, p]) for p in range(2)], axis=0)
            if g == 1:
                o0, o1 = ot[j, 0], ot[j, 1]
                cs = _lhs_combos(o0[:, :TH], o1[:, :TH], o0[:, TH:], o1[:, TH:])
                for k in range(7):
                    ao_v[2 * k + j // 2][zero, :, (j % 2) * 128:(j % 2 + 1) * 128] = (
                        _u32(cs[k].astype(BF16).T))

        if last:
            fd = (NFC - 1) * FC
        else:
            fu = pl.multiple_of(i * FC, FC)
            fd = pl.multiple_of(jnp.maximum(i - 1, 0) * FC, FC)
        ffn = {}

        def matvec(key, w, vb, due):
            t = (w.astype(F32).reshape(FR // 8, 8, 256)
                 * jnp.concatenate([vb, vb], axis=1).reshape(FR // 8, 8, 256))
            t = jnp.sum(t, axis=0)
            ffn[key] = t if key not in ffn else ffn[key] + t
            sch.need(due, [ffn[key]])

        def ffn_up(w_ref, name, cp, rb, due):
            rs = slice(rb * FR, (rb + 1) * FR)
            matvec((name, cp), w_ref[rs, pl.ds(fu + cp * 256, 256)], xb_v[rs, :], due)

        def ffn_mid():
            hg, hu = [_round(jnp.sum(jnp.concatenate([ffn[nm, 0], ffn[nm, 1]], axis=1),
                                     axis=0, keepdims=True)) for nm in 'gu']
            lane_bcast(hb_v, _round(_round(_silu(hg)) * hu))

        def ffn_down(cp, rb, due):
            cs_ = slice(cp * 256, (cp + 1) * 256)
            if rb == 0:
                ffn['y', cp] = y_acc[:, cs_]
            matvec(('y', cp), wd_v[pl.ds(fd + rb * FR, FR), cs_],
                   hb_v[rb * FR:(rb + 1) * FR, :], due)
            if rb == FC // FR - 1:
                if last:
                    ffn['row', cp] = (
                        _round(jnp.sum(ffn['y', cp], axis=0, keepdims=True)) * router)
                else:
                    y_acc[:, cs_] = ffn['y', cp]

        d0, d1 = (2, 27) if last else (28, 36.5)
        nd_ = 4 * FC // FR
        for t in range(nd_):
            due = _eighths(d0 + (d1 - d0) * t / (nd_ - 1))
            sch.at(0, functools.partial(ffn_down, t % 4, t // 4, due))
        if not last:
            nu_ = 4 * D // FR
            for t in range(nu_):
                due = _eighths(37 + 16.5 * t / (nu_ - 1))
                name, w_ref = (('g', wg_v), ('u', wu_v))[(t // 2) % 2]
                sch.at(0, functools.partial(ffn_up, w_ref, name, t % 2, t // 4, due))
            sch.at(53, ffn_mid)
        lead = 0.5 if last else 0
        for j in range(NJ):
            s1 = 7 * j
            nds = (((1, 4), (1, 4), (1, 4), (2, 3)) if last
                   else ((1, 3), (0, 2), (0, 2), (0, 1)))[j]
            for g in range(2):
                for p in range(2):
                    sch.at(s1 if (j == 0 or g == 1) else s1 - 2, functools.partial(
                        sm, j, g, p, s1 + nds[g] + p - lead, 0.5))
                sch.at(s1 + nds[g], functools.partial(nd, j, g))
        for j in range(1, NJ):
            pq[j] = proj(sch, aq, j, b, early=pq)
        if last:
            def prod_a(k):
                return _dot(_bf(sch.gate(ao_v[2 * k][0])), _bf(bo[k, 0:128, 0:256]))
            part = _strassen(prod_a, sch.after)
        else:
            nxt = proj(sch, aq, 0, [_bf(bq[n_next, k]) for k in range(7)])
            for g in range(2):
                pq0_v[g] = nxt[g]

        er = 32 if last else 64
        rows = jax.lax.broadcasted_iota(I32, (er, 256), 0) + s0
        ne_ = T // er
        gates = {}

        def gate_part(c, e, due):
            r0 = e * er
            h, rh = r0 // TH, r0 % TH
            blk = ((1, 7), (8, 4))[h][c // 2]
            bb = _bf(bq[n, blk, rh // 2:(rh + er) // 2,
                        (c % 2) * 256:(c % 2 + 1) * 256]).astype(F32)
            if last:
                bb = bb + jnp.where(rows + r0 == idx, ffn['row', c], 0.0)
            gates[c, e] = _silu(bb)
            if due is not None:
                sch.need(due, [gates[c, e]])

        def epilogue(c, cc, e, due):
            r0 = e * er
            h, rh = r0 // TH, r0 % TH
            cs = slice(c * 256, (c + 1) * 256)
            rs = slice(rh, rh + er)
            if (c, e) not in gates:
                gate_part(c, e, None)
            xr = x_v[pl.ds(s0 + r0, er), cs].astype(F32)
            sv = jnp.concatenate([cc[2 * h][rs], cc[2 * h + 1][rs]], axis=1)
            res = xr + sv * gates[c, e]
            out_v[slot, r0:r0 + er, cs] = res.astype(BF16)
            if due is not None:
                sch.need(due, [res])

        def out_cols(c, h=None):
            cs = slice(c * 256, (c + 1) * 256)
            if h is None:
                return pltpu.make_async_copy(out_v.at[slot, :, cs],
                                             out_hbm.at[0, pl.ds(s0, T), cs], sem_o.at[NT + c])
            return pltpu.make_async_copy(
                out_v.at[slot, h * TH:(h + 1) * TH, cs],
                out_hbm.at[0, pl.ds(s0 + h * TH, TH), cs], sem_o.at[NT + c + h])

        e0, e1 = (1 if last else 0.5), 6.5
        end = sch.slot + 28 - (7 if last else 0)
        for e in range(ne_):
            sch.at(end - 8, functools.partial(
                gate_part, 3, e, _eighths(end - 7 + 4 * e / (ne_ - 1))))
        pending = []
        c = 0
        while c < 4:
            if last and c == 0:
                def prod(k):
                    return _dot(_bf(sch.gate(ao_v[2 * k + 1][0])),
                                _bf(bo[k, 128:256, 0:256]))
                cc2 = [u + v for u, v in zip(part, _strassen(prod, sch.after))]
                blocks = [(t, [v[:, t * 128:(t + 1) * 128] for v in cc2]) for t in range(2)]
            else:
                def prod(k):
                    return _dot(_bf(sch.gate(jnp.concatenate(
                        [ao_v[2 * k][0], ao_v[2 * k + 1][0]], axis=1))),
                                _bf(bo[k, :, c * 128:(c + 1) * 128]))
                blocks = [(c, _strassen(prod, sch.after))]
            if last:
                for t in pending:
                    out_cols(t).start()
            nb = len(blocks) * ne_
            for q in range(nb):
                t, cc = blocks[q // ne_]
                due = _eighths(sch.slot + e0 + (e1 - e0) * q / (nb - 1))
                epilogue(t, cc, q % ne_, due if t < 3 else None)
                if last and t == 3 and (q + 1) % (ne_ // 2) == 0:
                    out_cols(3, (q + 1) // (ne_ // 2) - 1).start()
            pending = [t for t, _ in blocks]
            c += len(blocks)
        if last:
            for t in range(NT - 1):
                out_copy((tile + 1 + t) & (NT - 1), t).wait()
            for t in range(3):
                out_cols(t).wait()
            for h in range(2):
                out_cols(3, h).wait()
        else:
            out_copy(n, slot).start()
        return n_next

    jax.lax.fori_loop(0, NT - 1, phase2, n_first)
    phase2(NT - 1, tile)


@jax.jit
def pallas_recurrent_scan__linear_kernel_hedgehog__moe_arch_mod__prompt_kernel(
    A_x: jax.Array,
    A_wqkv: jax.Array,
    A_w_phi: jax.Array,
    A_wo: jax.Array,
    B_x: jax.Array,
    B_w_r: jax.Array,
    B_w_gate: jax.Array,
    B_w_up: jax.Array,
    B_w_down: jax.Array,
):
    del B_x
    any_spec = pl.BlockSpec(memory_space=pl.ANY)
    return pl.pallas_call(
        _kernel,
        out_shape=jax.ShapeDtypeStruct((1, S, D), BF16),
        in_specs=[any_spec] * 8,
        out_specs=any_spec,
        scratch_shapes=[
            pltpu.VMEM((S, D), BF16),
            pltpu.VMEM((3, D, D), BF16),
            pltpu.VMEM((H, DH, DH), BF16),
            pltpu.VMEM((8, 128), BF16),
            pltpu.VMEM((D, D), BF16),
            pltpu.VMEM((D, F), BF16),
            pltpu.VMEM((D, F), BF16),
            pltpu.VMEM((F, D), BF16),
            pltpu.VMEM((NT, 9, TH // 2, DHALF), U32),
            pltpu.VMEM((7, 256, DHALF), U32),
            pltpu.VMEM((7, 256, DHALF), U32),
            pltpu.VMEM((7, 256, DHALF), U32),
            pltpu.VMEM((7, 256, DHALF), U32),
            pltpu.VMEM((NP, 64, 128), F32),
            pltpu.VMEM((NP, 128, 128), F32),
            pltpu.VMEM((NF, NP, 64, T), U32),
            pltpu.VMEM((NF, 8, 64, T), U32),
            pltpu.VMEM((NP, 32, 128), U32),
            pltpu.VMEM((128, D), BF16),
            pltpu.VMEM((8, DHALF), U32),
            pltpu.VMEM((NT, 1, T), F32),
            pltpu.VMEM((8, D), F32),
            pltpu.VMEM((D, 128), F32),
            pltpu.VMEM((FC, 128), F32),
            pltpu.VMEM((2, 128, T), F32),
            pltpu.VMEM((NT, T, D), BF16),
            pltpu.SMEM((1,), I32),
        ] + [pltpu.VMEM((1, TH // 2, 256), U32)] * 14
        + [pltpu.VMEM((7, TH // 2, DHALF), U32)] * 2,
        compiler_params=pltpu.CompilerParams(
            vmem_limit_bytes=100 * 1024 * 1024,
            disable_bounds_checks=True),
    )(A_x, A_wqkv, A_w_phi, A_wo, B_w_r.reshape(8, 128), B_w_gate, B_w_up, B_w_down)
```

```python
import functools

import jax
import jax.numpy as jnp
import jax.experimental.pallas as pl
import jax.experimental.pallas.tpu as pltpu

S, D, H, DH, F = 2048, 1024, 32, 32, 3584
T = 256
TH = T // 2
DHALF = D // 2
NT = S // T
NJ = 4
NP = D // 64
FC = 512
NFC = F // FC
FR = 64
NF = 2
ORDER = 'ph wr k0 x0 x1 k1 k2 k3 v0 v1 v2 v3 x2'
PROG = ('w:ph,wr P w:k0 f0 w:x0 U0 w:x1 L1:2.75:6:0:4:5.5 K0a '
        'w:k1 f1 L1:2:6:4:8:4.5 K1a S0a K0b S0b K1b '
        'w:k2,k3,v0 f2 S1a K2a f3 p0:14:18 S1b K2b S2a K3a S2b K3b '
        'w:v1,v2,v3,x2 p1:3:8 p2:16:21 p3:30:35 L2:6:52:0:8:5.5 V0a X0a V0b '
        'X0b V1a X1a S3a V1b X1b V2a X2a S3b V2b X2b V3a X3a V3b Y3b')
LOG2E = 1.4426950408889634
F32, BF16, U32, I32 = jnp.float32, jnp.bfloat16, jnp.uint32, jnp.int32

_NT_DIMS = (((1,), (1,)), ((), ()))


def _dot_nt(a, b):
    return jax.lax.dot_general(a, b, _NT_DIMS, preferred_element_type=F32)


def _dot(a, b):
    return jnp.dot(a, b, preferred_element_type=F32)


def _u32(v):
    return pltpu.bitcast(v, U32) if v.dtype != U32 else v


def _pack(v):
    return pltpu.bitcast(v.astype(BF16), U32)


def _recip(x):
    r = pl.reciprocal(x, approx=True)
    return r * (2.0 - x * r)


def _bf(v):
    return pltpu.bitcast(v, BF16)


def _round(v):
    return v.astype(BF16).astype(F32)


def _eighths(x):
    return round(x * 8) / 8


def _or_all(vals):
    ts = []
    for v in vals:
        u = _u32(v)
        for a in range(u.shape[0] // 8):
            for b in range(u.shape[1] // 128):
                ts.append(u[a * 8:(a + 1) * 8, b * 128:(b + 1) * 128])
    while len(ts) > 1:
        ts = [ts[i] | ts[i + 1] if i + 1 < len(ts) else ts[i] for i in range(0, len(ts), 2)]
    return ts[0]


def _gate(lhs_u32, deps, never):
    if not deps:
        return lhs_u32
    rows = []
    for r in range(lhs_u32.shape[0] // 8):
        row = lhs_u32[r * 8:(r + 1) * 8]
        cs = [c for (r_, c) in deps if r_ == r]
        if cs:
            row = jnp.concatenate(
                [jnp.where(never, _or_all(deps[r, c]), row[:, c * 128:(c + 1) * 128])
                 if c in cs else row[:, c * 128:(c + 1) * 128]
                 for c in range(lhs_u32.shape[1] // 128)], axis=1)
        rows.append(row)
    return jnp.concatenate(rows, axis=0)


class Sched:
    def __init__(self, never):
        self.never = never
        self.slot = 0
        self.gated = 0
        self.token = None
        self.jobs = {}
        self.deps = {}

    def at(self, slot, fn):
        self.jobs.setdefault(slot, []).append(fn)

    def need(self, pos, vals):
        slot, r = divmod(int(round(pos * 8)), 8)
        assert slot >= self.gated, (pos, self.slot)
        d = self.deps.setdefault(slot, {})
        c = (slot + r) % 4
        d.setdefault((r, c), []).extend(vals)

    def spread(self, vals, due, step=0.25):
        for t in range(4):
            self.need(due + t * step, [v[:, t * 128:(t + 1) * 128] for v in vals])

    def gate(self, lhs):
        nc = lhs.shape[1] // 128
        self.gated = self.slot + 1
        deps = {}
        for (r, c), v in self.deps.pop(self.slot, {}).items():
            deps.setdefault((r, c % nc), []).extend(v)
        return _gate(lhs, deps, self.never)

    def hold(self, u, blocks):
        if self.token is None:
            return u
        return _gate(u, {rc: [self.token] for rc in blocks}, self.never)

    def after(self, step, done):
        for fn in self.jobs.pop(self.slot, []):
            fn()
        self.slot += 1


def _layernorm(x):
    m = jnp.mean(x, axis=-1, keepdims=True)
    mb = _round(m)
    xc = x - mb
    dm = m - mb
    v = jnp.mean(xc * xc, axis=-1, keepdims=True) - dm * dm
    a = _round(_round(v) + 1e-5)
    sd = _round(a * jax.lax.rsqrt(a))
    inv = _recip(sd)
    return xc * inv, inv


def _lhs_combos(a11, a12, a21, a22):
    return [a11 + a22, a21 + a22, a11, a22, a11 + a12, a21 - a11, a12 - a22]


def _rhs_combos(b11, b12, b21, b22):
    return [b11 + b22, b11, b12 - b22, b21 - b11, b22, b11 + b12, b21 + b22]


def _strassen(prod, after):
    done = {}
    m1 = prod(0)
    after(0, done)
    m4 = prod(3)
    after(1, done)
    m5 = prod(4)
    after(2, done)
    m7 = prod(6)
    done[0] = m1 + m4 - m5 + m7
    after(3, done)
    m3 = prod(2)
    done[1] = m3 + m5
    after(4, done)
    m2 = prod(1)
    done[2] = m2 + m4
    after(5, done)
    m6 = prod(5)
    done[3] = m1 - m2 + m3 + m6
    after(6, done)
    return done[0], done[1], done[2], done[3]


def _allreduce_pair(x, op):
    x = op(x, pltpu.roll(x, 2, axis=0))
    return op(x, pltpu.roll(x, 4, axis=0))


def _feature_map(p, z=None):
    t = p.shape[1]
    p3 = p.reshape(8, 8, t)
    mx = _allreduce_pair(jnp.max(p3, axis=0), jnp.maximum)
    mn = _allreduce_pair(jnp.min(p3, axis=0), jnp.minimum)
    ep = jnp.exp2(p3 - mx[None])
    en = jnp.exp2(mn[None] - p3)
    rp = _recip(_allreduce_pair(jnp.sum(ep, axis=0), jnp.add))
    rn = _recip(_allreduce_pair(jnp.sum(en, axis=0), jnp.add))
    if z is not None:
        z4 = jnp.concatenate([z] * (t // 128), axis=1).reshape(2, 8, 8, t)
        den = rp * jnp.sum(ep * z4[0], axis=0) + rn * jnp.sum(en * z4[1], axis=0)
        inv = _recip(_allreduce_pair(den, jnp.add) + 1e-6)
        rp, rn = rp * inv, rn * inv
    pos = (ep * rp[None]).reshape(64, t)
    neg = (en * rn[None]).reshape(64, t)
    return jnp.concatenate([pos, neg], axis=0), (rp, rn)


def _silu(x):
    h = 0.5 * x
    return h + h * jnp.tanh(h)


def _kernel(*refs):
    pl.run_scoped(functools.partial(_body, *refs),
                  pltpu.SemaphoreType.DMA((NT + 18,)), pltpu.SemaphoreType.DMA((NT + 5,)))


def _body(x_hbm, wqkv_hbm, wphi_hbm, wo_hbm, wr_hbm, wg_hbm, wu_hbm, wd_hbm,
          out_hbm,
          x_v, w_v, wphi_v, wr_v, wo_v, wg_v, wu_v, wd_v,
          bq, ak, av, aq, bo, kv_acc, z_v, ph_v, vt_v, m_v, phit, wr2, r_v,
          y_acc, xb_v, hb_v, pq0_v, out_v, zero_s, *rest):
    ao_v, bp, (sem, sem_o) = rest[:-4], rest[-4:-2], rest[-2:]

    def x_copy(i):
        return pltpu.make_async_copy(x_hbm.at[0, pl.ds(i * T, T), :],
                                     x_v.at[pl.ds(i * T, T), :], sem.at[i])

    def w_copy(m, j):
        return pltpu.make_async_copy(
            wqkv_hbm.at[:, m * D + j * 256:m * D + (j + 1) * 256],
            w_v.at[m, :, j * 256:(j + 1) * 256], sem.at[NT + 6 + 4 * m + j])

    wphi_copy = pltpu.make_async_copy(wphi_hbm, wphi_v, sem.at[NT])
    wr_copy = pltpu.make_async_copy(wr_hbm, wr_v, sem.at[NT + 1])
    wo_copy = pltpu.make_async_copy(wo_hbm, wo_v, sem.at[NT + 2])
    wg_copy = pltpu.make_async_copy(wg_hbm, wg_v, sem.at[NT + 3])
    wu_copy = pltpu.make_async_copy(wu_hbm, wu_v, sem.at[NT + 4])
    wd_copy = pltpu.make_async_copy(wd_hbm, wd_v, sem.at[NT + 5])

    def out_copy(i, slot):
        return pltpu.make_async_copy(out_v.at[slot],
                                     out_hbm.at[0, pl.ds(i * T, T), :],
                                     sem_o.at[slot])

    def named_copy(nm):
        if nm in ('ph', 'wr'):
            return wphi_copy if nm == 'ph' else wr_copy
        t = int(nm[1])
        return x_copy(t) if nm[0] == 'x' else w_copy({'k': 1, 'v': 2}[nm[0]], t)

    for nm in ORDER.split():
        named_copy(nm).start()
    x_copy(NF + 1).start()
    wo_copy.start()
    for i in range(NF + 2, NT):
        x_copy(i).start()
    for j in range(NJ):
        w_copy(0, j).start()
    wg_copy.start()
    wu_copy.start()
    wd_copy.start()

    zero_s[0] = 0
    kv_acc[...] = jnp.zeros_like(kv_acc)
    y_acc[...] = jnp.zeros_like(y_acc)
    z_v[...] = jnp.zeros_like(z_v)
    hb_v[...] = jnp.zeros_like(hb_v)

    def build_phit():
        row = jax.lax.broadcasted_iota(I32, (128, DH), 0)
        col = jax.lax.broadcasted_iota(I32, (128, DH), 1)
        sel = jnp.where((row % 64) // 2 == col, 1.0, 0.0).astype(BF16)
        wall = wphi_v[...].reshape(H * DH, DH)
        ph = _dot_nt(sel, wall)
        row = jax.lax.broadcasted_iota(I32, (128, D), 0)
        col = jax.lax.broadcasted_iota(I32, (128, D), 1)
        keep = (2 * (row // 64) + row % 2) == ((col % 128) // DH)
        phit[...] = jnp.where(keep, ph * LOG2E, 0.0).astype(BF16)
        wr = wr_v[...].astype(F32)
        halves = [jnp.concatenate([jnp.broadcast_to(wr[4 * h + t:4 * h + t + 1], (16, 128))
                                   for t in range(4)], axis=1) for h in range(2)]
        odd = jax.lax.broadcasted_iota(I32, (16, DHALF), 0) % 2 == 1
        wr2[...] = _pack(jnp.where(odd, halves[1], halves[0]))

    def fold(which, dst, j, sch=None):
        wt = []
        for g in (2 * j, 2 * j + 1):
            r_ = _dot_nt(phit[:, g * 128:(g + 1) * 128],
                         w_v[which, :, g * 128:(g + 1) * 128])
            if sch is not None and g == 2 * j:
                sch.token = r_[0:8, 0:128]
            wt.append(r_)
        w0, w1 = wt
        cs = _lhs_combos(w0[:, :DHALF], w0[:, DHALF:], w1[:, :DHALF], w1[:, DHALF:])
        for k in range(7):
            dst.at[k][j * 64:(j + 1) * 64, :] = _pack(cs[k])

    def prep_v(j, sch):
        ws = [_u32(w_v[2, :, g * 128:(g + 1) * 128]) for g in (2 * j, 2 * j + 1)]
        ws = [sch.hold(w, [(8 * q, 0) for q in range(8)]) for w in ws]
        wt = [_bf(w).T for w in ws]
        f0, f1 = [w.astype(F32) for w in wt]
        w0, w1 = [_u32(w) for w in wt]
        cs = _lhs_combos(f0[:, :DHALF], f0[:, DHALF:], f1[:, :DHALF], f1[:, DHALF:])
        for k in range(7):
            u = w0[:, :DHALF] if k == 2 else w1[:, DHALF:] if k == 3 else _pack(cs[k])
            av.at[k][j * 64:(j + 1) * 64, :] = u
        return w0, w1

    def ln_chunk(n, c, sch=None, also=None, early=None):
        ys = []
        for h in range(2):
            r0 = n * T + h * TH + c * 16
            if not isinstance(r0, int):
                r0 = pl.multiple_of(r0, 16)
            xr = x_v[pl.ds(r0, 16), :].astype(F32)
            if sch is not None:
                xr = pltpu.bitcast(sch.hold(_u32(xr), [(0, 0), (1, 0)]), F32)
            y, inv = _layernorm(xr)
            ys.append(y)
            if early is not None and h == 0:
                early([jnp.broadcast_to(inv, (16, 128))])
        ya, yb = ys
        cs = (_rhs_combos(ya[:, :DHALF], yb[:, :DHALF], ya[:, DHALF:], yb[:, DHALF:])
              + [ya[:, DHALF:], yb[:, :DHALF]])
        out = []
        for k in range(9):
            dst = bq.at[n, k]
            u = _pack(cs[k])
            dst[c * 8:(c + 1) * 8, :] = u
            if also is not None and k < 7:
                dst = also.at[k]
                dst[c * 8:(c + 1) * 8, :] = u
            if isinstance(n, int):
                out.append(dst[c * 8:(c + 1) * 8, :])
        if isinstance(n, int):
            return out
        return [cs[k] for k in (0, 2, 3, 5, 6)]

    def wo_piece(e):
        r0 = pl.multiple_of((e // 8) * 256 + (e % 8) * 16, 16)
        o0 = pl.multiple_of(e * 8, 8)
        w0 = wo_v[pl.ds(r0, 16), :].astype(F32)
        w1 = wo_v[pl.ds(r0 + 128, 16), :].astype(F32)

        def cols(w, par):
            return jnp.concatenate(
                [w[:, (2 * q + par) * 128:(2 * q + par + 1) * 128] for q in range(4)], axis=1)
        cs = _rhs_combos(cols(w0, 0), cols(w0, 1), cols(w1, 0), cols(w1, 1))
        for k in range(7):
            bo.at[k][pl.ds(o0, 8), :] = _pack(cs[k])
        return [cs[k] for k in (0, 2, 3, 5, 6)]

    def proj(sch, a_ref, j, b, extra=None, early=None):
        def prod(k):
            lhs = sch.gate(a_ref[k, j * 64:(j + 1) * 64, :])
            if extra is not None and k in (1, 2, 3, 4):
                r_ = _dot_nt(_bf(jnp.concatenate([lhs, wr2[...]], axis=0)), b[k])
                extra[k] = r_[128:136]
                r_ = r_[0:128]
            else:
                r_ = _dot_nt(_bf(lhs), b[k])
            sch.token = r_[0:8, 0:128]
            return r_

        def after(step, done):
            if step == 4 and early is not None:
                early[j] = [jnp.concatenate([done[0], done[1]], axis=1), None]
            sch.after(step, done)
        c11, c12, c21, c22 = _strassen(prod, after)
        return (jnp.concatenate([c11, c12], axis=1),
                jnp.concatenate([c21, c22], axis=1))

    class KVTile:
        def __init__(self, sch, i, slot, src=None):
            self.sch, self.i, self.slot, self.src = sch, i, slot, src
            self.b = None
            self.pk, self.phis = {}, {}

        def operands(self):
            if self.src is not None:
                return [_bf(self.src[k]) for k in range(7)]
            if self.b is None:
                self.b = [_bf(bq[self.i, k]) for k in range(7)]
            return self.b

        def kproj(self, j):
            self.pk[j] = proj(self.sch, ak, j, self.operands())

        def vproj(self, j):
            ex = {} if j == 0 else None
            vs = proj(self.sch, av, j, self.operands(), ex)
            for g in range(2):
                for p in range(2):
                    vt_v.at[self.slot, 2 * j + g][p * 32:(p + 1) * 32, :] = _pack(
                        vs[g][p * 64:(p + 1) * 64])
            if j == 0:
                r_v[self.i] = jnp.concatenate(
                    [ex[1][0:1] + ex[1][1:2] + ex[3][1:2],
                     ex[4][0:1] + ex[4][1:2] + ex[2][0:1]], axis=1)

        def sm(self, j, g, p, due=None, step=0):
            phi, _ = _feature_map(self.pk[j][g][p * 64:(p + 1) * 64])
            z_v[4 * j + 2 * g + p] += phi[:, :128] + phi[:, 128:]
            if due is None:
                self.phis[j, g, p] = lambda: phi.astype(BF16)
                return
            dst = ph_v.at[self.i, 4 * j + 2 * g + p]
            for t in range(2):
                dst[t * 32:(t + 1) * 32, :] = _pack(phi[t * 64:(t + 1) * 64])
            self.phis[j, g, p] = lambda: _bf(dst[...])
            for t in range(2):
                self.sch.need(due - step * (1 - t), [dst[:, t * 128:(t + 1) * 128]])

        def kv(self, j, g):
            for p in range(2):
                if (j, g, p) not in self.phis:
                    self.sm(j, g, p)
                lhs = _bf(vt_v[self.slot, 2 * j + g, p * 32:(p + 1) * 32, :])
                kv_acc[4 * j + 2 * g + p] += _dot_nt(lhs, self.phis[j, g, p]())

    def first_tiles():
        sch = Sched(zero_s[0] > 0)
        tiles = {'a': KVTile(sch, 0, 0), 'b': KVTile(sch, 1, 1)}
        for op in PROG.split():
            kind, arg = op[0], op[1:2]
            if kind == 'w':
                for nm in op[2:].split(','):
                    named_copy(nm).wait()
            elif kind == 'P':
                build_phit()
            elif kind == 'f':
                fold(1, ak, int(arg))
            elif kind == 'p':
                _, rel, d0 = op.split(':')

                def job(j=int(arg), base=sch.slot + float(d0)):
                    ws = prep_v(j, sch)
                    for q in range(8):
                        sch.need(base + q * 0.375, [w[:, q * 128:(q + 1) * 128] for w in ws])
                sch.at(sch.slot + int(rel), job)
            elif kind == 'U':
                for c in range(8):
                    ln_chunk(int(arg), c)
            elif kind == 'L':
                l0, l1, c0, c1, lead = [float(v) for v in op.split(':')[1:]]
                for c in range(int(c0), int(c1)):
                    due = _eighths(sch.slot + l0 + (l1 - l0) * (c - c0) / (c1 - c0 - 1))
                    rel = int(due - lead)

                    def job(n=int(arg), c=c, due=due, held=rel >= sch.slot):
                        sch.spread(ln_chunk(n, c, sch if held else None,
                                            bp[0] if n == NF else None), due)
                    if rel >= sch.slot:
                        sch.at(rel, job)
                    else:
                        job()
            elif kind == 'S':
                st_ = 4.0 / 7
                for q in range(4):
                    tiles[op[2]].sm(int(arg), q // 2, q % 2,
                                    _eighths(sch.slot + 2.5 + st_ * (2 * q + 1)), _eighths(st_))
            elif kind == 'K':
                tiles[op[2]].kproj(int(arg))
            elif kind == 'V':
                tiles[op[2]].vproj(int(arg))
            elif kind == 'X':
                for g in range(2):
                    sch.at(sch.slot + 1 + g, functools.partial(tiles[op[2]].kv, int(arg), g))
            elif kind == 'Y':
                for g in range(2):
                    tiles[op[2]].kv(int(arg), g)
        assert not sch.jobs and not sch.deps

    def phase1_tile(i, par, sch):
        nxt = jnp.minimum(i + 1, NT - 1)
        o = sch.slot
        tl = KVTile(sch, i, par, bp[par])
        for c in range(8):
            due = o + min(14 * (c // 2) + (5 + par, 13)[c % 2], 54 + par)
            sch.spread(ln_chunk(nxt, c, None, bp[1 - par],
                                functools.partial(sch.need, due - 0.25)), due)
        for q, due in enumerate((2, 9, 16, 30, 37, 44)):
            sch.spread(wo_piece(jnp.minimum((i - NF) * 6 + q, 31)), o + due)
        for j in range(NJ if par == 0 else NJ - 1):
            for g in range(2):
                sch.at(o + 14 * (j + 1) + g, functools.partial(tl.kv, j, g))
        for j in range(NJ):
            tl.kproj(j)
            tl.vproj(j)
        if par == 1:
            for g in range(2):
                tl.kv(NJ - 1, g)

    def phase1(m, carry):
        sch = Sched(zero_s[0] > 0)
        for par in range(2):
            phase1_tile(NF + 2 * m + par, par, sch)
        return carry

    first_tiles()
    wo_copy.wait()
    for t in range(NF + 1, NT):
        x_copy(t).wait()
    jax.lax.fori_loop(0, (NT - NF) // 2, phase1, 0)

    for j in range(NJ):
        w_copy(0, j).wait()
    wg_copy.wait()
    wu_copy.wait()
    wd_copy.wait()
    sch = Sched(zero_s[0] > 0)
    row = jax.lax.broadcasted_iota(I32, (64, 128), 0)
    col = jax.lax.broadcasted_iota(I32, (64, 128), 1)
    keep = (row // DH) == (col % 2)
    for j in range(NJ):
        fold(0, aq, j, sch)
        for p in range(8 * j, 8 * j + 8) if j < 2 else ():
            kvp = pltpu.bitcast(sch.hold(_u32(kv_acc[p]), [(r, 0) for r in range(8)]), F32)
            mk = jnp.where(keep, kvp, 0.0)
            for t in range(2):
                m_v.at[p][t * 16:(t + 1) * 16, :] = _pack(mk[t * 32:(t + 1) * 32])
            sch.need(1 + p * 0.25, [m_v[p]])
            zp = pltpu.bitcast(sch.hold(_u32(z_v[p]), [(r, 0) for r in range(16)]), F32)
            z_v[p] = jnp.broadcast_to(jnp.sum(zp, axis=1, keepdims=True), (128, 128))

    r = _round(r_v[...].reshape(NT, T))
    rmax = jnp.max(jnp.max(r, axis=1, keepdims=True), axis=0, keepdims=True)
    pos = (jax.lax.broadcasted_iota(I32, (NT, T), 0) * T
           + jax.lax.broadcasted_iota(I32, (NT, T), 1))
    idx = jnp.min(jnp.where(r == rmax, pos, S))
    idx = jnp.clip(idx, 0, S - 1)
    tile = idx // T
    half = (idx % T) // TH
    sub = pl.multiple_of(((idx % TH) // 16) * 8, 8)
    xs = jnp.concatenate([bq[tile, 1 + 7 * half, pl.ds(sub, 8), :],
                          bq[tile, 7 - 3 * half, pl.ds(sub, 8), :]], axis=1)
    xs = jnp.where(jax.lax.broadcasted_iota(I32, (16, D), 0) == idx % 16,
                   _bf(xs).astype(F32), 0.0)
    xs = jnp.sum(xs, axis=0, keepdims=True)

    def lane_bcast(dst, row):
        for t in range(row.shape[1] // 128):
            dst[t * 128:(t + 1) * 128, :] = jnp.broadcast_to(
                row[:, t * 128:(t + 1) * 128], (128, 128)).T

    lane_bcast(xb_v, xs)
    router = _round(0.5 + 0.5 * jnp.tanh(0.5 * rmax))

    n_first = (tile + 1) & (NT - 1)
    first = proj(sch, aq, 0, [_bf(bq[n_first, k]) for k in range(7)])
    for g in range(2):
        pq0_v[g] = first[g]

    def phase2(i, n):
        last = isinstance(i, int)
        zero = zero_s[0]
        slot = i
        n_next = (n + 1) & (NT - 1)

        s0 = pl.multiple_of(n * T, T)
        b = [_bf(bq[n, k]) for k in range(7)]
        pq = [None] * NJ
        sch = Sched(zero > 0)
        ot = {}
        pq[0] = [pq0_v[g] for g in range(2)]
        phis = {}

        def sm(j, g, p, due, step):
            phi, scales = _feature_map(pq[j][g][p * 64:(p + 1) * 64], z_v[4 * j + 2 * g + p])
            phis[j, g, p] = phi.astype(BF16)
            for t in range(2):
                sch.need(max(due - step * (1 - t), sch.slot + 1),
                         [v[:, t * 128:(t + 1) * 128] for v in scales])

        def nd(j, g):
            ot[j, g] = jnp.concatenate(
                [_dot(_bf(m_v[4 * j + 2 * g + p]), phis[j, g, p]) for p in range(2)], axis=0)
            if g == 1:
                o0, o1 = ot[j, 0], ot[j, 1]
                cs = _lhs_combos(o0[:, :TH], o1[:, :TH], o0[:, TH:], o1[:, TH:])
                for k in range(7):
                    ao_v[2 * k + j // 2][zero, :, (j % 2) * 128:(j % 2 + 1) * 128] = (
                        _u32(cs[k].astype(BF16).T))

        if last:
            fd = (NFC - 1) * FC
        else:
            fu = pl.multiple_of(i * FC, FC)
            fd = pl.multiple_of(jnp.maximum(i - 1, 0) * FC, FC)
        ffn = {}

        def matvec(key, w, vb, due):
            t = (w.astype(F32).reshape(FR // 8, 8, 256)
                 * jnp.concatenate([vb, vb], axis=1).reshape(FR // 8, 8, 256))
            t = jnp.sum(t, axis=0)
            ffn[key] = t if key not in ffn else ffn[key] + t
            sch.need(due, [ffn[key]])

        def ffn_up(w_ref, name, cp, rb, due):
            rs = slice(rb * FR, (rb + 1) * FR)
            matvec((name, cp), w_ref[rs, pl.ds(fu + cp * 256, 256)], xb_v[rs, :], due)

        def ffn_mid():
            hg, hu = [_round(jnp.sum(jnp.concatenate([ffn[nm, 0], ffn[nm, 1]], axis=1),
                                     axis=0, keepdims=True)) for nm in 'gu']
            lane_bcast(hb_v, _round(_round(_silu(hg)) * hu))

        def ffn_down(cp, rb, due):
            cs_ = slice(cp * 256, (cp + 1) * 256)
            if rb == 0:
                ffn['y', cp] = y_acc[:, cs_]
            matvec(('y', cp), wd_v[pl.ds(fd + rb * FR, FR), cs_],
                   hb_v[rb * FR:(rb + 1) * FR, :], due)
            if rb == FC // FR - 1:
                if last:
                    ffn['row', cp] = (
                        _round(jnp.sum(ffn['y', cp], axis=0, keepdims=True)) * router)
                else:
                    y_acc[:, cs_] = ffn['y', cp]

        d0, d1 = (2, 27) if last else (28, 36.5)
        nd_ = 4 * FC // FR
        for t in range(nd_):
            due = _eighths(d0 + (d1 - d0) * t / (nd_ - 1))
            sch.at(0, functools.partial(ffn_down, t % 4, t // 4, due))
        if not last:
            nu_ = 4 * D // FR
            for t in range(nu_):
                due = _eighths(37 + 16.5 * t / (nu_ - 1))
                name, w_ref = (('g', wg_v), ('u', wu_v))[(t // 2) % 2]
                sch.at(0, functools.partial(ffn_up, w_ref, name, t % 2, t // 4, due))
            sch.at(53, ffn_mid)
        lead = 0.5 if last else 0
        for j in range(NJ):
            s1 = 7 * j
            nds = (((1, 4), (1, 4), (1, 4), (2, 3)) if last
                   else ((1, 3), (0, 2), (0, 2), (0, 1)))[j]
            for g in range(2):
                for p in range(2):
                    sch.at(s1 if (j == 0 or g == 1) else s1 - 2, functools.partial(
                        sm, j, g, p, s1 + nds[g] + p - lead, 0.5))
                sch.at(s1 + nds[g], functools.partial(nd, j, g))
        for j in range(1, NJ):
            pq[j] = proj(sch, aq, j, b, early=pq)
        if last:
            def prod_a(k):
                return _dot(_bf(sch.gate(ao_v[2 * k][0])), _bf(bo[k, 0:128, 0:256]))
            part = _strassen(prod_a, sch.after)
        else:
            nxt = proj(sch, aq, 0, [_bf(bq[n_next, k]) for k in range(7)])
            for g in range(2):
                pq0_v[g] = nxt[g]

        er = 32 if last else 64
        rows = jax.lax.broadcasted_iota(I32, (er, 256), 0) + s0
        ne_ = T // er
        gates = {}

        def gate_part(c, e, due):
            r0 = e * er
            h, rh = r0 // TH, r0 % TH
            blk = ((1, 7), (8, 4))[h][c // 2]
            bb = _bf(bq[n, blk, rh // 2:(rh + er) // 2,
                        (c % 2) * 256:(c % 2 + 1) * 256]).astype(F32)
            if last:
                bb = bb + jnp.where(rows + r0 == idx, ffn['row', c], 0.0)
            gates[c, e] = _silu(bb)
            if due is not None:
                sch.need(due, [gates[c, e]])

        def epilogue(c, cc, e, due):
            r0 = e * er
            h, rh = r0 // TH, r0 % TH
            cs = slice(c * 256, (c + 1) * 256)
            rs = slice(rh, rh + er)
            if (c, e) not in gates:
                gate_part(c, e, None)
            xr = x_v[pl.ds(s0 + r0, er), cs].astype(F32)
            sv = jnp.concatenate([cc[2 * h][rs], cc[2 * h + 1][rs]], axis=1)
            res = xr + sv * gates[c, e]
            out_v[slot, r0:r0 + er, cs] = res.astype(BF16)
            if due is not None:
                sch.need(due, [res])

        def out_cols(c, h=None):
            cs = slice(c * 256, (c + 1) * 256)
            if h is None:
                return pltpu.make_async_copy(out_v.at[slot, :, cs],
                                             out_hbm.at[0, pl.ds(s0, T), cs], sem_o.at[NT + c])
            return pltpu.make_async_copy(
                out_v.at[slot, h * TH:(h + 1) * TH, cs],
                out_hbm.at[0, pl.ds(s0 + h * TH, TH), cs], sem_o.at[NT + c + h])

        e0, e1 = (1 if last else 0.5), 6.5
        end = sch.slot + 28 - (7 if last else 0)
        for e in range(ne_):
            sch.at(end - 8, functools.partial(
                gate_part, 3, e, _eighths(end - 7 + 4 * e / (ne_ - 1))))
        pending = []
        c = 0
        while c < 4:
            if last and c == 0:
                def prod(k):
                    return _dot(_bf(sch.gate(ao_v[2 * k + 1][0])),
                                _bf(bo[k, 128:256, 0:256]))
                cc2 = [u + v for u, v in zip(part, _strassen(prod, sch.after))]
                blocks = [(t, [v[:, t * 128:(t + 1) * 128] for v in cc2]) for t in range(2)]
            else:
                def prod(k):
                    return _dot(_bf(sch.gate(jnp.concatenate(
                        [ao_v[2 * k][0], ao_v[2 * k + 1][0]], axis=1))),
                                _bf(bo[k, :, c * 128:(c + 1) * 128]))
                blocks = [(c, _strassen(prod, sch.after))]
            if last:
                for t in pending:
                    out_cols(t).start()
            nb = len(blocks) * ne_
            for q in range(nb):
                t, cc = blocks[q // ne_]
                due = _eighths(sch.slot + e0 + (e1 - e0) * q / (nb - 1))
                epilogue(t, cc, q % ne_, due if t < 3 else None)
                if last and t == 3 and (q + 1) % (ne_ // 2) == 0:
                    out_cols(3, (q + 1) // (ne_ // 2) - 1).start()
            pending = [t for t, _ in blocks]
            c += len(blocks)
        if last:
            for t in range(NT - 1):
                out_copy((tile + 1 + t) & (NT - 1), t).wait()
            for t in range(3):
                out_cols(t).wait()
            for h in range(2):
                out_cols(3, h).wait()
        else:
            out_copy(n, slot).start()
        return n_next

    jax.lax.fori_loop(0, NT - 1, phase2, n_first)
    phase2(NT - 1, tile)


@jax.jit
def pallas_recurrent_scan__linear_kernel_hedgehog__moe_arch_mod__prompt_kernel(
    A_x: jax.Array,
    A_wqkv: jax.Array,
    A_w_phi: jax.Array,
    A_wo: jax.Array,
    B_x: jax.Array,
    B_w_r: jax.Array,
    B_w_gate: jax.Array,
    B_w_up: jax.Array,
    B_w_down: jax.Array,
):
    del B_x
    any_spec = pl.BlockSpec(memory_space=pl.ANY)
    return pl.pallas_call(
        _kernel,
        out_shape=jax.ShapeDtypeStruct((1, S, D), BF16),
        in_specs=[any_spec] * 8,
        out_specs=any_spec,
        scratch_shapes=[
            pltpu.VMEM((S, D), BF16),
            pltpu.VMEM((3, D, D), BF16),
            pltpu.VMEM((H, DH, DH), BF16),
            pltpu.VMEM((8, 128), BF16),
            pltpu.VMEM((D, D), BF16),
            pltpu.VMEM((D, F), BF16),
            pltpu.VMEM((D, F), BF16),
            pltpu.VMEM((F, D), BF16),
            pltpu.VMEM((NT, 9, TH // 2, DHALF), U32),
            pltpu.VMEM((7, 256, DHALF), U32),
            pltpu.VMEM((7, 256, DHALF), U32),
            pltpu.VMEM((7, 256, DHALF), U32),
            pltpu.VMEM((7, 256, DHALF), U32),
            pltpu.VMEM((NP, 64, 128), F32),
            pltpu.VMEM((NP, 128, 128), F32),
            pltpu.VMEM((NF, NP, 64, T), U32),
            pltpu.VMEM((NF, 8, 64, T), U32),
            pltpu.VMEM((NP, 32, 128), U32),
            pltpu.VMEM((128, D), BF16),
            pltpu.VMEM((8, DHALF), U32),
            pltpu.VMEM((NT, 1, T), F32),
            pltpu.VMEM((8, D), F32),
            pltpu.VMEM((D, 128), F32),
            pltpu.VMEM((FC, 128), F32),
            pltpu.VMEM((2, 128, T), F32),
            pltpu.VMEM((NT, T, D), BF16),
            pltpu.SMEM((1,), I32),
        ] + [pltpu.VMEM((1, TH // 2, 256), U32)] * 14
        + [pltpu.VMEM((7, TH // 2, DHALF), U32)] * 2,
        compiler_params=pltpu.CompilerParams(
            vmem_limit_bytes=100 * 1024 * 1024,
            disable_bounds_checks=True),
    )(A_x, A_wqkv, A_w_phi, A_wo, B_w_r.reshape(8, 128), B_w_gate, B_w_up, B_w_down)
```

```python
import functools

import jax
import jax.numpy as jnp
import jax.experimental.pallas as pl
import jax.experimental.pallas.tpu as pltpu

S, D, H, DH, F = 2048, 1024, 32, 32, 3584
T = 256
TH = T // 2
DHALF = D // 2
NT = S // T
NJ = 4
NP = D // 64
FC = 512
NFC = F // FC
FR = 64
NF = 2
ORDER = 'ph wr k0 x0 x1 k1 k2 k3 v0 v1 v2 v3 x2'
PROG = ('w:ph,wr P w:k0 f0 w:x0 U0 w:x1 L1:3:6:0:4:5.5 K0a '
        'w:k1 f1 L1:2.5:6:4:8:4.5 K1a S1a K0b S0a K1b '
        'w:k2,k3,v0 f2 S0b K2a f3 p0:13:17 S1b K2b S2a K3a S2b K3b '
        'w:v1,v2,v3,x2 p1:3:8 p2:16:21 p3:30:35 L2:6:52:0:8:5.5 V0a X0a V0b '
        'X0b V1a X1a S3a V1b X1b V2a X2a S3b V2b X2b V3a X3a V3b Y3b')
LOG2E = 1.4426950408889634
F32, BF16, U32, I32 = jnp.float32, jnp.bfloat16, jnp.uint32, jnp.int32

_NT_DIMS = (((1,), (1,)), ((), ()))


def _dot_nt(a, b):
    return jax.lax.dot_general(a, b, _NT_DIMS, preferred_element_type=F32)


def _dot(a, b):
    return jnp.dot(a, b, preferred_element_type=F32)


def _u32(v):
    return pltpu.bitcast(v, U32) if v.dtype != U32 else v


def _pack(v):
    return pltpu.bitcast(v.astype(BF16), U32)


def _recip(x):
    r = pl.reciprocal(x, approx=True)
    return r * (2.0 - x * r)


def _bf(v):
    return pltpu.bitcast(v, BF16)


def _round(v):
    return v.astype(BF16).astype(F32)


def _eighths(x):
    return round(x * 8) / 8


def _or_all(vals):
    ts = []
    for v in vals:
        u = _u32(v)
        for a in range(u.shape[0] // 8):
            for b in range(u.shape[1] // 128):
                ts.append(u[a * 8:(a + 1) * 8, b * 128:(b + 1) * 128])
    while len(ts) > 1:
        ts = [ts[i] | ts[i + 1] if i + 1 < len(ts) else ts[i] for i in range(0, len(ts), 2)]
    return ts[0]


def _gate(lhs_u32, deps, never):
    if not deps:
        return lhs_u32
    rows = []
    for r in range(lhs_u32.shape[0] // 8):
        row = lhs_u32[r * 8:(r + 1) * 8]
        cs = [c for (r_, c) in deps if r_ == r]
        if cs:
            row = jnp.concatenate(
                [jnp.where(never, _or_all(deps[r, c]), row[:, c * 128:(c + 1) * 128])
                 if c in cs else row[:, c * 128:(c + 1) * 128]
                 for c in range(lhs_u32.shape[1] // 128)], axis=1)
        rows.append(row)
    return jnp.concatenate(rows, axis=0)


class Sched:
    def __init__(self, never):
        self.never = never
        self.slot = 0
        self.gated = 0
        self.token = None
        self.jobs = {}
        self.deps = {}

    def at(self, slot, fn):
        self.jobs.setdefault(slot, []).append(fn)

    def need(self, pos, vals):
        slot, r = divmod(int(round(pos * 8)), 8)
        assert slot >= self.gated, (pos, self.slot)
        d = self.deps.setdefault(slot, {})
        c = (slot + r) % 4
        d.setdefault((r, c), []).extend(vals)

    def spread(self, vals, due, step=0.25):
        for t in range(4):
            self.need(due + t * step, [v[:, t * 128:(t + 1) * 128] for v in vals])

    def gate(self, lhs):
        nc = lhs.shape[1] // 128
        self.gated = self.slot + 1
        deps = {}
        for (r, c), v in self.deps.pop(self.slot, {}).items():
            deps.setdefault((r, c % nc), []).extend(v)
        return _gate(lhs, deps, self.never)

    def hold(self, u, blocks):
        if self.token is None:
            return u
        return _gate(u, {rc: [self.token] for rc in blocks}, self.never)

    def after(self, step, done):
        for fn in self.jobs.pop(self.slot, []):
            fn()
        self.slot += 1


def _layernorm(x):
    m = jnp.mean(x, axis=-1, keepdims=True)
    mb = _round(m)
    xc = x - mb
    dm = m - mb
    v = jnp.mean(xc * xc, axis=-1, keepdims=True) - dm * dm
    a = _round(_round(v) + 1e-5)
    sd = _round(a * jax.lax.rsqrt(a))
    inv = _recip(sd)
    return xc * inv, inv


def _lhs_combos(a11, a12, a21, a22):
    return [a11 + a22, a21 + a22, a11, a22, a11 + a12, a21 - a11, a12 - a22]


def _rhs_combos(b11, b12, b21, b22):
    return [b11 + b22, b11, b12 - b22, b21 - b11, b22, b11 + b12, b21 + b22]


def _strassen(prod, after):
    done = {}
    m1 = prod(0)
    after(0, done)
    m4 = prod(3)
    after(1, done)
    m5 = prod(4)
    after(2, done)
    m7 = prod(6)
    done[0] = m1 + m4 - m5 + m7
    after(3, done)
    m3 = prod(2)
    done[1] = m3 + m5
    after(4, done)
    m2 = prod(1)
    done[2] = m2 + m4
    after(5, done)
    m6 = prod(5)
    done[3] = m1 - m2 + m3 + m6
    after(6, done)
    return done[0], done[1], done[2], done[3]


def _allreduce_pair(x, op):
    x = op(x, pltpu.roll(x, 2, axis=0))
    return op(x, pltpu.roll(x, 4, axis=0))


def _feature_map(p, z=None):
    t = p.shape[1]
    p3 = p.reshape(8, 8, t)
    mx = _allreduce_pair(jnp.max(p3, axis=0), jnp.maximum)
    mn = _allreduce_pair(jnp.min(p3, axis=0), jnp.minimum)
    ep = jnp.exp2(p3 - mx[None])
    en = jnp.exp2(mn[None] - p3)
    rp = _recip(_allreduce_pair(jnp.sum(ep, axis=0), jnp.add))
    rn = _recip(_allreduce_pair(jnp.sum(en, axis=0), jnp.add))
    if z is not None:
        z4 = jnp.concatenate([z] * (t // 128), axis=1).reshape(2, 8, 8, t)
        den = rp * jnp.sum(ep * z4[0], axis=0) + rn * jnp.sum(en * z4[1], axis=0)
        inv = _recip(_allreduce_pair(den, jnp.add) + 1e-6)
        rp, rn = rp * inv, rn * inv
    pos = (ep * rp[None]).reshape(64, t)
    neg = (en * rn[None]).reshape(64, t)
    return jnp.concatenate([pos, neg], axis=0), (rp, rn)


def _silu(x):
    h = 0.5 * x
    return h + h * jnp.tanh(h)


def _kernel(*refs):
    pl.run_scoped(functools.partial(_body, *refs),
                  pltpu.SemaphoreType.DMA((NT + 18,)), pltpu.SemaphoreType.DMA((NT + 5,)))


def _body(x_hbm, wqkv_hbm, wphi_hbm, wo_hbm, wr_hbm, wg_hbm, wu_hbm, wd_hbm,
          out_hbm,
          x_v, w_v, wphi_v, wr_v, wo_v, wg_v, wu_v, wd_v,
          bq, ak, av, aq, bo, kv_acc, z_v, ph_v, vt_v, m_v, phit, wrb, r_v,
          y_acc, xb_v, hb_v, pq0_v, out_v, zero_s, *rest):
    ao_v, bp, (sem, sem_o) = rest[:-4], rest[-4:-2], rest[-2:]

    def x_copy(i):
        return pltpu.make_async_copy(x_hbm.at[0, pl.ds(i * T, T), :],
                                     x_v.at[pl.ds(i * T, T), :], sem.at[i])

    def w_copy(m, j):
        return pltpu.make_async_copy(
            wqkv_hbm.at[:, m * D + j * 256:m * D + (j + 1) * 256],
            w_v.at[m, :, j * 256:(j + 1) * 256], sem.at[NT + 6 + 4 * m + j])

    wphi_copy = pltpu.make_async_copy(wphi_hbm, wphi_v, sem.at[NT])
    wr_copy = pltpu.make_async_copy(wr_hbm, wr_v, sem.at[NT + 1])
    wo_copy = pltpu.make_async_copy(wo_hbm, wo_v, sem.at[NT + 2])
    wg_copy = pltpu.make_async_copy(wg_hbm, wg_v, sem.at[NT + 3])
    wu_copy = pltpu.make_async_copy(wu_hbm, wu_v, sem.at[NT + 4])
    wd_copy = pltpu.make_async_copy(wd_hbm, wd_v, sem.at[NT + 5])

    def out_copy(i, slot):
        return pltpu.make_async_copy(out_v.at[slot],
                                     out_hbm.at[0, pl.ds(i * T, T), :],
                                     sem_o.at[slot])

    def named_copy(nm):
        if nm in ('ph', 'wr'):
            return wphi_copy if nm == 'ph' else wr_copy
        t = int(nm[1])
        return x_copy(t) if nm[0] == 'x' else w_copy({'k': 1, 'v': 2}[nm[0]], t)

    for nm in ORDER.split():
        named_copy(nm).start()
    x_copy(NF + 1).start()
    wo_copy.start()
    for i in range(NF + 2, NT):
        x_copy(i).start()
    for j in range(NJ):
        w_copy(0, j).start()
    wg_copy.start()
    wu_copy.start()
    wd_copy.start()

    zero_s[0] = 0
    kv_acc[...] = jnp.zeros_like(kv_acc)
    y_acc[...] = jnp.zeros_like(y_acc)
    z_v[...] = jnp.zeros_like(z_v)
    r_v[...] = jnp.full(r_v.shape, -jnp.inf, F32)
    hb_v[...] = jnp.zeros_like(hb_v)

    def build_phit():
        row = jax.lax.broadcasted_iota(I32, (128, DH), 0)
        col = jax.lax.broadcasted_iota(I32, (128, DH), 1)
        sel = jnp.where((row % 64) // 2 == col, 1.0, 0.0).astype(BF16)
        wall = wphi_v[...].reshape(H * DH, DH)
        ph = _dot_nt(sel, wall)
        row = jax.lax.broadcasted_iota(I32, (128, D), 0)
        col = jax.lax.broadcasted_iota(I32, (128, D), 1)
        keep = (2 * (row // 64) + row % 2) == ((col % 128) // DH)
        phit[...] = jnp.where(keep, ph * LOG2E, 0.0).astype(BF16)
        wr = wr_v[...].astype(F32)
        wrb[...] = jnp.concatenate([jnp.broadcast_to(wr[t:t + 1], (8, 128))
                                    for t in range(8)], axis=1)

    def fold(which, dst, j, sch=None):
        wt = []
        for g in (2 * j, 2 * j + 1):
            r_ = _dot_nt(phit[:, g * 128:(g + 1) * 128],
                         w_v[which, :, g * 128:(g + 1) * 128])
            if sch is not None and g == 2 * j:
                sch.token = r_[0:8, 0:128]
            wt.append(r_)
        w0, w1 = wt
        cs = _lhs_combos(w0[:, :DHALF], w0[:, DHALF:], w1[:, :DHALF], w1[:, DHALF:])
        for k in range(7):
            dst.at[k][j * 64:(j + 1) * 64, :] = _pack(cs[k])

    def prep_v(j, sch):
        ws = [_u32(w_v[2, :, g * 128:(g + 1) * 128]) for g in (2 * j, 2 * j + 1)]
        ws = [sch.hold(w, [(8 * q, 0) for q in range(8)]) for w in ws]
        wt = [_bf(w).T for w in ws]
        f0, f1 = [w.astype(F32) for w in wt]
        w0, w1 = [_u32(w) for w in wt]
        cs = _lhs_combos(f0[:, :DHALF], f0[:, DHALF:], f1[:, :DHALF], f1[:, DHALF:])
        for k in range(7):
            u = w0[:, :DHALF] if k == 2 else w1[:, DHALF:] if k == 3 else _pack(cs[k])
            av.at[k][j * 64:(j + 1) * 64, :] = u
        return w0, w1

    def ln_chunk(n, c, sch=None, also=None, early=None, late=None):
        ys = []
        for h in range(2):
            r0 = n * T + h * TH + c * 16
            if not isinstance(r0, int):
                r0 = pl.multiple_of(r0, 16)
            xr = x_v[pl.ds(r0, 16), :].astype(F32)
            if sch is not None:
                xr = pltpu.bitcast(sch.hold(_u32(xr), [(0, 0), (1, 0)]), F32)
            y, inv = _layernorm(xr)
            ys.append(y)
            if early is not None and h == 0:
                early([jnp.broadcast_to(inv, (16, 128))])
            w8 = wrb[...]
            sc = jnp.sum(y * jnp.concatenate([w8, w8], axis=0), axis=-1, keepdims=True)
            r_v.at[n][:, 2 * c + h:2 * c + h + 1] = sc
            if late is not None:
                late([jnp.broadcast_to(sc, (16, 128))])
        ya, yb = ys
        cs = (_rhs_combos(ya[:, :DHALF], yb[:, :DHALF], ya[:, DHALF:], yb[:, DHALF:])
              + [ya[:, DHALF:], yb[:, :DHALF]])
        out = []
        for k in range(9):
            dst = bq.at[n, k]
            u = _pack(cs[k])
            dst[c * 8:(c + 1) * 8, :] = u
            if also is not None and k < 7:
                dst = also.at[k]
                dst[c * 8:(c + 1) * 8, :] = u
            if isinstance(n, int):
                out.append(dst[c * 8:(c + 1) * 8, :])
        if isinstance(n, int):
            return out
        return [cs[k] for k in (0, 2, 3, 5, 6)]

    def wo_piece(e):
        r0 = pl.multiple_of((e // 8) * 256 + (e % 8) * 16, 16)
        o0 = pl.multiple_of(e * 8, 8)
        w0 = wo_v[pl.ds(r0, 16), :].astype(F32)
        w1 = wo_v[pl.ds(r0 + 128, 16), :].astype(F32)

        def cols(w, par):
            return jnp.concatenate(
                [w[:, (2 * q + par) * 128:(2 * q + par + 1) * 128] for q in range(4)], axis=1)
        cs = _rhs_combos(cols(w0, 0), cols(w0, 1), cols(w1, 0), cols(w1, 1))
        for k in range(7):
            bo.at[k][pl.ds(o0, 8), :] = _pack(cs[k])
        return [cs[k] for k in (0, 2, 3, 5, 6)]

    def proj(sch, a_ref, j, b, early=None):
        def prod(k):
            r_ = _dot_nt(_bf(sch.gate(a_ref[k, j * 64:(j + 1) * 64, :])), b[k])
            sch.token = r_[0:8, 0:128]
            return r_

        def after(step, done):
            if step == 4 and early is not None:
                early[j] = [jnp.concatenate([done[0], done[1]], axis=1), None]
            sch.after(step, done)
        c11, c12, c21, c22 = _strassen(prod, after)
        return (jnp.concatenate([c11, c12], axis=1),
                jnp.concatenate([c21, c22], axis=1))

    class KVTile:
        def __init__(self, sch, i, slot, src=None):
            self.sch, self.i, self.slot, self.src = sch, i, slot, src
            self.b = None
            self.pk, self.phis = {}, {}

        def operands(self):
            if self.src is not None:
                return [_bf(self.src[k]) for k in range(7)]
            if self.b is None:
                self.b = [_bf(bq[self.i, k]) for k in range(7)]
            return self.b

        def kproj(self, j):
            self.pk[j] = proj(self.sch, ak, j, self.operands())

        def vproj(self, j):
            vs = proj(self.sch, av, j, self.operands())
            for g in range(2):
                for p in range(2):
                    vt_v.at[self.slot, 2 * j + g][p * 32:(p + 1) * 32, :] = _pack(
                        vs[g][p * 64:(p + 1) * 64])

        def sm(self, j, g, p, due=None, step=0):
            phi, _ = _feature_map(self.pk[j][g][p * 64:(p + 1) * 64])
            z_v[4 * j + 2 * g + p] += phi[:, :128] + phi[:, 128:]
            if due is None:
                self.phis[j, g, p] = lambda: phi.astype(BF16)
                return
            dst = ph_v.at[self.i, 4 * j + 2 * g + p]
            for t in range(2):
                dst[t * 32:(t + 1) * 32, :] = _pack(phi[t * 64:(t + 1) * 64])
            self.phis[j, g, p] = lambda: _bf(dst[...])
            for t in range(2):
                self.sch.need(due - step * (1 - t), [dst[:, t * 128:(t + 1) * 128]])

        def kv(self, j, g):
            for p in range(2):
                if (j, g, p) not in self.phis:
                    self.sm(j, g, p)
                lhs = _bf(vt_v[self.slot, 2 * j + g, p * 32:(p + 1) * 32, :])
                kv_acc[4 * j + 2 * g + p] += _dot_nt(lhs, self.phis[j, g, p]())

    def first_tiles():
        sch = Sched(zero_s[0] > 0)
        tiles = {'a': KVTile(sch, 0, 0), 'b': KVTile(sch, 1, 1)}
        for op in PROG.split():
            kind, arg = op[0], op[1:2]
            if kind == 'w':
                for nm in op[2:].split(','):
                    named_copy(nm).wait()
            elif kind == 'P':
                build_phit()
            elif kind == 'f':
                fold(1, ak, int(arg))
            elif kind == 'p':
                _, rel, d0 = op.split(':')

                def job(j=int(arg), base=sch.slot + float(d0)):
                    ws = prep_v(j, sch)
                    for q in range(8):
                        sch.need(base + q * 0.375, [w[:, q * 128:(q + 1) * 128] for w in ws])
                sch.at(sch.slot + int(rel), job)
            elif kind == 'U':
                for c in range(8):
                    ln_chunk(int(arg), c)
            elif kind == 'L':
                l0, l1, c0, c1, lead = [float(v) for v in op.split(':')[1:]]
                for c in range(int(c0), int(c1)):
                    due = _eighths(sch.slot + l0 + (l1 - l0) * (c - c0) / (c1 - c0 - 1))
                    rel = int(due - lead)

                    def job(n=int(arg), c=c, due=due, held=rel >= sch.slot):
                        late = functools.partial(sch.need, due + 2)
                        sch.spread(ln_chunk(n, c, sch if held else None,
                                            bp[0] if n == NF else None, None,
                                            late if n == NF else None), due)
                    if rel >= sch.slot:
                        sch.at(rel, job)
                    else:
                        job()
            elif kind == 'S':
                st_ = 4.0 / 7
                for q in range(4):
                    tiles[op[2]].sm(int(arg), q // 2, q % 2,
                                    _eighths(sch.slot + 2.5 + st_ * (2 * q + 1)), _eighths(st_))
            elif kind == 'K':
                tiles[op[2]].kproj(int(arg))
            elif kind == 'V':
                tiles[op[2]].vproj(int(arg))
            elif kind == 'X':
                for g in range(2):
                    sch.at(sch.slot + 1 + g, functools.partial(tiles[op[2]].kv, int(arg), g))
            elif kind == 'Y':
                for g in range(2):
                    tiles[op[2]].kv(int(arg), g)
        assert not sch.jobs and not sch.deps

    def phase1_tile(i, par, sch):
        nxt = jnp.minimum(i + 1, NT - 1)
        o = sch.slot
        tl = KVTile(sch, i, par, bp[par])
        for c in range(8):
            due = o + min(14 * (c // 2) + (5, 13)[c % 2], 54 + par)
            sch.spread(ln_chunk(nxt, c, None, bp[1 - par],
                                functools.partial(sch.need, due - 0.25),
                                functools.partial(sch.need, min(due + 3, 111.875))),
                       due, 0.125)
        for q, due in enumerate((2, 9, 16, 30, 37, 44)):
            sch.spread(wo_piece(jnp.minimum((i - NF) * 6 + q, 31)), o + due)
        for j in range(NJ if par == 0 else NJ - 1):
            for g in range(2):
                sch.at(o + 14 * (j + 1) + g, functools.partial(tl.kv, j, g))
        for j in range(NJ):
            tl.kproj(j)
            tl.vproj(j)
        if par == 1:
            for g in range(2):
                tl.kv(NJ - 1, g)

    def phase1(m, carry):
        sch = Sched(zero_s[0] > 0)
        for par in range(2):
            phase1_tile(NF + 2 * m + par, par, sch)
        return carry

    first_tiles()
    wo_copy.wait()
    for t in range(NF + 1, NT):
        x_copy(t).wait()
    jax.lax.fori_loop(0, (NT - NF) // 2, phase1, 0)

    for j in range(NJ):
        w_copy(0, j).wait()
    wg_copy.wait()
    wu_copy.wait()
    wd_copy.wait()
    sch = Sched(zero_s[0] > 0)
    row = jax.lax.broadcasted_iota(I32, (64, 128), 0)
    col = jax.lax.broadcasted_iota(I32, (64, 128), 1)
    keep = (row // DH) == (col % 2)
    for j in range(NJ):
        fold(0, aq, j, sch)
        for p in range(8 * j, 8 * j + 8) if j < 2 else ():
            kvp = pltpu.bitcast(sch.hold(_u32(kv_acc[p]), [(r, 0) for r in range(8)]), F32)
            mk = jnp.where(keep, kvp, 0.0)
            for t in range(2):
                m_v.at[p][t * 16:(t + 1) * 16, :] = _pack(mk[t * 32:(t + 1) * 32])
            sch.need(1 + p * 0.25, [m_v[p]])
            zp = pltpu.bitcast(sch.hold(_u32(z_v[p]), [(r, 0) for r in range(16)]), F32)
            z_v[p] = jnp.broadcast_to(jnp.sum(zp, axis=1, keepdims=True), (128, 128))

    r = _round(r_v[...].reshape(NT * 16, 128))
    rmax = jnp.max(jnp.max(r, axis=0, keepdims=True), axis=1, keepdims=True)
    rw = jax.lax.broadcasted_iota(I32, (NT * 16, 128), 0)
    ln = jax.lax.broadcasted_iota(I32, (NT * 16, 128), 1)
    pos = (rw // 16) * T + (ln % 2) * TH + (ln // 2) * 16 + rw % 16
    idx = jnp.min(jnp.where(r == rmax, pos, S))
    idx = jnp.clip(idx, 0, S - 1)
    tile = idx // T
    half = (idx % T) // TH
    sub = pl.multiple_of(((idx % TH) // 16) * 8, 8)
    xs = jnp.concatenate([bq[tile, 1 + 7 * half, pl.ds(sub, 8), :],
                          bq[tile, 7 - 3 * half, pl.ds(sub, 8), :]], axis=1)
    xs = jnp.where(jax.lax.broadcasted_iota(I32, (16, D), 0) == idx % 16,
                   _bf(xs).astype(F32), 0.0)
    xs = jnp.sum(xs, axis=0, keepdims=True)

    def lane_bcast(dst, row):
        for t in range(row.shape[1] // 128):
            dst[t * 128:(t + 1) * 128, :] = jnp.broadcast_to(
                row[:, t * 128:(t + 1) * 128], (128, 128)).T

    lane_bcast(xb_v, xs)
    router = _round(0.5 + 0.5 * jnp.tanh(0.5 * rmax))

    n_first = (tile + 1) & (NT - 1)
    first = proj(sch, aq, 0, [_bf(bq[n_first, k]) for k in range(7)])
    for g in range(2):
        pq0_v[g] = first[g]

    def phase2(i, n):
        last = isinstance(i, int)
        zero = zero_s[0]
        slot = i
        n_next = (n + 1) & (NT - 1)

        s0 = pl.multiple_of(n * T, T)
        b = [_bf(bq[n, k]) for k in range(7)]
        pq = [None] * NJ
        sch = Sched(zero > 0)
        ot = {}
        pq[0] = [pq0_v[g] for g in range(2)]
        phis = {}

        def sm(j, g, p, due, step):
            phi, scales = _feature_map(pq[j][g][p * 64:(p + 1) * 64], z_v[4 * j + 2 * g + p])
            phis[j, g, p] = phi.astype(BF16)
            for t in range(2):
                sch.need(max(due - step * (1 - t), sch.slot + 1),
                         [v[:, t * 128:(t + 1) * 128] for v in scales])

        def nd(j, g):
            ot[j, g] = jnp.concatenate(
                [_dot(_bf(m_v[4 * j + 2 * g + p]), phis[j, g, p]) for p in range(2)], axis=0)
            if g == 1:
                o0, o1 = ot[j, 0], ot[j, 1]
                cs = _lhs_combos(o0[:, :TH], o1[:, :TH], o0[:, TH:], o1[:, TH:])
                for k in range(7):
                    ao_v[2 * k + j // 2][zero, :, (j % 2) * 128:(j % 2 + 1) * 128] = (
                        _u32(cs[k].astype(BF16).T))

        if last:
            fd = (NFC - 1) * FC
        else:
            fu = pl.multiple_of(i * FC, FC)
            fd = pl.multiple_of(jnp.maximum(i - 1, 0) * FC, FC)
        ffn = {}

        def matvec(key, w, vb, due):
            t = (w.astype(F32).reshape(FR // 8, 8, 256)
                 * jnp.concatenate([vb, vb], axis=1).reshape(FR // 8, 8, 256))
            t = jnp.sum(t, axis=0)
            ffn[key] = t if key not in ffn else ffn[key] + t
            sch.need(due, [ffn[key]])

        def ffn_up(w_ref, name, cp, rb, due):
            rs = slice(rb * FR, (rb + 1) * FR)
            matvec((name, cp), w_ref[rs, pl.ds(fu + cp * 256, 256)], xb_v[rs, :], due)

        def ffn_mid():
            hg, hu = [_round(jnp.sum(jnp.concatenate([ffn[nm, 0], ffn[nm, 1]], axis=1),
                                     axis=0, keepdims=True)) for nm in 'gu']
            lane_bcast(hb_v, _round(_round(_silu(hg)) * hu))

        def ffn_down(cp, rb, due):
            cs_ = slice(cp * 256, (cp + 1) * 256)
            if rb == 0:
                ffn['y', cp] = y_acc[:, cs_]
            matvec(('y', cp), wd_v[pl.ds(fd + rb * FR, FR), cs_],
                   hb_v[rb * FR:(rb + 1) * FR, :], due)
            if rb == FC // FR - 1:
                if last:
                    ffn['row', cp] = (
                        _round(jnp.sum(ffn['y', cp], axis=0, keepdims=True)) * router)
                else:
                    y_acc[:, cs_] = ffn['y', cp]

        d0, d1 = (2, 27) if last else (28, 36.5)
        nd_ = 4 * FC // FR
        for t in range(nd_):
            due = _eighths(d0 + (d1 - d0) * t / (nd_ - 1))
            sch.at(0, functools.partial(ffn_down, t % 4, t // 4, due))
        if not last:
            nu_ = 4 * D // FR
            for t in range(nu_):
                due = _eighths(37 + 16.5 * t / (nu_ - 1))
                name, w_ref = (('g', wg_v), ('u', wu_v))[(t // 2) % 2]
                sch.at(0, functools.partial(ffn_up, w_ref, name, t % 2, t // 4, due))
            sch.at(53, ffn_mid)
        lead = 0.5 if last else 0
        for j in range(NJ):
            s1 = 7 * j
            nds = (((1, 4), (1, 4), (1, 4), (2, 3)) if last
                   else ((1, 3), (0, 2), (0, 2), (0, 1)))[j]
            for g in range(2):
                for p in range(2):
                    sch.at(s1 if (j == 0 or g == 1) else s1 - 2, functools.partial(
                        sm, j, g, p, s1 + nds[g] + p - lead, 0.5))
                sch.at(s1 + nds[g], functools.partial(nd, j, g))
        for j in range(1, NJ):
            pq[j] = proj(sch, aq, j, b, early=pq)
        if last:
            def prod_a(k):
                return _dot(_bf(sch.gate(ao_v[2 * k][0])), _bf(bo[k, 0:128, 0:256]))
            part = _strassen(prod_a, sch.after)
        else:
            nxt = proj(sch, aq, 0, [_bf(bq[n_next, k]) for k in range(7)])
            for g in range(2):
                pq0_v[g] = nxt[g]

        er = 32 if last else 64
        rows = jax.lax.broadcasted_iota(I32, (er, 256), 0) + s0
        ne_ = T // er
        gates = {}

        def gate_part(c, e, due):
            r0 = e * er
            h, rh = r0 // TH, r0 % TH
            blk = ((1, 7), (8, 4))[h][c // 2]
            bb = _bf(bq[n, blk, rh // 2:(rh + er) // 2,
                        (c % 2) * 256:(c % 2 + 1) * 256]).astype(F32)
            if last:
                bb = bb + jnp.where(rows + r0 == idx, ffn['row', c], 0.0)
            gates[c, e] = _silu(bb)
            if due is not None:
                sch.need(due, [gates[c, e]])

        def epilogue(c, cc, e, due):
            r0 = e * er
            h, rh = r0 // TH, r0 % TH
            cs = slice(c * 256, (c + 1) * 256)
            rs = slice(rh, rh + er)
            if (c, e) not in gates:
                gate_part(c, e, None)
            xr = x_v[pl.ds(s0 + r0, er), cs].astype(F32)
            sv = jnp.concatenate([cc[2 * h][rs], cc[2 * h + 1][rs]], axis=1)
            res = xr + sv * gates[c, e]
            out_v[slot, r0:r0 + er, cs] = res.astype(BF16)
            if due is not None:
                sch.need(due, [res])

        def out_cols(c, h=None):
            cs = slice(c * 256, (c + 1) * 256)
            if h is None:
                return pltpu.make_async_copy(out_v.at[slot, :, cs],
                                             out_hbm.at[0, pl.ds(s0, T), cs], sem_o.at[NT + c])
            return pltpu.make_async_copy(
                out_v.at[slot, h * TH:(h + 1) * TH, cs],
                out_hbm.at[0, pl.ds(s0 + h * TH, TH), cs], sem_o.at[NT + c + h])

        e0, e1 = (1 if last else 0.5), 6.5
        end = sch.slot + 28 - (7 if last else 0)
        for e in range(ne_):
            sch.at(end - 8, functools.partial(
                gate_part, 3, e, _eighths(end - 7 + 4 * e / (ne_ - 1))))
        pending = []
        c = 0
        while c < 4:
            if last and c == 0:
                def prod(k):
                    return _dot(_bf(sch.gate(ao_v[2 * k + 1][0])),
                                _bf(bo[k, 128:256, 0:256]))
                cc2 = [u + v for u, v in zip(part, _strassen(prod, sch.after))]
                blocks = [(t, [v[:, t * 128:(t + 1) * 128] for v in cc2]) for t in range(2)]
            else:
                def prod(k):
                    return _dot(_bf(sch.gate(jnp.concatenate(
                        [ao_v[2 * k][0], ao_v[2 * k + 1][0]], axis=1))),
                                _bf(bo[k, :, c * 128:(c + 1) * 128]))
                blocks = [(c, _strassen(prod, sch.after))]
            if last:
                for t in pending:
                    out_cols(t).start()
            nb = len(blocks) * ne_
            for q in range(nb):
                t, cc = blocks[q // ne_]
                due = _eighths(sch.slot + e0 + (e1 - e0) * q / (nb - 1))
                epilogue(t, cc, q % ne_, due if t < 3 else None)
                if last and t == 3 and (q + 1) % (ne_ // 2) == 0:
                    out_cols(3, (q + 1) // (ne_ // 2) - 1).start()
            pending = [t for t, _ in blocks]
            c += len(blocks)
        if last:
            for t in range(NT - 1):
                out_copy((tile + 1 + t) & (NT - 1), t).wait()
            for t in range(3):
                out_cols(t).wait()
            for h in range(2):
                out_cols(3, h).wait()
        else:
            out_copy(n, slot).start()
        return n_next

    jax.lax.fori_loop(0, NT - 1, phase2, n_first)
    phase2(NT - 1, tile)


@jax.jit
def pallas_recurrent_scan__linear_kernel_hedgehog__moe_arch_mod__prompt_kernel(
    A_x: jax.Array,
    A_wqkv: jax.Array,
    A_w_phi: jax.Array,
    A_wo: jax.Array,
    B_x: jax.Array,
    B_w_r: jax.Array,
    B_w_gate: jax.Array,
    B_w_up: jax.Array,
    B_w_down: jax.Array,
):
    del B_x
    any_spec = pl.BlockSpec(memory_space=pl.ANY)
    return pl.pallas_call(
        _kernel,
        out_shape=jax.ShapeDtypeStruct((1, S, D), BF16),
        in_specs=[any_spec] * 8,
        out_specs=any_spec,
        scratch_shapes=[
            pltpu.VMEM((S, D), BF16),
            pltpu.VMEM((3, D, D), BF16),
            pltpu.VMEM((H, DH, DH), BF16),
            pltpu.VMEM((8, 128), BF16),
            pltpu.VMEM((D, D), BF16),
            pltpu.VMEM((D, F), BF16),
            pltpu.VMEM((D, F), BF16),
            pltpu.VMEM((F, D), BF16),
            pltpu.VMEM((NT, 9, TH // 2, DHALF), U32),
            pltpu.VMEM((7, 256, DHALF), U32),
            pltpu.VMEM((7, 256, DHALF), U32),
            pltpu.VMEM((7, 256, DHALF), U32),
            pltpu.VMEM((7, 256, DHALF), U32),
            pltpu.VMEM((NP, 64, 128), F32),
            pltpu.VMEM((NP, 128, 128), F32),
            pltpu.VMEM((NF, NP, 64, T), U32),
            pltpu.VMEM((NF, 8, 64, T), U32),
            pltpu.VMEM((NP, 32, 128), U32),
            pltpu.VMEM((128, D), BF16),
            pltpu.VMEM((8, D), F32),
            pltpu.VMEM((NT, 16, 128), F32),
            pltpu.VMEM((8, D), F32),
            pltpu.VMEM((D, 128), F32),
            pltpu.VMEM((FC, 128), F32),
            pltpu.VMEM((2, 128, T), F32),
            pltpu.VMEM((NT, T, D), BF16),
            pltpu.SMEM((1,), I32),
        ] + [pltpu.VMEM((1, TH // 2, 256), U32)] * 14
        + [pltpu.VMEM((7, TH // 2, DHALF), U32)] * 2,
        compiler_params=pltpu.CompilerParams(
            vmem_limit_bytes=100 * 1024 * 1024,
            disable_bounds_checks=True),
    )(A_x, A_wqkv, A_w_phi, A_wo, B_w_r.reshape(8, 128), B_w_gate, B_w_up, B_w_down)
```

```python
import functools

import jax
import jax.numpy as jnp
import jax.experimental.pallas as pl
import jax.experimental.pallas.tpu as pltpu

S, D, H, DH, F = 2048, 1024, 32, 32, 3584
T = 256
TH = T // 2
DHALF = D // 2
NT = S // T
NJ = 4
NP = D // 64
FC = 512
NFC = F // FC
FR = 64
NF = 2
ORDER = 'ph wr x0 k0 x1 k1 k2 k3 v0 v1 v2 v3 x2'
PROG = ('w:ph,wr P w:x0 U0 w:k0 f0 w:x1 L1:3:6:0:4:5.5 K0a '
        'w:k1 f1 L1:2.5:6:4:8:4.5 K1a S1a K0b S0a K1b '
        'w:k2,k3,v0 f2 S0b K2a f3 p0:13:17 S1b K2b S2a K3a S2b K3b '
        'w:v1,v2,v3,x2 p1:3:8 p2:16:21 p3:30:35 L2:6:52:0:8:5.5 V0a X0a V0b '
        'X0b V1a X1a S3a V1b X1b V2a X2a S3b V2b X2b V3a X3a V3b Y3b')
LOG2E = 1.4426950408889634
F32, BF16, U32, I32 = jnp.float32, jnp.bfloat16, jnp.uint32, jnp.int32

_NT_DIMS = (((1,), (1,)), ((), ()))


def _dot_nt(a, b):
    return jax.lax.dot_general(a, b, _NT_DIMS, preferred_element_type=F32)


def _dot(a, b):
    return jnp.dot(a, b, preferred_element_type=F32)


def _u32(v):
    return pltpu.bitcast(v, U32) if v.dtype != U32 else v


def _pack(v):
    return pltpu.bitcast(v.astype(BF16), U32)


def _recip(x):
    r = pl.reciprocal(x, approx=True)
    return r * (2.0 - x * r)


def _bf(v):
    return pltpu.bitcast(v, BF16)


def _round(v):
    return v.astype(BF16).astype(F32)


def _eighths(x):
    return round(x * 8) / 8


def _or_all(vals):
    ts = []
    for v in vals:
        u = _u32(v)
        for a in range(u.shape[0] // 8):
            for b in range(u.shape[1] // 128):
                ts.append(u[a * 8:(a + 1) * 8, b * 128:(b + 1) * 128])
    while len(ts) > 1:
        ts = [ts[i] | ts[i + 1] if i + 1 < len(ts) else ts[i] for i in range(0, len(ts), 2)]
    return ts[0]


def _gate(lhs_u32, deps, never):
    if not deps:
        return lhs_u32
    rows = []
    for r in range(lhs_u32.shape[0] // 8):
        row = lhs_u32[r * 8:(r + 1) * 8]
        cs = [c for (r_, c) in deps if r_ == r]
        if cs:
            row = jnp.concatenate(
                [jnp.where(never, _or_all(deps[r, c]), row[:, c * 128:(c + 1) * 128])
                 if c in cs else row[:, c * 128:(c + 1) * 128]
                 for c in range(lhs_u32.shape[1] // 128)], axis=1)
        rows.append(row)
    return jnp.concatenate(rows, axis=0)


class Sched:
    def __init__(self, never):
        self.never = never
        self.slot = 0
        self.gated = 0
        self.token = None
        self.jobs = {}
        self.deps = {}

    def at(self, slot, fn):
        self.jobs.setdefault(slot, []).append(fn)

    def need(self, pos, vals):
        slot, r = divmod(int(round(pos * 8)), 8)
        assert slot >= self.gated, (pos, self.slot)
        d = self.deps.setdefault(slot, {})
        c = (slot + r) % 4
        d.setdefault((r, c), []).extend(vals)

    def spread(self, vals, due, step=0.25):
        for t in range(4):
            self.need(due + t * step, [v[:, t * 128:(t + 1) * 128] for v in vals])

    def gate(self, lhs):
        nc = lhs.shape[1] // 128
        self.gated = self.slot + 1
        deps = {}
        for (r, c), v in self.deps.pop(self.slot, {}).items():
            deps.setdefault((r, c % nc), []).extend(v)
        return _gate(lhs, deps, self.never)

    def hold(self, u, blocks):
        if self.token is None:
            return u
        return _gate(u, {rc: [self.token] for rc in blocks}, self.never)

    def after(self, step, done):
        for fn in self.jobs.pop(self.slot, []):
            fn()
        self.slot += 1


def _layernorm(x):
    m = jnp.mean(x, axis=-1, keepdims=True)
    mb = _round(m)
    xc = x - mb
    dm = m - mb
    v = jnp.mean(xc * xc, axis=-1, keepdims=True) - dm * dm
    a = _round(_round(v) + 1e-5)
    sd = _round(a * jax.lax.rsqrt(a))
    inv = _recip(sd)
    return xc * inv, inv


def _lhs_combos(a11, a12, a21, a22):
    return [a11 + a22, a21 + a22, a11, a22, a11 + a12, a21 - a11, a12 - a22]


def _rhs_combos(b11, b12, b21, b22):
    return [b11 + b22, b11, b12 - b22, b21 - b11, b22, b11 + b12, b21 + b22]


def _strassen(prod, after):
    done = {}
    m1 = prod(0)
    after(0, done)
    m4 = prod(3)
    after(1, done)
    m5 = prod(4)
    after(2, done)
    m7 = prod(6)
    done[0] = m1 + m4 - m5 + m7
    after(3, done)
    m3 = prod(2)
    done[1] = m3 + m5
    after(4, done)
    m2 = prod(1)
    done[2] = m2 + m4
    after(5, done)
    m6 = prod(5)
    done[3] = m1 - m2 + m3 + m6
    after(6, done)
    return done[0], done[1], done[2], done[3]


def _allreduce_pair(x, op):
    x = op(x, pltpu.roll(x, 2, axis=0))
    return op(x, pltpu.roll(x, 4, axis=0))


def _feature_map(p, z=None):
    t = p.shape[1]
    p3 = p.reshape(8, 8, t)
    mx = _allreduce_pair(jnp.max(p3, axis=0), jnp.maximum)
    mn = _allreduce_pair(jnp.min(p3, axis=0), jnp.minimum)
    ep = jnp.exp2(p3 - mx[None])
    en = jnp.exp2(mn[None] - p3)
    rp = _recip(_allreduce_pair(jnp.sum(ep, axis=0), jnp.add))
    rn = _recip(_allreduce_pair(jnp.sum(en, axis=0), jnp.add))
    if z is not None:
        z4 = jnp.concatenate([z] * (t // 128), axis=1).reshape(2, 8, 8, t)
        den = rp * jnp.sum(ep * z4[0], axis=0) + rn * jnp.sum(en * z4[1], axis=0)
        inv = _recip(_allreduce_pair(den, jnp.add) + 1e-6)
        rp, rn = rp * inv, rn * inv
    pos = (ep * rp[None]).reshape(64, t)
    neg = (en * rn[None]).reshape(64, t)
    return jnp.concatenate([pos, neg], axis=0), (rp, rn)


def _silu(x):
    h = 0.5 * x
    return h + h * jnp.tanh(h)


def _kernel(*refs):
    pl.run_scoped(functools.partial(_body, *refs),
                  pltpu.SemaphoreType.DMA((NT + 18,)), pltpu.SemaphoreType.DMA((NT + 5,)))


def _body(x_hbm, wqkv_hbm, wphi_hbm, wo_hbm, wr_hbm, wg_hbm, wu_hbm, wd_hbm,
          out_hbm,
          x_v, w_v, wphi_v, wr_v, wo_v, wg_v, wu_v, wd_v,
          bq, ak, av, aq, bo, kv_acc, z_v, ph_v, vt_v, m_v, phit, wrb, r_v,
          y_acc, xb_v, hb_v, pq0_v, out_v, zero_s, *rest):
    ao_v, bp, (sem, sem_o) = rest[:-4], rest[-4:-2], rest[-2:]

    def x_copy(i):
        return pltpu.make_async_copy(x_hbm.at[0, pl.ds(i * T, T), :],
                                     x_v.at[pl.ds(i * T, T), :], sem.at[i])

    def w_copy(m, j):
        return pltpu.make_async_copy(
            wqkv_hbm.at[:, m * D + j * 256:m * D + (j + 1) * 256],
            w_v.at[m, :, j * 256:(j + 1) * 256], sem.at[NT + 6 + 4 * m + j])

    wphi_copy = pltpu.make_async_copy(wphi_hbm, wphi_v, sem.at[NT])
    wr_copy = pltpu.make_async_copy(wr_hbm, wr_v, sem.at[NT + 1])
    wo_copy = pltpu.make_async_copy(wo_hbm, wo_v, sem.at[NT + 2])
    wg_copy = pltpu.make_async_copy(wg_hbm, wg_v, sem.at[NT + 3])
    wu_copy = pltpu.make_async_copy(wu_hbm, wu_v, sem.at[NT + 4])
    wd_copy = pltpu.make_async_copy(wd_hbm, wd_v, sem.at[NT + 5])

    def out_copy(i, slot):
        return pltpu.make_async_copy(out_v.at[slot],
                                     out_hbm.at[0, pl.ds(i * T, T), :],
                                     sem_o.at[slot])

    def named_copy(nm):
        if nm in ('ph', 'wr'):
            return wphi_copy if nm == 'ph' else wr_copy
        t = int(nm[1])
        return x_copy(t) if nm[0] == 'x' else w_copy({'k': 1, 'v': 2}[nm[0]], t)

    for nm in ORDER.split():
        named_copy(nm).start()
    x_copy(NF + 1).start()
    wo_copy.start()
    for i in range(NF + 2, NT):
        x_copy(i).start()
    for j in range(NJ):
        w_copy(0, j).start()
    wg_copy.start()
    wu_copy.start()
    wd_copy.start()

    zero_s[0] = 0
    kv_acc[...] = jnp.zeros_like(kv_acc)
    y_acc[...] = jnp.zeros_like(y_acc)
    z_v[...] = jnp.zeros_like(z_v)
    r_v[...] = jnp.full(r_v.shape, -jnp.inf, F32)
    hb_v[...] = jnp.zeros_like(hb_v)

    def build_phit():
        row = jax.lax.broadcasted_iota(I32, (128, DH), 0)
        col = jax.lax.broadcasted_iota(I32, (128, DH), 1)
        sel = jnp.where((row % 64) // 2 == col, 1.0, 0.0).astype(BF16)
        wall = wphi_v[...].reshape(H * DH, DH)
        ph = _dot_nt(sel, wall)
        row = jax.lax.broadcasted_iota(I32, (128, D), 0)
        col = jax.lax.broadcasted_iota(I32, (128, D), 1)
        keep = (2 * (row // 64) + row % 2) == ((col % 128) // DH)
        phit[...] = jnp.where(keep, ph * LOG2E, 0.0).astype(BF16)
        wr = wr_v[...].astype(F32)
        wrb[...] = jnp.concatenate([jnp.broadcast_to(wr[t:t + 1], (8, 128))
                                    for t in range(8)], axis=1)

    def fold(which, dst, j, sch=None):
        wt = []
        for g in (2 * j, 2 * j + 1):
            r_ = _dot_nt(phit[:, g * 128:(g + 1) * 128],
                         w_v[which, :, g * 128:(g + 1) * 128])
            if sch is not None and g == 2 * j:
                sch.token = r_[0:8, 0:128]
            wt.append(r_)
        w0, w1 = wt
        cs = _lhs_combos(w0[:, :DHALF], w0[:, DHALF:], w1[:, :DHALF], w1[:, DHALF:])
        for k in range(7):
            dst.at[k][j * 64:(j + 1) * 64, :] = _pack(cs[k])

    def prep_v(j, sch):
        ws = [_u32(w_v[2, :, g * 128:(g + 1) * 128]) for g in (2 * j, 2 * j + 1)]
        ws = [sch.hold(w, [(8 * q, 0) for q in range(8)]) for w in ws]
        wt = [_bf(w).T for w in ws]
        f0, f1 = [w.astype(F32) for w in wt]
        w0, w1 = [_u32(w) for w in wt]
        cs = _lhs_combos(f0[:, :DHALF], f0[:, DHALF:], f1[:, :DHALF], f1[:, DHALF:])
        for k in range(7):
            u = w0[:, :DHALF] if k == 2 else w1[:, DHALF:] if k == 3 else _pack(cs[k])
            av.at[k][j * 64:(j + 1) * 64, :] = u
        return w0, w1

    def ln_chunk(n, c, sch=None, also=None, early=None, late=None):
        ys = []
        for h in range(2):
            r0 = n * T + h * TH + c * 16
            if not isinstance(r0, int):
                r0 = pl.multiple_of(r0, 16)
            xr = x_v[pl.ds(r0, 16), :].astype(F32)
            if sch is not None:
                xr = pltpu.bitcast(sch.hold(_u32(xr), [(0, 0), (1, 0)]), F32)
            y, inv = _layernorm(xr)
            ys.append(y)
            if early is not None and h == 0:
                early([jnp.broadcast_to(inv, (16, 128))])
            w8 = wrb[...]
            sc = jnp.sum(y * jnp.concatenate([w8, w8], axis=0), axis=-1, keepdims=True)
            r_v.at[n][:, 2 * c + h:2 * c + h + 1] = sc
            if late is not None:
                late([jnp.broadcast_to(sc, (16, 128))])
        ya, yb = ys
        cs = (_rhs_combos(ya[:, :DHALF], yb[:, :DHALF], ya[:, DHALF:], yb[:, DHALF:])
              + [ya[:, DHALF:], yb[:, :DHALF]])
        out = []
        for k in range(9):
            dst = bq.at[n, k]
            u = _pack(cs[k])
            dst[c * 8:(c + 1) * 8, :] = u
            if also is not None and k < 7:
                dst = also.at[k]
                dst[c * 8:(c + 1) * 8, :] = u
            if isinstance(n, int):
                out.append(dst[c * 8:(c + 1) * 8, :])
        if isinstance(n, int):
            return out
        return [cs[k] for k in (0, 2, 3, 5, 6)]

    def wo_piece(e):
        r0 = pl.multiple_of((e // 8) * 256 + (e % 8) * 16, 16)
        o0 = pl.multiple_of(e * 8, 8)
        w0 = wo_v[pl.ds(r0, 16), :].astype(F32)
        w1 = wo_v[pl.ds(r0 + 128, 16), :].astype(F32)

        def cols(w, par):
            return jnp.concatenate(
                [w[:, (2 * q + par) * 128:(2 * q + par + 1) * 128] for q in range(4)], axis=1)
        cs = _rhs_combos(cols(w0, 0), cols(w0, 1), cols(w1, 0), cols(w1, 1))
        for k in range(7):
            bo.at[k][pl.ds(o0, 8), :] = _pack(cs[k])
        return [cs[k] for k in (0, 2, 3, 5, 6)]

    def proj(sch, a_ref, j, b, early=None):
        def prod(k):
            r_ = _dot_nt(_bf(sch.gate(a_ref[k, j * 64:(j + 1) * 64, :])), b[k])
            sch.token = r_[0:8, 0:128]
            return r_

        def after(step, done):
            if step == 4 and early is not None:
                early[j] = [jnp.concatenate([done[0], done[1]], axis=1), None]
            sch.after(step, done)
        c11, c12, c21, c22 = _strassen(prod, after)
        return (jnp.concatenate([c11, c12], axis=1),
                jnp.concatenate([c21, c22], axis=1))

    class KVTile:
        def __init__(self, sch, i, slot, src=None):
            self.sch, self.i, self.slot, self.src = sch, i, slot, src
            self.b = None
            self.pk, self.phis = {}, {}

        def operands(self):
            if self.src is not None:
                return [_bf(self.src[k]) for k in range(7)]
            if self.b is None:
                self.b = [_bf(bq[self.i, k]) for k in range(7)]
            return self.b

        def kproj(self, j):
            self.pk[j] = proj(self.sch, ak, j, self.operands())

        def vproj(self, j):
            vs = proj(self.sch, av, j, self.operands())
            for g in range(2):
                for p in range(2):
                    vt_v.at[self.slot, 2 * j + g][p * 32:(p + 1) * 32, :] = _pack(
                        vs[g][p * 64:(p + 1) * 64])

        def sm(self, j, g, p, due=None, step=0):
            phi, _ = _feature_map(self.pk[j][g][p * 64:(p + 1) * 64])
            z_v[4 * j + 2 * g + p] += phi[:, :128] + phi[:, 128:]
            if due is None:
                self.phis[j, g, p] = lambda: phi.astype(BF16)
                return
            dst = ph_v.at[self.i, 4 * j + 2 * g + p]
            for t in range(2):
                dst[t * 32:(t + 1) * 32, :] = _pack(phi[t * 64:(t + 1) * 64])
            self.phis[j, g, p] = lambda: _bf(dst[...])
            for t in range(2):
                self.sch.need(due - step * (1 - t), [dst[:, t * 128:(t + 1) * 128]])

        def kv(self, j, g):
            for p in range(2):
                if (j, g, p) not in self.phis:
                    self.sm(j, g, p)
                lhs = _bf(vt_v[self.slot, 2 * j + g, p * 32:(p + 1) * 32, :])
                kv_acc[4 * j + 2 * g + p] += _dot_nt(lhs, self.phis[j, g, p]())

    def first_tiles():
        sch = Sched(zero_s[0] > 0)
        tiles = {'a': KVTile(sch, 0, 0), 'b': KVTile(sch, 1, 1)}
        for op in PROG.split():
            kind, arg = op[0], op[1:2]
            if kind == 'w':
                for nm in op[2:].split(','):
                    named_copy(nm).wait()
            elif kind == 'P':
                build_phit()
            elif kind == 'f':
                fold(1, ak, int(arg))
            elif kind == 'p':
                _, rel, d0 = op.split(':')

                def job(j=int(arg), base=sch.slot + float(d0)):
                    ws = prep_v(j, sch)
                    for q in range(8):
                        sch.need(base + q * 0.375, [w[:, q * 128:(q + 1) * 128] for w in ws])
                sch.at(sch.slot + int(rel), job)
            elif kind == 'U':
                for c in range(8):
                    ln_chunk(int(arg), c)
            elif kind == 'L':
                l0, l1, c0, c1, lead = [float(v) for v in op.split(':')[1:]]
                for c in range(int(c0), int(c1)):
                    due = _eighths(sch.slot + l0 + (l1 - l0) * (c - c0) / (c1 - c0 - 1))
                    rel = int(due - lead)

                    def job(n=int(arg), c=c, due=due, held=rel >= sch.slot):
                        late = functools.partial(sch.need, due + 2)
                        sch.spread(ln_chunk(n, c, sch if held else None,
                                            bp[0] if n == NF else None, None,
                                            late if n == NF else None), due)
                    if rel >= sch.slot:
                        sch.at(rel, job)
                    else:
                        job()
            elif kind == 'S':
                st_ = 4.0 / 7
                for q in range(4):
                    tiles[op[2]].sm(int(arg), q // 2, q % 2,
                                    _eighths(sch.slot + 2.5 + st_ * (2 * q + 1)), _eighths(st_))
            elif kind == 'K':
                tiles[op[2]].kproj(int(arg))
            elif kind == 'V':
                tiles[op[2]].vproj(int(arg))
            elif kind == 'X':
                for g in range(2):
                    sch.at(sch.slot + 1 + g, functools.partial(tiles[op[2]].kv, int(arg), g))
            elif kind == 'Y':
                for g in range(2):
                    tiles[op[2]].kv(int(arg), g)
        assert not sch.jobs and not sch.deps

    def phase1_tile(i, par, sch):
        nxt = jnp.minimum(i + 1, NT - 1)
        o = sch.slot
        tl = KVTile(sch, i, par, bp[par])
        for c in range(8):
            due = o + min(14 * (c // 2) + (5, 13)[c % 2], 54 + par)
            sch.spread(ln_chunk(nxt, c, None, bp[1 - par],
                                functools.partial(sch.need, due - 0.25),
                                functools.partial(sch.need, min(due + 3, 111.875))),
                       due, 0.125)
        for q, due in enumerate((2, 9, 16, 30, 37, 44)):
            sch.spread(wo_piece(jnp.minimum((i - NF) * 6 + q, 31)), o + due)
        for j in range(NJ if par == 0 else NJ - 1):
            for g in range(2):
                sch.at(o + 14 * (j + 1) + g, functools.partial(tl.kv, j, g))
        for j in range(NJ):
            tl.kproj(j)
            tl.vproj(j)
        if par == 1:
            for g in range(2):
                tl.kv(NJ - 1, g)

    def phase1(m, carry):
        sch = Sched(zero_s[0] > 0)
        for par in range(2):
            phase1_tile(NF + 2 * m + par, par, sch)
        return carry

    first_tiles()
    wo_copy.wait()
    for t in range(NF + 1, NT):
        x_copy(t).wait()
    jax.lax.fori_loop(0, (NT - NF) // 2, phase1, 0)

    for j in range(NJ):
        w_copy(0, j).wait()
    wg_copy.wait()
    wu_copy.wait()
    wd_copy.wait()
    sch = Sched(zero_s[0] > 0)
    row = jax.lax.broadcasted_iota(I32, (64, 128), 0)
    col = jax.lax.broadcasted_iota(I32, (64, 128), 1)
    keep = (row // DH) == (col % 2)
    for j in range(NJ):
        fold(0, aq, j, sch)
        for p in range(8 * j, 8 * j + 8) if j < 2 else ():
            kvp = pltpu.bitcast(sch.hold(_u32(kv_acc[p]), [(r, 0) for r in range(8)]), F32)
            mk = jnp.where(keep, kvp, 0.0)
            for t in range(2):
                m_v.at[p][t * 16:(t + 1) * 16, :] = _pack(mk[t * 32:(t + 1) * 32])
            sch.need(1 + p * 0.25, [m_v[p]])
            zp = pltpu.bitcast(sch.hold(_u32(z_v[p]), [(r, 0) for r in range(16)]), F32)
            z_v[p] = jnp.broadcast_to(jnp.sum(zp, axis=1, keepdims=True), (128, 128))

    r = _round(r_v[...].reshape(NT * 16, 128))
    rmax = jnp.max(jnp.max(r, axis=0, keepdims=True), axis=1, keepdims=True)
    rw = jax.lax.broadcasted_iota(I32, (NT * 16, 128), 0)
    ln = jax.lax.broadcasted_iota(I32, (NT * 16, 128), 1)
    pos = (rw // 16) * T + (ln % 2) * TH + (ln // 2) * 16 + rw % 16
    idx = jnp.min(jnp.where(r == rmax, pos, S))
    idx = jnp.clip(idx, 0, S - 1)
    tile = idx // T
    half = (idx % T) // TH
    sub = pl.multiple_of(((idx % TH) // 16) * 8, 8)
    xs = jnp.concatenate([bq[tile, 1 + 7 * half, pl.ds(sub, 8), :],
                          bq[tile, 7 - 3 * half, pl.ds(sub, 8), :]], axis=1)
    xs = jnp.where(jax.lax.broadcasted_iota(I32, (16, D), 0) == idx % 16,
                   _bf(xs).astype(F32), 0.0)
    xs = jnp.sum(xs, axis=0, keepdims=True)

    def lane_bcast(dst, row):
        for t in range(row.shape[1] // 128):
            dst[t * 128:(t + 1) * 128, :] = jnp.broadcast_to(
                row[:, t * 128:(t + 1) * 128], (128, 128)).T

    lane_bcast(xb_v, xs)
    router = _round(0.5 + 0.5 * jnp.tanh(0.5 * rmax))

    n_first = (tile + 1) & (NT - 1)
    first = proj(sch, aq, 0, [_bf(bq[n_first, k]) for k in range(7)])
    for g in range(2):
        pq0_v[g] = first[g]

    def phase2(i, n):
        last = isinstance(i, int)
        zero = zero_s[0]
        slot = i
        n_next = (n + 1) & (NT - 1)

        s0 = pl.multiple_of(n * T, T)
        b = [_bf(bq[n, k]) for k in range(7)]
        pq = [None] * NJ
        sch = Sched(zero > 0)
        ot = {}
        pq[0] = [pq0_v[g] for g in range(2)]
        phis = {}

        def sm(j, g, p, due, step):
            phi, scales = _feature_map(pq[j][g][p * 64:(p + 1) * 64], z_v[4 * j + 2 * g + p])
            phis[j, g, p] = phi.astype(BF16)
            for t in range(2):
                sch.need(max(due - step * (1 - t), sch.slot + 1),
                         [v[:, t * 128:(t + 1) * 128] for v in scales])

        def nd(j, g):
            ot[j, g] = jnp.concatenate(
                [_dot(_bf(m_v[4 * j + 2 * g + p]), phis[j, g, p]) for p in range(2)], axis=0)
            if g == 1:
                o0, o1 = ot[j, 0], ot[j, 1]
                cs = _lhs_combos(o0[:, :TH], o1[:, :TH], o0[:, TH:], o1[:, TH:])
                for k in range(7):
                    ao_v[2 * k + j // 2][zero, :, (j % 2) * 128:(j % 2 + 1) * 128] = (
                        _u32(cs[k].astype(BF16).T))

        if last:
            fd = (NFC - 1) * FC
        else:
            fu = pl.multiple_of(i * FC, FC)
            fd = pl.multiple_of(jnp.maximum(i - 1, 0) * FC, FC)
        ffn = {}

        def matvec(key, w, vb, due):
            t = (w.astype(F32).reshape(FR // 8, 8, 256)
                 * jnp.concatenate([vb, vb], axis=1).reshape(FR // 8, 8, 256))
            t = jnp.sum(t, axis=0)
            ffn[key] = t if key not in ffn else ffn[key] + t
            sch.need(due, [ffn[key]])

        def ffn_up(w_ref, name, cp, rb, due):
            rs = slice(rb * FR, (rb + 1) * FR)
            matvec((name, cp), w_ref[rs, pl.ds(fu + cp * 256, 256)], xb_v[rs, :], due)

        def ffn_mid():
            hg, hu = [_round(jnp.sum(jnp.concatenate([ffn[nm, 0], ffn[nm, 1]], axis=1),
                                     axis=0, keepdims=True)) for nm in 'gu']
            lane_bcast(hb_v, _round(_round(_silu(hg)) * hu))

        def ffn_down(cp, rb, due):
            cs_ = slice(cp * 256, (cp + 1) * 256)
            if rb == 0:
                ffn['y', cp] = y_acc[:, cs_]
            matvec(('y', cp), wd_v[pl.ds(fd + rb * FR, FR), cs_],
                   hb_v[rb * FR:(rb + 1) * FR, :], due)
            if rb == FC // FR - 1:
                if last:
                    ffn['row', cp] = (
                        _round(jnp.sum(ffn['y', cp], axis=0, keepdims=True)) * router)
                else:
                    y_acc[:, cs_] = ffn['y', cp]

        d0, d1 = (21, 33) if last else (28, 36.5)
        nd_ = 4 * FC // FR
        for t in range(nd_):
            due = _eighths(d0 + (d1 - d0) * t / (nd_ - 1))
            sch.at(0, functools.partial(ffn_down, t % 4, t // 4, due))
        if not last:
            nu_ = 4 * D // FR
            for t in range(nu_):
                due = _eighths(37 + 16.5 * t / (nu_ - 1))
                name, w_ref = (('g', wg_v), ('u', wu_v))[(t // 2) % 2]
                sch.at(0, functools.partial(ffn_up, w_ref, name, t % 2, t // 4, due))
            sch.at(53, ffn_mid)
        for j in range(NJ):
            s1 = 7 * j
            nds = (((1, 3), (0, 3), (0, 3), (1, 2)) if last
                   else ((1, 3), (0, 2), (0, 2), (0, 1)))[j]
            for g in range(2):
                for p in range(2):
                    sch.at(s1 if (j == 0 or g == 1) else s1 - 2, functools.partial(
                        sm, j, g, p, s1 + nds[g] + p, 0.5))
                sch.at(s1 + nds[g], functools.partial(nd, j, g))
        for j in range(1, NJ):
            pq[j] = proj(sch, aq, j, b, early=pq)
        if last:
            def prod_a(k):
                return _dot(_bf(sch.gate(ao_v[2 * k][0])), _bf(bo[k, 0:128, 0:256]))
            part = _strassen(prod_a, sch.after)
        else:
            nxt = proj(sch, aq, 0, [_bf(bq[n_next, k]) for k in range(7)])
            for g in range(2):
                pq0_v[g] = nxt[g]

        er = 64
        rows = jax.lax.broadcasted_iota(I32, (er, 256), 0) + s0
        ne_ = T // er
        gates = {}

        def gate_part(c, e, due):
            r0 = e * er
            h, rh = r0 // TH, r0 % TH
            blk = ((1, 7), (8, 4))[h][c // 2]
            bb = _bf(bq[n, blk, rh // 2:(rh + er) // 2,
                        (c % 2) * 256:(c % 2 + 1) * 256]).astype(F32)
            if last:
                bb = bb + jnp.where(rows + r0 == idx, ffn['row', c], 0.0)
            gates[c, e] = _silu(bb)
            if due is not None:
                sch.need(due, [gates[c, e]])

        def epilogue(c, cc, e, due):
            r0 = e * er
            h, rh = r0 // TH, r0 % TH
            cs = slice(c * 256, (c + 1) * 256)
            rs = slice(rh, rh + er)
            if (c, e) not in gates:
                gate_part(c, e, None)
            xr = x_v[pl.ds(s0 + r0, er), cs].astype(F32)
            sv = jnp.concatenate([cc[2 * h][rs], cc[2 * h + 1][rs]], axis=1)
            res = xr + sv * gates[c, e]
            out_v[slot, r0:r0 + er, cs] = res.astype(BF16)
            if due is not None:
                sch.need(due, [res])

        def out_cols(c, h=None):
            cs = slice(c * 256, (c + 1) * 256)
            if h is None:
                return pltpu.make_async_copy(out_v.at[slot, :, cs],
                                             out_hbm.at[0, pl.ds(s0, T), cs], sem_o.at[NT + c])
            return pltpu.make_async_copy(
                out_v.at[slot, h * TH:(h + 1) * TH, cs],
                out_hbm.at[0, pl.ds(s0 + h * TH, TH), cs], sem_o.at[NT + c + h])

        e0, e1 = (1 if last else 0.5), 6.5
        end = sch.slot + 28 - (7 if last else 0)
        for e in range(ne_):
            sch.at(end - 8, functools.partial(
                gate_part, 3, e, _eighths(end - 7 + 4 * e / (ne_ - 1))))
        pending = []
        c = 0
        while c < 4:
            if last and c == 0:
                def prod(k):
                    return _dot(_bf(sch.gate(ao_v[2 * k + 1][0])),
                                _bf(bo[k, 128:256, 0:256]))
                cc2 = [u + v for u, v in zip(part, _strassen(prod, sch.after))]
                blocks = [(t, [v[:, t * 128:(t + 1) * 128] for v in cc2]) for t in range(2)]
            else:
                def prod(k):
                    return _dot(_bf(sch.gate(jnp.concatenate(
                        [ao_v[2 * k][0], ao_v[2 * k + 1][0]], axis=1))),
                                _bf(bo[k, :, c * 128:(c + 1) * 128]))
                blocks = [(c, _strassen(prod, sch.after))]
            if last:
                for t in pending:
                    out_cols(t).start()
            nb = len(blocks) * ne_
            for q in range(nb):
                t, cc = blocks[q // ne_]
                due = _eighths(sch.slot + e0 + (e1 - e0) * q / (nb - 1))
                epilogue(t, cc, q % ne_, due if t < 3 else None)
                if last and t == 3 and (q + 1) % (ne_ // 2) == 0:
                    out_cols(3, (q + 1) // (ne_ // 2) - 1).start()
            pending = [t for t, _ in blocks]
            c += len(blocks)
        if last:
            for t in range(NT - 1):
                out_copy((tile + 1 + t) & (NT - 1), t).wait()
            for t in range(3):
                out_cols(t).wait()
            for h in range(2):
                out_cols(3, h).wait()
        else:
            out_copy(n, slot).start()
        return n_next

    jax.lax.fori_loop(0, NT - 1, phase2, n_first)
    phase2(NT - 1, tile)


@jax.jit
def pallas_recurrent_scan__linear_kernel_hedgehog__moe_arch_mod__prompt_kernel(
    A_x: jax.Array,
    A_wqkv: jax.Array,
    A_w_phi: jax.Array,
    A_wo: jax.Array,
    B_x: jax.Array,
    B_w_r: jax.Array,
    B_w_gate: jax.Array,
    B_w_up: jax.Array,
    B_w_down: jax.Array,
):
    del B_x
    any_spec = pl.BlockSpec(memory_space=pl.ANY)
    return pl.pallas_call(
        _kernel,
        out_shape=jax.ShapeDtypeStruct((1, S, D), BF16),
        in_specs=[any_spec] * 8,
        out_specs=any_spec,
        scratch_shapes=[
            pltpu.VMEM((S, D), BF16),
            pltpu.VMEM((3, D, D), BF16),
            pltpu.VMEM((H, DH, DH), BF16),
            pltpu.VMEM((8, 128), BF16),
            pltpu.VMEM((D, D), BF16),
            pltpu.VMEM((D, F), BF16),
            pltpu.VMEM((D, F), BF16),
            pltpu.VMEM((F, D), BF16),
            pltpu.VMEM((NT, 9, TH // 2, DHALF), U32),
            pltpu.VMEM((7, 256, DHALF), U32),
            pltpu.VMEM((7, 256, DHALF), U32),
            pltpu.VMEM((7, 256, DHALF), U32),
            pltpu.VMEM((7, 256, DHALF), U32),
            pltpu.VMEM((NP, 64, 128), F32),
            pltpu.VMEM((NP, 128, 128), F32),
            pltpu.VMEM((NF, NP, 64, T), U32),
            pltpu.VMEM((NF, 8, 64, T), U32),
            pltpu.VMEM((NP, 32, 128), U32),
            pltpu.VMEM((128, D), BF16),
            pltpu.VMEM((8, D), F32),
            pltpu.VMEM((NT, 16, 128), F32),
            pltpu.VMEM((8, D), F32),
            pltpu.VMEM((D, 128), F32),
            pltpu.VMEM((FC, 128), F32),
            pltpu.VMEM((2, 128, T), F32),
            pltpu.VMEM((NT, T, D), BF16),
            pltpu.SMEM((1,), I32),
        ] + [pltpu.VMEM((1, TH // 2, 256), U32)] * 14
        + [pltpu.VMEM((7, TH // 2, DHALF), U32)] * 2,
        compiler_params=pltpu.CompilerParams(
            vmem_limit_bytes=100 * 1024 * 1024,
            disable_bounds_checks=True),
    )(A_x, A_wqkv, A_w_phi, A_wo, B_w_r.reshape(8, 128), B_w_gate, B_w_up, B_w_down)
```
